```python
import jax
import jax.numpy as jnp

def _softmax(x, axis=-1):
    return jax.nn.softmax(x, axis=axis)
def _gelu(x):
    return jax.nn.gelu(x, approximate=True)
def _silu(x):
    return jax.nn.silu(x)
def _sigmoid(x):
    return jax.nn.sigmoid(x)
def _layernorm(x, axis=-1, eps=1e-5):
    m = jnp.mean(x, axis=axis, keepdims=True)
    v = jnp.var(x, axis=axis, keepdims=True)
    return (x - m) / jnp.sqrt(v + eps)
def _scatter_add(tgt, idx, src, axis=0):
    return tgt.at[idx].add(src)
def _segment_sum(src, seg, n):
    return jax.ops.segment_sum(src, seg, n)
class _Rng:
    def __init__(self, key):
        self._k = key
    def _next(self):
        self._k, sub = jax.random.split(self._k)
        return sub
    def normal(self, shape):
        return jax.random.normal(self._next(), shape, dtype=jnp.bfloat16)
    def randint(self, lo, hi, shape):
        return jax.random.randint(self._next(), shape, lo, hi, dtype=jnp.int32)
    def uniform(self, shape, lo=0.0, hi=1.0):
        return jax.random.uniform(self._next(), shape, jnp.bfloat16, lo, hi)
    def permutation(self, n):
        return jax.random.permutation(self._next(), n)


kernel_name = 'recurrent_scan__ssm_conv_s4__moe_arch_mod__prompt'

def setup_inputs():
    _rng = _Rng(jax.random.key(int.from_bytes(__import__("os").urandom(4), "little")))
    _w = (lambda a: (lambda t: t.astype(jnp.bfloat16) if jnp.issubdtype(t.dtype, jnp.floating) else t)(jnp.asarray(a)))
    def _A_setup():
        B, L, D, N = 1, 2048, 576, 128
        A_re = -jnp.exp((lambda *s: _rng.normal(s) * 0.05)(D, N))
        A_im = jnp.pi * (lambda *s: _rng.normal(s) * 0.05)(D, N)
        B_re = (lambda *s: _rng.normal(s) * 0.05)(D, N)
        B_im = (lambda *s: _rng.normal(s) * 0.05)(D, N)
        C_re = (lambda *s: _rng.normal(s) * 0.05)(D, N)
        C_im = (lambda *s: _rng.normal(s) * 0.05)(D, N)
        log_dt = (lambda *s: _rng.normal(s) * 0.05)(D) * 0.5 - 4.0
        Dskip = (lambda *s: _rng.normal(s) * 0.05)(D)
        return {
            "u": _w((lambda *s: _rng.normal(s) * 0.05)(B, L, D)),
            "A_re": _w(A_re),
            "A_im": _w(A_im),
            "B_re": _w(B_re),
            "B_im": _w(B_im),
            "C_re": _w(C_re),
            "C_im": _w(C_im),
            "log_dt": _w(log_dt),
            "Dskip": _w(Dskip),
        }
    _A_in = _A_setup()

    def _B_setup():
        B, S, D, F, C = 1, 2048, 576, 4608, 8
        return {
            "x": _w((lambda *s: _rng.normal(s) * 0.05)(B, S, D)),
            "w_r": _w((lambda *s: _rng.normal(s) * 0.05)(D)),
            "w_gate": _w((lambda *s: _rng.normal(s) * 0.05)(D, F)),
            "w_up": _w((lambda *s: _rng.normal(s) * 0.05)(D, F)),
            "w_down": _w((lambda *s: _rng.normal(s) * 0.05)(F, D)),
        }
    _B_in = _B_setup()

    return {
        "A_u": _A_in["u"],
        "A_A_re": _A_in["A_re"],
        "A_A_im": _A_in["A_im"],
        "A_B_re": _A_in["B_re"],
        "A_B_im": _A_in["B_im"],
        "A_C_re": _A_in["C_re"],
        "A_C_im": _A_in["C_im"],
        "A_log_dt": _A_in["log_dt"],
        "A_Dskip": _A_in["Dskip"],
        "B_x": _B_in["x"],
        "B_w_r": _B_in["w_r"],
        "B_w_gate": _B_in["w_gate"],
        "B_w_up": _B_in["w_up"],
        "B_w_down": _B_in["w_down"],
    }

def reference(A_u, A_A_re, A_A_im, A_B_re, A_B_im, A_C_re, A_C_im, A_log_dt, A_Dskip, B_x, B_w_r, B_w_gate, B_w_up, B_w_down):
    def _A_ref(u, A_re, A_im, B_re, B_im, C_re, C_im, log_dt, Dskip):
        Bsz, L, D = u.shape
        dt = jnp.exp(log_dt)[:, None]
        A = A_re + 1j * A_im
        Bc = B_re + 1j * B_im
        Cc = C_re + 1j * C_im
        logdA = dt * A
        dB = dt * Bc
        l = (lambda x, dt: x.astype(dt))(jnp.arange(L), A_re.dtype)
        P = jnp.exp(logdA[:, :, None] * l[None, None, :])
        K = jnp.einsum("dn,dnl,dn->dl", Cc, P, dB).real
        L2 = 2 * L
        Kp = jnp.pad(K, ((0, 0), (0, L)))
        up = (lambda x, *d: x.transpose(*d))(u, 0, 2, 1)
        up = jnp.pad(up, ((0, 0), (0, 0), (0, L)))
        Kf = (lambda x, axes=(-2,-1): jnp.fft.rfft2(x.astype(jnp.float32), axes=axes))(Kp[:, None, :], axes=(-2, -1))
        Uf = (lambda x, axes=(-2,-1): jnp.fft.rfft2(x.astype(jnp.float32), axes=axes))(up[:, :, None, :], axes=(-2, -1))
        Yf = Uf * Kf[None, :, :, :]
        y = (lambda x, s, axes=(-2,-1): jnp.fft.irfft2(x, s=s, axes=axes).astype(jnp.bfloat16))(Yf, (1, L2), axes=(-2, -1))[:, :, 0, :L]
        y = (lambda x, *d: x.transpose(*d))(y, 0, 2, 1) + u * Dskip[None, None, :]
        return y

    def _B_ref(x, w_r, w_gate, w_up, w_down):
        B, S, D = x.shape
        C = 8
        r = x @ w_r
        idx = jnp.argsort(-r, axis=-1)[:, :C]
        idx_e = jnp.repeat(idx.reshape(B, C, 1), D, axis=2)
        x_sel = jnp.take_along_axis(x, idx_e, axis=1)
        g = _silu(x_sel @ w_gate)
        u = x_sel @ w_up
        y = (g * u) @ w_down
        r_sel = _sigmoid(jnp.take_along_axis(r, idx, axis=1))
        y = y * r_sel.reshape(B, C, 1)
        b_off = (jnp.arange(B) * S).reshape(B, 1)
        flat_idx = (idx + b_off).reshape(B * C)
        zero = (x * 0.0).reshape(B * S, D)
        upd = _scatter_add(zero, flat_idx, y.reshape(B * C, D), axis=0)
        return x + upd.reshape(B, S, D)

    x = A_u
    xn = _layernorm(x, axis=-1)
    s = _A_ref(xn, A_A_re, A_A_im, A_B_re, A_B_im, A_C_re, A_C_im, A_log_dt, A_Dskip)
    g = _silu(_B_ref(xn, B_w_r, B_w_gate, B_w_up, B_w_down))
    return x + s * g
```

```python
import jax
import jax.numpy as jnp
import numpy as np
from jax import lax
import jax.experimental.pallas as pl
import jax.experimental.pallas.tpu as pltpu

_D, _L, _N, _F, _C = 576, 2048, 128, 4608, 8
_T = 128
_NB = _L // _T
_EPS = 1e-5
_CH_A = 16
_CH_C = 32
_OUT_CHUNKS = ((0, 128), (128, 128), (256, 128), (384, 128), (512, 64))

f32, bf16, i32 = jnp.float32, jnp.bfloat16, jnp.int32


def _dft_constants():
    theta = (np.pi / 2 + 2 * np.pi * np.arange(_T)) / _T
    ang = np.arange(_T)[:, None] * theta[None, :]
    fwd = np.concatenate([np.cos(ang), np.sin(ang)], axis=1)
    return fwd.astype(bf16), (fwd.T / _T).astype(bf16)


_FWD, _INV = _dft_constants()


def _lag_step(j):
    return max(1, (1 << (j * _T).bit_length()) >> 8)


def _round_lag(p, st):
    if st == 1:
        return p
    return (p + (st // 2 - 1) + ((p >> (st.bit_length() - 1)) & 1)) & ~(st - 1)


assert np.array_equal(
    np.concatenate([j * _T + _round_lag(np.arange(_T), _lag_step(j)) for j in range(_NB)]),
    np.arange(_L).astype(bf16).astype(np.int64))


def _cmul(a, b):
    return a[0] * b[0] - a[1] * b[1], a[0] * b[1] + a[1] * b[0]


def _csq(a):
    return a[0] * a[0] - a[1] * a[1], (a[0] + a[0]) * a[1]


def _silu(x):
    h = 0.5 * x
    return h + h * jnp.tanh(h)


def _rnd(x):
    return x.astype(bf16).astype(f32)


def _dot(a, b):
    return jnp.dot(a, b, preferred_element_type=f32)


def _dot_nt(a, b):
    return lax.dot_general(a, b, (((1,), (1,)), ((), ())), preferred_element_type=f32)


def _column(v):
    return jnp.broadcast_to(v.reshape(1, _D), (_T, _D)).T


def _filter_taps(dt, ar, ai, br, bi, cr, ci):
    zr, zi = dt * ar, dt * ai
    w = _cmul((cr, ci), (dt * br, dt * bi))
    mag = jnp.exp(zr)
    a1 = (mag * jnp.cos(zi), mag * jnp.sin(zi))
    a2 = _csq(a1)
    a4 = _csq(a2)
    a8 = _csq(a4)
    e = [(jnp.ones_like(zr), jnp.zeros_like(zr)), (a8[0], -a8[1])]
    for s in range(2, 16):
        e.append(_csq(e[s // 2]) if s % 2 == 0 else _cmul(e[s // 2], e[s - s // 2]))
    t = _csq(e[8])
    a128 = (t[0], -t[1])
    a256 = _csq(a128)
    a512 = _csq(a256)
    a1024 = _csq(a512)
    g = {(0, 1): _cmul(w, a1), (0, 2): _cmul(w, a2)}
    for r in (3, 4):
        g[0, r] = _cmul(g[0, r - 2], a2)
    for r in (5, 6, 7, 8):
        g[0, r] = _cmul(g[0, r - 4], a4)
    for j0, mult in ((1, a128), (2, a256), (4, a512), (8, a1024)):
        for j in range(j0, 2 * j0):
            for r in range(_lag_step(j), 9, _lag_step(j)):
                g[j, r] = _cmul(g[j - j0, r], mult)
    keys = sorted(g)
    stack = lambda xs: jnp.concatenate(
        [jnp.concatenate([x[p] for x in xs], axis=0).astype(bf16) for p in (0, 1)], axis=1)
    v = _dot_nt(stack([g[k] for k in keys]), stack(e))

    lane = lax.broadcasted_iota(i32, (8, _T), 1)
    row = lax.broadcasted_iota(i32, (8, _T), 0)
    idx_lo = (lane & ~7) + row
    idx_8 = ((_round_lag(lane, 8) - 8) & (_T - 1)) + row
    tap = {}
    for n, k in enumerate(keys):
        tap[k] = jnp.take_along_axis(v[8 * n:8 * n + 8], idx_8 if k[1] == 8 else idx_lo,
                                     axis=1, mode="promise_in_bounds")
    blocks = []
    for j in range(_NB):
        st = _lag_step(j)
        q = _round_lag(lane, st)
        blk = tap[j, 8]
        for r in range(st, 8, st):
            blk = jnp.where((q & 7) == r, tap[j, r], blk)
        blocks.append(jnp.where(q == 0, tap[j - 1, 8] if j else 0.0, blk))
    return blocks, jnp.sum(w[0], axis=1, keepdims=True)


def _block_conv(k, u):
    p = []
    for b in range(_NB):
        acc = _cmul(k[0], u[b])
        for j in range(1, b + 1):
            t = _cmul(k[j], u[b - j])
            acc = (acc[0] + t[0], acc[1] + t[1])
        p.append(acc)
    return [p[0]] + [(p[b][0] + p[b - 1][1], p[b][1] - p[b - 1][0]) for b in range(1, _NB)]


def _kernel(x_hbm, ar_hbm, ai_hbm, br_hbm, bi_hbm, cr_hbm, ci_hbm, ldt_hbm, dsk_hbm, wr_hbm,
            wg_hbm, wu_hbm, wd_hbm, fwd_hbm, inv_hbm, o_hbm,
            x_v, xn_v, k_v, s_v, o_v, par_v, ldt_v, dsk_v, wr_v, wg_v, wu_v, wd_v, fwd_v, inv_v,
            dt_v, c0_v, sem):
    copies = {}

    def start(name, src, dst):
        copies[name] = pltpu.make_async_copy(src, dst, sem.at[len(copies)])
        copies[name].start()

    def wait(*names):
        for name in names:
            copies[name].wait()

    start("ldt", ldt_hbm, ldt_v)
    start("dsk", dsk_hbm, dsk_v)
    for n, src in enumerate((ar_hbm, ai_hbm, br_hbm, bi_hbm, cr_hbm, ci_hbm)):
        start(("par", n), src, par_v.at[n])
    wait("ldt")
    start("x", x_hbm, x_v)
    start("wr", wr_hbm, wr_v)
    start("fwd", fwd_hbm, fwd_v)
    start("inv", inv_hbm, inv_v)
    dt_v[...] = _column(_rnd(jnp.exp(ldt_v[...].astype(f32))))
    wait("dsk")
    c0_v[...] = _column(dsk_v[...].astype(f32))
    wait(*[("par", n) for n in range(6)])
    start("wg", wg_hbm, wg_v)
    start("wu", wu_hbm, wu_v)

    def phase_a(i, carry):
        rows = pl.ds(pl.multiple_of(i * _CH_A, _CH_A), _CH_A)
        par = [dt_v[rows, :]] + [par_v[n, rows, :].astype(f32) for n in range(6)]
        parts = [_filter_taps(*[p[8 * h:8 * h + 8] for p in par]) for h in range(_CH_A // 8)]
        for j in range(_NB):
            k_v[rows, j * _T:(j + 1) * _T] = jnp.concatenate(
                [p[0][j] for p in parts], axis=0).astype(bf16)
        c0_v[rows, :] += jnp.concatenate([p[1] for p in parts], axis=0)
        return carry

    lax.fori_loop(0, _D // _CH_A, phase_a, 0)

    wait("x", "wr")
    ones = jnp.ones((8, _D), bf16)
    wt = 256

    def phase_b(i, carry):
        cols = pl.ds(pl.multiple_of(i * wt, wt), wt)
        x = x_v[:, cols]
        mean = _dot(ones, x)[0:1] / _D
        m = _rnd(mean)
        xc = x.astype(f32) - m
        var = jnp.sum(xc * xc, axis=0, keepdims=True) / _D - (mean - m) * (mean - m)
        sd = _rnd(jnp.sqrt(_rnd(_rnd(jnp.maximum(var, 0.0)) + _rnd(jnp.full_like(var, _EPS)))))
        xn_v[:, cols] = (xc * (1.0 / sd)).astype(bf16)
        return carry

    lax.fori_loop(0, _L // wt, phase_b, 0)

    wr = jnp.broadcast_to(wr_v[...].astype(f32).reshape(1, _D), (8, _D)).astype(bf16)
    score = _rnd(_dot(wr, xn_v[...])) + 0.0
    bits = pltpu.bitcast(score, i32) >> 16
    rank = jnp.where(bits < 0, ~bits, bits + 0x8000)
    tok = lax.broadcasted_iota(i32, (8, _L), 1)
    key = pltpu.bitcast((1 << 28) + rank * _L + (_L - 1 - tok), f32)
    row = lax.broadcasted_iota(i32, (8, _T), 0)
    live = []
    for h in range(_NB // 8):
        t = key[:, 8 * h * _T:(8 * h + 1) * _T]
        for s in range(1, 8):
            t = jnp.where(row == s, key[:, (8 * h + s) * _T:(8 * h + s + 1) * _T], t)
        live.append(t)
    top = jnp.zeros((8, _T), f32)
    for c in range(_C):
        best = jnp.max(jnp.max(jnp.maximum(live[0], live[1]), axis=0, keepdims=True),
                       axis=1, keepdims=True)
        top = jnp.where(row == c, best, top)
        live = [jnp.where(t == best, 0.0, t) for t in live]
    onehot = jnp.concatenate(
        [jnp.where(key[:, b * _T:(b + 1) * _T] == top, 1.0, 0.0) for b in range(_NB)],
        axis=1).astype(bf16)
    top_rank = (pltpu.bitcast(top, i32) - (1 << 28)) >> 11
    top_score = pltpu.bitcast(
        jnp.where(top_rank >= 0x8000, top_rank - 0x8000, ~top_rank) << 16, f32)
    route_w = _rnd(jax.nn.sigmoid(top_score))
    x_sel = _dot_nt(onehot, xn_v[...]).astype(bf16)

    wait("fwd", "inv")
    for n, (r0, nr) in enumerate(_OUT_CHUNKS):
        start(("wd", n), wd_hbm.at[pl.ds(r0, nr)], wd_v.at[pl.ds(r0, nr)])

    def phase_c(i, carry):
        rows = pl.ds(pl.multiple_of(i * _CH_C, _CH_C), _CH_C)
        stacked = lambda ref: jnp.concatenate(
            [ref[rows, b * _T:(b + 1) * _T] for b in range(_NB)], axis=0)
        kf = _dot(stacked(k_v), fwd_v[...])
        uf = _dot(stacked(xn_v), fwd_v[...])
        pick = lambda z, h: [(z[b * _CH_C + 8 * h:b * _CH_C + 8 * h + 8, :_T],
                              z[b * _CH_C + 8 * h:b * _CH_C + 8 * h + 8, _T:]) for b in range(_NB)]
        w = [_block_conv(pick(kf, h), pick(uf, h)) for h in range(_CH_C // 8)]
        wf = jnp.concatenate(
            [jnp.concatenate([wh[b][p] for b in range(_NB) for wh in w], axis=0).astype(bf16)
             for p in (0, 1)], axis=1)
        y = _dot(wf, inv_v[...])
        for b in range(_NB):
            s_v[rows, b * _T:(b + 1) * _T] = y[b * _CH_C:(b + 1) * _CH_C]
        return carry

    lax.fori_loop(0, _D // _CH_C, phase_c, 0)

    wait("wg")
    gate = _rnd(_silu(_rnd(_dot(x_sel, wg_v[...]))))
    wait("wu")
    hid = (gate * _rnd(_dot(x_sel, wu_v[...]))).astype(bf16)

    for n, (r0, nr) in enumerate(_OUT_CHUNKS):
        rows = pl.ds(r0, nr)
        wait(("wd", n))
        y = _rnd(_dot_nt(hid, wd_v[rows, :])) * route_w[:, :nr]
        upd = _dot(y.T.astype(bf16), onehot)
        xn = xn_v[rows, :].astype(f32)
        s = s_v[rows, :] + xn * jnp.concatenate([c0_v[rows, :]] * _NB, axis=1)
        o_v[rows, :] = (x_v[rows, :].astype(f32) + s * _silu(xn + upd)).astype(bf16)
        start(("o", n), o_v.at[rows], o_hbm.at[rows])
    wait(*[("o", n) for n in range(len(_OUT_CHUNKS))])


@jax.jit
def pallas_recurrent_scan__ssm_conv_s4__moe_arch_mod__prompt_kernel(
    A_u: jax.Array,
    A_A_re: jax.Array,
    A_A_im: jax.Array,
    A_B_re: jax.Array,
    A_B_im: jax.Array,
    A_C_re: jax.Array,
    A_C_im: jax.Array,
    A_log_dt: jax.Array,
    A_Dskip: jax.Array,
    B_x: jax.Array,
    B_w_r: jax.Array,
    B_w_gate: jax.Array,
    B_w_up: jax.Array,
    B_w_down: jax.Array,
):
    del B_x
    assert A_u.shape == (1, _L, _D) and A_A_re.shape == (_D, _N) and B_w_gate.shape == (_D, _F)
    assert A_u.dtype == bf16 and A_A_re.dtype == bf16
    hbm = pl.BlockSpec(memory_space=pl.ANY)
    vmem = pltpu.VMEM
    out = pl.pallas_call(
        _kernel,
        out_shape=jax.ShapeDtypeStruct((_D, _L), bf16),
        in_specs=[hbm] * 15,
        out_specs=hbm,
        scratch_shapes=[
            vmem((_D, _L), bf16), vmem((_D, _L), bf16), vmem((_D, _L), bf16),
            vmem((_D, _L), f32), vmem((_D, _L), bf16),
            vmem((6, _D, _N), bf16), vmem((_D,), bf16), vmem((_D,), bf16), vmem((_D,), bf16),
            vmem((_D, _F), bf16), vmem((_D, _F), bf16), vmem((_D, _F), bf16),
            vmem((_T, 2 * _T), bf16), vmem((2 * _T, _T), bf16),
            vmem((_D, _T), f32), vmem((_D, _T), f32),
            pltpu.SemaphoreType.DMA((14 + 2 * len(_OUT_CHUNKS),)),
        ],
        compiler_params=pltpu.CompilerParams(vmem_limit_bytes=100 * 2**20),
    )(A_u.reshape(_L, _D).T, A_A_re, A_A_im, A_B_re, A_B_im, A_C_re, A_C_im, A_log_dt, A_Dskip,
      B_w_r, B_w_gate, B_w_up, B_w_down.T, _FWD, _INV)
    return out.T.reshape(1, _L, _D)
```

```python
import jax
import jax.numpy as jnp
import numpy as np
from jax import lax
import jax.experimental.pallas as pl
import jax.experimental.pallas.tpu as pltpu

_D, _L, _N, _F, _C = 576, 2048, 128, 4608, 8
_T = 128
_NB = _L // _T
_EPS = 1e-5
_GA = 2
_GC = 2
_NG = _D // 16
_NCH = _NG // _GC
_R = _GC * _NB
_ROW_K, _ROW_X, _ROW_W, _ROW_P, _ROWS = 0, _R, 2 * _R, 6 * _R, 6 * _R + _NB
_OUT_CHUNKS = ((0, 128), (128, 128), (256, 128), (384, 128), (512, 64))

f32, bf16, i32 = jnp.float32, jnp.bfloat16, jnp.int32


def _dft_constants():
    theta = (np.pi / 2 + 2 * np.pi * np.arange(_T)) / _T
    ang = np.arange(_T)[:, None] * theta[None, :]
    c, s = np.cos(ang), np.sin(ang)
    fwd = np.concatenate([c, s], axis=1)
    return fwd.astype(bf16), (fwd.T / _T).astype(np.float32)


_FWD, _INV = _dft_constants()


def _lag_step(j):
    return max(1, (1 << (j * _T).bit_length()) >> 8)


def _round_lag(p, st):
    if st == 1:
        return p
    return (p + (st // 2 - 1) + ((p >> (st.bit_length() - 1)) & 1)) & ~(st - 1)


assert np.array_equal(
    np.concatenate([j * _T + _round_lag(np.arange(_T), _lag_step(j)) for j in range(_NB)]),
    np.arange(_L).astype(bf16).astype(np.int64))

_TAPS = [(j, r) for j in range(_NB) for r in range(_lag_step(j), 9, _lag_step(j))]


def _cmul(a, b):
    return a[0] * b[0] - a[1] * b[1], a[0] * b[1] + a[1] * b[0]


def _csq(a):
    return a[0] * a[0] - a[1] * a[1], (a[0] + a[0]) * a[1]


def _silu(x):
    h = 0.5 * x
    return h + h * jnp.tanh(h)


def _rnd(x):
    return x.astype(bf16).astype(f32)


def _dot(a, b):
    return jnp.dot(a, b, preferred_element_type=f32)


def _dot_nt(a, b):
    return lax.dot_general(a, b, (((1,), (1,)), ((), ())), preferred_element_type=f32)


def _column(v):
    return jnp.broadcast_to(v.reshape(1, _D), (_T, _D)).T


def _even_odd(x):
    b = pltpu.bitcast(x, i32)
    return pltpu.bitcast(b << 16, f32), pltpu.bitcast(b & -65536, f32)


def _interleave(even, odd):
    return pltpu.bitcast(pltpu.pack_elementwise([even, odd], packed_dtype=bf16), i32)


def _fine_powers(dt, ar, ai, br, bi, cr, ci):
    zr, zi = dt * ar, dt * ai
    w = _cmul((cr, ci), (dt * br, dt * bi))
    mag = jnp.exp(zr)
    a1 = (mag * jnp.cos(zi), mag * jnp.sin(zi))
    a2 = _csq(a1)
    a4 = _csq(a2)
    a8 = _csq(a4)
    e = [(jnp.ones_like(zr), jnp.zeros_like(zr)), (a8[0], -a8[1])]
    for s in range(2, 16):
        e.append(_csq(e[s // 2]) if s % 2 == 0 else _cmul(e[s // 2], e[s - s // 2]))
    t = _csq(e[8])
    return e, [_cmul(w, a1), _cmul(w, a2), a2, a4, (t[0], -t[1])], w[0]


def _coarse_powers(g1, g2, a2, a4, a128):
    g = {(0, 1): g1, (0, 2): g2}
    for r in (3, 4):
        g[0, r] = _cmul(g[0, r - 2], a2)
    for r in (5, 6, 7, 8):
        g[0, r] = _cmul(g[0, r - 4], a4)
    mult = a128
    for j0 in (1, 2, 4, 8):
        for j in range(j0, 2 * j0):
            for r in range(_lag_step(j), 9, _lag_step(j)):
                g[j, r] = _cmul(g[j - j0, r], mult)
        mult = _csq(mult)
    return [g[k] for k in _TAPS]


def _lag_blocks(v):
    lane = lax.broadcasted_iota(i32, (8, _T), 1)
    row = lax.broadcasted_iota(i32, (8, _T), 0)
    idx_lo = (lane & ~7) + row
    idx_8 = ((_round_lag(lane, 8) - 8) & (_T - 1)) + row
    tap = {k: jnp.take_along_axis(v[8 * n:8 * n + 8], idx_8 if k[1] == 8 else idx_lo,
                                  axis=1, mode="promise_in_bounds")
           for n, k in enumerate(_TAPS)}
    blocks = []
    for j in range(_NB):
        st = _lag_step(j)
        q = _round_lag(lane, st)
        blk = tap[j, 8]
        for r in range(st, 8, st):
            blk = jnp.where((q & 7) == r, tap[j, r], blk)
        blocks.append(jnp.where(q == 0, tap[j - 1, 8] if j else jnp.zeros_like(blk), blk))
    return blocks


def _kernel(x_hbm, ar_hbm, ai_hbm, br_hbm, bi_hbm, cr_hbm, ci_hbm, ldt_hbm, dsk_hbm, wr_hbm,
            wg_hbm, wu_hbm, wd_hbm, fwd_hbm, inv_hbm, o_hbm,
            x_v, o_v, par_v, ldt_v, dsk_v, wr_v, wg_v, wu_v, wd_v, fwd_v, inv_v,
            dt_v, c0_v, k0_v, arena, s_v, e_a, seed_a, e_b, seed_b, spec_a, spec_b, sem):
    copies = {}

    def start(name, src, dst):
        copies[name] = pltpu.make_async_copy(src, dst, sem.at[len(copies)])
        copies[name].start()

    def wait(*names):
        for name in names:
            copies[name].wait()

    with jax.named_scope("init"):
        start("ldt", ldt_hbm, ldt_v)
        start("dsk", dsk_hbm, dsk_v)
        for n, src in enumerate((ar_hbm, ai_hbm, br_hbm, bi_hbm, cr_hbm, ci_hbm)):
            start(("par", n), src, par_v.at[n])
        arena[0, _ROW_W:_ROW_P] = jnp.zeros((_ROW_P - _ROW_W, 8, _T), i32)
        wait("ldt")
        start("x", x_hbm, x_v)
        start("wr", wr_hbm, wr_v)
        start("fwd", fwd_hbm, fwd_v)
        start("inv", inv_hbm, inv_v)
        dt_v[...] = _column(jnp.exp(ldt_v[...].astype(f32))).astype(bf16)
        wait("dsk")
        c0_v[...] = _column(dsk_v[...].astype(f32))
        wait(*[("par", n) for n in range(6)])
        start("wg", wg_hbm, wg_v)
        start("wu", wu_hbm, wu_v)

    def fine(grp, u, e_ref, seed_ref):
        rows = pl.ds(pl.multiple_of(grp * 16, 16), 16)
        par = [_even_odd(dt_v[rows, :])] + [_even_odd(par_v[n, rows, :]) for n in range(6)]
        for h in range(2):
            e, seeds, w_re = _fine_powers(*[p[h] for p in par])
            for p in range(2):
                e_ref[u, h, p] = jnp.concatenate([x[p] for x in e], axis=0)
                seed_ref[u, h, p] = jnp.concatenate([x[p] for x in seeds], axis=0)
            k0_v[pl.ds(grp * 16 + h, 8, stride=2), :] = jnp.broadcast_to(
                jnp.sum(w_re, axis=1, keepdims=True), (8, _T))

    def coarse(chunk, row0, u, e_ref, seed_ref):
        v = []
        for h in range(2):
            g = _coarse_powers(*[(seed_ref[u, h, 0, 8 * n:8 * n + 8], seed_ref[u, h, 1, 8 * n:8 * n + 8])
                                 for n in range(5)])
            v.append(_dot_nt(jnp.concatenate([x[0] for x in g], axis=0), e_ref[u, h, 0])
                     + _dot_nt(jnp.concatenate([x[1] for x in g], axis=0), e_ref[u, h, 1]))
        for j, blk in enumerate(_lag_blocks(_interleave(*v))):
            arena[chunk, _ROW_K + row0 + j] = blk

    def phase_a(i, carry):
        for half, (cur, nxt) in enumerate((((e_a, seed_a), (e_b, seed_b)),
                                           ((e_b, seed_b), (e_a, seed_a)))):
            for u in range(_GA):
                n = half * _GA + u
                coarse(i * (2 * _GA // _GC) + n // _GC, (n % _GC) * _NB, u, *cur)
                fine(jnp.minimum(i * 2 * _GA + n + _GA, _NG - 1), u, *nxt)
        return carry

    with jax.named_scope("A"):
        for u in range(_GA):
            fine(u, u, e_a, seed_a)
        lax.fori_loop(0, _NG // (2 * _GA), phase_a, 0)

    def xn_block(b):
        return pltpu.bitcast(
            jnp.concatenate([arena[g // _GC, _ROW_X + (g % _GC) * _NB + b] for g in range(_NG)],
                            axis=0), bf16)

    ones = jnp.ones((8, _D), bf16)
    wt = 2

    def phase_b(i, carry):
        x = x_v[:, pl.ds(pl.multiple_of(i * wt * _T, wt * _T), wt * _T)]
        mean = _dot(ones, x)[0:1] / _D
        m = _rnd(mean)
        xc = x.astype(f32) - m
        var = jnp.sum(xc * xc, axis=0, keepdims=True) / _D - (mean - m) * (mean - m)
        sd = _rnd(jnp.sqrt(_rnd(_rnd(jnp.maximum(var, 0.0)) + _rnd(jnp.full_like(var, _EPS)))))
        xn = pltpu.bitcast((xc * (1.0 / sd)).astype(bf16), i32)
        for g in range(_NG):
            for b in range(wt):
                arena[g // _GC, _ROW_X + (g % _GC) * _NB + i * wt + b] = (
                    xn[8 * g:8 * g + 8, b * _T:(b + 1) * _T])
        return carry

    with jax.named_scope("B"):
        wait("x", "wr", "fwd", "inv")
        lax.fori_loop(0, _L // (wt * _T), phase_b, 0)

    def spectra(rows, dst):
        z = _dot(jnp.concatenate(rows, axis=0), fwd_v[...])
        for is_x in range(2):
            for h in range(2 * _GC):
                o = (is_x * _R + (h // 2) * _NB) * 16 + 8 * (h % 2)
                t = [(z[o + 16 * b:o + 16 * b + 8, :_T], z[o + 16 * b:o + 16 * b + 8, _T:])
                     for b in range(_NB)]
                if is_x:
                    t = [t[0]] + [(t[b][0] + t[b - 1][1], t[b][1] - t[b - 1][0])
                                  for b in range(1, _NB)]
                for b, (re, im) in enumerate(t):
                    planes = (re + im, im, re) if is_x else (re, re + im, im - re)
                    for p, val in enumerate(planes):
                        dst[(h * 6 + is_x * 3 + p) * _NB + b] = val

    def w_row(c, r):
        return jnp.concatenate(
            [pltpu.bitcast(arena[c, _ROW_W + q * 2 * _R + r], f32) for q in range(2)], axis=1)

    with jax.named_scope("topk"):
        xn = jnp.concatenate([xn_block(b) for b in range(_NB)], axis=1)
        wr = jnp.broadcast_to(wr_v[...].astype(f32).reshape(1, _D), (8, _D)).astype(bf16)
        score = _rnd(_dot(wr, xn)) + 0.0
        spectra([pltpu.bitcast(arena[0, r], bf16) for r in range(2 * _R)], spec_a)
        bits = pltpu.bitcast(score, i32) >> 16
        rank = jnp.where(bits < 0, ~bits, bits + 0x8000)
        tok = lax.broadcasted_iota(i32, (8, _L), 1)
        key = pltpu.bitcast((1 << 28) + rank * _L + (_L - 1 - tok), f32)
        row = lax.broadcasted_iota(i32, (8, _T), 0)
        live = []
        for h in range(_NB // 8):
            t = key[:, 8 * h * _T:(8 * h + 1) * _T]
            for s in range(1, 8):
                t = jnp.where(row == s, key[:, (8 * h + s) * _T:(8 * h + s + 1) * _T], t)
            live.append(t)
        top = jnp.zeros((8, _T), f32)
        for c in range(_C):
            best = jnp.max(jnp.max(jnp.maximum(live[0], live[1]), axis=0, keepdims=True),
                           axis=1, keepdims=True)
            top = jnp.where(row == c, best, top)
            live = [jnp.where(t == best, 0.0, t) for t in live]
        onehot = jnp.concatenate(
            [jnp.where(key[:, b * _T:(b + 1) * _T] == top, 1.0, 0.0) for b in range(_NB)],
            axis=1).astype(bf16)
        top_rank = (pltpu.bitcast(top, i32) - (1 << 28)) >> 11
        top_score = pltpu.bitcast(
            jnp.where(top_rank >= 0x8000, top_rank - 0x8000, ~top_rank) << 16, f32)
        route_w = _rnd(jax.nn.sigmoid(top_score))
        x_sel = _dot_nt(onehot, xn).astype(bf16)

    def conv_step(c, cur, nxt):
        c_next, c_prev = jnp.minimum(c + 1, _NCH - 1), jnp.maximum(c - 1, 0)
        zero = c >> 8
        fwd_rows, inv_rows = [None] * (2 * _R), [None] * (2 * _R)
        todo = sorted([(8 * r, 0, r) for r in range(2 * _R)]
                      + [(16 * (_R + r if r < _R // 2 else r - _R // 2), 1, r) for r in range(2 * _R)])
        pace = 0.95 * (3 * _NB * (_NB + 1) * _GC) / (24 * _R)

        def read_operands(done):
            while todo and done >= (todo[0][0] - 128) * pace:
                _, is_fwd, r = todo.pop(0)
                if is_fwd:
                    fwd_rows[r] = pltpu.bitcast(arena[c_next, r], bf16)
                else:
                    inv_rows[r] = w_row(c_prev, r)

        done = 0
        read_operands(done)
        for h in range(2 * _GC):
            for p in range(3):
                k, u = [], []
                for lo, hi in ((0, 9), (9, 13), (13, 16)):
                    base = {b: pltpu.bitcast(arena[c + zero, _ROW_P + b], f32)
                            for b in range(lo, hi) if p}
                    for b in range(lo, hi):
                        k.append(cur[zero + (h * 6 + p) * _NB + b])
                        u.append(cur[zero + (h * 6 + 3 + p) * _NB + b])
                        acc = k[0] * u[b]
                        for j in range(1, b + 1):
                            acc = acc + k[j] * u[b - j]
                        if p == 0:
                            arena[c, _ROW_P + b] = pltpu.bitcast(acc, i32)
                        else:
                            arena[c, _ROW_W + (p - 1) * 2 * _R + ((h // 2) * _NB + b) * 2 + h % 2] = (
                                pltpu.bitcast(base[b] - acc if p == 1 else base[b] + acc, i32))
                        done += b + 1
                    read_operands(done)
        assert not todo
        s_v[c_prev] = _dot(jnp.concatenate(inv_rows, axis=0), inv_v[...])
        spectra(fwd_rows, nxt)

    def phase_c(i, carry):
        pl.when(i % 2 == 0)(lambda: conv_step(i, spec_a, spec_b))
        pl.when(i % 2 == 1)(lambda: conv_step(i, spec_b, spec_a))
        return carry

    with jax.named_scope("C"):
        for n, (r0, nr) in enumerate(_OUT_CHUNKS):
            start(("wd", n), wd_hbm.at[pl.ds(r0, nr)], wd_v.at[pl.ds(r0, nr)])
        lax.fori_loop(0, _NCH, phase_c, 0)

    with jax.named_scope("G"):
        s_v[_NCH - 1] = _dot(
            jnp.concatenate([w_row(_NCH - 1, r) for r in range(2 * _R)], axis=0), inv_v[...])
        wait("wg", "wu")
        gate = _rnd(_silu(_rnd(_dot(x_sel, wg_v[...]))))
        hid = (gate * _rnd(_dot(x_sel, wu_v[...]))).astype(bf16)

    for n, (r0, nr) in enumerate(_OUT_CHUNKS):
      with jax.named_scope("D%d" % n):
        wait(("wd", n))
        y = _rnd(_dot_nt(hid, wd_v[pl.ds(r0, nr), :])) * route_w[:, :nr]
        upd = _dot(y.T.astype(bf16), onehot)
        for g in range(r0 // 16, (r0 + nr) // 16):
            rows = pl.ds(16 * g, 16)
            c0 = c0_v[rows, :] + k0_v[rows, :]
            for b in range(_NB):
                cols = pl.ds(b * _T, _T)
                r = (g % _GC) * _NB + b
                xn_t = pltpu.bitcast(arena[g // _GC, _ROW_X + r], bf16).astype(f32)
                s = s_v[g // _GC, pl.ds(16 * r, 16), :] + xn_t * c0
                gated = _silu(xn_t + upd[16 * g - r0:16 * g - r0 + 16, b * _T:(b + 1) * _T])
                o_v[rows, cols] = (x_v[rows, cols].astype(f32) + s * gated).astype(bf16)
        start(("o", n), o_v.at[pl.ds(r0, nr)], o_hbm.at[pl.ds(r0, nr)])
    with jax.named_scope("end"):
        wait(*[("o", n) for n in range(len(_OUT_CHUNKS))])


@jax.jit
def pallas_recurrent_scan__ssm_conv_s4__moe_arch_mod__prompt_kernel(
    A_u: jax.Array,
    A_A_re: jax.Array,
    A_A_im: jax.Array,
    A_B_re: jax.Array,
    A_B_im: jax.Array,
    A_C_re: jax.Array,
    A_C_im: jax.Array,
    A_log_dt: jax.Array,
    A_Dskip: jax.Array,
    B_x: jax.Array,
    B_w_r: jax.Array,
    B_w_gate: jax.Array,
    B_w_up: jax.Array,
    B_w_down: jax.Array,
):
    del B_x
    assert A_u.shape == (1, _L, _D) and A_A_re.shape == (_D, _N) and B_w_gate.shape == (_D, _F)
    assert A_u.dtype == bf16 and A_A_re.dtype == bf16
    hbm = pl.BlockSpec(memory_space=pl.ANY)
    vmem = pltpu.VMEM
    out = pl.pallas_call(
        _kernel,
        out_shape=jax.ShapeDtypeStruct((_D, _L), bf16),
        in_specs=[hbm] * 15,
        out_specs=hbm,
        scratch_shapes=[
            vmem((_D, _L), bf16), vmem((_D, _L), bf16),
            vmem((6, _D, _N), bf16), vmem((_D,), bf16), vmem((_D,), bf16), vmem((_D,), bf16),
            vmem((_D, _F), bf16), vmem((_D, _F), bf16), vmem((_D, _F), bf16),
            vmem((_T, 2 * _T), bf16), vmem((2 * _T, _T), f32),
            vmem((_D, _T), bf16), vmem((_D, _T), f32), vmem((_D, _T), f32),
            vmem((_NCH, _ROWS, 8, _T), i32), vmem((_NCH, 16 * _R, _T), f32),
            *[vmem((_GA, 2, 2, _T, _N), f32), vmem((_GA, 2, 2, 40, _N), f32)] * 2,
            *[vmem((2 * _GC * 6 * _NB, 8, _T), f32)] * 2,
            pltpu.SemaphoreType.DMA((14 + 2 * len(_OUT_CHUNKS),)),
        ],
        compiler_params=pltpu.CompilerParams(vmem_limit_bytes=100 * 2**20),
    )(A_u.reshape(_L, _D).T, A_A_re, A_A_im, A_B_re, A_B_im, A_C_re, A_C_im, A_log_dt, A_Dskip,
      B_w_r, B_w_gate, B_w_up, B_w_down.T, _FWD, _INV)
    return out.T.reshape(1, _L, _D)
```

```python
import jax
import jax.numpy as jnp
import numpy as np
from jax import lax
import jax.experimental.pallas as pl
import jax.experimental.pallas.tpu as pltpu

_D, _L, _N, _F, _C = 576, 2048, 128, 4608, 8
_T = 128
_NB = _L // _T
_EPS = 1e-5
_GA = 4
_GC = 2
_NG = _D // 16
_NCH = _NG // _GC
_R = _GC * _NB
_ROW_K, _ROW_X, _ROW_W, _ROW_P, _ROWS = 0, _R, 2 * _R, 6 * _R, 6 * _R + _NB
_OUT_CHUNKS = ((0, 128), (128, 128), (256, 128), (384, 128), (512, 64))

f32, bf16, i32 = jnp.float32, jnp.bfloat16, jnp.int32


def _dft_constants():
    theta = (np.pi / 2 + 2 * np.pi * np.arange(_T)) / _T
    ang = np.arange(_T)[:, None] * theta[None, :]
    c, s = np.cos(ang), np.sin(ang)
    fwd = np.concatenate([c, s], axis=1)
    return fwd.astype(bf16), (fwd.T / _T).astype(np.float32)


_FWD, _INV = _dft_constants()


def _lag_step(j):
    return max(1, (1 << (j * _T).bit_length()) >> 8)


def _round_lag(p, st):
    if st == 1:
        return p
    return (p + (st // 2 - 1) + ((p >> (st.bit_length() - 1)) & 1)) & ~(st - 1)


assert np.array_equal(
    np.concatenate([j * _T + _round_lag(np.arange(_T), _lag_step(j)) for j in range(_NB)]),
    np.arange(_L).astype(bf16).astype(np.int64))

_PAIRS = (((0, 1), (0, 5)), ((0, 2), (0, 6)), ((0, 3), (0, 7)), ((0, 4), (0, 8)), ((1, 2), (1, 6)),
          ((1, 4), (1, 8)), ((2, 4), (2, 8)), ((3, 4), (3, 8)), ((4, 8), (5, 8)), ((6, 8), (7, 8)))
_TAPS = [k for pair in _PAIRS for k in pair]


def _cmul(a, b):
    return a[0] * b[0] - a[1] * b[1], a[0] * b[1] + a[1] * b[0]


def _csq(a):
    return a[0] * a[0] - a[1] * a[1], (a[0] + a[0]) * a[1]


def _silu(x):
    h = 0.5 * x
    return h + h * jnp.tanh(h)


def _rnd(x):
    return x.astype(bf16).astype(f32)


def _dot(a, b):
    return jnp.dot(a, b, preferred_element_type=f32)


def _dot_nt(a, b):
    return lax.dot_general(a, b, (((1,), (1,)), ((), ())), preferred_element_type=f32)


def _column(v):
    return jnp.broadcast_to(v.reshape(1, _D), (_T, _D)).T


def _even_odd(x):
    b = pltpu.bitcast(x, i32)
    return pltpu.bitcast(b << 16, f32), pltpu.bitcast(b & -65536, f32)


def _interleave(even, odd):
    return pltpu.bitcast(pltpu.pack_elementwise([even, odd], packed_dtype=bf16), i32)


def _modes(dt, ar, ai, br, bi, cr, ci):
    zr, zi = dt * ar, dt * ai
    mag = jnp.exp(zr)
    return _cmul((cr, ci), (dt * br, dt * bi)) + (mag * jnp.cos(zi), mag * jnp.sin(zi))


def _vandermonde(w, a1):
    row = lax.broadcasted_iota(i32, (8, _N), 0)
    a = {1: a1}
    for n in range(9):
        a[2 << n] = _csq(a[1 << n])

    def conj(z):
        return z[0], -z[1]

    def mix(z0, z1):
        rolled = [pltpu.roll(x, 4, 0) for x in z1]
        return ([jnp.where(row < 4, x, y) for x, y in zip(z0, rolled)],
                [jnp.where(row < 4, y, x) for x, y in zip(z0, rolled)])

    def dup(z):
        return [[jnp.take_along_axis(x, (row & 3) + 4 * q, axis=0, mode="promise_in_bounds")
                 for x in z] for q in range(2)]

    def stack(zs, p):
        return jnp.concatenate([z[p] for z in zs], axis=0)

    wa = _cmul(w, a1)
    out = []
    for e0, m8, m32, g0, m1, m256, m_top, m512 in zip(
            mix((1.0, 0.0), conj(a[128])), dup(conj(a[8])), dup(conj(a[32])),
            mix(wa, _cmul(wa, a[4])), dup(a1), dup(a[256]),
            mix(_cmul(a[256], a[4]), a[512]), dup(a[512])):
        e = [e0]
        for s in range(1, 16):
            e.append(_cmul(e[s - 1], m8) if s < 4 else _cmul(e[s - 4], m32))
        g = [g0]
        for _ in range(3):
            g.append(_cmul(g[-1], m1))
        g += [_cmul(g[1], m256), _cmul(g[3], m256)]
        g += [_cmul(g[3], m512), _cmul(g[5], m512)]
        g.append(_cmul(g[7], m_top))
        g.append(_cmul(g[8], m512))
        out.append(_dot_nt(stack(g, 0), stack(e, 0)) + _dot_nt(stack(g, 1), stack(e, 1)))
    return out


def _unmix(lo, hi):
    row = lax.broadcasted_iota(i32, (8, _T), 0)
    out = []
    for m in range(len(_PAIRS)):
        x, y = lo[8 * m:8 * m + 8], hi[8 * m:8 * m + 8]
        out += [jnp.where(row < 4, x, y), pltpu.roll(jnp.where(row < 4, y, x), 4, 0)]
    return out


def _lag_blocks(tap, store):
    lane = lax.broadcasted_iota(i32, (8, _T), 1)
    row = lax.broadcasted_iota(i32, (8, _T), 0)
    for h in range(2):
        def take(big, r, fine):
            s = ((_T * h + fine) >> 3) & 31
            return jnp.take_along_axis(tap(_TAPS.index((big, r))),
                                       ((s & 15) << 3) + (row ^ ((s >> 4) << 2)),
                                       axis=1, mode="promise_in_bounds")

        top = [take(big, 8, _round_lag(lane, 8) - 8) for big in range(_NB // 2)]
        for big, blk in enumerate(top):
            st = _lag_step(2 * big + h)
            lag = _round_lag(lane, st)
            if h == 0:
                blk = jnp.where(lag == 0, top[big - 1] if big else jnp.zeros_like(blk), blk)
            for r in range(st, 8, st):
                blk = jnp.where((lag & 7) == r, take(big, r, lane), blk)
            store(2 * big + h, blk)


def _kernel(x_hbm, ar_hbm, ai_hbm, br_hbm, bi_hbm, cr_hbm, ci_hbm, ldt_hbm, dsk_hbm, wr_hbm,
            wg_hbm, wu_hbm, wd_hbm, fwd_hbm, inv_hbm, o_hbm,
            x_v, o_v, par_v, ldt_v, dsk_v, wr_v, wg_v, wu_v, wd_v, fwd_v, inv_v,
            dt_v, c0_v, k0_v, arena, s_v, mode_v, tap_v, xc_v, stat_v, spec_a, spec_b, sem):
    copies = {}

    def start(name, src, dst):
        copies[name] = pltpu.make_async_copy(src, dst, sem.at[len(copies)])
        copies[name].start()

    def wait(*names):
        for name in names:
            copies[name].wait()

    with jax.named_scope("init"):
        start("ldt", ldt_hbm, ldt_v)
        start("dsk", dsk_hbm, dsk_v)
        for n, src in enumerate((ar_hbm, ai_hbm, br_hbm, bi_hbm, cr_hbm, ci_hbm)):
            start(("par", n), src, par_v.at[n])
        arena[0, _ROW_W:_ROW_P] = jnp.zeros((_ROW_P - _ROW_W, 8, _T), i32)
        tap_v[...] = jnp.zeros(tap_v.shape, i32)
        wait("ldt")
        start("x", x_hbm, x_v)
        start("wr", wr_hbm, wr_v)
        start("fwd", fwd_hbm, fwd_v)
        start("inv", inv_hbm, inv_v)
        dt_v[...] = _column(jnp.exp(ldt_v[...].astype(f32))).astype(bf16)
        wait("dsk")
        c0_v[...] = _column(dsk_v[...].astype(f32))
        wait(*[("par", n) for n in range(6)])
        start("wg", wg_hbm, wg_v)
        start("wu", wu_hbm, wu_v)

    def modes(step):
        for u in range(_GA):
            grp = step * _GA + u
            rows = pl.ds(pl.multiple_of(grp * 16, 16), 16)
            par = [_even_odd(dt_v[rows, :])] + [_even_odd(par_v[n, rows, :]) for n in range(6)]
            for h in range(2):
                z = _modes(*[p[h] for p in par])
                for n in range(4):
                    mode_v[u, h, n] = z[n]
                k0_v[pl.ds(grp * 16 + h, 8, stride=2), :] = jnp.broadcast_to(
                    jnp.sum(z[0], axis=1, keepdims=True), (8, _T))

    def spread(step):
        for u in range(_GA):
            def store(j, blk):
                arena[step * (_GA // _GC) + u // _GC, _ROW_K + (u % _GC) * _NB + j] = blk
            _lag_blocks(lambda n: tap_v[u, n], store)

    def phase_a(i, carry):
        spread(jnp.maximum(i - 1, 0))
        for u in range(_GA):
            even, odd = [_vandermonde((mode_v[u, h, 0], mode_v[u, h, 1]),
                                      (mode_v[u, h, 2], mode_v[u, h, 3])) for h in range(2)]
            for n, v in enumerate(_unmix(_interleave(even[0], odd[0]), _interleave(even[1], odd[1]))):
                tap_v[u, n] = v
        modes(jnp.minimum(i + 1, _NG // _GA - 1))
        return carry

    with jax.named_scope("A"):
        modes(0)
        lax.fori_loop(0, _NG // _GA, phase_a, 0)

    def centre(b):
        mean = stat_v[0, b] / _D
        m = _rnd(mean)
        acc = [None] * 4
        for g in range(_NG):
            x = x_v[pl.ds(16 * g, 16), pl.ds(pl.multiple_of(b * _T, _T), _T)]
            for h, xh in enumerate(_even_odd(x)):
                xc = xh - m
                xc_v[2 * g + h] = xc
                n = (2 * g + h) % 4
                acc[n] = xc * xc if acc[n] is None else acc[n] + xc * xc
        var = jnp.sum((acc[0] + acc[1]) + (acc[2] + acc[3]), axis=0, keepdims=True) / _D
        var = jnp.maximum(var - (mean - m) * (mean - m), 0.0)
        return 1.0 / _rnd(jnp.sqrt(_rnd(_rnd(var) + _rnd(jnp.full_like(var, _EPS)))))

    def phase_b(b, inv_sd):
        xn = [_interleave(xc_v[2 * g] * inv_sd, xc_v[2 * g + 1] * inv_sd) for g in range(_NG)]
        for g in range(_NG):
            arena[g // _GC, _ROW_X + (g % _GC) * _NB + b] = xn[g]
        stat_v[1, b] = _dot(wr, pltpu.bitcast(jnp.concatenate(xn, axis=0), bf16))
        return centre(jnp.minimum(b + 1, _NB - 1))

    with jax.named_scope("B"):
        wait("x", "wr", "fwd", "inv")
        spread(_NG // _GA - 1)
        wr = jnp.broadcast_to(wr_v[...].astype(f32).reshape(1, _D), (8, _D)).astype(bf16)
        total = _dot(jnp.ones((8, _D), bf16), x_v[...])
        for b in range(_NB):
            stat_v[0, b] = total[:, b * _T:(b + 1) * _T]
        lax.fori_loop(0, _NB, phase_b, centre(0))

    def spectra(rows, dst):
        z = _dot(jnp.concatenate(rows, axis=0), fwd_v[...])
        for is_x in range(2):
            for h in range(2 * _GC):
                o = (is_x * _R + (h // 2) * _NB) * 16 + 8 * (h % 2)
                t = [(z[o + 16 * b:o + 16 * b + 8, :_T], z[o + 16 * b:o + 16 * b + 8, _T:])
                     for b in range(_NB)]
                if is_x:
                    t = [t[0]] + [(t[b][0] + t[b - 1][1], t[b][1] - t[b - 1][0])
                                  for b in range(1, _NB)]
                for b, (re, im) in enumerate(t):
                    planes = (re + im, im, re) if is_x else (re, re + im, im - re)
                    for p, val in enumerate(planes):
                        dst[(h * 6 + is_x * 3 + p) * _NB + b] = val

    def w_row(c, r):
        return jnp.concatenate(
            [pltpu.bitcast(arena[c, _ROW_W + q * 2 * _R + r], f32) for q in range(2)], axis=1)

    with jax.named_scope("topk"):
        spectra([pltpu.bitcast(arena[0, r], bf16) for r in range(2 * _R)], spec_a)
        row = lax.broadcasted_iota(i32, (8, _T), 0)
        lane = lax.broadcasted_iota(i32, (8, _T), 1)
        live = []
        for h in range(_NB // 8):
            score = stat_v[1, 8 * h]
            for s in range(1, 8):
                score = jnp.where(row == s, stat_v[1, 8 * h + s], score)
            bits = pltpu.bitcast(_rnd(score) + 0.0, i32) >> 16
            rank = jnp.where(bits < 0, ~bits, bits + 0x8000)
            token = (8 * h + row) * _T + lane
            live.append(pltpu.bitcast((1 << 28) + rank * _L + (_L - 1 - token), f32))
        top = jnp.zeros((8, _T), f32)
        for c in range(_C):
            best = jnp.max(jnp.max(jnp.maximum(live[0], live[1]), axis=0, keepdims=True),
                           axis=1, keepdims=True)
            top = jnp.where(row == c, best, top)
            live = [jnp.where(t == best, 0.0, t) for t in live]
        top = pltpu.bitcast(top, i32) - (1 << 28)
        top_token = _L - 1 - (top & (_L - 1))
        top_rank = top >> 11
        top_score = pltpu.bitcast(
            jnp.where(top_rank >= 0x8000, top_rank - 0x8000, ~top_rank) << 16, f32)
        route_w = _rnd(jax.nn.sigmoid(top_score))
        onehot = jnp.concatenate(
            [jnp.where(top_token == b * _T + lane, 1.0, 0.0) for b in range(_NB)], axis=1)
        blocks = [top_token[c, 0] >> 7 for c in range(_C)]
        routed = jnp.concatenate(
            [pltpu.bitcast(jnp.concatenate(
                [arena[g // _GC, _ROW_X + (g % _GC) * _NB + b] for g in range(_NG)], axis=0), bf16)
             for b in blocks], axis=1)
        pick = jnp.concatenate(
            [jnp.where((row == c) & ((top_token & (_T - 1)) == lane), 1.0, 0.0) for c in range(_C)],
            axis=1).astype(bf16)
        x_sel = _dot_nt(pick, routed).astype(bf16)

    def conv_step(c, cur, nxt):
        c_next, c_prev = jnp.minimum(c + 1, _NCH - 1), jnp.maximum(c - 1, 0)
        zero = c >> 8
        fwd_rows, inv_rows = [None] * (2 * _R), [None] * (2 * _R)
        todo = sorted([(8 * r, 0, r) for r in range(2 * _R)]
                      + [(16 * (_R + r if r < _R // 2 else r - _R // 2), 1, r) for r in range(2 * _R)])
        pace = 0.95 * (3 * _NB * (_NB + 1) * _GC) / (24 * _R)

        def read_operands(done):
            while todo and done >= (todo[0][0] - 128) * pace:
                _, is_fwd, r = todo.pop(0)
                if is_fwd:
                    fwd_rows[r] = pltpu.bitcast(arena[c_next, r], bf16)
                else:
                    inv_rows[r] = w_row(c_prev, r)

        done = 0
        read_operands(done)
        for h in range(2 * _GC):
            for p in range(3):
                k, u = [], []
                for lo, hi in ((0, 9), (9, 13), (13, 16)):
                    base = {b: pltpu.bitcast(arena[c + zero, _ROW_P + b], f32)
                            for b in range(lo, hi) if p}
                    for b in range(lo, hi):
                        k.append(cur[zero + (h * 6 + p) * _NB + b])
                        u.append(cur[zero + (h * 6 + 3 + p) * _NB + b])
                        acc = k[0] * u[b]
                        for j in range(1, b + 1):
                            acc = acc + k[j] * u[b - j]
                        if p == 0:
                            arena[c, _ROW_P + b] = pltpu.bitcast(acc, i32)
                        else:
                            arena[c, _ROW_W + (p - 1) * 2 * _R + ((h // 2) * _NB + b) * 2 + h % 2] = (
                                pltpu.bitcast(base[b] - acc if p == 1 else base[b] + acc, i32))
                        done += b + 1
                    read_operands(done)
        assert not todo
        s_v[c_prev] = _dot(jnp.concatenate(inv_rows, axis=0), inv_v[...])
        spectra(fwd_rows, nxt)

    def phase_c(i, carry):
        pl.when(i % 2 == 0)(lambda: conv_step(i, spec_a, spec_b))
        pl.when(i % 2 == 1)(lambda: conv_step(i, spec_b, spec_a))
        return carry

    with jax.named_scope("C"):
        for n, (r0, nr) in enumerate(_OUT_CHUNKS):
            start(("wd", n), wd_hbm.at[pl.ds(r0, nr)], wd_v.at[pl.ds(r0, nr)])
        lax.fori_loop(0, _NCH, phase_c, 0)

    with jax.named_scope("G"):
        s_v[_NCH - 1] = _dot(
            jnp.concatenate([w_row(_NCH - 1, r) for r in range(2 * _R)], axis=0), inv_v[...])
        wait("wg", "wu")
        gate = _rnd(_silu(_rnd(_dot(x_sel, wg_v[...]))))
        hid = (gate * _rnd(_dot(x_sel, wu_v[...]))).astype(bf16)

    for n, (r0, nr) in enumerate(_OUT_CHUNKS):
      with jax.named_scope("D%d" % n):
        wait(("wd", n))
        y = _rnd(_dot_nt(hid, wd_v[pl.ds(r0, nr), :])) * route_w[:, :nr]
        upd = _dot(_rnd(y).T, onehot)
        for g in range(r0 // 16, (r0 + nr) // 16):
            rows = pl.ds(16 * g, 16)
            c0 = c0_v[rows, :] + k0_v[rows, :]
            for b in range(_NB):
                cols = pl.ds(b * _T, _T)
                r = (g % _GC) * _NB + b
                xn_t = pltpu.bitcast(arena[g // _GC, _ROW_X + r], bf16).astype(f32)
                s = s_v[g // _GC, pl.ds(16 * r, 16), :] + xn_t * c0
                gated = _silu(xn_t + upd[16 * g - r0:16 * g - r0 + 16, b * _T:(b + 1) * _T])
                o_v[rows, cols] = (x_v[rows, cols].astype(f32) + s * gated).astype(bf16)
        start(("o", n), o_v.at[pl.ds(r0, nr)], o_hbm.at[pl.ds(r0, nr)])
    with jax.named_scope("end"):
        wait(*[("o", n) for n in range(len(_OUT_CHUNKS))])


@jax.jit
def pallas_recurrent_scan__ssm_conv_s4__moe_arch_mod__prompt_kernel(
    A_u: jax.Array,
    A_A_re: jax.Array,
    A_A_im: jax.Array,
    A_B_re: jax.Array,
    A_B_im: jax.Array,
    A_C_re: jax.Array,
    A_C_im: jax.Array,
    A_log_dt: jax.Array,
    A_Dskip: jax.Array,
    B_x: jax.Array,
    B_w_r: jax.Array,
    B_w_gate: jax.Array,
    B_w_up: jax.Array,
    B_w_down: jax.Array,
):
    del B_x
    assert A_u.shape == (1, _L, _D) and A_A_re.shape == (_D, _N) and B_w_gate.shape == (_D, _F)
    assert A_u.dtype == bf16 and A_A_re.dtype == bf16
    hbm = pl.BlockSpec(memory_space=pl.ANY)
    vmem = pltpu.VMEM
    out = pl.pallas_call(
        _kernel,
        out_shape=jax.ShapeDtypeStruct((_D, _L), bf16),
        in_specs=[hbm] * 15,
        out_specs=hbm,
        scratch_shapes=[
            vmem((_D, _L), bf16), vmem((_D, _L), bf16),
            vmem((6, _D, _N), bf16), vmem((_D,), bf16), vmem((_D,), bf16), vmem((_D,), bf16),
            vmem((_D, _F), bf16), vmem((_D, _F), bf16), vmem((_D, _F), bf16),
            vmem((_T, 2 * _T), bf16), vmem((2 * _T, _T), f32),
            vmem((_D, _T), bf16), vmem((_D, _T), f32), vmem((_D, _T), f32),
            vmem((_NCH, _ROWS, 8, _T), i32), vmem((_NCH, 16 * _R, _T), f32),
            vmem((_GA, 2, 4, 8, _N), f32), vmem((_GA, len(_TAPS), 8, _T), i32),
            vmem((2 * _NG, 8, _T), f32), vmem((2, _NB, 8, _T), f32),
            *[vmem((2 * _GC * 6 * _NB, 8, _T), f32)] * 2,
            pltpu.SemaphoreType.DMA((14 + 2 * len(_OUT_CHUNKS),)),
        ],
        compiler_params=pltpu.CompilerParams(vmem_limit_bytes=100 * 2**20),
    )(A_u.reshape(_L, _D).T, A_A_re, A_A_im, A_B_re, A_B_im, A_C_re, A_C_im, A_log_dt, A_Dskip,
      B_w_r, B_w_gate, B_w_up, B_w_down.T, _FWD, _INV)
    return out.T.reshape(1, _L, _D)
```

```python
import jax
import jax.numpy as jnp
import numpy as np
from jax import lax
import jax.experimental.pallas as pl
import jax.experimental.pallas.tpu as pltpu

_D, _L, _N, _F, _C = 576, 2048, 128, 4608, 8
_T = 128
_NB = _L // _T
_EPS = 1e-5
_GA = 4
_GC = 2
_NG = _D // 16
_NCH = _NG // _GC
_R = _GC * _NB
_ROW_X, _ROW_W, _ROW_P, _ROWS = 0, _R, 5 * _R + 8, 5 * _R + 8 + 24
_PLANE, _WQ = _NB + 2, 2 * _R + 2
_NO, _TAIL = divmod(_D, _T)
_NF = 3
_FCH = _F // _NF
_LN_STEP = 4
_WD_STEP = 1
_PACE, _LEAD, _G0 = 0.8, 32, 160
_KU, _KP, _KARA, _KB = 4, 3, 1, ((0, 4), (4, 6), (6, 8))
_ROW_SEL = 5 * _R + 3
_LAG = 140
_DSTEP = 14
_BATCH = ((0, 9), (9, 13), (13, 16))

f32, bf16, i32 = jnp.float32, jnp.bfloat16, jnp.int32


def _dft_constants():
    theta = (np.pi / 2 + 2 * np.pi * np.arange(_T)) / _T
    ang = np.arange(_T)[:, None] * theta[None, :]
    c, s = np.cos(ang), np.sin(ang)
    fwd = np.concatenate([c, s], axis=1)
    return fwd.astype(bf16), (fwd.T * (2 / _T)).astype(np.float32)


_FWD, _INV = _dft_constants()


def _lag_step(j):
    return max(1, (1 << (j * _T).bit_length()) >> 8)


def _round_lag(p, st):
    if st == 1:
        return p
    return (p + (st // 2 - 1) + ((p >> (st.bit_length() - 1)) & 1)) & ~(st - 1)


assert np.array_equal(
    np.concatenate([j * _T + _round_lag(np.arange(_T), _lag_step(j)) for j in range(_NB)]),
    np.arange(_L).astype(bf16).astype(np.int64))

_PAIRS = (((0, 1), (0, 5)), ((0, 2), (0, 6)), ((0, 3), (0, 7)), ((0, 4), (0, 8)), ((1, 2), (1, 6)),
          ((1, 4), (1, 8)), ((2, 4), (2, 8)), ((3, 4), (3, 8)), ((4, 8), (5, 8)), ((6, 8), (7, 8)))
_TAPS = [k for pair in _PAIRS for k in pair]


def _cmul(a, b):
    return a[0] * b[0] - a[1] * b[1], a[0] * b[1] + a[1] * b[0]


def _csq(a):
    return a[0] * a[0] - a[1] * a[1], (a[0] + a[0]) * a[1]


def _silu(x):
    h = 0.5 * x
    return h + h * jnp.tanh(h)


def _rnd(x):
    return x.astype(bf16).astype(f32)


def _dot(a, b):
    return jnp.dot(a, b, preferred_element_type=f32)


def _dot_nt(a, b):
    return lax.dot_general(a, b, (((1,), (1,)), ((), ())), preferred_element_type=f32)


def _column(v):
    return jnp.broadcast_to(v.reshape(1, _D), (_T, _D)).T


def _even_odd(x):
    b = pltpu.bitcast(x, i32)
    return pltpu.bitcast(b << 16, f32), pltpu.bitcast(b & -65536, f32)


def _interleave(even, odd):
    return pltpu.bitcast(pltpu.pack_elementwise([even, odd], packed_dtype=bf16), i32)


def _modes(dt, ar, ai, br, bi, cr, ci):
    zr, zi = dt * ar, dt * ai
    mag = jnp.exp(zr)
    return _cmul((cr, ci), (dt * br, dt * bi)) + (mag * jnp.cos(zi), mag * jnp.sin(zi))


def _seeds(w, a1):
    a = {1: a1}
    for n in range(9):
        a[2 << n] = _csq(a[1 << n])
    row = lax.broadcasted_iota(i32, (8, _N), 0)

    def conj(z):
        return z[0], -z[1]

    def mix(z0, z1):
        rolled = [pltpu.roll(x, 4, 0) for x in z1]
        return ([jnp.where(row < 4, x, y) for x, y in zip(z0, rolled)],
                [jnp.where(row < 4, y, x) for x, y in zip(z0, rolled)])

    def dup(z):
        return [[jnp.take_along_axis(x, (row & 3) + 4 * q, axis=0, mode="promise_in_bounds")
                 for x in z] for q in range(2)]

    wa = _cmul(w, a[1])
    return zip(mix((1.0, 0.0), conj(a[128])), dup(conj(a[8])), dup(conj(a[32])),
               mix(wa, _cmul(wa, a[4])), dup(a[1]), dup(a[256]),
               mix(_cmul(a[256], a[4]), a[512]), dup(a[512]))


def _vandermonde(e0, m8, m32, g0, m1, m256, m_top, m512):
    e = [e0]
    for s in range(1, 16):
        e.append(_cmul(e[s - 1], m8) if s < 4 else _cmul(e[s - 4], m32))
    g = [g0]
    for _ in range(3):
        g.append(_cmul(g[-1], m1))
    g += [_cmul(g[1], m256), _cmul(g[3], m256)]
    g += [_cmul(g[3], m512), _cmul(g[5], m512)]
    g.append(_cmul(g[7], m_top))
    g.append(_cmul(g[8], m512))
    re, im = [_dot_nt(jnp.concatenate([z[p] for z in g], axis=0),
                      jnp.concatenate([z[p] for z in e], axis=0)) for p in range(2)]
    return re + im


def _unmix(lo, hi):
    row = lax.broadcasted_iota(i32, (8, _T), 0)
    out = []
    for m in range(len(_PAIRS)):
        x, y = lo[8 * m:8 * m + 8], hi[8 * m:8 * m + 8]
        out += [jnp.where(row < 4, x, y), pltpu.roll(jnp.where(row < 4, y, x), 4, 0)]
    return out


def _lag_blocks(tap, lag0):
    lane = lax.broadcasted_iota(i32, (8, _T), 1)
    row = lax.broadcasted_iota(i32, (8, _T), 0)
    for h in range(2):
        def take(big, r, fine):
            s = ((_T * h + fine) >> 3) & 31
            return jnp.take_along_axis(tap(_TAPS.index((big, r))),
                                       ((s & 15) << 3) + (row ^ ((s >> 4) << 2)),
                                       axis=1, mode="promise_in_bounds")

        top = [take(big, 8, _round_lag(lane, 8) - 8) for big in range(_NB // 2)]
        for big, blk in enumerate(top):
            st = _lag_step(2 * big + h)
            lag = _round_lag(lane, st)
            if h == 0:
                blk = jnp.where(lag == 0, top[big - 1] if big else lag0, blk)
            for r in range(st, 8, st):
                blk = jnp.where((lag & 7) == r, take(big, r, lane), blk)
            yield 2 * big + h, blk


def _kernel(x_hbm, ar_hbm, ai_hbm, br_hbm, bi_hbm, cr_hbm, ci_hbm, ldt_hbm, dsk_hbm, wr_hbm,
            wg_hbm, wu_hbm, wd_hbm, fwd_hbm, inv_hbm, o_hbm,
            x_v, o_v, par_v, ldt_v, dsk_v, wr_v, wg_v, wu_v, wd_v, fwd_v, inv_v,
            skip_v, k0_v, arena, s_v, dt_v, mode_v, tap_v, k_v, xc_v, stat_v, key_v, hid_v, y_v, col_v,
            spec_a, spec_b, kf_v, sem, w_sem, o_sem):
    row = lax.broadcasted_iota(i32, (8, _T), 0)
    lane = lax.broadcasted_iota(i32, (8, _T), 1)
    copies = {}

    def start(name, src, dst):
        copies[name] = pltpu.make_async_copy(src, dst, sem.at[len(copies)])
        copies[name].start()

    def wait(*names):
        for name in names:
            copies[name].wait()

    def hidden_copies(n):
        cols = pl.ds(pl.multiple_of(n * _FCH, _FCH), _FCH)
        return [pltpu.make_async_copy(w.at[:, cols], v.at[:, cols], w_sem.at[2 * n + k])
                for k, (w, v) in enumerate(((wg_hbm, wg_v), (wu_hbm, wu_v)))]

    def chunk_rows(n, size):
        return pl.ds(pl.multiple_of(n * _T, _T), size)

    def down_copy(n, size=_T):
        return pltpu.make_async_copy(wd_hbm.at[chunk_rows(n, size)], wd_v.at[chunk_rows(n, size)],
                                     w_sem.at[2 * _NF + n])

    def out_copy(n, size=_T):
        return pltpu.make_async_copy(o_v.at[chunk_rows(n, size)], o_hbm.at[chunk_rows(n, size)],
                                     o_sem.at[n])

    with jax.named_scope("init"):
        start("ldt", ldt_hbm, ldt_v)
        start("dsk", dsk_hbm, dsk_v)
        for part, rows in enumerate((pl.ds(0, 16 * _GA), pl.ds(16 * _GA, _D - 16 * _GA))):
            for n, src in enumerate((ar_hbm, ai_hbm, br_hbm, bi_hbm, cr_hbm, ci_hbm)):
                start((part, n), src.at[rows], par_v.at[n, rows])
        start("fwd", fwd_hbm, fwd_v)
        arena[0, _ROW_W:_ROW_P] = jnp.zeros((_ROW_P - _ROW_W, 8, _T), i32)
        tap_v[...] = jnp.zeros(tap_v.shape, i32)
        k_v[...] = jnp.zeros(k_v.shape, i32)
        key_v[...] = jnp.zeros(key_v.shape, f32)
        wait("ldt")
        dt = pltpu.bitcast(_column(jnp.exp(ldt_v[...].astype(f32))).astype(bf16), i32)
        for g in range(_NG):
            dt_v[g] = dt[8 * g:8 * g + 8]
        wait("dsk")
        skip_v[...] = _column(dsk_v[...].astype(f32)).astype(bf16)
        wait(*[(0, n) for n in range(6)])

    def compact(ref, k, h):
        out = ref[k, 8 * h]
        for s in range(1, 8):
            out = jnp.where(row == s, ref[k, 8 * h + s], out)
        return out

    def layer_norm():
        wait("x", "wr", "inv")
        for cp in hidden_copies(1):
            cp.start()

        def moments(b, carry):
            cols = pl.ds(pl.multiple_of(b * _T, _T), _T)
            pivot = jnp.broadcast_to(_even_odd(x_v[:16, cols])[0][:1], (8, _T))
            s1, s2 = [None] * 2, [None] * 2
            for g in range(_NG):
                for h, x in enumerate(_even_odd(x_v[pl.ds(16 * g, 16), cols])):
                    d = x - pivot
                    xc_v[b, 2 * g + h] = d
                    s1[h] = s1[h] + d if g else d
                    s2[h] = s2[h] + d * d if g else d * d
            for k, s in enumerate((s1, s2)):
                stat_v[k, b] = jnp.broadcast_to(jnp.sum(s[0] + s[1], axis=0, keepdims=True), (8, _T))
            stat_v[2, b] = pivot
            return carry

        lax.fori_loop(0, _NB, moments, 0, unroll=2)
        for h in range(_NB // 8):
            m1, m2, pivot = compact(stat_v, 0, h) / _D, compact(stat_v, 1, h) / _D, compact(stat_v, 2, h)
            var = jnp.maximum(m2 - m1 * m1, 0.0)
            shift = _rnd(pivot + m1) - pivot
            gain = 0.5 / _rnd(jnp.sqrt(_rnd(_rnd(var) + _rnd(jnp.full_like(var, _EPS)))))
            for s in range(8):
                stat_v[0, 8 * h + s] = jnp.broadcast_to(shift[s:s + 1], (8, _T))
                stat_v[1, 8 * h + s] = jnp.broadcast_to(gain[s:s + 1], (8, _T))
        wr = jnp.broadcast_to(wr_v[...].astype(f32).reshape(1, _D), (8, _D)).astype(bf16)

        def scale(b, carry):
            shift, gain = stat_v[0, b], stat_v[1, b]
            xn = [_interleave(*[(xc_v[b, 2 * g + h] - shift) * gain for h in range(2)])
                  for g in range(_NG)]
            for g in range(_NG):
                arena[g // _GC, _ROW_X + (g % _GC) * _NB + b] = xn[g]
            stat_v[2, b] = _dot(wr, pltpu.bitcast(jnp.concatenate(xn, axis=0), bf16))
            return carry

        lax.fori_loop(0, _NB, scale, 0, unroll=8)
        for h in range(_NB // 8):
            bits = pltpu.bitcast(_rnd(2.0 * compact(stat_v, 2, h)) + 0.0, i32) >> 16
            rank = jnp.where(bits < 0, ~bits, bits + 0x8000)
            token = (8 * h + row) * _T + lane
            key_v[h] = pltpu.bitcast((1 << 28) + rank * _L + (_L - 1 - token), f32)

    def pop_best(c):
        best = jnp.max(jnp.max(jnp.maximum(key_v[0], key_v[1]), axis=0, keepdims=True),
                       axis=1, keepdims=True)
        key_v[2] = jnp.where(row == c, best, key_v[2])
        for h in range(2):
            key_v[h] = jnp.where(key_v[h] == best, 0.0, key_v[h])

    def modes(step):
        for u in range(_GA):
            grp = step * _GA + u
            rows = pl.ds(pl.multiple_of(grp * 16, 16), 16)
            par = [_even_odd(dt_v[grp])] + [_even_odd(par_v[n, rows, :]) for n in range(6)]
            k0 = []
            for h, skip in enumerate(_even_odd(skip_v[rows, :])):
                z = _modes(*[p[h] for p in par])
                for n in range(4):
                    mode_v[u, h, n] = z[n]
                k0.append(skip + jnp.sum(z[0], axis=1, keepdims=True))
            k0_v[grp] = _interleave(*k0)

    def dft(rows):
        z = _dot(jnp.concatenate([pltpu.bitcast(r, bf16) for r in rows], axis=0), fwd_v[...])
        return [[(z[o:o + 8, :_T], z[o:o + 8, _T:])
                 for o in range((h // 2) * 16 * _NB + 8 * (h % 2), (h // 2 + 1) * 16 * _NB, 16)]
                for h in range(2 * len(rows) // _NB)]

    def spread(step, u):
        for j, blk in _lag_blocks(lambda n: tap_v[u, n], k0_v[step * _GA + u]):
            k_v[u, j] = blk

    def filter_spectra(step, us, zero=0):
        for h, blocks in enumerate(dft([k_v[u + zero, j] for u in us for j in range(_NB)])):
            for j, (re, im) in enumerate(blocks):
                for p, val in enumerate((re, re + im, im - re)):
                    kf_v[2 * (step * _GA + us[0]) + h, p * _PLANE + j] = val

    def phase_a(i, carry):
        pl.when(i == _LN_STEP)(layer_norm)
        for c in range(2):
            pop_best(2 * (i - _LN_STEP) + c)
        for u in range(_GA):
            if u == 0:
                filter_spectra(jnp.maximum(i - 2, 0), range(_GA // 2, _GA), i >> 8)
            if u == _GA // 2:
                filter_spectra(jnp.maximum(i - 1, 0), range(_GA // 2), i >> 8)
            spread(jnp.maximum(i - 1, 0), u)
            v = [[_vandermonde(*seeds) for seeds in _seeds(
                (mode_v[u, h, 0], mode_v[u, h, 1]), (mode_v[u, h, 2], mode_v[u, h, 3]))]
                 for h in range(2)]
            for n, tap in enumerate(_unmix(*map(_interleave, *v))):
                tap_v[u, n] = tap
        modes(jnp.minimum(i + 1, _NG // _GA - 1))
        return carry

    with jax.named_scope("A"):
        modes(0)
        start("x", x_hbm, x_v)
        start("wr", wr_hbm, wr_v)
        start("inv", inv_hbm, inv_v)
        wait("fwd", *[(1, n) for n in range(6)])
        for cp in hidden_copies(0):
            cp.start()
        lax.fori_loop(0, _NG // _GA, phase_a, 0)

    def input_spectra(rows, dst):
        z = dft(rows)
        for h, t in enumerate(z):
            for b, (re, im) in enumerate(t):
                if b:
                    re, im = re + t[b - 1][1], im - t[b - 1][0]
                for p, val in enumerate((re + im, im, re)):
                    dst[(h * 3 + p) * _PLANE + b] = val
        return z

    def w_row(c, r):
        return jnp.concatenate(
            [pltpu.bitcast(arena[c, _ROW_W + q * _WQ + r], f32) for q in range(2)], axis=1)

    def routed_tokens():
        return _L - 1 - (pltpu.bitcast(key_v[2], i32) & (_L - 1))

    with jax.named_scope("topk"):
        for n in range(2, _NF):
            for cp in hidden_copies(n):
                cp.start()
        token = routed_tokens()
        blocks = jnp.concatenate(
            [pltpu.bitcast(jnp.concatenate(
                [arena[g // _GC, _ROW_X + (g % _GC) * _NB + (token[c, 0] >> 7)]
                 for g in range(_NG)], axis=0), bf16) for c in range(_C)], axis=1)
        pick = jnp.concatenate(
            [jnp.where((row == c) & ((token & (_T - 1)) == lane), 2.0, 0.0) for c in range(_C)],
            axis=1).astype(bf16)
        x_sel = jnp.concatenate([_dot_nt(pick, blocks), jnp.zeros((8, _T - _TAIL), f32)], axis=1)
        for n in range(_NO + 1):
            arena[1, _ROW_SEL + n] = pltpu.bitcast(x_sel[:, n * _T:(n + 1) * _T], i32)
            arena[0, _ROW_SEL + n] = pltpu.bitcast(
                jnp.concatenate([x_sel[:, n * _T:(n + 1) * _T]] * 2, axis=0).astype(bf16), i32)
        input_spectra([arena[0, _ROW_X + r] for r in range(_R)], spec_a)
        filter_spectra(_NG // _GA - 2, range(_GA // 2, _GA))
        for u in range(_GA):
            spread(_NG // _GA - 1, u)
        filter_spectra(_NG // _GA - 1, range(_GA))

    def conv_step(c, cur, nxt):
        c_next, c_prev = jnp.minimum(c + 1, _NCH - 1), jnp.maximum(c - 1, 0)
        zero = c >> 8
        fwd_rows, inv_rows, pre = [], [], []

        def project(n):
            cols = pl.ds(pl.multiple_of(c * (_F // _NCH) + n // 2 * _T, _T), _T)
            x_sel = jnp.concatenate(
                [pltpu.bitcast(arena[zero, _ROW_SEL + r], bf16) for r in range(_NO + 1)], axis=1)
            pre.append(_rnd(_dot(x_sel[:, :_D], (wu_v if n % 2 else wg_v)[:, cols])[:8]))
            if n % 2:
                hid_v[:, cols] = _rnd(_silu(pre[-2])) * pre[-1]

        def transform():
            y = _dot(jnp.concatenate(inv_rows, axis=0), inv_v[...])
            s_v[c_prev] = y
            pre.append((y, input_spectra(fwd_rows, nxt)))

        def drain(r):
            y, z = pre[-1]
            arena[c, _ROW_SEL - 1] = pltpu.bitcast(y[8 * r:8 * r + 8] + z[2 * (r // _R) + 1][r % _R // 2][r // 8 % 2], i32)

        dots = 2 * _F // (_NCH * _T)
        todo = sorted(
            [(_G0 // dots * n, lambda n=n: project(n)) for n in range(dots)]
            + [(_G0 + 8 * r, lambda r=r: inv_rows.append(w_row(c_prev, r))) for r in range(2 * _R)]
            + [(_G0 + 16 * r, lambda r=r: fwd_rows.append(arena[c_next, _ROW_X + r])) for r in range(_R)]
            + [(_G0 + 16 * _R, transform)]
            + [(_G0 + _LAG + 8 * r, lambda r=r: drain(r)) for r in range(2 * _R - 17, 2 * _R, 8)], key=lambda job: job[0])
        pace = _PACE * (3 * _NB * (_NB + 1) * _GC) / (_G0 + 16 * _R)

        def read_operands(done):
            while todo and done >= (todo[0][0] - _LEAD) * pace:
                todo.pop(0)[1]()

        done = 0
        read_operands(done)
        def conv(k, u):
            acc = k[0] * u[-1]
            for j in range(1, len(k)):
                acc = acc + k[j] * u[-1 - j]
            return acc

        for h in range(2 * _GC if _KARA else 0):
            for part in range(3):
                for plane in range(3):
                    off = c >> (8 + part)
                    kf = lambda b: kf_v[c * 2 * _GC + h + off, plane * _PLANE + b]
                    uf = lambda b: cur[off + (h * 3 + plane) * _PLANE + b]
                    base = [pltpu.bitcast(arena[c + zero, _ROW_P + plane * 8 + m], f32)
                            for m in range(8) if part and plane]
                    k, u, out = [], [], []
                    for m in range(8):
                        if part == 0:
                            k.append(kf(2 * m))
                            u.append(uf(2 * m) + uf(2 * m + 1))
                        elif part == 1:
                            k.append(kf(2 * m) - kf(2 * m - 1) if m else kf(0))
                            u.append(uf(2 * m + 1))
                        else:
                            k.append(kf(2 * m) - kf(2 * m + 1))
                            u.append(uf(2 * m))
                        y = conv(k, u)
                        if plane:
                            y = p[m] - y if plane == 1 else p[m] + y
                        out.append(y)
                        if part == 0 or plane == 0:
                            arena[c, _ROW_P + plane * 8 + m] = pltpu.bitcast(y, i32)
                        else:
                            b = 2 * m + part - 1
                            arena[c, _ROW_W + (plane - 1) * _WQ + ((h // 2) * _NB + b) * 2 + h % 2] = (
                                pltpu.bitcast(base[m] - y, i32))
                    if plane == 0:
                        p = out
                    done += 136 / 3
                    read_operands(done)
        for h in range(0 if _KARA else 2 * _GC):
            for p in range(3):
                k, u = [], []
                for lo, hi in _BATCH:
                    base = {b: pltpu.bitcast(arena[c + zero, _ROW_P + b], f32)
                            for b in range(lo, hi) if p}
                    for b in range(lo, hi):
                        if _KP == 3 or p == 0:
                            k.append(kf_v[c * 2 * _GC + h, p * _PLANE + b])
                        else:
                            re, im = [kf_v[c * 2 * _GC + h + (c >> (8 + p)), q * _PLANE + b] for q in range(2)]
                            k.append(im + re if p == 1 else im - re)
                        u.append(cur[zero + (h * 3 + p) * _PLANE + b])
                        acc = k[0] * u[b]
                        for j in range(1, b + 1):
                            acc = acc + k[j] * u[b - j]
                        if p == 0:
                            arena[c, _ROW_P + b] = pltpu.bitcast(acc, i32)
                        else:
                            arena[c, _ROW_W + (p - 1) * _WQ + ((h // 2) * _NB + b) * 2 + h % 2] = (
                                pltpu.bitcast(base[b] - acc if p == 1 else base[b] + acc, i32))
                        done += b + 1
                    read_operands(done)
        assert not todo

    def phase_c(part, carry):
        for cp in hidden_copies(part):
            cp.wait()

        @pl.when(part == _WD_STEP)
        def _():
            for n in range(_NO):
                down_copy(n).start()
            down_copy(_NO, _TAIL).start()

        def step(i, carry):
            lax.cond(i & 1 == 0, lambda: conv_step(i, spec_a, spec_b), lambda: conv_step(i, spec_b, spec_a))
            return carry

        return lax.fori_loop(part * (_NCH // _NF), (part + 1) * (_NCH // _NF), step, carry)

    with jax.named_scope("C"):
        lax.fori_loop(0, _NF, phase_c, 0)

    def hidden_at(t, zero=0):
        return (pl.ds(pl.multiple_of(_D + 8 * (t // _NB) + 8 * zero, 8), 8),
                pl.ds((t % _NB) * _T, _T))

    def down(n, size, hid):
        rank = (pltpu.bitcast(key_v[2], i32) - (1 << 28)) >> 11
        score = pltpu.bitcast(jnp.where(rank >= 0x8000, rank - 0x8000, ~rank) << 16, f32)
        y = _rnd(_dot_nt(hid, wd_v[chunk_rows(n, size), :]))
        y_v[:, :size] = 0.5 * (pltpu.bitcast(arena[1, _ROW_SEL + n], f32)[:, :size] + _rnd(y * _rnd(jax.nn.sigmoid(score))[:, :size]))

    def columns(size):
        col = jnp.concatenate([y_v[...], jnp.zeros((_T - _C, _T), f32)], axis=0).T
        col = pltpu.bitcast(col[:size].astype(bf16), i32)
        for c in range(_C):
            col_v[c, :size // 2] = jnp.broadcast_to(col[:, c:c + 1], (size // 2, _T))

    def scatter(n, size, zero):
        token = routed_tokens()
        for c in range(_C):
            hit = (token & (_T - 1))[c:c + 1] == lane
            where = [(n * (_T // (16 * _GC)) + g // _GC,
                      _ROW_X + (g % _GC) * _NB + (token[c, 0] >> 7)) for g in range(size // 16)]
            old = [arena[at] for at in where]
            for g, at in enumerate(where):
                arena[at] = jnp.where(hit, col_v[c + zero, 8 * g:8 * g + 8], old[g])

    def finish(n, g):
        rows = pl.ds(pl.multiple_of(n * _T + 16 * g, 16), 16)
        c = n * (_T // (16 * _GC)) + g // _GC
        for b in range(_NB):
            cols = pl.ds(b * _T, _T)
            r = (g % _GC) * _NB + b
            h = pltpu.bitcast(arena[c, _ROW_X + r], bf16).astype(f32)
            gated = s_v[c, pl.ds(16 * r, 16), :] * (h + h * jnp.tanh(h))
            o_v[rows, cols] = (x_v[rows, cols].astype(f32) + gated).astype(bf16)
            yield

    def phase_d(n, size):
        down_copy(n + 2, size).wait()
        columns(_T)
        hid, step = {}, 0

        def read_hidden():
            for t in range(len(hid), len(hid) + 4):
                hid[t] = o_v[hidden_at(t, zero)]

        read_hidden()
        for g in range(_T // 16):
            for _ in finish(n, g):
                step += 1
                if step % _DSTEP == 0 and len(hid) < _F // _T:
                    read_hidden()
        down(n + 2, size, jnp.concatenate([hid[t] for t in sorted(hid)], axis=1))
        scatter(n + 1, _T, zero)
        out_copy(n).start()

    with jax.named_scope("D0"):
        zero = routed_tokens()[0, 0] >> 11
        y_v[...] = jnp.zeros((8, _T), f32)
        hid = hid_v[...].astype(bf16)
        for t in range(_F // _T):
            o_v[hidden_at(t)] = hid[:, t * _T:(t + 1) * _T]
        down_copy(0).wait()
        down_copy(1).wait()
        down(0, _T, hid)
        columns(_T)
        down(1, _T, hid)
        s_v[_NCH - 1] = _dot(
            jnp.concatenate([w_row(_NCH - 1, r) for r in range(2 * _R)], axis=0), inv_v[...])
        scatter(0, _T, zero)
    with jax.named_scope("D1"):
        lax.fori_loop(0, _NO - 2, lambda n, carry: phase_d(n, _T), None)
    with jax.named_scope("D2"):
        phase_d(_NO - 2, _TAIL)
        columns(_TAIL)
        for g in range(_T // 16):
            list(finish(_NO - 1, g))
        scatter(_NO, _TAIL, zero)
        out_copy(_NO - 1).start()
        for g in range(_TAIL // 16):
            list(finish(_NO, g))
        out_copy(_NO, _TAIL).start()
    with jax.named_scope("end"):
        for n in range(_NO):
            out_copy(n).wait()
        out_copy(_NO, _TAIL).wait()


@jax.jit
def pallas_recurrent_scan__ssm_conv_s4__moe_arch_mod__prompt_kernel(
    A_u: jax.Array,
    A_A_re: jax.Array,
    A_A_im: jax.Array,
    A_B_re: jax.Array,
    A_B_im: jax.Array,
    A_C_re: jax.Array,
    A_C_im: jax.Array,
    A_log_dt: jax.Array,
    A_Dskip: jax.Array,
    B_x: jax.Array,
    B_w_r: jax.Array,
    B_w_gate: jax.Array,
    B_w_up: jax.Array,
    B_w_down: jax.Array,
):
    del B_x
    assert A_u.shape == (1, _L, _D) and A_A_re.shape == (_D, _N) and B_w_gate.shape == (_D, _F)
    assert A_u.dtype == bf16 and A_A_re.dtype == bf16
    hbm = pl.BlockSpec(memory_space=pl.ANY)
    vmem = pltpu.VMEM
    out = pl.pallas_call(
        _kernel,
        out_shape=jax.ShapeDtypeStruct((_D, _L), bf16),
        in_specs=[hbm] * 15,
        out_specs=hbm,
        scratch_shapes=[
            vmem((_D, _L), bf16), vmem((_D + 32, _L), bf16),
            vmem((6, _D, _N), bf16), vmem((_D,), bf16), vmem((_D,), bf16), vmem((_D,), bf16),
            vmem((_D, _F), bf16), vmem((_D, _F), bf16), vmem((_D, _F), bf16),
            vmem((_T, 2 * _T), bf16), vmem((2 * _T, _T), f32),
            vmem((_D, _T), bf16), vmem((_NG, 8, _T), i32),
            vmem((_NCH, _ROWS, 8, _T), i32), vmem((_NCH, 16 * _R, _T), f32),
            vmem((_NG, 8, _T), i32), vmem((_GA, 2, 4, 8, _N), f32), vmem((_GA, len(_TAPS), 8, _T), i32),
            vmem((_GA, _NB, 8, _T), i32),
            vmem((_NB, 2 * _NG, 8, _T), f32), vmem((3, _NB, 8, _T), f32), vmem((3, 8, _T), f32),
            vmem((8, _F), f32), vmem((8, _T), f32),
            vmem((_C, _T // 2, _T), i32),
            *[vmem((2 * _GC * 3 * _PLANE, 8, _T), f32)] * 2, vmem((2 * _NG, 3 * _PLANE, 8, _T), f32),
            pltpu.SemaphoreType.DMA((18,)), pltpu.SemaphoreType.DMA((2 * _NF + _NO + 1,)),
            pltpu.SemaphoreType.DMA((_NO + 1,)),
        ],
        compiler_params=pltpu.CompilerParams(vmem_limit_bytes=100 * 2**20),
    )(A_u.reshape(_L, _D).T, A_A_re, A_A_im, A_B_re, A_B_im, A_C_re, A_C_im, A_log_dt, A_Dskip,
      B_w_r, B_w_gate, B_w_up, B_w_down.T, _FWD, _INV)
    return out.T.reshape(1, _L, _D)
```

```python
import jax
import jax.numpy as jnp
import numpy as np
from jax import lax
import jax.experimental.pallas as pl
import jax.experimental.pallas.tpu as pltpu

_D, _L, _N, _F, _C = 576, 2048, 128, 4608, 8
_T = 128
_NB = _L // _T
_EPS = 1e-5
_GA = 4
_GC = 2
_NG = _D // 16
_NCH = _NG // _GC
_R = _GC * _NB
_ROW_X, _ROW_W, _ROW_P, _ROWS = 0, _R, 5 * _R + 8, 5 * _R + 8 + 24
_PLANE, _WQ = _NB + 2, 2 * _R + 2
_ROW_SEL = 5 * _R + 3
_KT = -(-_D // _T)
_NO, _OCH = 6, _D // 6
_NF = 3
_FCH = _F // _NF
_LN_STEP = 4
_WD_STEP = 1
_PACE, _PACE1, _LEAD, _LAG, _G1, _S0, _S1 = 0.85, 0.8, 32, 140, 32, 450, 30

f32, bf16, i32 = jnp.float32, jnp.bfloat16, jnp.int32


def _dft_constants():
    theta = (np.pi / 2 + 2 * np.pi * np.arange(_T)) / _T
    ang = np.arange(_T)[:, None] * theta[None, :]
    c, s = np.cos(ang), np.sin(ang)
    fwd = np.concatenate([c, s], axis=1)
    return fwd.astype(bf16), (fwd.T * (2 / _T)).astype(np.float32)


_FWD, _INV = _dft_constants()


def _lag_step(j):
    return max(1, (1 << (j * _T).bit_length()) >> 8)


def _round_lag(p, st):
    if st == 1:
        return p
    return (p + (st // 2 - 1) + ((p >> (st.bit_length() - 1)) & 1)) & ~(st - 1)


assert np.array_equal(
    np.concatenate([j * _T + _round_lag(np.arange(_T), _lag_step(j)) for j in range(_NB)]),
    np.arange(_L).astype(bf16).astype(np.int64))

_PAIRS = (((0, 1), (0, 5)), ((0, 2), (0, 6)), ((0, 3), (0, 7)), ((0, 4), (0, 8)), ((1, 2), (1, 6)),
          ((1, 4), (1, 8)), ((2, 4), (2, 8)), ((3, 4), (3, 8)), ((4, 8), (5, 8)), ((6, 8), (7, 8)))
_TAPS = [k for pair in _PAIRS for k in pair]


def _aligned(i, n):
    return i if isinstance(i, int) else pl.multiple_of(i, n)


def _cmul(a, b):
    return a[0] * b[0] - a[1] * b[1], a[0] * b[1] + a[1] * b[0]


def _csq(a):
    return a[0] * a[0] - a[1] * a[1], (a[0] + a[0]) * a[1]


def _silu(x):
    h = 0.5 * x
    return h + h * jnp.tanh(h)


def _rnd(x):
    return x.astype(bf16).astype(f32)


def _dot(a, b):
    return jnp.dot(a, b, preferred_element_type=f32)


def _dot_nt(a, b):
    return lax.dot_general(a, b, (((1,), (1,)), ((), ())), preferred_element_type=f32)


def _column(v):
    return jnp.broadcast_to(v.reshape(1, _D), (_T, _D)).T


def _even_odd(x):
    b = pltpu.bitcast(x, i32)
    return pltpu.bitcast(b << 16, f32), pltpu.bitcast(b & -65536, f32)


def _interleave(even, odd):
    return pltpu.bitcast(pltpu.pack_elementwise([even, odd], packed_dtype=bf16), i32)


def _modes(dt, ar, ai, br, bi, cr, ci):
    zr, zi = dt * ar, dt * ai
    mag = jnp.exp(zr)
    return _cmul((cr, ci), (dt * br, dt * bi)) + (mag * jnp.cos(zi), mag * jnp.sin(zi))


def _seeds(w, a1):
    a = {1: a1}
    for n in range(9):
        a[2 << n] = _csq(a[1 << n])
    row = lax.broadcasted_iota(i32, (8, _N), 0)

    def conj(z):
        return z[0], -z[1]

    def mix(z0, z1):
        rolled = [pltpu.roll(x, 4, 0) for x in z1]
        return ([jnp.where(row < 4, x, y) for x, y in zip(z0, rolled)],
                [jnp.where(row < 4, y, x) for x, y in zip(z0, rolled)])

    def dup(z):
        return [[jnp.take_along_axis(x, (row & 3) + 4 * q, axis=0, mode="promise_in_bounds")
                 for x in z] for q in range(2)]

    wa = _cmul(w, a[1])
    return zip(mix((1.0, 0.0), conj(a[128])), dup(conj(a[8])), dup(conj(a[32])),
               mix(wa, _cmul(wa, a[4])), dup(a[1]), dup(a[256]),
               mix(_cmul(a[256], a[4]), a[512]), dup(a[512]))


def _vandermonde(e0, m8, m32, g0, m1, m256, m_top, m512):
    e = [e0]
    for s in range(1, 16):
        e.append(_cmul(e[s - 1], m8) if s < 4 else _cmul(e[s - 4], m32))
    g = [g0]
    for _ in range(3):
        g.append(_cmul(g[-1], m1))
    g += [_cmul(g[1], m256), _cmul(g[3], m256)]
    g += [_cmul(g[3], m512), _cmul(g[5], m512)]
    g.append(_cmul(g[7], m_top))
    g.append(_cmul(g[8], m512))
    re, im = [_dot_nt(jnp.concatenate([z[p] for z in g], axis=0),
                      jnp.concatenate([z[p] for z in e], axis=0)) for p in range(2)]
    return re + im


def _unmix(lo, hi):
    row = lax.broadcasted_iota(i32, (8, _T), 0)
    out = []
    for m in range(len(_PAIRS)):
        x, y = lo[8 * m:8 * m + 8], hi[8 * m:8 * m + 8]
        out += [jnp.where(row < 4, x, y), pltpu.roll(jnp.where(row < 4, y, x), 4, 0)]
    return out


def _lag_blocks(tap, lag0):
    lane = lax.broadcasted_iota(i32, (8, _T), 1)
    row = lax.broadcasted_iota(i32, (8, _T), 0)
    for h in range(2):
        def take(big, r, fine):
            s = ((_T * h + fine) >> 3) & 31
            return jnp.take_along_axis(tap(_TAPS.index((big, r))),
                                       ((s & 15) << 3) + (row ^ ((s >> 4) << 2)),
                                       axis=1, mode="promise_in_bounds")

        top = [take(big, 8, _round_lag(lane, 8) - 8) for big in range(_NB // 2)]
        for big, blk in enumerate(top):
            st = _lag_step(2 * big + h)
            lag = _round_lag(lane, st)
            if h == 0:
                blk = jnp.where(lag == 0, top[big - 1] if big else lag0, blk)
            for r in range(st, 8, st):
                blk = jnp.where((lag & 7) == r, take(big, r, lane), blk)
            yield 2 * big + h, blk


def _kernel(x_hbm, ar_hbm, ai_hbm, br_hbm, bi_hbm, cr_hbm, ci_hbm, ldt_hbm, dsk_hbm, wr_hbm,
            wg_hbm, wu_hbm, wd_hbm, fwd_hbm, inv_hbm, o_hbm,
            x_v, o_v, par_v, ldt_v, dsk_v, wr_v, wg_v, wu_v, wd_v, fwd_v, inv_v,
            skip_v, k0_v, arena, s_v, dt_v, mode_v, tap_v, k_v, xc_v, stat_v, key_v, sel_v, hid_v,
            spec_a, spec_b, kf_v, sem, w_sem, o_sem):
    row = lax.broadcasted_iota(i32, (8, _T), 0)
    lane = lax.broadcasted_iota(i32, (8, _T), 1)
    copies = {}

    def start(name, src, dst):
        copies[name] = pltpu.make_async_copy(src, dst, sem.at[len(copies)])
        copies[name].start()

    def wait(*names):
        for name in names:
            copies[name].wait()

    def hidden_copies(n):
        cols = pl.ds(_aligned(n * _FCH, _FCH), _FCH)
        return [pltpu.make_async_copy(w.at[:, cols], v.at[:, cols], w_sem.at[2 * n + k])
                for k, (w, v) in enumerate(((wg_hbm, wg_v), (wu_hbm, wu_v)))]

    def chunk_rows(n):
        return pl.ds(_aligned(n * _OCH, 32), _OCH)

    def down_copy(n):
        return pltpu.make_async_copy(wd_hbm.at[chunk_rows(n)], wd_v.at[chunk_rows(n)],
                                     w_sem.at[2 * _NF + n])

    def out_copy(n):
        return pltpu.make_async_copy(o_v.at[chunk_rows(n)], o_hbm.at[chunk_rows(n)], o_sem.at[n])

    with jax.named_scope("init"):
        start("ldt", ldt_hbm, ldt_v)
        start("dsk", dsk_hbm, dsk_v)
        for part, rows in enumerate((pl.ds(0, 16 * _GA), pl.ds(16 * _GA, _D - 16 * _GA))):
            for n, src in enumerate((ar_hbm, ai_hbm, br_hbm, bi_hbm, cr_hbm, ci_hbm)):
                start((part, n), src.at[rows], par_v.at[n, rows])
        start("fwd", fwd_hbm, fwd_v)
        arena[0, _ROW_W:_ROW_P] = jnp.zeros((_ROW_P - _ROW_W, 8, _T), i32)
        tap_v[...] = jnp.zeros(tap_v.shape, i32)
        k_v[...] = jnp.zeros(k_v.shape, i32)
        key_v[...] = jnp.zeros(key_v.shape, f32)
        wait("ldt")
        dt = pltpu.bitcast(_column(jnp.exp(ldt_v[...].astype(f32))).astype(bf16), i32)
        for g in range(_NG):
            dt_v[g] = dt[8 * g:8 * g + 8]
        wait("dsk")
        skip_v[...] = _column(dsk_v[...].astype(f32)).astype(bf16)
        wait(*[(0, n) for n in range(6)])

    def compact(ref, k, h):
        out = ref[k, 8 * h]
        for s in range(1, 8):
            out = jnp.where(row == s, ref[k, 8 * h + s], out)
        return out

    def layer_norm():
        wait("x", "wr", "inv")
        for cp in hidden_copies(1):
            cp.start()

        def moments(b, carry):
            cols = pl.ds(_aligned(b * _T, _T), _T)
            pivot = jnp.broadcast_to(_even_odd(x_v[:16, cols])[0][:1], (8, _T))
            s1, s2 = [None] * 2, [None] * 2
            for g in range(_NG):
                for h, x in enumerate(_even_odd(x_v[pl.ds(16 * g, 16), cols])):
                    d = x - pivot
                    xc_v[b, 2 * g + h] = d
                    s1[h] = s1[h] + d if g else d
                    s2[h] = s2[h] + d * d if g else d * d
            for k, s in enumerate((s1, s2)):
                stat_v[k, b] = jnp.broadcast_to(jnp.sum(s[0] + s[1], axis=0, keepdims=True), (8, _T))
            stat_v[2, b] = pivot
            return carry

        lax.fori_loop(0, _NB, moments, 0, unroll=2)
        for h in range(_NB // 8):
            m1, m2, pivot = compact(stat_v, 0, h) / _D, compact(stat_v, 1, h) / _D, compact(stat_v, 2, h)
            var = jnp.maximum(m2 - m1 * m1, 0.0)
            shift = _rnd(pivot + m1) - pivot
            gain = 0.5 / _rnd(jnp.sqrt(_rnd(_rnd(var) + _rnd(jnp.full_like(var, _EPS)))))
            for s in range(8):
                stat_v[0, 8 * h + s] = jnp.broadcast_to(shift[s:s + 1], (8, _T))
                stat_v[1, 8 * h + s] = jnp.broadcast_to(gain[s:s + 1], (8, _T))
        wr = jnp.broadcast_to(wr_v[...].astype(f32).reshape(1, _D), (8, _D)).astype(bf16)

        def scale(b, carry):
            shift, gain = stat_v[0, b], stat_v[1, b]
            xn = [_interleave(*[(xc_v[b, 2 * g + h] - shift) * gain for h in range(2)])
                  for g in range(_NG)]
            for g in range(_NG):
                arena[g // _GC, _ROW_X + (g % _GC) * _NB + b] = xn[g]
            stat_v[2, b] = _dot(wr, pltpu.bitcast(jnp.concatenate(xn, axis=0), bf16))
            return carry

        lax.fori_loop(0, _NB, scale, 0, unroll=8)
        for h in range(_NB // 8):
            bits = pltpu.bitcast(_rnd(2.0 * compact(stat_v, 2, h)) + 0.0, i32) >> 16
            rank = jnp.where(bits < 0, ~bits, bits + 0x8000)
            token = (8 * h + row) * _T + lane
            key_v[h] = pltpu.bitcast((1 << 28) + rank * _L + (_L - 1 - token), f32)

    def pop_best(c):
        best = jnp.max(jnp.max(jnp.maximum(key_v[0], key_v[1]), axis=0, keepdims=True),
                       axis=1, keepdims=True)
        key_v[2] = jnp.where(row == c, best, key_v[2])
        for h in range(2):
            key_v[h] = jnp.where(key_v[h] == best, 0.0, key_v[h])

    def modes(step):
        for u in range(_GA):
            grp = step * _GA + u
            rows = pl.ds(_aligned(grp * 16, 16), 16)
            par = [_even_odd(dt_v[grp])] + [_even_odd(par_v[n, rows, :]) for n in range(6)]
            k0 = []
            for h, skip in enumerate(_even_odd(skip_v[rows, :])):
                z = _modes(*[p[h] for p in par])
                for n in range(4):
                    mode_v[u, h, n] = z[n]
                k0.append(skip + jnp.sum(z[0], axis=1, keepdims=True))
            k0_v[grp] = _interleave(*k0)

    def dft(rows):
        z = _dot(jnp.concatenate([pltpu.bitcast(r, bf16) for r in rows], axis=0), fwd_v[...])
        return [[(z[o:o + 8, :_T], z[o:o + 8, _T:])
                 for o in range((h // 2) * 16 * _NB + 8 * (h % 2), (h // 2 + 1) * 16 * _NB, 16)]
                for h in range(2 * len(rows) // _NB)]

    def spread(step, u):
        for j, blk in _lag_blocks(lambda n: tap_v[u, n], k0_v[step * _GA + u]):
            k_v[u, j] = blk

    def filter_spectra(step, us, zero=0):
        for h, blocks in enumerate(dft([k_v[u + zero, j] for u in us for j in range(_NB)])):
            for j, (re, im) in enumerate(blocks):
                for p, val in enumerate((re, re + im, im - re)):
                    kf_v[2 * (step * _GA + us[0]) + h, p * _PLANE + j] = val

    def phase_a(i, carry):
        pl.when(i == _LN_STEP)(layer_norm)
        for c in range(2):
            pop_best(2 * (i - _LN_STEP) + c)
        for u in range(_GA):
            if u == 0:
                filter_spectra(jnp.maximum(i - 2, 0), range(_GA // 2, _GA), i >> 8)
            if u == _GA // 2:
                filter_spectra(jnp.maximum(i - 1, 0), range(_GA // 2), i >> 8)
            spread(jnp.maximum(i - 1, 0), u)
            v = [[_vandermonde(*seeds) for seeds in _seeds(
                (mode_v[u, h, 0], mode_v[u, h, 1]), (mode_v[u, h, 2], mode_v[u, h, 3]))]
                 for h in range(2)]
            for n, tap in enumerate(_unmix(*map(_interleave, *v))):
                tap_v[u, n] = tap
        modes(jnp.minimum(i + 1, _NG // _GA - 1))
        return carry

    with jax.named_scope("A"):
        modes(0)
        start("x", x_hbm, x_v)
        start("wr", wr_hbm, wr_v)
        start("inv", inv_hbm, inv_v)
        wait("fwd", *[(1, n) for n in range(6)])
        for cp in hidden_copies(0):
            cp.start()
        lax.fori_loop(0, _NG // _GA, phase_a, 0)

    def input_spectra(rows, dst):
        z = dft(rows)
        for h, t in enumerate(z):
            for b, (re, im) in enumerate(t):
                if b:
                    re, im = re + t[b - 1][1], im - t[b - 1][0]
                for p, val in enumerate((re + im, im, re)):
                    dst[(h * 3 + p) * _PLANE + b] = val
        return z

    def w_row(c, r):
        return jnp.concatenate(
            [pltpu.bitcast(arena[c, _ROW_W + q * _WQ + r], f32) for q in range(2)], axis=1)

    def routed_tokens():
        return _L - 1 - (pltpu.bitcast(key_v[2], i32) & (_L - 1))

    with jax.named_scope("topk"):
        for n in range(2, _NF):
            for cp in hidden_copies(n):
                cp.start()
        token = routed_tokens()
        blocks = jnp.concatenate(
            [pltpu.bitcast(jnp.concatenate(
                [arena[g // _GC, _ROW_X + (g % _GC) * _NB + (token[c, 0] >> 7)]
                 for g in range(_NG)], axis=0), bf16) for c in range(_C)], axis=1)
        pick = jnp.concatenate(
            [jnp.where((row == c) & ((token & (_T - 1)) == lane), 2.0, 0.0) for c in range(_C)],
            axis=1).astype(bf16)
        x_sel = _dot_nt(pick, blocks)
        for n in range(_NO):
            sel_v[n] = x_sel[:, n * _OCH:(n + 1) * _OCH]
        x_sel = jnp.concatenate([x_sel, jnp.zeros((8, _KT * _T - _D), f32)], axis=1)
        for n in range(_KT):
            arena[0, _ROW_SEL + n] = pltpu.bitcast(
                jnp.concatenate([x_sel[:, n * _T:(n + 1) * _T]] * 2, axis=0).astype(bf16), i32)
        input_spectra([arena[0, _ROW_X + r] for r in range(_R)], spec_a)
        filter_spectra(_NG // _GA - 2, range(_GA // 2, _GA))
        for u in range(_GA):
            spread(_NG // _GA - 1, u)
        filter_spectra(_NG // _GA - 1, range(_GA))

    def hidden_jobs(c):
        width = _F // (_NCH - _NO)
        gate = []

        def project(n):
            cols = pl.ds(_aligned(c * width + n // 2 * _T, _T), _T)
            x_sel = jnp.concatenate(
                [pltpu.bitcast(arena[c >> 8, _ROW_SEL + r], bf16) for r in range(_KT)], axis=1)
            gate.append(_rnd(_dot(x_sel[:, :_D], (wu_v if n % 2 else wg_v)[:, cols])[:8]))
            if n % 2:
                hid_v[:, cols] = (_rnd(_silu(gate[-2])) * gate[-1]).astype(bf16)

        return [(40 * n, lambda n=n: project(n)) for n in range(2 * width // _T)]

    def hidden_at(t, zero=0):
        return pl.ds(_aligned(_D + 8 * (t // _NB + zero), 8), 8), pl.ds((t % _NB) * _T, _T)

    def finish(n):
        for k in range(_OCH // 16 * _NB):
            c, r = n * (_OCH // (16 * _GC)) + k // _R, k % _R
            rows = pl.ds(_aligned(n * _OCH + 16 * (k // _NB), 16), 16)
            cols = pl.ds((k % _NB) * _T, _T)
            h = pltpu.bitcast(arena[c, _ROW_X + r], bf16).astype(f32)
            gated = s_v[c, pl.ds(16 * r, 16), :] * (h + h * jnp.tanh(h))
            o_v[rows, cols] = (x_v[rows, cols].astype(f32) + gated).astype(bf16)
            yield k

    def output_jobs(c):
        n = c - (_NCH - _NO)
        hid = [o_v[hidden_at(t, c >> 8)] for t in range(4)]
        for k in finish(jnp.maximum(n - 1, 0)):
            if k % 12 == 11:
                hid += [o_v[hidden_at(t, c >> 8)] for t in range(len(hid), len(hid) + 4)]
        rank = (pltpu.bitcast(key_v[2], i32) - (1 << 28)) >> 11
        score = pltpu.bitcast(jnp.where(rank >= 0x8000, rank - 0x8000, ~rank) << 16, f32)
        y = _rnd(_dot_nt(jnp.concatenate(hid, axis=1), wd_v[chunk_rows(n), :]))
        y = 0.5 * (sel_v[n] + _rnd(y * _rnd(jax.nn.sigmoid(score))[:, :_OCH]))
        col = jnp.concatenate([y, jnp.zeros((_T - _C, _OCH), f32)], axis=0).T
        col = pltpu.bitcast(col.astype(bf16), i32)
        token = routed_tokens()

        def scatter(t):
            hit = ((token & (_T - 1)) == lane)[t:t + 1]
            new = jnp.broadcast_to(col[:, t:t + 1], (_OCH // 2, _T))
            where = [(n * (_OCH // (16 * _GC)) + g // _GC,
                      _ROW_X + (g % _GC) * _NB + (token[t, 0] >> 7)) for g in range(_OCH // 16)]
            old = [arena[at] for at in where]
            for g, at in enumerate(where):
                arena[at] = jnp.where(hit, new[8 * g:8 * g + 8], old[g])

        return [(_S0 + _S1 * t, lambda t=t: scatter(t)) for t in range(_C)]

    def conv_step(c, cur, nxt, ffn_jobs, delay, pace):
        c_next, c_prev = jnp.minimum(c + 1, _NCH - 1), jnp.maximum(c - 1, 0)
        zero = c >> 8
        fwd_rows, inv_rows, results = [], [], []

        def transform():
            y = _dot(jnp.concatenate(inv_rows, axis=0), inv_v[...])
            s_v[c_prev] = y
            results.extend((y, input_spectra(fwd_rows, nxt)))

        def drain(r):
            y, z = results
            arena[c, _ROW_SEL - 1] = pltpu.bitcast(
                y[8 * r:8 * r + 8] + z[2 * (r // _R) + 1][r % _R // 2][r // 8 % 2], i32)

        jobs = sorted(
            ffn_jobs(c)
            + [(delay + 8 * r, lambda r=r: inv_rows.append(w_row(c_prev, r))) for r in range(2 * _R)]
            + [(delay + 16 * r, lambda r=r: fwd_rows.append(arena[c_next, _ROW_X + r]))
               for r in range(_R)]
            + [(delay + 16 * _R, transform)]
            + [(delay + _LAG + 8 * r, lambda r=r: drain(r)) for r in range(2 * _R - 17, 2 * _R, 8)],
            key=lambda job: job[0])

        def run_jobs(done):
            while jobs and done * (delay + 16 * _R) >= (jobs[0][0] - _LEAD) * pace * 18 * _GC:
                jobs.pop(0)[1]()

        run_jobs(0)
        for h in range(2 * _GC):
            for part in range(3):
                for plane in range(3):
                    kf = lambda b: kf_v[c * 2 * _GC + h + (zero >> part), plane * _PLANE + b]
                    uf = lambda b: cur[(zero >> part) + (h * 3 + plane) * _PLANE + b]
                    base = [pltpu.bitcast(arena[c + zero, _ROW_P + plane * 8 + m], f32)
                            for m in range(8) if part and plane]
                    k, u, out = [], [], []
                    for m in range(8):
                        if part == 0:
                            k.append(kf(2 * m))
                            u.append(uf(2 * m) + uf(2 * m + 1))
                        elif part == 1:
                            k.append(kf(2 * m) - kf(2 * m - 1) if m else kf(0))
                            u.append(uf(2 * m + 1))
                        else:
                            k.append(kf(2 * m) - kf(2 * m + 1))
                            u.append(uf(2 * m))
                        y = k[0] * u[m]
                        for j in range(1, m + 1):
                            y = y + k[j] * u[m - j]
                        if plane:
                            y = shared[m] - y if plane == 1 else shared[m] + y
                        out.append(y)
                        if part == 0 or plane == 0:
                            arena[c, _ROW_P + plane * 8 + m] = pltpu.bitcast(y, i32)
                        else:
                            b = 2 * m + part - 1
                            arena[c, _ROW_W + (plane - 1) * _WQ + ((h // 2) * _NB + b) * 2 + h % 2] = (
                                pltpu.bitcast(base[m] - y, i32))
                    if plane == 0:
                        shared = out
                    run_jobs((h * 3 + part) * 3 + plane + 1)
        assert not jobs

    def either(c, *args):
        lax.cond(c & 1 == 0, lambda: conv_step(c, spec_a, spec_b, *args),
                 lambda: conv_step(c, spec_b, spec_a, *args))

    def phase_c(part, carry):
        for cp in hidden_copies(part):
            cp.wait()

        @pl.when(part == _WD_STEP)
        def _():
            for n in range(_NO):
                down_copy(n).start()

        steps = (_NCH - _NO) // _NF
        return lax.fori_loop(part * steps, (part + 1) * steps,
                             lambda c, carry: either(c, hidden_jobs, 240, _PACE), carry)

    def phase_d(n, carry):
        down_copy(n).wait()
        either(n + _NCH - _NO, output_jobs, _G1, _PACE1)
        pl.when(n > 0)(lambda: out_copy(n - 1).start())

    with jax.named_scope("C"):
        lax.fori_loop(0, _NF, phase_c, None)
    with jax.named_scope("D"):
        for t in range(_F // _T):
            o_v[hidden_at(t)] = hid_v[:, t * _T:(t + 1) * _T]
        lax.fori_loop(0, _NO, phase_d, None)
    with jax.named_scope("tail"):
        s_v[_NCH - 1] = _dot(
            jnp.concatenate([w_row(_NCH - 1, r) for r in range(2 * _R)], axis=0), inv_v[...])
        list(finish(_NO - 1))
        out_copy(_NO - 1).start()
    with jax.named_scope("end"):
        for n in range(_NO):
            out_copy(n).wait()


@jax.jit
def pallas_recurrent_scan__ssm_conv_s4__moe_arch_mod__prompt_kernel(
    A_u: jax.Array,
    A_A_re: jax.Array,
    A_A_im: jax.Array,
    A_B_re: jax.Array,
    A_B_im: jax.Array,
    A_C_re: jax.Array,
    A_C_im: jax.Array,
    A_log_dt: jax.Array,
    A_Dskip: jax.Array,
    B_x: jax.Array,
    B_w_r: jax.Array,
    B_w_gate: jax.Array,
    B_w_up: jax.Array,
    B_w_down: jax.Array,
):
    del B_x
    assert A_u.shape == (1, _L, _D) and A_A_re.shape == (_D, _N) and B_w_gate.shape == (_D, _F)
    assert A_u.dtype == bf16 and A_A_re.dtype == bf16
    hbm = pl.BlockSpec(memory_space=pl.ANY)
    vmem = pltpu.VMEM
    out = pl.pallas_call(
        _kernel,
        out_shape=jax.ShapeDtypeStruct((_D, _L), bf16),
        in_specs=[hbm] * 15,
        out_specs=hbm,
        scratch_shapes=[
            vmem((_D, _L), bf16), vmem((_D + 32, _L), bf16),
            vmem((6, _D, _N), bf16), vmem((_D,), bf16), vmem((_D,), bf16), vmem((_D,), bf16),
            vmem((_D, _F), bf16), vmem((_D, _F), bf16), vmem((_D, _F), bf16),
            vmem((_T, 2 * _T), bf16), vmem((2 * _T, _T), f32),
            vmem((_D, _T), bf16), vmem((_NG, 8, _T), i32),
            vmem((_NCH, _ROWS, 8, _T), i32), vmem((_NCH, 16 * _R, _T), f32),
            vmem((_NG, 8, _T), i32), vmem((_GA, 2, 4, 8, _N), f32), vmem((_GA, len(_TAPS), 8, _T), i32),
            vmem((_GA, _NB, 8, _T), i32),
            vmem((_NB, 2 * _NG, 8, _T), f32), vmem((3, _NB, 8, _T), f32), vmem((3, 8, _T), f32),
            vmem((_NO, 8, _OCH), f32), vmem((8, _F), bf16),
            *[vmem((2 * _GC * 3 * _PLANE, 8, _T), f32)] * 2, vmem((2 * _NG, 3 * _PLANE, 8, _T), f32),
            pltpu.SemaphoreType.DMA((18,)), pltpu.SemaphoreType.DMA((2 * _NF + _NO,)),
            pltpu.SemaphoreType.DMA((_NO,)),
        ],
        compiler_params=pltpu.CompilerParams(vmem_limit_bytes=100 * 2**20),
    )(A_u.reshape(_L, _D).T, A_A_re, A_A_im, A_B_re, A_B_im, A_C_re, A_C_im, A_log_dt, A_Dskip,
      B_w_r, B_w_gate, B_w_up, B_w_down.T, _FWD, _INV)
    return out.T.reshape(1, _L, _D)
```

```python
import jax
import jax.numpy as jnp
import numpy as np
from jax import lax
import jax.experimental.pallas as pl
import jax.experimental.pallas.tpu as pltpu

_D, _L, _N, _F, _C = 576, 2048, 128, 4608, 8
_T = 128
_NB = _L // _T
_EPS = 1e-5
_GA = 4
_GC = 2
_NG = _D // 16
_NCH = _NG // _GC
_R = _GC * _NB
_ROW_X, _ROW_W, _ROW_P, _ROWS = 0, _R, 5 * _R + 8, 5 * _R + 8 + 24
_PLANE, _WQ = _NB + 2, 2 * _R + 2
_ROW_SEL = 5 * _R + 3
_MERGE = 1
_KT = -(-_D // _T)
_NO, _OCH = 6, _D // 6
_NF = 3
_FCH = _F // _NF
_LN_STEP = 4
_WD_STEP = 1
_PACE, _PACE1, _LEAD, _LAG, _G1, _S0, _S1 = 0.87, 0.8, 32, 140, 32, 520, 20

f32, bf16, i32 = jnp.float32, jnp.bfloat16, jnp.int32


def _dft_constants():
    theta = (np.pi / 2 + 2 * np.pi * np.arange(_T)) / _T
    ang = np.arange(_T)[:, None] * theta[None, :]
    c, s = np.cos(ang), np.sin(ang)
    fwd = np.concatenate([c, s], axis=1)
    return fwd.astype(bf16), (fwd.T * (2 / _T)).astype(np.float32)


_FWD, _INV = _dft_constants()


def _lag_step(j):
    return max(1, (1 << (j * _T).bit_length()) >> 8)


def _round_lag(p, st):
    if st == 1:
        return p
    return (p + (st // 2 - 1) + ((p >> (st.bit_length() - 1)) & 1)) & ~(st - 1)


assert np.array_equal(
    np.concatenate([j * _T + _round_lag(np.arange(_T), _lag_step(j)) for j in range(_NB)]),
    np.arange(_L).astype(bf16).astype(np.int64))

_PAIRS = (((0, 1), (0, 5)), ((0, 2), (0, 6)), ((0, 3), (0, 7)), ((0, 4), (0, 8)), ((1, 2), (1, 6)),
          ((1, 4), (1, 8)), ((2, 4), (2, 8)), ((3, 4), (3, 8)), ((4, 8), (5, 8)), ((6, 8), (7, 8)))
_TAPS = [k for pair in _PAIRS for k in pair]


def _aligned(i, n):
    return i if isinstance(i, int) else pl.multiple_of(i, n)


def _cmul(a, b):
    return a[0] * b[0] - a[1] * b[1], a[0] * b[1] + a[1] * b[0]


def _csq(a):
    return a[0] * a[0] - a[1] * a[1], (a[0] + a[0]) * a[1]


def _silu(x):
    h = 0.5 * x
    return h + h * jnp.tanh(h)


def _rnd(x):
    return x.astype(bf16).astype(f32)


def _dot(a, b):
    return jnp.dot(a, b, preferred_element_type=f32)


def _dot_nt(a, b):
    return lax.dot_general(a, b, (((1,), (1,)), ((), ())), preferred_element_type=f32)


def _column(v):
    return jnp.broadcast_to(v.reshape(1, _D), (_T, _D)).T


def _even_odd(x):
    b = pltpu.bitcast(x, i32)
    return pltpu.bitcast(b << 16, f32), pltpu.bitcast(b & -65536, f32)


def _interleave(even, odd):
    return pltpu.bitcast(pltpu.pack_elementwise([even, odd], packed_dtype=bf16), i32)


def _modes(dt, ar, ai, br, bi, cr, ci):
    zr, zi = dt * ar, dt * ai
    mag = jnp.exp(zr)
    return _cmul((cr, ci), (dt * br, dt * bi)) + (mag * jnp.cos(zi), mag * jnp.sin(zi))


def _seeds(w, a1):
    a = {1: a1}
    for n in range(9):
        a[2 << n] = _csq(a[1 << n])
    row = lax.broadcasted_iota(i32, (8, _N), 0)

    def conj(z):
        return z[0], -z[1]

    def mix(z0, z1):
        rolled = [pltpu.roll(x, 4, 0) for x in z1]
        return ([jnp.where(row < 4, x, y) for x, y in zip(z0, rolled)],
                [jnp.where(row < 4, y, x) for x, y in zip(z0, rolled)])

    def dup(z):
        return [[jnp.take_along_axis(x, (row & 3) + 4 * q, axis=0, mode="promise_in_bounds")
                 for x in z] for q in range(2)]

    wa = _cmul(w, a[1])
    return zip(mix((1.0, 0.0), conj(a[128])), dup(conj(a[8])), dup(conj(a[32])),
               mix(wa, _cmul(wa, a[4])), dup(a[1]), dup(a[256]),
               mix(_cmul(a[256], a[4]), a[512]), dup(a[512]))


def _vandermonde(e0, m8, m32, g0, m1, m256, m_top, m512):
    e = [e0]
    for s in range(1, 16):
        e.append(_cmul(e[s - 1], m8) if s < 4 else _cmul(e[s - 4], m32))
    g = [g0]
    for _ in range(3):
        g.append(_cmul(g[-1], m1))
    g += [_cmul(g[1], m256), _cmul(g[3], m256)]
    g += [_cmul(g[3], m512), _cmul(g[5], m512)]
    g.append(_cmul(g[7], m_top))
    g.append(_cmul(g[8], m512))
    re, im = [_dot_nt(jnp.concatenate([z[p] for z in g], axis=0),
                      jnp.concatenate([z[p] for z in e], axis=0)) for p in range(2)]
    return re + im


def _unmix(lo, hi):
    row = lax.broadcasted_iota(i32, (8, _T), 0)
    out = []
    for m in range(len(_PAIRS)):
        x, y = lo[8 * m:8 * m + 8], hi[8 * m:8 * m + 8]
        out += [jnp.where(row < 4, x, y), pltpu.roll(jnp.where(row < 4, y, x), 4, 0)]
    return out


def _lag_blocks(tap, lag0):
    lane = lax.broadcasted_iota(i32, (8, _T), 1)
    row = lax.broadcasted_iota(i32, (8, _T), 0)
    for h in range(2):
        def take(big, r, fine):
            s = ((_T * h + fine) >> 3) & 31
            return jnp.take_along_axis(tap(_TAPS.index((big, r))),
                                       ((s & 15) << 3) + (row ^ ((s >> 4) << 2)),
                                       axis=1, mode="promise_in_bounds")

        top = [take(big, 8, _round_lag(lane, 8) - 8) for big in range(_NB // 2)]
        for big, blk in enumerate(top):
            st = _lag_step(2 * big + h)
            lag = _round_lag(lane, st)
            if h == 0:
                blk = jnp.where(lag == 0, top[big - 1] if big else lag0, blk)
            for r in range(st, 8, st):
                blk = jnp.where((lag & 7) == r, take(big, r, lane), blk)
            yield 2 * big + h, blk


def _kernel(x_hbm, ar_hbm, ai_hbm, br_hbm, bi_hbm, cr_hbm, ci_hbm, ldt_hbm, dsk_hbm, wr_hbm,
            wg_hbm, wu_hbm, wd_hbm, fwd_hbm, inv_hbm, o_hbm,
            x_v, o_v, par_v, ldt_v, dsk_v, wr_v, wg_v, wu_v, wd_v, fwd_v, inv_v,
            skip_v, k0_v, arena, s_v, dt_v, mode_v, tap_v, k_v, xc_v, stat_v, key_v, sel_v, hid_v,
            spec_a, spec_b, kf_v, sem, w_sem, o_sem):
    row = lax.broadcasted_iota(i32, (8, _T), 0)
    lane = lax.broadcasted_iota(i32, (8, _T), 1)
    copies = {}

    def start(name, src, dst):
        copies[name] = pltpu.make_async_copy(src, dst, sem.at[len(copies)])
        copies[name].start()

    def wait(*names):
        for name in names:
            copies[name].wait()

    def hidden_copies(n):
        cols = pl.ds(_aligned(n * _FCH, _FCH), _FCH)
        return [pltpu.make_async_copy(w.at[:, cols], v.at[:, cols], w_sem.at[2 * n + k])
                for k, (w, v) in enumerate(((wg_hbm, wg_v), (wu_hbm, wu_v)))]

    def chunk_rows(n):
        return pl.ds(_aligned(n * _OCH, 32), _OCH)

    def down_copy(n):
        return pltpu.make_async_copy(wd_hbm.at[chunk_rows(n)], wd_v.at[chunk_rows(n)],
                                     w_sem.at[2 * _NF + n])

    def out_copy(n):
        return pltpu.make_async_copy(o_v.at[chunk_rows(n)], o_hbm.at[chunk_rows(n)], o_sem.at[n])

    def start_parameters(part, rows):
        for n, src in enumerate((ar_hbm, ai_hbm, br_hbm, bi_hbm, cr_hbm, ci_hbm)):
            start((part, n), src.at[rows], par_v.at[n, rows])

    with jax.named_scope("init"):
        start("ldt", ldt_hbm, ldt_v)
        start("dsk", dsk_hbm, dsk_v)
        start_parameters(0, pl.ds(0, 32 * _GA))
        start("fwd", fwd_hbm, fwd_v)
        arena[0, _ROW_W:_ROW_P] = jnp.zeros((_ROW_P - _ROW_W, 8, _T), i32)
        tap_v[...] = jnp.zeros(tap_v.shape, i32)
        k_v[...] = jnp.zeros(k_v.shape, i32)
        key_v[...] = jnp.zeros(key_v.shape, f32)
        wait("ldt")
        start_parameters(1, pl.ds(32 * _GA, _D - 32 * _GA))
        start("x", x_hbm, x_v)
        start("wr", wr_hbm, wr_v)
        start("inv", inv_hbm, inv_v)
        dt = pltpu.bitcast(_column(jnp.exp(ldt_v[...].astype(f32))).astype(bf16), i32)
        for g in range(_NG):
            dt_v[g] = dt[8 * g:8 * g + 8]
        wait("dsk")
        skip_v[...] = _column(dsk_v[...].astype(f32)).astype(bf16)
        wait(*[(0, n) for n in range(6)])

    def compact(ref, k, h):
        out = ref[k, 8 * h]
        for s in range(1, 8):
            out = jnp.where(row == s, ref[k, 8 * h + s], out)
        return out

    def layer_norm():
        wait("x", "wr", "inv")
        for cp in hidden_copies(1):
            cp.start()

        def moments(b, carry):
            cols = pl.ds(_aligned(b * _T, _T), _T)
            pivot = jnp.broadcast_to(_even_odd(x_v[:16, cols])[0][:1], (8, _T))
            s1, s2 = [None] * 2, [None] * 2
            for g in range(_NG):
                for h, x in enumerate(_even_odd(x_v[pl.ds(16 * g, 16), cols])):
                    d = x - pivot
                    xc_v[b, 2 * g + h] = d
                    s1[h] = s1[h] + d if g else d
                    s2[h] = s2[h] + d * d if g else d * d
            for k, s in enumerate((s1, s2)):
                stat_v[k, b] = jnp.broadcast_to(jnp.sum(s[0] + s[1], axis=0, keepdims=True), (8, _T))
            stat_v[2, b] = pivot
            return carry

        lax.fori_loop(0, _NB, moments, 0, unroll=2)
        for h in range(_NB // 8):
            m1, m2, pivot = compact(stat_v, 0, h) / _D, compact(stat_v, 1, h) / _D, compact(stat_v, 2, h)
            var = jnp.maximum(m2 - m1 * m1, 0.0)
            shift = _rnd(pivot + m1) - pivot
            gain = 0.5 / _rnd(jnp.sqrt(_rnd(_rnd(var) + _rnd(jnp.full_like(var, _EPS)))))
            for s in range(8):
                stat_v[0, 8 * h + s] = jnp.broadcast_to(shift[s:s + 1], (8, _T))
                stat_v[1, 8 * h + s] = jnp.broadcast_to(gain[s:s + 1], (8, _T))
        wr = jnp.broadcast_to(wr_v[...].astype(f32).reshape(1, _D), (8, _D)).astype(bf16)

        def scale(b, carry):
            shift, gain = stat_v[0, b], stat_v[1, b]
            xn = [_interleave(*[(xc_v[b, 2 * g + h] - shift) * gain for h in range(2)])
                  for g in range(_NG)]
            for g in range(_NG):
                arena[g // _GC, _ROW_X + (g % _GC) * _NB + b] = xn[g]
            stat_v[2, b] = _dot(wr, pltpu.bitcast(jnp.concatenate(xn, axis=0), bf16))
            return carry

        lax.fori_loop(0, _NB, scale, 0, unroll=8)
        for h in range(_NB // 8):
            bits = pltpu.bitcast(_rnd(2.0 * compact(stat_v, 2, h)) + 0.0, i32) >> 16
            rank = jnp.where(bits < 0, ~bits, bits + 0x8000)
            token = (8 * h + row) * _T + lane
            key_v[h] = pltpu.bitcast((1 << 28) + rank * _L + (_L - 1 - token), f32)

    def pop_best(c):
        best = jnp.max(jnp.max(jnp.maximum(key_v[0], key_v[1]), axis=0, keepdims=True),
                       axis=1, keepdims=True)
        key_v[2] = jnp.where(row == c, best, key_v[2])
        for h in range(2):
            key_v[h] = jnp.where(key_v[h] == best, 0.0, key_v[h])

    def modes(step):
        for u in range(_GA):
            grp = step * _GA + u
            rows = pl.ds(_aligned(grp * 16, 16), 16)
            par = [_even_odd(dt_v[grp])] + [_even_odd(par_v[n, rows, :]) for n in range(6)]
            k0 = []
            for h, skip in enumerate(_even_odd(skip_v[rows, :])):
                z = _modes(*[p[h] for p in par])
                for n in range(4):
                    mode_v[u, h, n] = z[n]
                k0.append(skip + jnp.sum(z[0], axis=1, keepdims=True))
            k0_v[grp] = _interleave(*k0)

    def dft(rows):
        z = _dot(jnp.concatenate([pltpu.bitcast(r, bf16) for r in rows], axis=0), fwd_v[...])
        return [[(z[o:o + 8, :_T], z[o:o + 8, _T:])
                 for o in range((h // 2) * 16 * _NB + 8 * (h % 2), (h // 2 + 1) * 16 * _NB, 16)]
                for h in range(2 * len(rows) // _NB)]

    def spread(step, u):
        for j, blk in _lag_blocks(lambda n: tap_v[u, n], k0_v[step * _GA + u]):
            k_v[u, j] = blk

    def filter_spectra(step, us, zero=0):
        for h, blocks in enumerate(dft([k_v[u + zero, j] for u in us for j in range(_NB)])):
            for j, (re, im) in enumerate(blocks):
                for p, val in enumerate((re, re + im, im - re)):
                    kf_v[2 * (step * _GA + us[0]) + h, p * _PLANE + j] = val

    def filter_step(i, zero, extra=lambda u: None):
        for u in range(_GA):
            if u == 0:
                filter_spectra(jnp.maximum(i - 2, 0), range(_GA // 2, _GA), zero)
            if u == _GA // 2:
                filter_spectra(jnp.maximum(i - 1, 0), range(_GA // 2), zero)
            spread(jnp.maximum(i - 1, 0), u)
            v = [[_vandermonde(*seeds) for seeds in _seeds(
                (mode_v[u, h, 0], mode_v[u, h, 1]), (mode_v[u, h, 2], mode_v[u, h, 3]))]
                 for h in range(2)]
            for n, tap in enumerate(_unmix(*map(_interleave, *v))):
                tap_v[u, n] = tap
            extra(u)

    def phase_a(i, carry):
        @pl.when(i == 1)
        def _():
            wait(*[(1, n) for n in range(6)])
            for cp in hidden_copies(0):
                cp.start()

        pl.when(i == _LN_STEP)(layer_norm)
        for c in range(2):
            pop_best(2 * (i - _LN_STEP) + c)
        filter_step(i, i >> 8)
        modes(i + 1)

    with jax.named_scope("A"):
        modes(0)
        wait("fwd")
        lax.fori_loop(0, _NG // _GA - 1, phase_a, None)

    def input_spectra(rows, dst):
        z = dft(rows)
        for h, t in enumerate(z):
            for b, (re, im) in enumerate(t):
                if b:
                    re, im = re + t[b - 1][1], im - t[b - 1][0]
                for p, val in enumerate((re + im, im, re)):
                    dst[(h * 3 + p) * _PLANE + b] = val
        return z

    def w_row(c, r):
        return jnp.concatenate(
            [pltpu.bitcast(arena[c, _ROW_W + q * _WQ + r], f32) for q in range(2)], axis=1)

    def routed_tokens():
        return _L - 1 - (pltpu.bitcast(key_v[2], i32) & (_L - 1))

    with jax.named_scope("topk"):
        for n in range(2, _NF):
            for cp in hidden_copies(n):
                cp.start()
        token = routed_tokens()
        picked = []

        def gather(u):
            tokens = range(u * _C // _GA, (u + 1) * _C // _GA)
            blocks = jnp.concatenate(
                [pltpu.bitcast(jnp.concatenate(
                    [arena[g // _GC, _ROW_X + (g % _GC) * _NB + (token[t, 0] >> 7)]
                     for g in range(_NG)], axis=0), bf16) for t in tokens], axis=1)
            pick = jnp.concatenate(
                [jnp.where((row == t) & ((token & (_T - 1)) == lane), 2.0, 0.0) for t in tokens],
                axis=1).astype(bf16)
            picked.append(_dot_nt(pick, blocks))

        filter_step(_NG // _GA - 1, token[0, 0] >> 11, gather if _MERGE else lambda u: None)
        for u in range(0 if _MERGE else _GA):
            gather(u)
        x_sel = sum(picked[1:], picked[0])
        for n in range(_NO):
            sel_v[n] = x_sel[:, n * _OCH:(n + 1) * _OCH]
        x_sel = jnp.concatenate([x_sel, jnp.zeros((8, _KT * _T - _D), f32)], axis=1)
        for n in range(_KT):
            arena[0, _ROW_SEL + n] = pltpu.bitcast(
                jnp.concatenate([x_sel[:, n * _T:(n + 1) * _T]] * 2, axis=0).astype(bf16), i32)
        input_spectra([arena[0, _ROW_X + r] for r in range(_R)], spec_a)
        filter_spectra(_NG // _GA - 2, range(_GA // 2, _GA))
        for u in range(_GA):
            spread(_NG // _GA - 1, u)
        filter_spectra(_NG // _GA - 1, range(_GA))

    def hidden_jobs(c):
        width = _F // (_NCH - _NO)
        gate = []

        def project(n):
            cols = pl.ds(_aligned(c * width + n // 2 * _T, _T), _T)
            x_sel = jnp.concatenate(
                [pltpu.bitcast(arena[c >> 8, _ROW_SEL + r], bf16) for r in range(_KT)], axis=1)
            gate.append(_rnd(_dot(x_sel[:, :_D], (wu_v if n % 2 else wg_v)[:, cols])[:8]))
            if n % 2:
                hid_v[:, cols] = (_rnd(_silu(gate[-2])) * gate[-1]).astype(bf16)

        return [(40 * n, lambda n=n: project(n)) for n in range(2 * width // _T)]

    def hidden_at(t, zero=0):
        return pl.ds(_aligned(_D + 8 * (t // _NB + zero), 8), 8), pl.ds((t % _NB) * _T, _T)

    def finish(n):
        for k in range(_OCH // 16 * _NB):
            c, r = n * (_OCH // (16 * _GC)) + k // _R, k % _R
            rows = pl.ds(_aligned(n * _OCH + 16 * (k // _NB), 16), 16)
            cols = pl.ds((k % _NB) * _T, _T)
            h = pltpu.bitcast(arena[c, _ROW_X + r], bf16).astype(f32)
            gated = s_v[c, pl.ds(16 * r, 16), :] * (h + h * jnp.tanh(h))
            o_v[rows, cols] = (x_v[rows, cols].astype(f32) + gated).astype(bf16)
            yield k

    def output_jobs(c):
        n = c - (_NCH - _NO)
        hid = [o_v[hidden_at(t, c >> 8)] for t in range(4)]
        for k in finish(jnp.maximum(n - 1, 0)):
            if k % 12 == 11:
                hid += [o_v[hidden_at(t, c >> 8)] for t in range(len(hid), len(hid) + 4)]
        rank = (pltpu.bitcast(key_v[2], i32) - (1 << 28)) >> 11
        score = pltpu.bitcast(jnp.where(rank >= 0x8000, rank - 0x8000, ~rank) << 16, f32)
        y = _rnd(_dot_nt(jnp.concatenate(hid, axis=1), wd_v[chunk_rows(n), :]))
        y = 0.5 * (sel_v[n] + _rnd(y * _rnd(jax.nn.sigmoid(score))[:, :_OCH]))
        col = jnp.concatenate([y, jnp.zeros((_T - _C, _OCH), f32)], axis=0).T
        col = pltpu.bitcast(col.astype(bf16), i32)
        token = routed_tokens()

        def scatter(t):
            hit = ((token & (_T - 1)) == lane)[t:t + 1]
            new = jnp.broadcast_to(col[:, t:t + 1], (_OCH // 2, _T))
            where = [(n * (_OCH // (16 * _GC)) + g // _GC,
                      _ROW_X + (g % _GC) * _NB + (token[t, 0] >> 7)) for g in range(_OCH // 16)]
            old = [arena[at] for at in where]
            for g, at in enumerate(where):
                arena[at] = jnp.where(hit, new[8 * g:8 * g + 8], old[g])

        return [(_S0 + _S1 * t, lambda t=t: scatter(t)) for t in range(_C)]

    def conv_step(c, cur, nxt, ffn_jobs, delay, pace):
        c_next, c_prev = jnp.minimum(c + 1, _NCH - 1), jnp.maximum(c - 1, 0)
        zero = c >> 8
        fwd_rows, inv_rows, results = [], [], []

        def transform():
            y = _dot(jnp.concatenate(inv_rows, axis=0), inv_v[...])
            s_v[c_prev] = y
            results.extend((y, input_spectra(fwd_rows, nxt)))

        def drain(r):
            y, z = results
            arena[c, _ROW_SEL - 1] = pltpu.bitcast(
                y[8 * r:8 * r + 8] + z[2 * (r // _R) + 1][r % _R // 2][r // 8 % 2], i32)

        jobs = sorted(
            ffn_jobs(c)
            + [(delay + 8 * r, lambda r=r: inv_rows.append(w_row(c_prev, r))) for r in range(2 * _R)]
            + [(delay + 16 * r, lambda r=r: fwd_rows.append(arena[c_next, _ROW_X + r]))
               for r in range(_R)]
            + [(delay + 16 * _R, transform)]
            + [(delay + _LAG + 8 * r, lambda r=r: drain(r)) for r in range(2 * _R - 17, 2 * _R, 8)],
            key=lambda job: job[0])

        def run_jobs(done):
            while jobs and done * (delay + 16 * _R) >= (jobs[0][0] - _LEAD) * pace * 18 * _GC:
                jobs.pop(0)[1]()

        run_jobs(0)
        for h in range(2 * _GC):
            for part in range(3):
                for plane in range(3):
                    kf = lambda b: kf_v[c * 2 * _GC + h + (zero >> part), plane * _PLANE + b]
                    uf = lambda b: cur[(zero >> part) + (h * 3 + plane) * _PLANE + b]
                    base = [pltpu.bitcast(arena[c + zero, _ROW_P + plane * 8 + m], f32)
                            for m in range(8) if part and plane]
                    k, u, out = [], [], []
                    for m in range(8):
                        if part == 0:
                            k.append(kf(2 * m))
                            u.append(uf(2 * m) + uf(2 * m + 1))
                        elif part == 1:
                            k.append(kf(2 * m) - kf(2 * m - 1) if m else kf(0))
                            u.append(uf(2 * m + 1))
                        else:
                            k.append(kf(2 * m) - kf(2 * m + 1))
                            u.append(uf(2 * m))
                        y = k[0] * u[m]
                        for j in range(1, m + 1):
                            y = y + k[j] * u[m - j]
                        if plane:
                            y = shared[m] - y if plane == 1 else shared[m] + y
                        out.append(y)
                        if part == 0 or plane == 0:
                            arena[c, _ROW_P + plane * 8 + m] = pltpu.bitcast(y, i32)
                        else:
                            b = 2 * m + part - 1
                            arena[c, _ROW_W + (plane - 1) * _WQ + ((h // 2) * _NB + b) * 2 + h % 2] = (
                                pltpu.bitcast(base[m] - y, i32))
                    if plane == 0:
                        shared = out
                    run_jobs((h * 3 + part) * 3 + plane + 1)
        assert not jobs

    def either(c, *args):
        lax.cond(c & 1 == 0, lambda: conv_step(c, spec_a, spec_b, *args),
                 lambda: conv_step(c, spec_b, spec_a, *args))

    def phase_c(part, carry):
        for cp in hidden_copies(part):
            cp.wait()

        @pl.when(part == _WD_STEP)
        def _():
            for n in range(_NO):
                down_copy(n).start()

        steps = (_NCH - _NO) // _NF
        return lax.fori_loop(part * steps, (part + 1) * steps,
                             lambda c, carry: either(c, hidden_jobs, 240, _PACE), carry)

    def phase_d(n, carry):
        down_copy(n).wait()
        either(n + _NCH - _NO, output_jobs, _G1, _PACE1)
        pl.when(n > 0)(lambda: out_copy(n - 1).start())

    with jax.named_scope("C"):
        lax.fori_loop(0, _NF, phase_c, None)
    with jax.named_scope("D"):
        for t in range(_F // _T):
            o_v[hidden_at(t)] = hid_v[:, t * _T:(t + 1) * _T]
        lax.fori_loop(0, _NO, phase_d, None)
    with jax.named_scope("tail"):
        s_v[_NCH - 1] = _dot(
            jnp.concatenate([w_row(_NCH - 1, r) for r in range(2 * _R)], axis=0), inv_v[...])
        for k in finish(_NO - 1):
            if k % _R == _R - 1:
                rows = pl.ds((_NO - 1) * _OCH + k // _R * 16 * _GC, 16 * _GC)
                start(("out", k // _R), o_v.at[rows], o_hbm.at[rows])
    with jax.named_scope("end"):
        for n in range(_NO - 1):
            out_copy(n).wait()
        wait(*[("out", k) for k in range(_OCH // (16 * _GC))])


@jax.jit
def pallas_recurrent_scan__ssm_conv_s4__moe_arch_mod__prompt_kernel(
    A_u: jax.Array,
    A_A_re: jax.Array,
    A_A_im: jax.Array,
    A_B_re: jax.Array,
    A_B_im: jax.Array,
    A_C_re: jax.Array,
    A_C_im: jax.Array,
    A_log_dt: jax.Array,
    A_Dskip: jax.Array,
    B_x: jax.Array,
    B_w_r: jax.Array,
    B_w_gate: jax.Array,
    B_w_up: jax.Array,
    B_w_down: jax.Array,
):
    del B_x
    assert A_u.shape == (1, _L, _D) and A_A_re.shape == (_D, _N) and B_w_gate.shape == (_D, _F)
    assert A_u.dtype == bf16 and A_A_re.dtype == bf16
    hbm = pl.BlockSpec(memory_space=pl.ANY)
    vmem = pltpu.VMEM
    out = pl.pallas_call(
        _kernel,
        out_shape=jax.ShapeDtypeStruct((_D, _L), bf16),
        in_specs=[hbm] * 15,
        out_specs=hbm,
        scratch_shapes=[
            vmem((_D, _L), bf16), vmem((_D + 32, _L), bf16),
            vmem((6, _D, _N), bf16), vmem((_D,), bf16), vmem((_D,), bf16), vmem((_D,), bf16),
            vmem((_D, _F), bf16), vmem((_D, _F), bf16), vmem((_D, _F), bf16),
            vmem((_T, 2 * _T), bf16), vmem((2 * _T, _T), f32),
            vmem((_D, _T), bf16), vmem((_NG, 8, _T), i32),
            vmem((_NCH, _ROWS, 8, _T), i32), vmem((_NCH, 16 * _R, _T), f32),
            vmem((_NG, 8, _T), i32), vmem((_GA, 2, 4, 8, _N), f32), vmem((_GA, len(_TAPS), 8, _T), i32),
            vmem((_GA, _NB, 8, _T), i32),
            vmem((_NB, 2 * _NG, 8, _T), f32), vmem((3, _NB, 8, _T), f32), vmem((3, 8, _T), f32),
            vmem((_NO, 8, _OCH), f32), vmem((8, _F), bf16),
            *[vmem((2 * _GC * 3 * _PLANE, 8, _T), f32)] * 2, vmem((2 * _NG, 3 * _PLANE, 8, _T), f32),
            pltpu.SemaphoreType.DMA((21,)), pltpu.SemaphoreType.DMA((2 * _NF + _NO,)),
            pltpu.SemaphoreType.DMA((_NO,)),
        ],
        compiler_params=pltpu.CompilerParams(vmem_limit_bytes=100 * 2**20),
    )(A_u.reshape(_L, _D).T, A_A_re, A_A_im, A_B_re, A_B_im, A_C_re, A_C_im, A_log_dt, A_Dskip,
      B_w_r, B_w_gate, B_w_up, B_w_down.T, _FWD, _INV)
    return out.T.reshape(1, _L, _D)
```

```python
import jax
import jax.numpy as jnp
import numpy as np
from jax import lax
import jax.experimental.pallas as pl
import jax.experimental.pallas.tpu as pltpu

_D, _L, _N, _F, _C = 576, 2048, 128, 4608, 8
_T = 128
_NB = _L // _T
_EPS = 1e-5
_GA = 4
_GC = 2
_NG = _D // 16
_NCH = _NG // _GC
_R = _GC * _NB
_ROW_X, _ROW_W, _ROW_P, _ROWS = 0, _R, 5 * _R + 8, 5 * _R + 8 + 24
_PLANE, _WQ = _NB + 2, 2 * _R + 2
_ROW_SEL = 5 * _R + 3
_MERGE = 1
_KT = -(-_D // _T)
_NO, _OCH = 6, _D // 6
_NF = 3
_FCH = _F // _NF
_LN_STEP = 4
_WD_STEP = 1
_PACE, _PACE1, _LEAD, _LAG, _G1, _S0, _S1 = 0.87, 0.8, 32, 140, 32, 520, 20

f32, bf16, i32 = jnp.float32, jnp.bfloat16, jnp.int32


def _dft_constants():
    theta = (np.pi / 2 + 2 * np.pi * np.arange(_T)) / _T
    ang = np.arange(_T)[:, None] * theta[None, :]
    c, s = np.cos(ang), np.sin(ang)
    fwd = np.concatenate([c, s], axis=1)
    bits = fwd.astype(bf16).view(np.uint16).astype(np.uint32)
    words = (bits[0::2] | bits[1::2] << 16).view(np.int32)
    return words, (fwd.T * (2 / _T)).astype(np.float32)


_FWD, _INV = _dft_constants()


def _lag_step(j):
    return max(1, (1 << (j * _T).bit_length()) >> 8)


def _round_lag(p, st):
    if st == 1:
        return p
    return (p + (st // 2 - 1) + ((p >> (st.bit_length() - 1)) & 1)) & ~(st - 1)


assert np.array_equal(
    np.concatenate([j * _T + _round_lag(np.arange(_T), _lag_step(j)) for j in range(_NB)]),
    np.arange(_L).astype(bf16).astype(np.int64))

_PAIRS = (((0, 1), (0, 5)), ((0, 2), (0, 6)), ((0, 3), (0, 7)), ((0, 4), (0, 8)), ((1, 2), (1, 6)),
          ((1, 4), (1, 8)), ((2, 4), (2, 8)), ((3, 4), (3, 8)), ((4, 8), (5, 8)), ((6, 8), (7, 8)))
_TAPS = [k for pair in _PAIRS for k in pair]


def _aligned(i, n):
    return i if isinstance(i, int) else pl.multiple_of(i, n)


def _cmul(a, b):
    return a[0] * b[0] - a[1] * b[1], a[0] * b[1] + a[1] * b[0]


def _csq(a):
    return a[0] * a[0] - a[1] * a[1], (a[0] + a[0]) * a[1]


def _silu(x):
    h = 0.5 * x
    return h + h * jnp.tanh(h)


def _rnd(x):
    return x.astype(bf16).astype(f32)


def _dot(a, b):
    return jnp.dot(a, b, preferred_element_type=f32)


def _dot_nt(a, b):
    return lax.dot_general(a, b, (((1,), (1,)), ((), ())), preferred_element_type=f32)


def _column(v):
    return jnp.broadcast_to(v.reshape(1, _D), (_T, _D)).T


def _even_odd(x):
    return pltpu.bitcast(x << 16, f32), pltpu.bitcast(x & -65536, f32)


def _interleave(even, odd):
    return pltpu.bitcast(pltpu.pack_elementwise([even, odd], packed_dtype=bf16), i32)


def _modes(dt, ar, ai, br, bi, cr, ci):
    zr, zi = dt * ar, dt * ai
    mag = jnp.exp(zr)
    return _cmul((cr, ci), (dt * br, dt * bi)) + (mag * jnp.cos(zi), mag * jnp.sin(zi))


def _seeds(w, a1):
    a = {1: a1}
    for n in range(9):
        a[2 << n] = _csq(a[1 << n])
    row = lax.broadcasted_iota(i32, (8, _N), 0)

    def conj(z):
        return z[0], -z[1]

    def mix(z0, z1):
        rolled = [pltpu.roll(x, 4, 0) for x in z1]
        return ([jnp.where(row < 4, x, y) for x, y in zip(z0, rolled)],
                [jnp.where(row < 4, y, x) for x, y in zip(z0, rolled)])

    def dup(z):
        return [[jnp.take_along_axis(x, (row & 3) + 4 * q, axis=0, mode="promise_in_bounds")
                 for x in z] for q in range(2)]

    wa = _cmul(w, a[1])
    return zip(mix((1.0, 0.0), conj(a[128])), dup(conj(a[8])), dup(conj(a[32])),
               mix(wa, _cmul(wa, a[4])), dup(a[1]), dup(a[256]),
               mix(_cmul(a[256], a[4]), a[512]), dup(a[512]))


def _vandermonde(e0, m8, m32, g0, m1, m256, m_top, m512):
    e = [e0]
    for s in range(1, 16):
        e.append(_cmul(e[s - 1], m8) if s < 4 else _cmul(e[s - 4], m32))
    g = [g0]
    for _ in range(3):
        g.append(_cmul(g[-1], m1))
    g += [_cmul(g[1], m256), _cmul(g[3], m256)]
    g += [_cmul(g[3], m512), _cmul(g[5], m512)]
    g.append(_cmul(g[7], m_top))
    g.append(_cmul(g[8], m512))
    re, im = [_dot_nt(jnp.concatenate([z[p] for z in g], axis=0),
                      jnp.concatenate([z[p] for z in e], axis=0)) for p in range(2)]
    return re + im


def _unmix(lo, hi):
    row = lax.broadcasted_iota(i32, (8, _T), 0)
    out = []
    for m in range(len(_PAIRS)):
        x, y = lo[8 * m:8 * m + 8], hi[8 * m:8 * m + 8]
        out += [jnp.where(row < 4, x, y), pltpu.roll(jnp.where(row < 4, y, x), 4, 0)]
    return out


def _lag_blocks(tap, lag0):
    lane = lax.broadcasted_iota(i32, (8, _T), 1)
    row = lax.broadcasted_iota(i32, (8, _T), 0)
    for h in range(2):
        def take(big, r, fine):
            s = ((_T * h + fine) >> 3) & 31
            return jnp.take_along_axis(tap(_TAPS.index((big, r))),
                                       ((s & 15) << 3) + (row ^ ((s >> 4) << 2)),
                                       axis=1, mode="promise_in_bounds")

        top = [take(big, 8, _round_lag(lane, 8) - 8) for big in range(_NB // 2)]
        for big, blk in enumerate(top):
            st = _lag_step(2 * big + h)
            lag = _round_lag(lane, st)
            if h == 0:
                blk = jnp.where(lag == 0, top[big - 1] if big else lag0, blk)
            for r in range(st, 8, st):
                blk = jnp.where((lag & 7) == r, take(big, r, lane), blk)
            yield 2 * big + h, blk


def _kernel(x_hbm, ar_hbm, ai_hbm, br_hbm, bi_hbm, cr_hbm, ci_hbm, ldt_hbm, dsk_hbm, wr_hbm,
            wg_hbm, wu_hbm, wd_hbm, fwd_hbm, inv_hbm, o_hbm,
            x_v, o_v, par_v, ldt_v, dsk_v, wr_v, wg_v, wu_v, wd_v, fwd_v, inv_v,
            skip_v, k0_v, arena, s_v, dt_v, mode_v, tap_v, k_v, xc_v, stat_v, key_v, sel_v, hid_v,
            spec_a, spec_b, kf_v, sem, w_sem, o_sem):
    row = lax.broadcasted_iota(i32, (8, _T), 0)
    lane = lax.broadcasted_iota(i32, (8, _T), 1)
    groups = {}

    def start(name, src, dst):
        slot, pairs = groups.setdefault(name, (len(groups), []))
        pairs.append((src, dst))
        pltpu.make_async_copy(src, dst, sem.at[slot]).start()

    def wait(name):
        slot, pairs = groups[name]
        for src, dst in pairs:
            pltpu.make_async_copy(src, dst, sem.at[slot]).wait()

    def hidden_copies(n):
        cols = pl.ds(_aligned(n * _FCH, _FCH), _FCH)
        return [pltpu.make_async_copy(w.bitcast(i32).at[:, cols], v.at[:, cols], w_sem.at[n])
                for w, v in ((wg_hbm, wg_v), (wu_hbm, wu_v))]

    def chunk_rows(n):
        return pl.ds(_aligned(n * _OCH, 32), _OCH)

    def down_copy(n):
        rows = pl.ds(_aligned(n * (_OCH // 2), 16), _OCH // 2)
        return pltpu.make_async_copy(wd_hbm.bitcast(i32).at[rows], wd_v.at[n], w_sem.at[_NF + n])

    def out_copy(n):
        return pltpu.make_async_copy(o_v.at[chunk_rows(n)], o_hbm.at[chunk_rows(n)], o_sem)

    def start_parameters(part, rows):
        for n, src in enumerate((ar_hbm, ai_hbm, br_hbm, bi_hbm, cr_hbm, ci_hbm)):
            start(part, src.bitcast(i32).at[rows], par_v.at[n, rows])

    with jax.named_scope("init"):
        start("vectors", ldt_hbm, ldt_v)
        start("vectors", dsk_hbm, dsk_v)
        start_parameters(0, pl.ds(0, 16 * _GA))
        start(0, fwd_hbm, fwd_v)
        arena[0, _ROW_W:_ROW_P] = jnp.zeros((_ROW_P - _ROW_W, 8, _T), i32)
        tap_v[...] = jnp.zeros(tap_v.shape, i32)
        k_v[...] = jnp.zeros(k_v.shape, i32)
        key_v[...] = jnp.zeros(key_v.shape, f32)
        wait("vectors")
        start_parameters(1, pl.ds(16 * _GA, _D // 2 - 16 * _GA))
        start("x", x_hbm.bitcast(i32), x_v)
        start("x", wr_hbm, wr_v)
        start("x", inv_hbm, inv_v)
        dt_v[...] = pltpu.bitcast(_column(jnp.exp(ldt_v[...].astype(f32))).astype(bf16), i32)
        skip_v[...] = pltpu.bitcast(_column(dsk_v[...].astype(f32)).astype(bf16), i32)
        wait(0)

    def compact(ref, k, h):
        out = ref[k, 8 * h]
        for s in range(1, 8):
            out = jnp.where(row == s, ref[k, 8 * h + s], out)
        return out

    def layer_norm():
        wait("x")
        for cp in hidden_copies(1):
            cp.start()

        def moments(b, carry):
            cols = pl.ds(_aligned(b * _T, _T), _T)
            pivot = jnp.broadcast_to(_even_odd(x_v[:8, cols])[0][:1], (8, _T))
            s1, s2 = [None] * 2, [None] * 2
            for g in range(_NG):
                words = x_v[pl.ds(8 * g, 8), cols]
                x = pltpu.bitcast(words, bf16).astype(f32)
                xc_v[b, g] = x
                for h in range(2):
                    d = x[8 * h:8 * h + 8] - pivot
                    s1[h] = s1[h] + d if g else d
                    s2[h] = s2[h] + d * d if g else d * d
            for k, s in enumerate((s1, s2)):
                stat_v[k, b] = jnp.broadcast_to(jnp.sum(s[0] + s[1], axis=0, keepdims=True), (8, _T))
            stat_v[2, b] = pivot
            return carry

        lax.fori_loop(0, _NB, moments, 0, unroll=2)
        for h in range(_NB // 8):
            m1, m2, pivot = compact(stat_v, 0, h) / _D, compact(stat_v, 1, h) / _D, compact(stat_v, 2, h)
            var = jnp.maximum(m2 - m1 * m1, 0.0)
            shift = _rnd(pivot + m1)
            gain = 0.5 / _rnd(jnp.sqrt(_rnd(_rnd(var) + _rnd(jnp.full_like(var, _EPS)))))
            for s in range(8):
                stat_v[0, 8 * h + s] = jnp.broadcast_to(shift[s:s + 1], (8, _T))
                stat_v[1, 8 * h + s] = jnp.broadcast_to(gain[s:s + 1], (8, _T))
        wr = jnp.broadcast_to(wr_v[...].astype(f32).reshape(1, _D), (8, _D)).astype(bf16)

        def scale(b, carry):
            shift, gain = stat_v[0, b], stat_v[1, b]
            xn = [_interleave(*[(xc_v[b, g, pl.ds(h, 8, stride=2), :] - shift) * gain for h in range(2)])
                  for g in range(_NG)]
            for g in range(_NG):
                arena[g // _GC, _ROW_X + (g % _GC) * _NB + b] = xn[g]
            stat_v[2, b] = _dot(wr, pltpu.bitcast(jnp.concatenate(xn, axis=0), bf16))
            return carry

        lax.fori_loop(0, _NB, scale, 0, unroll=8)
        for h in range(_NB // 8):
            bits = pltpu.bitcast(_rnd(2.0 * compact(stat_v, 2, h)) + 0.0, i32) >> 16
            rank = jnp.where(bits < 0, ~bits, bits + 0x8000)
            token = (8 * h + row) * _T + lane
            key_v[h] = pltpu.bitcast((1 << 28) + rank * _L + (_L - 1 - token), f32)

    def pop_best(c):
        best = jnp.max(jnp.max(jnp.maximum(key_v[0], key_v[1]), axis=0, keepdims=True),
                       axis=1, keepdims=True)
        key_v[2] = jnp.where(row == c, best, key_v[2])
        for h in range(2):
            key_v[h] = jnp.where(key_v[h] == best, 0.0, key_v[h])

    def modes(step):
        for u in range(_GA):
            grp = step * _GA + u
            rows = pl.ds(_aligned(grp * 8, 8), 8)
            par = [_even_odd(dt_v[rows, :])] + [_even_odd(par_v[n, rows, :]) for n in range(6)]
            k0 = []
            for h, skip in enumerate(_even_odd(skip_v[rows, :])):
                z = _modes(*[p[h] for p in par])
                for n in range(4):
                    mode_v[u, h, n] = z[n]
                k0.append(skip + jnp.sum(z[0], axis=1, keepdims=True))
            k0_v[grp] = _interleave(*k0)

    def dft(rows):
        z = _dot(jnp.concatenate([pltpu.bitcast(r, bf16) for r in rows], axis=0), pltpu.bitcast(fwd_v[...], bf16))
        return [[(z[o:o + 8, :_T], z[o:o + 8, _T:])
                 for o in range((h // 2) * 16 * _NB + 8 * (h % 2), (h // 2 + 1) * 16 * _NB, 16)]
                for h in range(2 * len(rows) // _NB)]

    def spread(step, u):
        for j, blk in _lag_blocks(lambda n: tap_v[u, n], k0_v[step * _GA + u]):
            k_v[u, j] = blk

    def filter_spectra(step, us, zero=0):
        for h, blocks in enumerate(dft([k_v[u + zero, j] for u in us for j in range(_NB)])):
            for j, (re, im) in enumerate(blocks):
                for p, val in enumerate((re, re + im, im - re)):
                    kf_v[2 * (step * _GA + us[0]) + h, p * _PLANE + j] = val

    def filter_step(i, zero, extra=lambda u: None):
        for u in range(_GA):
            if u == 0:
                filter_spectra(jnp.maximum(i - 2, 0), range(_GA // 2, _GA), zero)
            if u == _GA // 2:
                filter_spectra(jnp.maximum(i - 1, 0), range(_GA // 2), zero)
            spread(jnp.maximum(i - 1, 0), u)
            v = [[_vandermonde(*seeds) for seeds in _seeds(
                (mode_v[u, h, 0], mode_v[u, h, 1]), (mode_v[u, h, 2], mode_v[u, h, 3]))]
                 for h in range(2)]
            for n, tap in enumerate(_unmix(*map(_interleave, *v))):
                tap_v[u, n] = tap
            extra(u)

    def phase_a(i, carry):
        @pl.when(i == 1)
        def _():
            wait(1)
            for cp in hidden_copies(0):
                cp.start()

        pl.when(i == _LN_STEP)(layer_norm)
        for c in range(2):
            pop_best(2 * (i - _LN_STEP) + c)
        filter_step(i, i >> 8)
        modes(i + 1)

    with jax.named_scope("A"):
        modes(0)
        lax.fori_loop(0, _NG // _GA - 1, phase_a, None)

    def input_spectra(rows, dst):
        z = dft(rows)
        for h, t in enumerate(z):
            for b, (re, im) in enumerate(t):
                if b:
                    re, im = re + t[b - 1][1], im - t[b - 1][0]
                for p, val in enumerate((re + im, im, re)):
                    dst[(h * 3 + p) * _PLANE + b] = val
        return z

    def w_row(c, r):
        return jnp.concatenate(
            [pltpu.bitcast(arena[c, _ROW_W + q * _WQ + r], f32) for q in range(2)], axis=1)

    def routed_tokens():
        return _L - 1 - (pltpu.bitcast(key_v[2], i32) & (_L - 1))

    with jax.named_scope("topk"):
        for n in range(2, _NF):
            for cp in hidden_copies(n):
                cp.start()
        token = routed_tokens()
        picked = []

        def gather(u):
            tokens = range(u * _C // _GA, (u + 1) * _C // _GA)
            blocks = jnp.concatenate(
                [pltpu.bitcast(jnp.concatenate(
                    [arena[g // _GC, _ROW_X + (g % _GC) * _NB + (token[t, 0] >> 7)]
                     for g in range(_NG)], axis=0), bf16) for t in tokens], axis=1)
            pick = jnp.concatenate(
                [jnp.where((row == t) & ((token & (_T - 1)) == lane), 2.0, 0.0) for t in tokens],
                axis=1).astype(bf16)
            picked.append(_dot_nt(pick, blocks))

        filter_step(_NG // _GA - 1, token[0, 0] >> 11, gather if _MERGE else lambda u: None)
        for u in range(0 if _MERGE else _GA):
            gather(u)
        x_sel = sum(picked[1:], picked[0])
        for n in range(_NO):
            sel_v[n] = x_sel[:, n * _OCH:(n + 1) * _OCH]
        x_sel = jnp.concatenate([x_sel, jnp.zeros((8, _KT * _T - _D), f32)], axis=1)
        for n in range(_KT):
            arena[0, _ROW_SEL + n] = pltpu.bitcast(
                jnp.concatenate([x_sel[:, n * _T:(n + 1) * _T]] * 2, axis=0).astype(bf16), i32)
        input_spectra([arena[0, _ROW_X + r] for r in range(_R)], spec_a)
        filter_spectra(_NG // _GA - 2, range(_GA // 2, _GA))
        for u in range(_GA):
            spread(_NG // _GA - 1, u)
        filter_spectra(_NG // _GA - 1, range(_GA))

    def hidden_jobs(c):
        width = _F // (_NCH - _NO)
        gate = []

        def project(n):
            cols = pl.ds(_aligned(c * width + n // 2 * _T, _T), _T)
            x_sel = jnp.concatenate(
                [pltpu.bitcast(arena[c >> 8, _ROW_SEL + r], bf16) for r in range(_KT)], axis=1)
            gate.append(_rnd(_dot(x_sel[:, :_D], pltpu.bitcast((wu_v if n % 2 else wg_v)[:, cols], bf16))[:8]))
            if n % 2:
                hid_v[:, cols] = (_rnd(_silu(gate[-2])) * gate[-1]).astype(bf16)

        return [(40 * n, lambda n=n: project(n)) for n in range(2 * width // _T)]

    def hidden_at(t, zero=0):
        return pl.ds(_aligned(_D + 8 * (t // _NB + zero), 8), 8), pl.ds((t % _NB) * _T, _T)

    def finish(n):
        for k in range(_OCH // 16 * _NB):
            c, r = n * (_OCH // (16 * _GC)) + k // _R, k % _R
            rows = pl.ds(_aligned(n * _OCH + 16 * (k // _NB), 16), 16)
            cols = pl.ds((k % _NB) * _T, _T)
            h = pltpu.bitcast(arena[c, _ROW_X + r], bf16).astype(f32)
            gated = s_v[c, pl.ds(16 * r, 16), :] * (h + h * jnp.tanh(h))
            o_v[rows, cols] = (xc_v[k % _NB, n * (_OCH // 16) + k // _NB] + gated).astype(bf16)
            yield k

    def output_jobs(c):
        n = c - (_NCH - _NO)
        hid = [o_v[hidden_at(t, c >> 8)] for t in range(4)]
        for k in finish(jnp.maximum(n - 1, 0)):
            if k % 12 == 11:
                hid += [o_v[hidden_at(t, c >> 8)] for t in range(len(hid), len(hid) + 4)]
        rank = (pltpu.bitcast(key_v[2], i32) - (1 << 28)) >> 11
        score = pltpu.bitcast(jnp.where(rank >= 0x8000, rank - 0x8000, ~rank) << 16, f32)
        y = _rnd(_dot_nt(jnp.concatenate(hid, axis=1), pltpu.bitcast(wd_v[n], bf16)))
        y = 0.5 * (sel_v[n] + _rnd(y * _rnd(jax.nn.sigmoid(score))[:, :_OCH]))
        col = jnp.concatenate([y, jnp.zeros((_T - _C, _OCH), f32)], axis=0).T
        col = pltpu.bitcast(col.astype(bf16), i32)
        token = routed_tokens()

        def scatter(t):
            hit = ((token & (_T - 1)) == lane)[t:t + 1]
            new = jnp.broadcast_to(col[:, t:t + 1], (_OCH // 2, _T))
            where = [(n * (_OCH // (16 * _GC)) + g // _GC,
                      _ROW_X + (g % _GC) * _NB + (token[t, 0] >> 7)) for g in range(_OCH // 16)]
            old = [arena[at] for at in where]
            for g, at in enumerate(where):
                arena[at] = jnp.where(hit, new[8 * g:8 * g + 8], old[g])

        return [(_S0 + _S1 * t, lambda t=t: scatter(t)) for t in range(_C)]

    def conv_step(c, cur, nxt, ffn_jobs, delay, pace):
        c_next, c_prev = jnp.minimum(c + 1, _NCH - 1), jnp.maximum(c - 1, 0)
        zero = c >> 8
        fwd_rows, inv_rows, results = [], [], []

        def transform():
            y = _dot(jnp.concatenate(inv_rows, axis=0), inv_v[...])
            s_v[c_prev] = y
            results.extend((y, input_spectra(fwd_rows, nxt)))

        def drain(r):
            y, z = results
            arena[c, _ROW_SEL - 1] = pltpu.bitcast(
                y[8 * r:8 * r + 8] + z[2 * (r // _R) + 1][r % _R // 2][r // 8 % 2], i32)

        jobs = sorted(
            ffn_jobs(c)
            + [(delay + 8 * r, lambda r=r: inv_rows.append(w_row(c_prev, r))) for r in range(2 * _R)]
            + [(delay + 16 * r, lambda r=r: fwd_rows.append(arena[c_next, _ROW_X + r]))
               for r in range(_R)]
            + [(delay + 16 * _R, transform)]
            + [(delay + _LAG + 8 * r, lambda r=r: drain(r)) for r in range(2 * _R - 17, 2 * _R, 8)],
            key=lambda job: job[0])

        def run_jobs(done):
            while jobs and done * (delay + 16 * _R) >= (jobs[0][0] - _LEAD) * pace * 18 * _GC:
                jobs.pop(0)[1]()

        run_jobs(0)
        for h in range(2 * _GC):
            for part in range(3):
                for plane in range(3):
                    kf = lambda b: kf_v[c * 2 * _GC + h + (zero >> part), plane * _PLANE + b]
                    uf = lambda b: cur[(zero >> part) + (h * 3 + plane) * _PLANE + b]
                    base = [pltpu.bitcast(arena[c + zero, _ROW_P + plane * 8 + m], f32)
                            for m in range(8) if part and plane]
                    k, u, out = [], [], []
                    for m in range(8):
                        if part == 0:
                            k.append(kf(2 * m))
                            u.append(uf(2 * m) + uf(2 * m + 1))
                        elif part == 1:
                            k.append(kf(2 * m) - kf(2 * m - 1) if m else kf(0))
                            u.append(uf(2 * m + 1))
                        else:
                            k.append(kf(2 * m) - kf(2 * m + 1))
                            u.append(uf(2 * m))
                        y = k[0] * u[m]
                        for j in range(1, m + 1):
                            y = y + k[j] * u[m - j]
                        if plane:
                            y = shared[m] - y if plane == 1 else shared[m] + y
                        out.append(y)
                        if part == 0 or plane == 0:
                            arena[c, _ROW_P + plane * 8 + m] = pltpu.bitcast(y, i32)
                        else:
                            b = 2 * m + part - 1
                            arena[c, _ROW_W + (plane - 1) * _WQ + ((h // 2) * _NB + b) * 2 + h % 2] = (
                                pltpu.bitcast(base[m] - y, i32))
                    if plane == 0:
                        shared = out
                    run_jobs((h * 3 + part) * 3 + plane + 1)
        assert not jobs

    def either(c, *args):
        lax.cond(c & 1 == 0, lambda: conv_step(c, spec_a, spec_b, *args),
                 lambda: conv_step(c, spec_b, spec_a, *args))

    def phase_c(part, carry):
        for cp in hidden_copies(part):
            cp.wait()

        @pl.when(part == _WD_STEP)
        def _():
            for n in range(_NO):
                down_copy(n).start()

        steps = (_NCH - _NO) // _NF
        return lax.fori_loop(part * steps, (part + 1) * steps,
                             lambda c, carry: either(c, hidden_jobs, 240, _PACE), carry)

    def phase_d(n, carry):
        down_copy(n).wait()
        either(n + _NCH - _NO, output_jobs, _G1, _PACE1)
        pl.when(n > 0)(lambda: out_copy(n - 1).start())

    with jax.named_scope("C"):
        lax.fori_loop(0, _NF, phase_c, None)
    with jax.named_scope("D"):
        for t in range(_F // _T):
            o_v[hidden_at(t)] = hid_v[:, t * _T:(t + 1) * _T]
        lax.fori_loop(0, _NO, phase_d, None)
    with jax.named_scope("tail"):
        s_v[_NCH - 1] = _dot(
            jnp.concatenate([w_row(_NCH - 1, r) for r in range(2 * _R)], axis=0), inv_v[...])
        for k in finish(_NO - 1):
            if k % _R == _R - 1:
                rows = pl.ds((_NO - 1) * _OCH + k // _R * 16 * _GC, 16 * _GC)
                start("out", o_v.at[rows], o_hbm.at[rows])
    with jax.named_scope("end"):
        for n in range(_NO - 1):
            out_copy(n).wait()
        wait("out")


@jax.jit
def pallas_recurrent_scan__ssm_conv_s4__moe_arch_mod__prompt_kernel(
    A_u: jax.Array,
    A_A_re: jax.Array,
    A_A_im: jax.Array,
    A_B_re: jax.Array,
    A_B_im: jax.Array,
    A_C_re: jax.Array,
    A_C_im: jax.Array,
    A_log_dt: jax.Array,
    A_Dskip: jax.Array,
    B_x: jax.Array,
    B_w_r: jax.Array,
    B_w_gate: jax.Array,
    B_w_up: jax.Array,
    B_w_down: jax.Array,
):
    del B_x
    assert A_u.shape == (1, _L, _D) and A_A_re.shape == (_D, _N) and B_w_gate.shape == (_D, _F)
    assert A_u.dtype == bf16 and A_A_re.dtype == bf16
    hbm = pl.BlockSpec(memory_space=pl.ANY)
    vmem = pltpu.VMEM
    out = pl.pallas_call(
        _kernel,
        out_shape=jax.ShapeDtypeStruct((_D, _L), bf16),
        in_specs=[hbm] * 15,
        out_specs=hbm,
        scratch_shapes=[
            vmem((_D // 2, _L), i32), vmem((_D + 32, _L), bf16),
            vmem((6, _D // 2, _N), i32), vmem((_D,), bf16), vmem((_D,), bf16), vmem((_D,), bf16),
            vmem((_D // 2, _F), i32), vmem((_D // 2, _F), i32), vmem((_NO, _OCH // 2, _F), i32),
            vmem((_T // 2, 2 * _T), i32), vmem((2 * _T, _T), f32),
            vmem((_D // 2, _T), i32), vmem((_NG, 8, _T), i32),
            vmem((_NCH, _ROWS, 8, _T), i32), vmem((_NCH, 16 * _R, _T), f32),
            vmem((_D // 2, _T), i32), vmem((_GA, 2, 4, 8, _N), f32), vmem((_GA, len(_TAPS), 8, _T), i32),
            vmem((_GA, _NB, 8, _T), i32),
            vmem((_NB, _NG, 16, _T), f32), vmem((3, _NB, 8, _T), f32), vmem((3, 8, _T), f32),
            vmem((_NO, 8, _OCH), f32), vmem((8, _F), bf16),
            *[vmem((2 * _GC * 3 * _PLANE, 8, _T), f32)] * 2, vmem((2 * _NG, 3 * _PLANE, 8, _T), f32),
            pltpu.SemaphoreType.DMA((5,)), pltpu.SemaphoreType.DMA((_NF + _NO,)),
            pltpu.SemaphoreType.DMA(()),
        ],
        compiler_params=pltpu.CompilerParams(vmem_limit_bytes=100 * 2**20),
    )(A_u.reshape(_L, _D).T, A_A_re, A_A_im, A_B_re, A_B_im, A_C_re, A_C_im, A_log_dt, A_Dskip,
      B_w_r, B_w_gate, B_w_up, B_w_down.T, _FWD, _INV)
    return out.T.reshape(1, _L, _D)
```

```python
import jax
import jax.numpy as jnp
import numpy as np
from jax import lax
import jax.experimental.pallas as pl
import jax.experimental.pallas.tpu as pltpu

_D, _L, _N, _F, _C = 576, 2048, 128, 4608, 8
_T = 128
_NB = _L // _T
_EPS = 1e-5
_GA = 4
_GC = 2
_NG = _D // 16
_NCH = _NG // _GC
_R = _GC * _NB
_ROW_X, _ROW_W, _ROW_P, _ROWS = 0, _R, 5 * _R + 8, 5 * _R + 8 + 24
_PLANE, _WQ = _NB + 1, 2 * _R + 1
_ROW_SEL = 5 * _R + 3
_MERGE, _HOLD, _PRIO, _G2, _PACE2 = 1, 3, 0, 400, 0.83
_KT = -(-_D // _T)
_NO, _OCH = 6, _D // 6
_NF = 3
_FCH = _F // _NF
_LN_STEP = 4
_WD_STEP = 1
_PACE, _PACE1, _LEAD, _LAG, _G1, _S0, _S1 = 0.87, 0.8, 32, 140, 32, 520, 20

f32, bf16, i32 = jnp.float32, jnp.bfloat16, jnp.int32


def _dft_constants():
    theta = (np.pi / 2 + 2 * np.pi * np.arange(_T)) / _T
    ang = np.arange(_T)[:, None] * theta[None, :]
    c, s = np.cos(ang), np.sin(ang)
    fwd = np.concatenate([c, s], axis=1)
    bits = fwd.astype(bf16).view(np.uint16).astype(np.uint32)
    words = (bits[0::2] | bits[1::2] << 16).view(np.int32)
    return words, (fwd.T * (2 / _T)).astype(np.float32)


_FWD, _INV = _dft_constants()


def _lag_step(j):
    return max(1, (1 << (j * _T).bit_length()) >> 8)


def _round_lag(p, st):
    if st == 1:
        return p
    return (p + (st // 2 - 1) + ((p >> (st.bit_length() - 1)) & 1)) & ~(st - 1)


assert np.array_equal(
    np.concatenate([j * _T + _round_lag(np.arange(_T), _lag_step(j)) for j in range(_NB)]),
    np.arange(_L).astype(bf16).astype(np.int64))

_PAIRS = (((0, 1), (0, 5)), ((0, 2), (0, 6)), ((0, 3), (0, 7)), ((0, 4), (0, 8)), ((1, 2), (1, 6)),
          ((1, 4), (1, 8)), ((2, 4), (2, 8)), ((3, 4), (3, 8)), ((4, 8), (5, 8)), ((6, 8), (7, 8)))
_TAPS = [k for pair in _PAIRS for k in pair]


def _aligned(i, n):
    return i if isinstance(i, int) else pl.multiple_of(i, n)


def _cmul(a, b):
    return a[0] * b[0] - a[1] * b[1], a[0] * b[1] + a[1] * b[0]


def _csq(a):
    return a[0] * a[0] - a[1] * a[1], (a[0] + a[0]) * a[1]


def _silu(x):
    h = 0.5 * x
    return h + h * jnp.tanh(h)


def _rnd(x):
    return x.astype(bf16).astype(f32)


def _dot(a, b):
    return jnp.dot(a, b, preferred_element_type=f32)


def _dot_nt(a, b):
    return lax.dot_general(a, b, (((1,), (1,)), ((), ())), preferred_element_type=f32)


def _column(v):
    return jnp.broadcast_to(v.reshape(1, _D), (_T, _D)).T


def _even_odd(x):
    return pltpu.bitcast(x << 16, f32), pltpu.bitcast(x & -65536, f32)


def _interleave(even, odd):
    return pltpu.bitcast(pltpu.pack_elementwise([even, odd], packed_dtype=bf16), i32)


def _modes(dt, ar, ai, br, bi, cr, ci):
    zr, zi = dt * ar, dt * ai
    mag = jnp.exp(zr)
    return _cmul((cr, ci), (dt * br, dt * bi)) + (mag * jnp.cos(zi), mag * jnp.sin(zi))


def _seeds(w, a1):
    a = {1: a1}
    for n in range(9):
        a[2 << n] = _csq(a[1 << n])
    row = lax.broadcasted_iota(i32, (8, _N), 0)

    def conj(z):
        return z[0], -z[1]

    def mix(z0, z1):
        rolled = [pltpu.roll(x, 4, 0) for x in z1]
        return ([jnp.where(row < 4, x, y) for x, y in zip(z0, rolled)],
                [jnp.where(row < 4, y, x) for x, y in zip(z0, rolled)])

    def dup(z):
        return [[jnp.take_along_axis(x, (row & 3) + 4 * q, axis=0, mode="promise_in_bounds")
                 for x in z] for q in range(2)]

    wa = _cmul(w, a[1])
    return zip(mix((1.0, 0.0), conj(a[128])), dup(conj(a[8])), dup(conj(a[32])),
               mix(wa, _cmul(wa, a[4])), dup(a[1]), dup(a[256]),
               mix(_cmul(a[256], a[4]), a[512]), dup(a[512]))


def _vandermonde(e0, m8, m32, g0, m1, m256, m_top, m512):
    e = [e0]
    for s in range(1, 16):
        e.append(_cmul(e[s - 1], m8) if s < 4 else _cmul(e[s - 4], m32))
    g = [g0]
    for _ in range(3):
        g.append(_cmul(g[-1], m1))
    g += [_cmul(g[1], m256), _cmul(g[3], m256)]
    g += [_cmul(g[3], m512), _cmul(g[5], m512)]
    g.append(_cmul(g[7], m_top))
    g.append(_cmul(g[8], m512))
    re, im = [_dot_nt(jnp.concatenate([z[p] for z in g], axis=0),
                      jnp.concatenate([z[p] for z in e], axis=0)) for p in range(2)]
    return re + im


def _unmix(lo, hi):
    row = lax.broadcasted_iota(i32, (8, _T), 0)
    out = []
    for m in range(len(_PAIRS)):
        x, y = lo[8 * m:8 * m + 8], hi[8 * m:8 * m + 8]
        out += [jnp.where(row < 4, x, y), pltpu.roll(jnp.where(row < 4, y, x), 4, 0)]
    return out


def _lag_blocks(tap, lag0):
    lane = lax.broadcasted_iota(i32, (8, _T), 1)
    row = lax.broadcasted_iota(i32, (8, _T), 0)
    for h in range(2):
        def take(big, r, fine):
            s = ((_T * h + fine) >> 3) & 31
            return jnp.take_along_axis(tap(_TAPS.index((big, r))),
                                       ((s & 15) << 3) + (row ^ ((s >> 4) << 2)),
                                       axis=1, mode="promise_in_bounds")

        top = [take(big, 8, _round_lag(lane, 8) - 8) for big in range(_NB // 2)]
        for big, blk in enumerate(top):
            st = _lag_step(2 * big + h)
            lag = _round_lag(lane, st)
            if h == 0:
                blk = jnp.where(lag == 0, top[big - 1] if big else lag0, blk)
            for r in range(st, 8, st):
                blk = jnp.where((lag & 7) == r, take(big, r, lane), blk)
            yield 2 * big + h, blk


def _kernel(x_hbm, ar_hbm, ai_hbm, br_hbm, bi_hbm, cr_hbm, ci_hbm, ldt_hbm, dsk_hbm, wr_hbm,
            wg_hbm, wu_hbm, wd_hbm, fwd_hbm, inv_hbm, o_hbm,
            x_v, o_v, par_v, ldt_v, dsk_v, wr_v, wg_v, wu_v, wd_v, fwd_v, inv_v,
            skip_v, k0_v, arena, s_v, dt_v, mode_v, tap_v, k_v, xc_v, stat_v, key_v, sel_v, hid_v,
            spec_a, spec_b, kf_v, sem, w_sem, o_sem):
    row = lax.broadcasted_iota(i32, (8, _T), 0)
    lane = lax.broadcasted_iota(i32, (8, _T), 1)
    groups = {}

    def start(name, src, dst):
        slot, pairs = groups.setdefault(name, (len(groups), []))
        pairs.append((src, dst))
        pltpu.make_async_copy(src, dst, sem.at[slot]).start()

    def wait(name):
        slot, pairs = groups[name]
        for src, dst in pairs:
            pltpu.make_async_copy(src, dst, sem.at[slot]).wait()

    def hidden_copies(n):
        cols = pl.ds(_aligned(n * _FCH, _FCH), _FCH)
        return [pltpu.make_async_copy(w.bitcast(i32).at[:, cols], v.at[:, cols], w_sem.at[n])
                for w, v in ((wg_hbm, wg_v), (wu_hbm, wu_v))]

    def chunk_rows(n):
        return pl.ds(_aligned(n * _OCH, 32), _OCH)

    def down_copy(n):
        rows = pl.ds(_aligned(n * (_OCH // 2), 16), _OCH // 2)
        return pltpu.make_async_copy(wd_hbm.bitcast(i32).at[rows], wd_v.at[n], w_sem.at[_NF + n])

    def out_copy(n):
        return pltpu.make_async_copy(o_v.at[chunk_rows(n)], o_hbm.at[chunk_rows(n)], o_sem)

    def start_parameters(part, rows):
        for n, src in enumerate((ar_hbm, ai_hbm, br_hbm, bi_hbm, cr_hbm, ci_hbm)):
            start(part, src.bitcast(i32).at[rows], par_v.at[n, rows])

    with jax.named_scope("init"):
        start("vectors", ldt_hbm, ldt_v)
        start("vectors", dsk_hbm, dsk_v)
        start_parameters(0, pl.ds(0, 16 * _GA))
        start(0, fwd_hbm, fwd_v)
        arena[0, _ROW_W:_ROW_P] = jnp.zeros((_ROW_P - _ROW_W, 8, _T), i32)
        tap_v[...] = jnp.zeros(tap_v.shape, i32)
        k_v[...] = jnp.zeros(k_v.shape, i32)
        key_v[...] = jnp.zeros(key_v.shape, f32)
        wait("vectors")
        start_parameters(1, pl.ds(16 * _GA, _D // 2 - 16 * _GA))
        start("x", x_hbm.bitcast(i32), x_v)
        start("x", wr_hbm, wr_v)
        start("x", inv_hbm, inv_v)
        dt_v[...] = pltpu.bitcast(_column(jnp.exp(ldt_v[...].astype(f32))).astype(bf16), i32)
        skip_v[...] = pltpu.bitcast(_column(dsk_v[...].astype(f32)).astype(bf16), i32)
        wait(0)

    def compact(ref, k, h):
        out = ref[k, 8 * h]
        for s in range(1, 8):
            out = jnp.where(row == s, ref[k, 8 * h + s], out)
        return out

    def layer_norm():
        wait("x")
        for cp in hidden_copies(1):
            cp.start()

        def moments(b, carry):
            cols = pl.ds(_aligned(b * _T, _T), _T)
            pivot = jnp.broadcast_to(_even_odd(x_v[:8, cols])[0][:1], (8, _T))
            s1, s2 = [None] * 2, [None] * 2
            for g in range(_NG):
                words = x_v[pl.ds(8 * g, 8), cols]
                x = pltpu.bitcast(words, bf16).astype(f32)
                xc_v[b, g] = x
                for h in range(2):
                    d = x[8 * h:8 * h + 8] - pivot
                    s1[h] = s1[h] + d if g else d
                    s2[h] = s2[h] + d * d if g else d * d
            for k, s in enumerate((s1, s2)):
                stat_v[k, b] = jnp.broadcast_to(jnp.sum(s[0] + s[1], axis=0, keepdims=True), (8, _T))
            stat_v[2, b] = pivot
            return carry

        lax.fori_loop(0, _NB, moments, 0, unroll=4)
        for h in range(_NB // 8):
            m1, m2, pivot = compact(stat_v, 0, h) / _D, compact(stat_v, 1, h) / _D, compact(stat_v, 2, h)
            var = jnp.maximum(m2 - m1 * m1, 0.0)
            shift = _rnd(pivot + m1)
            gain = 0.5 / _rnd(jnp.sqrt(_rnd(_rnd(var) + _rnd(jnp.full_like(var, _EPS)))))
            for s in range(8):
                stat_v[0, 8 * h + s] = jnp.broadcast_to(shift[s:s + 1], (8, _T))
                stat_v[1, 8 * h + s] = jnp.broadcast_to(gain[s:s + 1], (8, _T))
        wr = jnp.broadcast_to(wr_v[...].astype(f32).reshape(1, _D), (8, _D)).astype(bf16)

        def scale(b, carry):
            shift, gain = stat_v[0, b], stat_v[1, b]
            xn = [_interleave(*[(xc_v[b, g, pl.ds(h, 8, stride=2), :] - shift) * gain for h in range(2)])
                  for g in range(_NG)]
            for g in range(_NG):
                arena[g // _GC, _ROW_X + (g % _GC) * _NB + b] = xn[g]
            stat_v[2, b] = _dot(wr, pltpu.bitcast(jnp.concatenate(xn, axis=0), bf16))
            return carry

        lax.fori_loop(0, _NB, scale, 0, unroll=16)
        for h in range(_NB // 8):
            bits = pltpu.bitcast(_rnd(2.0 * compact(stat_v, 2, h)) + 0.0, i32) >> 16
            rank = jnp.where(bits < 0, ~bits, bits + 0x8000)
            token = (8 * h + row) * _T + lane
            key_v[h] = pltpu.bitcast((1 << 28) + rank * _L + (_L - 1 - token), f32)

    def pop_best(c):
        best = jnp.max(jnp.max(jnp.maximum(key_v[0], key_v[1]), axis=0, keepdims=True),
                       axis=1, keepdims=True)
        key_v[2] = jnp.where(row == c, best, key_v[2])
        for h in range(2):
            key_v[h] = jnp.where(key_v[h] == best, 0.0, key_v[h])

    def modes(step):
        for u in range(_GA):
            grp = step * _GA + u
            rows = pl.ds(_aligned(grp * 8, 8), 8)
            par = [_even_odd(dt_v[rows, :])] + [_even_odd(par_v[n, rows, :]) for n in range(6)]
            k0 = []
            for h, skip in enumerate(_even_odd(skip_v[rows, :])):
                z = _modes(*[p[h] for p in par])
                for n in range(4):
                    mode_v[u, h, n] = z[n]
                k0.append(skip + jnp.sum(z[0], axis=1, keepdims=True))
            k0_v[grp] = _interleave(*k0)

    def dft(rows):
        z = _dot(jnp.concatenate([pltpu.bitcast(r, bf16) for r in rows], axis=0), pltpu.bitcast(fwd_v[...], bf16))
        return [[(z[o:o + 8, :_T], z[o:o + 8, _T:])
                 for o in range((h // 2) * 16 * _NB + 8 * (h % 2), (h // 2 + 1) * 16 * _NB, 16)]
                for h in range(2 * len(rows) // _NB)]

    def spread(step, u):
        for j, blk in _lag_blocks(lambda n: tap_v[u, n], k0_v[step * _GA + u]):
            k_v[u, j] = blk

    def filter_spectra(step, us, zero=0):
        for h, blocks in enumerate(dft([k_v[u + zero, j] for u in us for j in range(_NB)])):
            for j, (re, im) in enumerate(blocks):
                for p, val in enumerate((re, re + im, im - re)):
                    kf_v[2 * (step * _GA + us[0]) + h, p * _PLANE + j] = val

    def filter_step(i, zero, extra=lambda u: None):
        for u in range(_GA):
            if u == 0:
                filter_spectra(jnp.maximum(i - 2, 0), range(_GA // 2, _GA), zero)
            if u == _GA // 2:
                filter_spectra(jnp.maximum(i - 1, 0), range(_GA // 2), zero)
            spread(jnp.maximum(i - 1, 0), u)
            v = [[_vandermonde(*seeds) for seeds in _seeds(
                (mode_v[u, h, 0], mode_v[u, h, 1]), (mode_v[u, h, 2], mode_v[u, h, 3]))]
                 for h in range(2)]
            for n, tap in enumerate(_unmix(*map(_interleave, *v))):
                tap_v[u, n] = tap
            extra(u)

    def phase_a(i, carry):
        @pl.when(i == 1)
        def _():
            wait(1)
            for cp in hidden_copies(0):
                cp.start()

        pl.when(i == _LN_STEP)(layer_norm)
        for c in range(2):
            pop_best(2 * (i - _LN_STEP) + c)
        filter_step(i, i >> 8)
        modes(i + 1)

    with jax.named_scope("A"):
        modes(0)
        lax.fori_loop(0, _NG // _GA - 1, phase_a, None)

    def input_spectra(rows, dst):
        z = dft(rows)
        for h, t in enumerate(z):
            for b, (re, im) in enumerate(t):
                if b:
                    re, im = re + t[b - 1][1], im - t[b - 1][0]
                for p, val in enumerate((re + im, im, re)):
                    dst[(h * 3 + p) * _PLANE + b] = val
        return z

    def w_row(c, r):
        return jnp.concatenate(
            [pltpu.bitcast(arena[c, _ROW_W + q * _WQ + r], f32) for q in range(2)], axis=1)

    def routed_tokens():
        return _L - 1 - (pltpu.bitcast(key_v[2], i32) & (_L - 1))

    with jax.named_scope("topk"):
        for n in range(2, _NF):
            for cp in hidden_copies(n):
                cp.start()
        token = routed_tokens()
        picked = []

        def gather(u):
            tokens = range(u * _C // _GA, (u + 1) * _C // _GA)
            blocks = jnp.concatenate(
                [pltpu.bitcast(jnp.concatenate(
                    [arena[g // _GC, _ROW_X + (g % _GC) * _NB + (token[t, 0] >> 7)]
                     for g in range(_NG)], axis=0), bf16) for t in tokens], axis=1)
            pick = jnp.concatenate(
                [jnp.where((row == t) & ((token & (_T - 1)) == lane), 2.0, 0.0) for t in tokens],
                axis=1).astype(bf16)
            picked.append(_dot_nt(pick, blocks))

        filter_step(_NG // _GA - 1, token[0, 0] >> 11, gather if _MERGE else lambda u: None)
        for u in range(0 if _MERGE else _GA):
            gather(u)
        x_sel = sum(picked[1:], picked[0])
        for n in range(_NO):
            sel_v[n] = x_sel[:, n * _OCH:(n + 1) * _OCH]
        x_sel = jnp.concatenate([x_sel, jnp.zeros((8, _KT * _T - _D), f32)], axis=1)
        for n in range(_KT):
            arena[0, _ROW_SEL + n] = pltpu.bitcast(
                jnp.concatenate([x_sel[:, n * _T:(n + 1) * _T]] * 2, axis=0).astype(bf16), i32)
        input_spectra([arena[0, _ROW_X + r] for r in range(_R)], spec_a)
        filter_spectra(_NG // _GA - 2, range(_GA // 2, _GA))
        for u in range(_GA):
            spread(_NG // _GA - 1, u)
        filter_spectra(_NG // _GA - 1, range(_GA))

    def hidden_jobs(c):
        width = _F // (_NCH - _NO)
        gate = []

        def project(n):
            cols = pl.ds(_aligned(c * width + n // 2 * _T, _T), _T)
            x_sel = jnp.concatenate(
                [pltpu.bitcast(arena[c >> 8, _ROW_SEL + r], bf16) for r in range(_KT)], axis=1)
            gate.append(_rnd(_dot(x_sel[:, :_D], pltpu.bitcast((wu_v if n % 2 else wg_v)[:, cols], bf16))[:8]))
            if n % 2:
                hid_v[:, cols] = (_rnd(_silu(gate[-2])) * gate[-1]).astype(bf16)

        return [(40 * n, lambda n=n: project(n)) for n in range(2 * width // _T)]

    def hidden_at(t, zero=0):
        return pl.ds(_aligned(_D + 8 * (t // _NB + zero), 8), 8), pl.ds((t % _NB) * _T, _T)

    def finish(n):
        for k in range(_OCH // 16 * _NB):
            c, r = n * (_OCH // (16 * _GC)) + k // _R, k % _R
            rows = pl.ds(_aligned(n * _OCH + 16 * (k // _NB), 16), 16)
            cols = pl.ds((k % _NB) * _T, _T)
            h = pltpu.bitcast(arena[c, _ROW_X + r], bf16).astype(f32)
            gated = s_v[c, pl.ds(16 * r, 16), :] * (h + h * jnp.tanh(h))
            o_v[rows, cols] = (xc_v[k % _NB, n * (_OCH // 16) + k // _NB] + gated).astype(bf16)
            yield k

    def down_jobs(n, hid):
        rank = (pltpu.bitcast(key_v[2], i32) - (1 << 28)) >> 11
        score = pltpu.bitcast(jnp.where(rank >= 0x8000, rank - 0x8000, ~rank) << 16, f32)
        y = _rnd(_dot_nt(jnp.concatenate(hid, axis=1), pltpu.bitcast(wd_v[n], bf16)))
        y = 0.5 * (sel_v[n] + _rnd(y * _rnd(jax.nn.sigmoid(score))[:, :_OCH]))
        col = jnp.concatenate([y, jnp.zeros((_T - _C, _OCH), f32)], axis=0).T
        col = pltpu.bitcast(col.astype(bf16), i32)
        token = routed_tokens()

        def scatter(t):
            hit = ((token & (_T - 1)) == lane)[t:t + 1]
            new = jnp.broadcast_to(col[:, t:t + 1], (_OCH // 2, _T))
            where = [(n * (_OCH // (16 * _GC)) + g // _GC,
                      _ROW_X + (g % _GC) * _NB + (token[t, 0] >> 7)) for g in range(_OCH // 16)]
            old = [arena[at] for at in where]
            for g, at in enumerate(where):
                arena[at] = jnp.where(hit, new[8 * g:8 * g + 8], old[g])

        return [lambda t=t: scatter(t) for t in range(_C)]

    def first_output_jobs(c):
        hid, scatter = [], []

        def read():
            hid.extend(pltpu.bitcast(arena[c >> 8, _ROW_W + t], bf16)[:8]
                       for t in range(len(hid), len(hid) + 4))

        return ([(48 * k, read) for k in range(_F // (4 * _T))]
                + [(_G2 - 1, lambda: scatter.extend(down_jobs(0, hid)))]
                + [(_G2 + _S0 + _S1 * t, lambda t=t: scatter[t]()) for t in range(_C)])

    def output_jobs(c):
        n = c - (_NCH - _NO)
        hid = [o_v[hidden_at(t, c >> 8)] for t in range(4)]
        for k in finish(n - 1):
            if k % 12 == 11:
                hid += [o_v[hidden_at(t, c >> 8)] for t in range(len(hid), len(hid) + 4)]
        jobs = [(_S0 + _S1 * t, job) for t, job in enumerate(down_jobs(n, hid))]
        pl.when(n >= _HOLD)(lambda: out_copy(n - 1).start(priority=_PRIO))
        return jobs

    def conv_step(c, cur, nxt, ffn_jobs, delay, pace):
        c_next, c_prev = jnp.minimum(c + 1, _NCH - 1), jnp.maximum(c - 1, 0)
        zero = c >> 8
        fwd_rows, inv_rows, results = [], [], []

        def transform():
            y = _dot(jnp.concatenate(inv_rows, axis=0), inv_v[...])
            s_v[c_prev] = y
            results.extend((y, input_spectra(fwd_rows, nxt)))

        def drain(r):
            y, z = results
            arena[c, _ROW_SEL - 1] = pltpu.bitcast(
                y[8 * r:8 * r + 8] + z[2 * (r // _R) + 1][r % _R // 2][r // 8 % 2], i32)

        jobs = sorted(
            ffn_jobs(c)
            + [(delay + 8 * r, lambda r=r: inv_rows.append(w_row(c_prev, r))) for r in range(2 * _R)]
            + [(delay + 16 * r, lambda r=r: fwd_rows.append(arena[c_next, _ROW_X + r]))
               for r in range(_R)]
            + [(delay + 16 * _R, transform)]
            + [(delay + _LAG + 8 * r, lambda r=r: drain(r)) for r in range(2 * _R - 17, 2 * _R, 8)],
            key=lambda job: job[0])

        def run_jobs(done):
            while jobs and done * (delay + 16 * _R) >= (jobs[0][0] - _LEAD) * pace * 18 * _GC:
                jobs.pop(0)[1]()

        run_jobs(0)
        for h in range(2 * _GC):
            for part in range(3):
                for plane in range(3):
                    kf = lambda b: kf_v[c * 2 * _GC + h + (zero >> part), plane * _PLANE + b]
                    uf = lambda b: cur[(zero >> part) + (h * 3 + plane) * _PLANE + b]
                    base = [pltpu.bitcast(arena[c + zero, _ROW_P + plane * 8 + m], f32)
                            for m in range(8) if part and plane]
                    k, u, out = [], [], []
                    for m in range(8):
                        if part == 0:
                            k.append(kf(2 * m))
                            u.append(uf(2 * m) + uf(2 * m + 1))
                        elif part == 1:
                            k.append(kf(2 * m) - kf(2 * m - 1) if m else kf(0))
                            u.append(uf(2 * m + 1))
                        else:
                            k.append(kf(2 * m) - kf(2 * m + 1))
                            u.append(uf(2 * m))
                        y = k[0] * u[m]
                        for j in range(1, m + 1):
                            y = y + k[j] * u[m - j]
                        if plane:
                            y = shared[m] - y if plane == 1 else shared[m] + y
                        out.append(y)
                        if part == 0 or plane == 0:
                            arena[c, _ROW_P + plane * 8 + m] = pltpu.bitcast(y, i32)
                        else:
                            b = 2 * m + part - 1
                            arena[c, _ROW_W + (plane - 1) * _WQ + ((h // 2) * _NB + b) * 2 + h % 2] = (
                                pltpu.bitcast(base[m] - y, i32))
                    if plane == 0:
                        shared = out
                    run_jobs((h * 3 + part) * 3 + plane + 1)
        run_jobs(np.inf)

    def either(c, *args):
        lax.cond(c & 1 == 0, lambda: conv_step(c, spec_a, spec_b, *args),
                 lambda: conv_step(c, spec_b, spec_a, *args))

    def phase_c(part, carry):
        for cp in hidden_copies(part):
            cp.wait()

        @pl.when(part == _WD_STEP)
        def _():
            for n in range(_NO):
                down_copy(n).start()

        steps = (_NCH - _NO) // _NF
        return lax.fori_loop(part * steps, (part + 1) * steps,
                             lambda c, carry: either(c, hidden_jobs, 240, _PACE), carry)

    def phase_d(n, carry):
        down_copy(n).wait()

        @pl.when(n == _HOLD)
        def _():
            for k in range(_HOLD - 1):
                out_copy(k).start(priority=_PRIO)

        either(n + _NCH - _NO, output_jobs, _G1, _PACE1)

    with jax.named_scope("C"):
        lax.fori_loop(0, _NF, phase_c, None)
    with jax.named_scope("D"):
        for t in range(_F // _T):
            tile = hid_v[:, t * _T:(t + 1) * _T]
            o_v[hidden_at(t)] = tile
            arena[0, _ROW_W + t] = pltpu.bitcast(jnp.concatenate([tile] * 2, axis=0), i32)
        down_copy(0).wait()
        conv_step(_NCH - _NO + (routed_tokens()[0, 0] >> 11), spec_a, spec_b, first_output_jobs,
                  _G2, _PACE2)
        lax.fori_loop(1, _NO, phase_d, None)
    with jax.named_scope("tail"):
        s_v[_NCH - 1] = _dot(
            jnp.concatenate([w_row(_NCH - 1, r) for r in range(2 * _R)], axis=0), inv_v[...])
        for k in finish(_NO - 1):
            if k % _R == _R - 1:
                rows = pl.ds((_NO - 1) * _OCH + k // _R * 16 * _GC, 16 * _GC)
                start("out", o_v.at[rows], o_hbm.at[rows])
    with jax.named_scope("end"):
        for n in range(_NO - 1):
            out_copy(n).wait()
        wait("out")


@jax.jit
def pallas_recurrent_scan__ssm_conv_s4__moe_arch_mod__prompt_kernel(
    A_u: jax.Array,
    A_A_re: jax.Array,
    A_A_im: jax.Array,
    A_B_re: jax.Array,
    A_B_im: jax.Array,
    A_C_re: jax.Array,
    A_C_im: jax.Array,
    A_log_dt: jax.Array,
    A_Dskip: jax.Array,
    B_x: jax.Array,
    B_w_r: jax.Array,
    B_w_gate: jax.Array,
    B_w_up: jax.Array,
    B_w_down: jax.Array,
):
    del B_x
    assert A_u.shape == (1, _L, _D) and A_A_re.shape == (_D, _N) and B_w_gate.shape == (_D, _F)
    assert A_u.dtype == bf16 and A_A_re.dtype == bf16
    hbm = pl.BlockSpec(memory_space=pl.ANY)
    vmem = pltpu.VMEM
    out = pl.pallas_call(
        _kernel,
        out_shape=jax.ShapeDtypeStruct((_D, _L), bf16),
        in_specs=[hbm] * 15,
        out_specs=hbm,
        scratch_shapes=[
            vmem((_D // 2, _L), i32), vmem((_D + 32, _L), bf16),
            vmem((6, _D // 2, _N), i32), vmem((_D,), bf16), vmem((_D,), bf16), vmem((_D,), bf16),
            vmem((_D // 2, _F), i32), vmem((_D // 2, _F), i32), vmem((_NO, _OCH // 2, _F), i32),
            vmem((_T // 2, 2 * _T), i32), vmem((2 * _T, _T), f32),
            vmem((_D // 2, _T), i32), vmem((_NG, 8, _T), i32),
            vmem((_NCH, _ROWS, 8, _T), i32), vmem((_NCH, 16 * _R, _T), f32),
            vmem((_D // 2, _T), i32), vmem((_GA, 2, 4, 8, _N), f32), vmem((_GA, len(_TAPS), 8, _T), i32),
            vmem((_GA, _NB, 8, _T), i32),
            vmem((_NB, _NG, 16, _T), f32), vmem((3, _NB, 8, _T), f32), vmem((3, 8, _T), f32),
            vmem((_NO, 8, _OCH), f32), vmem((8, _F), bf16),
            *[vmem((2 * _GC * 3 * _PLANE, 8, _T), f32)] * 2, vmem((2 * _NG, 3 * _PLANE, 8, _T), f32),
            pltpu.SemaphoreType.DMA((5,)), pltpu.SemaphoreType.DMA((_NF + _NO,)),
            pltpu.SemaphoreType.DMA(()),
        ],
        compiler_params=pltpu.CompilerParams(vmem_limit_bytes=100 * 2**20),
    )(A_u.reshape(_L, _D).T, A_A_re, A_A_im, A_B_re, A_B_im, A_C_re, A_C_im, A_log_dt, A_Dskip,
      B_w_r, B_w_gate, B_w_up, B_w_down.T, _FWD, _INV)
    return out.T.reshape(1, _L, _D)
```

```python
import jax
import jax.numpy as jnp
import numpy as np
from jax import lax
import jax.experimental.pallas as pl
import jax.experimental.pallas.tpu as pltpu

_D, _L, _N, _F, _C = 576, 2048, 128, 4608, 8
_T = 128
_NB = _L // _T
_EPS = 1e-5
_GA = 4
_GC = 2
_NG = _D // 16
_NCH = _NG // _GC
_R = _GC * _NB
_ROW_X, _ROW_W, _ROW_P, _ROWS = 0, _R, 5 * _R + 8, 5 * _R + 8 + 24
_PLANE, _WQ = _NB + 1, 2 * _R + 1
_ROW_SEL = 5 * _R + 3
_MERGE, _HOLD, _PRIO, _G2, _PACE2 = 1, 3, 0, 400, 0.83
_FLAGS = None
_KT = -(-_D // _T)
_NO, _OCH = 6, _D // 6
_NF = 3
_FCH = _F // _NF
_LN_STEP = 4
_WD_STEP = 1
_PACE, _PACE1, _LEAD, _LAG, _G1, _S0, _S1 = 0.87, 0.8, 32, 140, 32, 520, 20

f32, bf16, i32 = jnp.float32, jnp.bfloat16, jnp.int32


def _dft_constants():
    theta = (np.pi / 2 + 2 * np.pi * np.arange(_T)) / _T
    ang = np.arange(_T)[:, None] * theta[None, :]
    c, s = np.cos(ang), np.sin(ang)
    fwd = np.concatenate([c, s], axis=1)
    bits = fwd.astype(bf16).view(np.uint16).astype(np.uint32)
    words = (bits[0::2] | bits[1::2] << 16).view(np.int32)
    return words


_FWD = _dft_constants()


def _lag_step(j):
    return max(1, (1 << (j * _T).bit_length()) >> 8)


def _round_lag(p, st):
    if st == 1:
        return p
    return (p + (st // 2 - 1) + ((p >> (st.bit_length() - 1)) & 1)) & ~(st - 1)


assert np.array_equal(
    np.concatenate([j * _T + _round_lag(np.arange(_T), _lag_step(j)) for j in range(_NB)]),
    np.arange(_L).astype(bf16).astype(np.int64))

_PAIRS = (((0, 1), (0, 5)), ((0, 2), (0, 6)), ((0, 3), (0, 7)), ((0, 4), (0, 8)), ((1, 2), (1, 6)),
          ((1, 4), (1, 8)), ((2, 4), (2, 8)), ((3, 4), (3, 8)), ((4, 8), (5, 8)), ((6, 8), (7, 8)))
_TAPS = [k for pair in _PAIRS for k in pair]


def _aligned(i, n):
    return i if isinstance(i, int) else pl.multiple_of(i, n)


def _cmul(a, b):
    return a[0] * b[0] - a[1] * b[1], a[0] * b[1] + a[1] * b[0]


def _csq(a):
    return a[0] * a[0] - a[1] * a[1], (a[0] + a[0]) * a[1]


def _silu(x):
    h = 0.5 * x
    return h + h * jnp.tanh(h)


def _rnd(x):
    return x.astype(bf16).astype(f32)


def _dot(a, b):
    return jnp.dot(a, b, preferred_element_type=f32)


def _dot_nt(a, b):
    return lax.dot_general(a, b, (((1,), (1,)), ((), ())), preferred_element_type=f32)


def _column(v):
    return jnp.broadcast_to(v.reshape(1, _D), (_T, _D)).T


def _even_odd(x):
    return pltpu.bitcast(x << 16, f32), pltpu.bitcast(x & -65536, f32)


def _interleave(even, odd):
    return pltpu.bitcast(pltpu.pack_elementwise([even, odd], packed_dtype=bf16), i32)


def _modes(dt, ar, ai, br, bi, cr, ci):
    zr, zi = dt * ar, dt * ai
    mag = jnp.exp(zr)
    return _cmul((cr, ci), (dt * br, dt * bi)) + (mag * jnp.cos(zi), mag * jnp.sin(zi))


def _seeds(w, a1):
    a = {1: a1}
    for n in range(9):
        a[2 << n] = _csq(a[1 << n])
    row = lax.broadcasted_iota(i32, (8, _N), 0)

    def conj(z):
        return z[0], -z[1]

    def mix(z0, z1):
        rolled = [pltpu.roll(x, 4, 0) for x in z1]
        return ([jnp.where(row < 4, x, y) for x, y in zip(z0, rolled)],
                [jnp.where(row < 4, y, x) for x, y in zip(z0, rolled)])

    def dup(z):
        return [[jnp.take_along_axis(x, (row & 3) + 4 * q, axis=0, mode="promise_in_bounds")
                 for x in z] for q in range(2)]

    wa = _cmul(w, a[1])
    return zip(mix((1.0, 0.0), conj(a[128])), dup(conj(a[8])), dup(conj(a[32])),
               mix(wa, _cmul(wa, a[4])), dup(a[1]), dup(a[256]),
               mix(_cmul(a[256], a[4]), a[512]), dup(a[512]))


def _vandermonde(e0, m8, m32, g0, m1, m256, m_top, m512):
    e = [e0]
    for s in range(1, 16):
        e.append(_cmul(e[s - 1], m8) if s < 4 else _cmul(e[s - 4], m32))
    g = [g0]
    for _ in range(3):
        g.append(_cmul(g[-1], m1))
    g += [_cmul(g[1], m256), _cmul(g[3], m256)]
    g += [_cmul(g[3], m512), _cmul(g[5], m512)]
    g.append(_cmul(g[7], m_top))
    g.append(_cmul(g[8], m512))
    re, im = [_dot_nt(jnp.concatenate([z[p] for z in g], axis=0),
                      jnp.concatenate([z[p] for z in e], axis=0)) for p in range(2)]
    return re + im


def _unmix(lo, hi):
    row = lax.broadcasted_iota(i32, (8, _T), 0)
    out = []
    for m in range(len(_PAIRS)):
        x, y = lo[8 * m:8 * m + 8], hi[8 * m:8 * m + 8]
        out += [jnp.where(row < 4, x, y), pltpu.roll(jnp.where(row < 4, y, x), 4, 0)]
    return out


def _lag_blocks(tap, lag0):
    lane = lax.broadcasted_iota(i32, (8, _T), 1)
    row = lax.broadcasted_iota(i32, (8, _T), 0)
    for h in range(2):
        def take(big, r, fine):
            s = ((_T * h + fine) >> 3) & 31
            return jnp.take_along_axis(tap(_TAPS.index((big, r))),
                                       ((s & 15) << 3) + (row ^ ((s >> 4) << 2)),
                                       axis=1, mode="promise_in_bounds")

        top = [take(big, 8, _round_lag(lane, 8) - 8) for big in range(_NB // 2)]
        for big, blk in enumerate(top):
            st = _lag_step(2 * big + h)
            lag = _round_lag(lane, st)
            if h == 0:
                blk = jnp.where(lag == 0, top[big - 1] if big else lag0, blk)
            for r in range(st, 8, st):
                blk = jnp.where((lag & 7) == r, take(big, r, lane), blk)
            yield 2 * big + h, blk


def _kernel(x_hbm, ar_hbm, ai_hbm, br_hbm, bi_hbm, cr_hbm, ci_hbm, ldt_hbm, dsk_hbm, wr_hbm,
            wg_hbm, wu_hbm, wd_hbm, fwd_hbm, o_hbm,
            x_v, o_v, par_v, ldt_v, dsk_v, wr_v, wg_v, wu_v, wd_v, fwd_v, inv_v,
            skip_v, k0_v, arena, s_v, dt_v, mode_v, tap_v, k_v, xc_v, stat_v, key_v, sel_v, hid_v,
            spec_a, spec_b, kf_v, sem, w_sem, o_sem):
    row = lax.broadcasted_iota(i32, (8, _T), 0)
    lane = lax.broadcasted_iota(i32, (8, _T), 1)
    groups = {}

    def start(name, src, dst):
        slot, pairs = groups.setdefault(name, (len(groups), []))
        pairs.append((src, dst))
        pltpu.make_async_copy(src, dst, sem.at[slot]).start()

    def wait(name):
        slot, pairs = groups[name]
        for src, dst in pairs:
            pltpu.make_async_copy(src, dst, sem.at[slot]).wait()

    def hidden_copies(n):
        cols = pl.ds(_aligned(n * _FCH, _FCH), _FCH)
        return [pltpu.make_async_copy(w.bitcast(i32).at[:, cols], v.at[:, cols], w_sem.at[n])
                for w, v in ((wg_hbm, wg_v), (wu_hbm, wu_v))]

    def chunk_rows(n):
        return pl.ds(_aligned(n * _OCH, 32), _OCH)

    def down_copy(n):
        rows = pl.ds(_aligned(n * (_OCH // 2), 16), _OCH // 2)
        return pltpu.make_async_copy(wd_hbm.bitcast(i32).at[rows], wd_v.at[n], w_sem.at[_NF + n])

    def out_copy(n):
        return pltpu.make_async_copy(o_v.at[chunk_rows(n)], o_hbm.at[chunk_rows(n)], o_sem)

    def start_parameters(part, rows):
        for n, src in enumerate((ar_hbm, ai_hbm, br_hbm, bi_hbm, cr_hbm, ci_hbm)):
            start(part, src.bitcast(i32).at[rows], par_v.at[n, rows])

    with jax.named_scope("init"):
        start("vectors", ldt_hbm, ldt_v)
        start("vectors", dsk_hbm, dsk_v)
        start_parameters(0, pl.ds(0, 16 * _GA))
        start(0, fwd_hbm, fwd_v)
        arena[0, _ROW_W:_ROW_P] = jnp.zeros((_ROW_P - _ROW_W, 8, _T), i32)
        tap_v[...] = jnp.zeros(tap_v.shape, i32)
        k_v[...] = jnp.zeros(k_v.shape, i32)
        key_v[...] = jnp.zeros(key_v.shape, f32)
        wait("vectors")
        start_parameters(1, pl.ds(16 * _GA, _D // 2 - 16 * _GA))
        start("x", x_hbm.bitcast(i32), x_v)
        start("x", wr_hbm, wr_v)
        dt_v[...] = pltpu.bitcast(_column(jnp.exp(ldt_v[...].astype(f32))).astype(bf16), i32)
        skip_v[...] = pltpu.bitcast(_column(dsk_v[...].astype(f32)).astype(bf16), i32)
        wait(0)

    def compact(ref, k, h):
        out = ref[k, 8 * h]
        for s in range(1, 8):
            out = jnp.where(row == s, ref[k, 8 * h + s], out)
        return out

    def layer_norm():
        wait("x")
        for cp in hidden_copies(1):
            cp.start()

        def moments(b, carry):
            cols = pl.ds(_aligned(b * _T, _T), _T)
            pivot = jnp.broadcast_to(_even_odd(x_v[:8, cols])[0][:1], (8, _T))
            s1, s2 = [None] * 2, [None] * 2
            for g in range(_NG):
                words = x_v[pl.ds(8 * g, 8), cols]
                x = pltpu.bitcast(words, bf16).astype(f32)
                xc_v[b, g] = x
                for h in range(2):
                    d = x[8 * h:8 * h + 8] - pivot
                    s1[h] = s1[h] + d if g else d
                    s2[h] = s2[h] + d * d if g else d * d
            for k, s in enumerate((s1, s2)):
                stat_v[k, b] = jnp.broadcast_to(jnp.sum(s[0] + s[1], axis=0, keepdims=True), (8, _T))
            stat_v[2, b] = pivot
            return carry

        lax.fori_loop(0, _NB, moments, 0, unroll=4)
        for h in range(_NB // 8):
            m1, m2, pivot = compact(stat_v, 0, h) / _D, compact(stat_v, 1, h) / _D, compact(stat_v, 2, h)
            var = jnp.maximum(m2 - m1 * m1, 0.0)
            shift = _rnd(pivot + m1)
            gain = 0.5 / _rnd(jnp.sqrt(_rnd(_rnd(var) + _rnd(jnp.full_like(var, _EPS)))))
            for s in range(8):
                stat_v[0, 8 * h + s] = jnp.broadcast_to(shift[s:s + 1], (8, _T))
                stat_v[1, 8 * h + s] = jnp.broadcast_to(gain[s:s + 1], (8, _T))
        inv_v[...] = pltpu.bitcast(
            (pltpu.bitcast(fwd_v[...], bf16).astype(f32).T * (2 / _T)).astype(bf16), i32)
        wr = jnp.broadcast_to(wr_v[...].astype(f32).reshape(1, _D), (8, _D)).astype(bf16)

        def scale(b, carry):
            shift, gain = stat_v[0, b], stat_v[1, b]
            xn = [_interleave(*[(xc_v[b, g, pl.ds(h, 8, stride=2), :] - shift) * gain for h in range(2)])
                  for g in range(_NG)]
            for g in range(_NG):
                arena[g // _GC, _ROW_X + (g % _GC) * _NB + b] = xn[g]
            stat_v[2, b] = _dot(wr, pltpu.bitcast(jnp.concatenate(xn, axis=0), bf16))
            return carry

        lax.fori_loop(0, _NB, scale, 0, unroll=16)
        for h in range(_NB // 8):
            bits = pltpu.bitcast(_rnd(2.0 * compact(stat_v, 2, h)) + 0.0, i32) >> 16
            rank = jnp.where(bits < 0, ~bits, bits + 0x8000)
            token = (8 * h + row) * _T + lane
            key_v[h] = pltpu.bitcast((1 << 28) + rank * _L + (_L - 1 - token), f32)

    def pop_best(c):
        best = jnp.max(jnp.max(jnp.maximum(key_v[0], key_v[1]), axis=0, keepdims=True),
                       axis=1, keepdims=True)
        key_v[2] = jnp.where(row == c, best, key_v[2])
        for h in range(2):
            key_v[h] = jnp.where(key_v[h] == best, 0.0, key_v[h])

    def modes(step):
        for u in range(_GA):
            grp = step * _GA + u
            rows = pl.ds(_aligned(grp * 8, 8), 8)
            par = [_even_odd(dt_v[rows, :])] + [_even_odd(par_v[n, rows, :]) for n in range(6)]
            k0 = []
            for h, skip in enumerate(_even_odd(skip_v[rows, :])):
                z = _modes(*[p[h] for p in par])
                for n in range(4):
                    mode_v[u, h, n] = z[n]
                k0.append(skip + jnp.sum(z[0], axis=1, keepdims=True))
            k0_v[grp] = _interleave(*k0)

    def dft(rows):
        z = _dot(jnp.concatenate([pltpu.bitcast(r, bf16) for r in rows], axis=0), pltpu.bitcast(fwd_v[...], bf16))
        return [[(z[o:o + 8, :_T], z[o:o + 8, _T:])
                 for o in range((h // 2) * 16 * _NB + 8 * (h % 2), (h // 2 + 1) * 16 * _NB, 16)]
                for h in range(2 * len(rows) // _NB)]

    def spread(step, u):
        for j, blk in _lag_blocks(lambda n: tap_v[u, n], k0_v[step * _GA + u]):
            k_v[u, j] = blk

    def filter_spectra(step, us, zero=0):
        for h, blocks in enumerate(dft([k_v[u + zero, j] for u in us for j in range(_NB)])):
            for j, (re, im) in enumerate(blocks):
                for p, val in enumerate((re, re + im, im - re)):
                    kf_v[2 * (step * _GA + us[0]) + h, p * _PLANE + j] = val

    def filter_step(i, zero, extra=lambda u: None):
        for u in range(_GA):
            if u == 0:
                filter_spectra(jnp.maximum(i - 2, 0), range(_GA // 2, _GA), zero)
            if u == _GA // 2:
                filter_spectra(jnp.maximum(i - 1, 0), range(_GA // 2), zero)
            spread(jnp.maximum(i - 1, 0), u)
            v = [[_vandermonde(*seeds) for seeds in _seeds(
                (mode_v[u, h, 0], mode_v[u, h, 1]), (mode_v[u, h, 2], mode_v[u, h, 3]))]
                 for h in range(2)]
            for n, tap in enumerate(_unmix(*map(_interleave, *v))):
                tap_v[u, n] = tap
            extra(u)

    def phase_a(i, carry):
        @pl.when(i == 1)
        def _():
            wait(1)
            for cp in hidden_copies(0):
                cp.start()

        pl.when(i == _LN_STEP)(layer_norm)
        for c in range(2):
            pop_best(2 * (i - _LN_STEP) + c)
        filter_step(i, i >> 8)
        modes(i + 1)

    with jax.named_scope("A"):
        modes(0)
        lax.fori_loop(0, _NG // _GA - 1, phase_a, None)

    def input_spectra(rows, dst):
        z = dft(rows)
        for h, t in enumerate(z):
            for b, (re, im) in enumerate(t):
                if b:
                    re, im = re + t[b - 1][1], im - t[b - 1][0]
                for p, val in enumerate((re + im, im, re)):
                    dst[(h * 3 + p) * _PLANE + b] = val
        return z

    def w_row(c, r):
        return jnp.concatenate(
            [pltpu.bitcast(arena[c, _ROW_W + q * _WQ + r], bf16) for q in range(2)], axis=1)

    def routed_tokens():
        return _L - 1 - (pltpu.bitcast(key_v[2], i32) & (_L - 1))

    with jax.named_scope("topk"):
        for n in range(2, _NF):
            for cp in hidden_copies(n):
                cp.start()
        token = routed_tokens()
        picked = []

        def gather(u):
            tokens = range(u * _C // _GA, (u + 1) * _C // _GA)
            blocks = jnp.concatenate(
                [pltpu.bitcast(jnp.concatenate(
                    [arena[g // _GC, _ROW_X + (g % _GC) * _NB + (token[t, 0] >> 7)]
                     for g in range(_NG)], axis=0), bf16) for t in tokens], axis=1)
            pick = jnp.concatenate(
                [jnp.where((row == t) & ((token & (_T - 1)) == lane), 2.0, 0.0) for t in tokens],
                axis=1).astype(bf16)
            picked.append(_dot_nt(pick, blocks))

        filter_step(_NG // _GA - 1, token[0, 0] >> 11, gather if _MERGE else lambda u: None)
        for u in range(0 if _MERGE else _GA):
            gather(u)
        x_sel = sum(picked[1:], picked[0])
        for n in range(_NO):
            sel_v[n] = x_sel[:, n * _OCH:(n + 1) * _OCH]
        x_sel = jnp.concatenate([x_sel, jnp.zeros((8, _KT * _T - _D), f32)], axis=1)
        for n in range(_KT):
            arena[0, _ROW_SEL + n] = pltpu.bitcast(
                jnp.concatenate([x_sel[:, n * _T:(n + 1) * _T]] * 2, axis=0).astype(bf16), i32)
        input_spectra([arena[0, _ROW_X + r] for r in range(_R)], spec_a)
        filter_spectra(_NG // _GA - 2, range(_GA // 2, _GA))
        for u in range(_GA):
            spread(_NG // _GA - 1, u)
        filter_spectra(_NG // _GA - 1, range(_GA))

    def hidden_jobs(c):
        width = _F // (_NCH - _NO)
        gate = []

        def project(n):
            cols = pl.ds(_aligned(c * width + n // 2 * _T, _T), _T)
            x_sel = jnp.concatenate(
                [pltpu.bitcast(arena[c >> 8, _ROW_SEL + r], bf16) for r in range(_KT)], axis=1)
            gate.append(_rnd(_dot(x_sel[:, :_D], pltpu.bitcast((wu_v if n % 2 else wg_v)[:, cols], bf16))[:8]))
            if n % 2:
                hid_v[:, cols] = (_rnd(_silu(gate[-2])) * gate[-1]).astype(bf16)

        return [(40 * n, lambda n=n: project(n)) for n in range(2 * width // _T)]

    def hidden_at(t, zero=0):
        return pl.ds(_aligned(_D + 8 * (t // _NB + zero), 8), 8), pl.ds((t % _NB) * _T, _T)

    def finish(n):
        for k in range(_OCH // 16 * _NB):
            c, r = n * (_OCH // (16 * _GC)) + k // _R, k % _R
            rows = pl.ds(_aligned(n * _OCH + 16 * (k // _NB), 16), 16)
            cols = pl.ds((k % _NB) * _T, _T)
            h = pltpu.bitcast(arena[c, _ROW_X + r], bf16).astype(f32)
            b = r % _NB
            s = s_v[c, pl.ds(16 * (r - b) + 32 * (b // 4 * 2 + b % 2) + b // 2 % 2, 16, stride=2), :]
            gated = s * (h + h * jnp.tanh(h))
            o_v[rows, cols] = (xc_v[k % _NB, n * (_OCH // 16) + k // _NB] + gated).astype(bf16)
            yield k

    def down_jobs(n, hid):
        rank = (pltpu.bitcast(key_v[2], i32) - (1 << 28)) >> 11
        score = pltpu.bitcast(jnp.where(rank >= 0x8000, rank - 0x8000, ~rank) << 16, f32)
        y = _rnd(_dot_nt(jnp.concatenate(hid, axis=1), pltpu.bitcast(wd_v[n], bf16)))
        y = 0.5 * (sel_v[n] + _rnd(y * _rnd(jax.nn.sigmoid(score))[:, :_OCH]))
        col = jnp.concatenate([y, jnp.zeros((_T - _C, _OCH), f32)], axis=0).T
        col = pltpu.bitcast(col.astype(bf16), i32)
        token = routed_tokens()

        def scatter(t):
            hit = ((token & (_T - 1)) == lane)[t:t + 1]
            new = jnp.broadcast_to(col[:, t:t + 1], (_OCH // 2, _T))
            where = [(n * (_OCH // (16 * _GC)) + g // _GC,
                      _ROW_X + (g % _GC) * _NB + (token[t, 0] >> 7)) for g in range(_OCH // 16)]
            old = [arena[at] for at in where]
            for g, at in enumerate(where):
                arena[at] = jnp.where(hit, new[8 * g:8 * g + 8], old[g])

        return [lambda t=t: scatter(t) for t in range(_C)]

    def first_output_jobs(c):
        hid, scatter = [], []

        def read():
            hid.extend(pltpu.bitcast(arena[c >> 8, _ROW_W + t], bf16)[:8]
                       for t in range(len(hid), len(hid) + 4))

        return ([(48 * k, read) for k in range(_F // (4 * _T))]
                + [(_G2 - 1, lambda: scatter.extend(down_jobs(0, hid)))]
                + [(_G2 + _S0 + _S1 * t, lambda t=t: scatter[t]()) for t in range(_C)])

    def output_jobs(c):
        n = c - (_NCH - _NO)
        hid = [o_v[hidden_at(t, c >> 8)] for t in range(4)]
        for k in finish(n - 1):
            if k % 12 == 11:
                hid += [o_v[hidden_at(t, c >> 8)] for t in range(len(hid), len(hid) + 4)]
        jobs = [(_S0 + _S1 * t, job) for t, job in enumerate(down_jobs(n, hid))]
        pl.when(n >= _HOLD)(lambda: out_copy(n - 1).start(priority=_PRIO))
        return jobs

    def conv_step(c, cur, nxt, ffn_jobs, delay, pace):
        c_next, c_prev = jnp.minimum(c + 1, _NCH - 1), jnp.maximum(c - 1, 0)
        zero = c >> 8
        fwd_rows, inv_rows, results = [], [], []

        def transform():
            y = _dot(jnp.concatenate(inv_rows, axis=0), pltpu.bitcast(inv_v[...], bf16))
            s_v[c_prev] = y
            results.extend((y, input_spectra(fwd_rows, nxt)))

        def drain(r):
            y, z = results
            arena[c, _ROW_SEL - 1] = pltpu.bitcast(
                y[8 * r:8 * r + 8] + z[2 * (r // _R) + 1][r % _R // 2][r // 8 % 2], i32)

        jobs = sorted(
            ffn_jobs(c)
            + [(delay + 16 * r, lambda r=r: inv_rows.append(w_row(c_prev, r))) for r in range(_R)]
            + [(delay + 16 * r, lambda r=r: fwd_rows.append(arena[c_next, _ROW_X + r]))
               for r in range(_R)]
            + [(delay + 16 * _R, transform)]
            + [(delay + _LAG + 8 * r, lambda r=r: drain(r)) for r in range(2 * _R - 17, 2 * _R, 8)],
            key=lambda job: job[0])

        def run_jobs(done):
            while jobs and done * (delay + 16 * _R) >= (jobs[0][0] - _LEAD) * pace * 18 * _GC:
                jobs.pop(0)[1]()

        run_jobs(0)
        for h in range(2 * _GC):
            for part in range(3):
                for plane in range(3):
                    kf = lambda b: kf_v[c * 2 * _GC + h + (zero >> part), plane * _PLANE + b]
                    uf = lambda b: cur[(zero >> part) + (h * 3 + plane) * _PLANE + b]
                    base = [pltpu.bitcast(arena[c + zero, _ROW_P + plane * 8 + m], f32)
                            for m in range(8) if part and plane]
                    k, u, out = [], [], []
                    for m in range(8):
                        if part == 0:
                            k.append(kf(2 * m))
                            u.append(uf(2 * m) + uf(2 * m + 1))
                        elif part == 1:
                            k.append(kf(2 * m) - kf(2 * m - 1) if m else kf(0))
                            u.append(uf(2 * m + 1))
                        else:
                            k.append(kf(2 * m) - kf(2 * m + 1))
                            u.append(uf(2 * m))
                        y = k[0] * u[m]
                        for j in range(1, m + 1):
                            y = y + k[j] * u[m - j]
                        if plane:
                            y = shared[m] - y if plane == 1 else shared[m] + y
                        out.append(y)
                        if part == 0 or plane == 0:
                            arena[c, _ROW_P + plane * 8 + m] = pltpu.bitcast(y, i32)
                        elif m % 2:
                            r = (h // 2) * _NB + (m - 1 + part - 1) * 2 + h % 2
                            arena[c, _ROW_W + (plane - 1) * _WQ + r] = _interleave(
                                base[m - 1] - out[m - 1], base[m] - y)
                    if plane == 0:
                        shared = out
                    run_jobs((h * 3 + part) * 3 + plane + 1)
        run_jobs(np.inf)

    def either(c, *args):
        lax.cond(c & 1 == 0, lambda: conv_step(c, spec_a, spec_b, *args),
                 lambda: conv_step(c, spec_b, spec_a, *args))

    def phase_c(part, carry):
        for cp in hidden_copies(part):
            cp.wait()

        @pl.when(part == _WD_STEP)
        def _():
            for n in range(_NO):
                down_copy(n).start()

        steps = (_NCH - _NO) // _NF
        return lax.fori_loop(part * steps, (part + 1) * steps,
                             lambda c, carry: either(c, hidden_jobs, 240, _PACE), carry)

    def phase_d(n, carry):
        down_copy(n).wait()

        @pl.when(n == _HOLD)
        def _():
            for k in range(_HOLD - 1):
                out_copy(k).start(priority=_PRIO)

        either(n + _NCH - _NO, output_jobs, _G1, _PACE1)

    with jax.named_scope("C"):
        lax.fori_loop(0, _NF, phase_c, None)
    with jax.named_scope("D"):
        for t in range(_F // _T):
            tile = hid_v[:, t * _T:(t + 1) * _T]
            o_v[hidden_at(t)] = tile
            arena[0, _ROW_W + t] = pltpu.bitcast(jnp.concatenate([tile] * 2, axis=0), i32)
        down_copy(0).wait()
        conv_step(_NCH - _NO + (routed_tokens()[0, 0] >> 11), spec_a, spec_b, first_output_jobs,
                  _G2, _PACE2)
        lax.fori_loop(1, _NO, phase_d, None)
    with jax.named_scope("tail"):
        s_v[_NCH - 1] = _dot(
            jnp.concatenate([w_row(_NCH - 1, r) for r in range(_R)], axis=0), pltpu.bitcast(inv_v[...], bf16))
        for k in finish(_NO - 1):
            if k % _R == _R - 1:
                rows = pl.ds((_NO - 1) * _OCH + k // _R * 16 * _GC, 16 * _GC)
                start("out", o_v.at[rows], o_hbm.at[rows])
    with jax.named_scope("end"):
        for n in range(_NO - 1):
            out_copy(n).wait()
        wait("out")


@jax.jit
def pallas_recurrent_scan__ssm_conv_s4__moe_arch_mod__prompt_kernel(
    A_u: jax.Array,
    A_A_re: jax.Array,
    A_A_im: jax.Array,
    A_B_re: jax.Array,
    A_B_im: jax.Array,
    A_C_re: jax.Array,
    A_C_im: jax.Array,
    A_log_dt: jax.Array,
    A_Dskip: jax.Array,
    B_x: jax.Array,
    B_w_r: jax.Array,
    B_w_gate: jax.Array,
    B_w_up: jax.Array,
    B_w_down: jax.Array,
):
    del B_x
    assert A_u.shape == (1, _L, _D) and A_A_re.shape == (_D, _N) and B_w_gate.shape == (_D, _F)
    assert A_u.dtype == bf16 and A_A_re.dtype == bf16
    hbm = pl.BlockSpec(memory_space=pl.ANY)
    vmem = pltpu.VMEM
    out = pl.pallas_call(
        _kernel,
        out_shape=jax.ShapeDtypeStruct((_D, _L), bf16),
        in_specs=[hbm] * 14,
        out_specs=hbm,
        scratch_shapes=[
            vmem((_D // 2, _L), i32), vmem((_D + 32, _L), bf16),
            vmem((6, _D // 2, _N), i32), vmem((_D,), bf16), vmem((_D,), bf16), vmem((_D,), bf16),
            vmem((_D // 2, _F), i32), vmem((_D // 2, _F), i32), vmem((_NO, _OCH // 2, _F), i32),
            vmem((_T // 2, 2 * _T), i32), vmem((_T, _T), i32),
            vmem((_D // 2, _T), i32), vmem((_NG, 8, _T), i32),
            vmem((_NCH, _ROWS, 8, _T), i32), vmem((_NCH, 16 * _R, _T), f32),
            vmem((_D // 2, _T), i32), vmem((_GA, 2, 4, 8, _N), f32), vmem((_GA, len(_TAPS), 8, _T), i32),
            vmem((_GA, _NB, 8, _T), i32),
            vmem((_NB, _NG, 16, _T), f32), vmem((3, _NB, 8, _T), f32), vmem((3, 8, _T), f32),
            vmem((_NO, 8, _OCH), f32), vmem((8, _F), bf16),
            *[vmem((2 * _GC * 3 * _PLANE, 8, _T), f32)] * 2, vmem((2 * _NG, 3 * _PLANE, 8, _T), f32),
            pltpu.SemaphoreType.DMA((5,)), pltpu.SemaphoreType.DMA((_NF + _NO,)),
            pltpu.SemaphoreType.DMA(()),
        ],
        compiler_params=pltpu.CompilerParams(vmem_limit_bytes=100 * 2**20, flags=_FLAGS),
    )(A_u.reshape(_L, _D).T, A_A_re, A_A_im, A_B_re, A_B_im, A_C_re, A_C_im, A_log_dt, A_Dskip,
      B_w_r, B_w_gate, B_w_up, B_w_down.T, _FWD)
    return out.T.reshape(1, _L, _D)
```

```python
import jax
import jax.numpy as jnp
import numpy as np
from jax import lax
import jax.experimental.pallas as pl
import jax.experimental.pallas.tpu as pltpu

_D, _L, _N, _F, _C = 576, 2048, 128, 4608, 8
_T = 128
_NB = _L // _T
_EPS = 1e-5
_GA = 4
_GC = 2
_NG = _D // 16
_NCH = _NG // _GC
_R = _GC * _NB
_ROW_X, _ROW_W, _ROW_P, _ROWS = 0, _R, 5 * _R + 8, 5 * _R + 8 + 24
_PLANE, _WQ = _NB + 1, 2 * _R + 1
_ROW_SEL = 5 * _R + 3
_MERGE, _HOLD, _PRIO, _G2, _PACE2 = 1, 3, 0, 400, 0.83
_FLAGS, _HALF = None, 0
_KT = -(-_D // _T)
_NO, _OCH = 6, _D // 6
_NF = 3
_FCH = _F // _NF
_LN_STEP = 4
_WD_STEP = 1
_PACE, _PACE1, _LEAD, _LAG, _G1, _S0, _S1 = 0.87, 0.8, 32, 140, 32, 520, 20

f32, bf16, i32 = jnp.float32, jnp.bfloat16, jnp.int32


def _dft_constants():
    theta = (np.pi / 2 + 2 * np.pi * np.arange(_T)) / _T
    ang = np.arange(_T)[:, None] * theta[None, :]
    c, s = np.cos(ang), np.sin(ang)
    fwd = np.concatenate([c, s], axis=1)
    bits = fwd.astype(bf16).view(np.uint16).astype(np.uint32)
    words = (bits[0::2] | bits[1::2] << 16).view(np.int32)
    return words


_FWD = _dft_constants()


def _lag_step(j):
    return max(1, (1 << (j * _T).bit_length()) >> 8)


def _round_lag(p, st):
    if st == 1:
        return p
    return (p + (st // 2 - 1) + ((p >> (st.bit_length() - 1)) & 1)) & ~(st - 1)


assert np.array_equal(
    np.concatenate([j * _T + _round_lag(np.arange(_T), _lag_step(j)) for j in range(_NB)]),
    np.arange(_L).astype(bf16).astype(np.int64))

_PAIRS = (((0, 1), (0, 5)), ((0, 2), (0, 6)), ((0, 3), (0, 7)), ((0, 4), (0, 8)), ((1, 2), (1, 6)),
          ((1, 4), (1, 8)), ((2, 4), (2, 8)), ((3, 4), (3, 8)), ((4, 8), (5, 8)), ((6, 8), (7, 8)))
_TAPS = [k for pair in _PAIRS for k in pair]


def _aligned(i, n):
    return i if isinstance(i, int) else pl.multiple_of(i, n)


def _cmul(a, b):
    return a[0] * b[0] - a[1] * b[1], a[0] * b[1] + a[1] * b[0]


def _csq(a):
    return a[0] * a[0] - a[1] * a[1], (a[0] + a[0]) * a[1]


def _silu(x):
    h = 0.5 * x
    return h + h * jnp.tanh(h)


def _rnd(x):
    return x.astype(bf16).astype(f32)


def _dot(a, b):
    return jnp.dot(a, b, preferred_element_type=f32)


def _dot_nt(a, b):
    return lax.dot_general(a, b, (((1,), (1,)), ((), ())), preferred_element_type=f32)


def _column(v):
    return jnp.broadcast_to(v.reshape(1, _D), (_T, _D)).T


def _even_odd(x):
    return pltpu.bitcast(x << 16, f32), pltpu.bitcast(x & -65536, f32)


def _interleave(even, odd):
    return pltpu.bitcast(pltpu.pack_elementwise([even, odd], packed_dtype=bf16), i32)


def _modes(dt, ar, ai, br, bi, cr, ci):
    zr, zi = dt * ar, dt * ai
    mag = jnp.exp(zr)
    return _cmul((cr, ci), (dt * br, dt * bi)) + (mag * jnp.cos(zi), mag * jnp.sin(zi))


def _seeds(w, a1):
    a = {1: a1}
    for n in range(9):
        a[2 << n] = _csq(a[1 << n])
    row = lax.broadcasted_iota(i32, (8, _N), 0)

    def conj(z):
        return z[0], -z[1]

    def mix(z0, z1):
        rolled = [pltpu.roll(x, 4, 0) for x in z1]
        return ([jnp.where(row < 4, x, y) for x, y in zip(z0, rolled)],
                [jnp.where(row < 4, y, x) for x, y in zip(z0, rolled)])

    def dup(z):
        return [[jnp.take_along_axis(x, (row & 3) + 4 * q, axis=0, mode="promise_in_bounds")
                 for x in z] for q in range(2)]

    wa = _cmul(w, a[1])
    return zip(mix((1.0, 0.0), conj(a[128])), dup(conj(a[8])), dup(conj(a[32])),
               mix(wa, _cmul(wa, a[4])), dup(a[1]), dup(a[256]),
               mix(_cmul(a[256], a[4]), a[512]), dup(a[512]))


def _vandermonde(e0, m8, m32, g0, m1, m256, m_top, m512):
    e = [e0]
    for s in range(1, 16):
        e.append(_cmul(e[s - 1], m8) if s < 4 else _cmul(e[s - 4], m32))
    g = [g0]
    for _ in range(3):
        g.append(_cmul(g[-1], m1))
    g += [_cmul(g[1], m256), _cmul(g[3], m256)]
    g += [_cmul(g[3], m512), _cmul(g[5], m512)]
    g.append(_cmul(g[7], m_top))
    g.append(_cmul(g[8], m512))
    re, im = [_dot_nt(jnp.concatenate([z[p] for z in g], axis=0),
                      jnp.concatenate([z[p] for z in e], axis=0)) for p in range(2)]
    return re + im


def _unmix(lo, hi):
    row = lax.broadcasted_iota(i32, (8, _T), 0)
    out = []
    for m in range(len(_PAIRS)):
        x, y = lo[8 * m:8 * m + 8], hi[8 * m:8 * m + 8]
        out += [jnp.where(row < 4, x, y), pltpu.roll(jnp.where(row < 4, y, x), 4, 0)]
    return out


def _lag_blocks(tap, lag0):
    lane = lax.broadcasted_iota(i32, (8, _T), 1)
    row = lax.broadcasted_iota(i32, (8, _T), 0)
    for h in range(2):
        def take(big, r, fine):
            s = ((_T * h + fine) >> 3) & 31
            return jnp.take_along_axis(tap(_TAPS.index((big, r))),
                                       ((s & 15) << 3) + (row ^ ((s >> 4) << 2)),
                                       axis=1, mode="promise_in_bounds")

        top = [take(big, 8, _round_lag(lane, 8) - 8) for big in range(_NB // 2)]
        for big, blk in enumerate(top):
            st = _lag_step(2 * big + h)
            lag = _round_lag(lane, st)
            if h == 0:
                blk = jnp.where(lag == 0, top[big - 1] if big else lag0, blk)
            for r in range(st, 8, st):
                blk = jnp.where((lag & 7) == r, take(big, r, lane), blk)
            yield 2 * big + h, blk


def _kernel(x_hbm, ar_hbm, ai_hbm, br_hbm, bi_hbm, cr_hbm, ci_hbm, ldt_hbm, dsk_hbm, wr_hbm,
            wg_hbm, wu_hbm, wd_hbm, fwd_hbm, o_hbm,
            x_v, o_v, par_v, ldt_v, dsk_v, wr_v, wg_v, wu_v, wd_v, fwd_v, inv_v,
            skip_v, k0_v, arena, s_v, dt_v, mode_v, tap_v, k_v, xc_v, stat_v, key_v, sel_v, hid_v,
            spec_a, spec_b, kf_v, sem, w_sem, o_sem):
    row = lax.broadcasted_iota(i32, (8, _T), 0)
    lane = lax.broadcasted_iota(i32, (8, _T), 1)
    groups = {}

    def start(name, src, dst):
        slot, pairs = groups.setdefault(name, (len(groups), []))
        pairs.append((src, dst))
        pltpu.make_async_copy(src, dst, sem.at[slot]).start()

    def wait(name):
        slot, pairs = groups[name]
        for src, dst in pairs:
            pltpu.make_async_copy(src, dst, sem.at[slot]).wait()

    def hidden_copies(n):
        cols = pl.ds(_aligned(n * _FCH, _FCH), _FCH)
        return [pltpu.make_async_copy(w.bitcast(i32).at[:, cols], v.at[:, cols], w_sem.at[n])
                for w, v in ((wg_hbm, wg_v), (wu_hbm, wu_v))]

    def chunk_rows(n):
        return pl.ds(_aligned(n * _OCH, 32), _OCH)

    def down_copy(n):
        rows = pl.ds(_aligned(n * (_OCH // 2), 16), _OCH // 2)
        return pltpu.make_async_copy(wd_hbm.bitcast(i32).at[rows], wd_v.at[n], w_sem.at[_NF + n])

    def out_copy(n):
        return pltpu.make_async_copy(o_v.at[chunk_rows(n)], o_hbm.at[chunk_rows(n)], o_sem)

    def start_parameters(part, rows):
        for n, src in enumerate((ar_hbm, ai_hbm, br_hbm, bi_hbm, cr_hbm, ci_hbm)):
            start(part, src.bitcast(i32).at[rows], par_v.at[n, rows])

    with jax.named_scope("init"):
        start("vectors", ldt_hbm, ldt_v)
        start("vectors", dsk_hbm, dsk_v)
        start_parameters(0, pl.ds(0, 16 * _GA))
        start(0, fwd_hbm, fwd_v)
        arena[0, _ROW_W:_ROW_P] = jnp.zeros((_ROW_P - _ROW_W, 8, _T), i32)
        tap_v[...] = jnp.zeros(tap_v.shape, i32)
        k_v[:_GA] = jnp.zeros((_GA, _NB, 8, _T), i32)
        key_v[...] = jnp.zeros(key_v.shape, f32)
        wait("vectors")
        start_parameters(1, pl.ds(16 * _GA, _D // 2 - 16 * _GA))
        start("x", x_hbm.bitcast(i32), x_v)
        start("x", wr_hbm, wr_v)
        dt_v[...] = pltpu.bitcast(_column(jnp.exp(ldt_v[...].astype(f32))).astype(bf16), i32)
        skip_v[...] = pltpu.bitcast(_column(dsk_v[...].astype(f32)).astype(bf16), i32)
        wait(0)

    def compact(ref, k, h):
        out = ref[k, 8 * h]
        for s in range(1, 8):
            out = jnp.where(row == s, ref[k, 8 * h + s], out)
        return out

    def layer_norm():
        wait("x")
        for cp in hidden_copies(1):
            cp.start()

        def moments(b, carry):
            cols = pl.ds(_aligned(b * _T, _T), _T)
            pivot = jnp.broadcast_to(_even_odd(x_v[:8, cols])[0][:1], (8, _T))
            s1, s2 = [None] * 2, [None] * 2
            for g in range(_NG):
                words = x_v[pl.ds(8 * g, 8), cols]
                x = pltpu.bitcast(words, bf16).astype(f32)
                xc_v[b, g] = x
                for h in range(2):
                    d = x[8 * h:8 * h + 8] - pivot
                    s1[h] = s1[h] + d if g else d
                    s2[h] = s2[h] + d * d if g else d * d
            for k, s in enumerate((s1, s2)):
                stat_v[k, b] = jnp.broadcast_to(jnp.sum(s[0] + s[1], axis=0, keepdims=True), (8, _T))
            stat_v[2, b] = pivot
            return carry

        lax.fori_loop(0, _NB, moments, 0, unroll=4)
        for h in range(_NB // 8):
            m1, m2, pivot = compact(stat_v, 0, h) / _D, compact(stat_v, 1, h) / _D, compact(stat_v, 2, h)
            var = jnp.maximum(m2 - m1 * m1, 0.0)
            shift = _rnd(pivot + m1)
            gain = 0.5 / _rnd(jnp.sqrt(_rnd(_rnd(var) + _rnd(jnp.full_like(var, _EPS)))))
            for s in range(8):
                stat_v[0, 8 * h + s] = jnp.broadcast_to(shift[s:s + 1], (8, _T))
                stat_v[1, 8 * h + s] = jnp.broadcast_to(gain[s:s + 1], (8, _T))
        inv_v[...] = pltpu.bitcast(
            (pltpu.bitcast(fwd_v[...], bf16).astype(f32).T * (2 / _T)).astype(bf16), i32)
        wr = jnp.broadcast_to(wr_v[...].astype(f32).reshape(1, _D), (8, _D)).astype(bf16)

        def scale(b, carry):
            shift, gain = stat_v[0, b], stat_v[1, b]
            xn = [_interleave(*[(xc_v[b, g, pl.ds(h, 8, stride=2), :] - shift) * gain for h in range(2)])
                  for g in range(_NG)]
            for g in range(_NG):
                arena[g // _GC, _ROW_X + (g % _GC) * _NB + b] = xn[g]
            stat_v[2, b] = _dot(wr, pltpu.bitcast(jnp.concatenate(xn, axis=0), bf16))
            return carry

        lax.fori_loop(0, _NB, scale, 0, unroll=16)
        for h in range(_NB // 8):
            bits = pltpu.bitcast(_rnd(2.0 * compact(stat_v, 2, h)) + 0.0, i32) >> 16
            rank = jnp.where(bits < 0, ~bits, bits + 0x8000)
            token = (8 * h + row) * _T + lane
            key_v[h] = pltpu.bitcast((1 << 28) + rank * _L + (_L - 1 - token), f32)

    def pop_best(c):
        best = jnp.max(jnp.max(jnp.maximum(key_v[0], key_v[1]), axis=0, keepdims=True),
                       axis=1, keepdims=True)
        key_v[2] = jnp.where(row == c, best, key_v[2])
        for h in range(2):
            key_v[h] = jnp.where(key_v[h] == best, 0.0, key_v[h])

    def modes(step):
        for u in range(_GA):
            grp = step * _GA + u
            rows = pl.ds(_aligned(grp * 8, 8), 8)
            par = [_even_odd(dt_v[rows, :])] + [_even_odd(par_v[n, rows, :]) for n in range(6)]
            k0 = []
            for h, skip in enumerate(_even_odd(skip_v[rows, :])):
                z = _modes(*[p[h] for p in par])
                for n in range(4):
                    mode_v[u, h, n] = z[n]
                k0.append(skip + jnp.sum(z[0], axis=1, keepdims=True))
            k0_v[grp] = _interleave(*k0)

    def dft(rows):
        z = _dot(jnp.concatenate([pltpu.bitcast(r, bf16) for r in rows], axis=0),
                 pltpu.bitcast(fwd_v[...], bf16))
        n = min(len(rows), _NB)
        return [[(z[o:o + 8, :_T], z[o:o + 8, _T:])
                 for o in range((h // 2) * 16 * n + 8 * (h % 2), (h // 2 + 1) * 16 * n, 16)]
                for h in range(2 * len(rows) // n)]

    def spread(step, u, slot):
        for j, blk in _lag_blocks(lambda n: tap_v[u, n], k0_v[step * _GA + u]):
            k_v[slot, j] = blk

    def filter_spectra(grp, rows):
        for h, blocks in enumerate(dft(rows)):
            for j, (re, im) in enumerate(blocks):
                for p, val in enumerate((re, re + im, im - re)):
                    kf_v[2 * grp + h, p * _PLANE + j] = val

    def filter_step(i, zero, extra=lambda u: None):
        for u in range(_GA):
            if u % (_GA // 2) == 0:
                old = (u + _GA // 2) % _GA
                filter_spectra(jnp.maximum(i - (1 if u else 2), 0) * _GA + old,
                               [k_v[old + k + zero, j] for k in range(_GA // 2) for j in range(_NB)])
            spread(jnp.maximum(i - 1, 0), u, u)
            v = [[_vandermonde(*seeds) for seeds in _seeds(
                (mode_v[u, h, 0], mode_v[u, h, 1]), (mode_v[u, h, 2], mode_v[u, h, 3]))]
                 for h in range(2)]
            for n, tap in enumerate(_unmix(*map(_interleave, *v))):
                tap_v[u, n] = tap
            extra(u)

    def phase_a(i, carry):
        @pl.when(i == 1)
        def _():
            wait(1)
            for cp in hidden_copies(0):
                cp.start()

        pl.when(i == _LN_STEP)(layer_norm)
        for c in range(2):
            pop_best(2 * (i - _LN_STEP) + c)
        filter_step(i, i >> 8)
        modes(i + 1)

    with jax.named_scope("A"):
        modes(0)
        lax.fori_loop(0, _NG // _GA - 1, phase_a, None)

    def input_spectra(rows, dst):
        z = dft(rows)
        for h, t in enumerate(z):
            for b, (re, im) in enumerate(t):
                if b:
                    re, im = re + t[b - 1][1], im - t[b - 1][0]
                for p, val in enumerate((re + im, im, re)):
                    dst[(h * 3 + p) * _PLANE + b] = val
        return z

    def w_row(c, r):
        return jnp.concatenate(
            [pltpu.bitcast(arena[c, _ROW_W + q * _WQ + r], bf16) for q in range(2)], axis=1)

    def routed_tokens():
        return _L - 1 - (pltpu.bitcast(key_v[2], i32) & (_L - 1))

    with jax.named_scope("topk"):
        for n in range(2, _NF):
            for cp in hidden_copies(n):
                cp.start()
        token = routed_tokens()
        picked = []

        def gather(u):
            tokens = range(u * _C // _GA, (u + 1) * _C // _GA)
            blocks = jnp.concatenate(
                [pltpu.bitcast(jnp.concatenate(
                    [arena[g // _GC, _ROW_X + (g % _GC) * _NB + (token[t, 0] >> 7)]
                     for g in range(_NG)], axis=0), bf16) for t in tokens], axis=1)
            pick = jnp.concatenate(
                [jnp.where((row == t) & ((token & (_T - 1)) == lane), 2.0, 0.0) for t in tokens],
                axis=1).astype(bf16)
            picked.append(_dot_nt(pick, blocks))

        filter_step(_NG // _GA - 1, token[0, 0] >> 11, gather if _MERGE else lambda u: None)
        for u in range(0 if _MERGE else _GA):
            gather(u)
        x_sel = sum(picked[1:], picked[0])
        for n in range(_NO):
            sel_v[n] = x_sel[:, n * _OCH:(n + 1) * _OCH]
        x_sel = jnp.concatenate([x_sel, jnp.zeros((8, _KT * _T - _D), f32)], axis=1)
        for n in range(_KT):
            arena[0, _ROW_SEL + n] = pltpu.bitcast(
                jnp.concatenate([x_sel[:, n * _T:(n + 1) * _T]] * 2, axis=0).astype(bf16), i32)
        input_spectra([arena[0, _ROW_X + r] for r in range(_R)], spec_a)
        for u in range(_GA):
            spread(_NG // _GA - 1, u, _GA + u)
        filter_spectra(_NG - 3 * _GA // 2,
                       [k_v[u, j] for u in range(_GA // 2, 2 * _GA) for j in range(_NB)])

    def hidden_jobs(c):
        width = _F // (_NCH - _NO)
        gate = []

        def project(n):
            cols = pl.ds(_aligned(c * width + n // 2 * _T, _T), _T)
            x_sel = jnp.concatenate(
                [pltpu.bitcast(arena[c >> 8, _ROW_SEL + r], bf16) for r in range(_KT)], axis=1)
            gate.append(_rnd(_dot(x_sel[:, :_D], pltpu.bitcast((wu_v if n % 2 else wg_v)[:, cols], bf16))[:8]))
            if n % 2:
                hid_v[:, cols] = (_rnd(_silu(gate[-2])) * gate[-1]).astype(bf16)

        return [(40 * n, lambda n=n: project(n)) for n in range(2 * width // _T)]

    def hidden_at(t, zero=0):
        return pl.ds(_aligned(_D + 8 * (t // _NB + zero), 8), 8), pl.ds((t % _NB) * _T, _T)

    def finish(n):
        for k in range(_OCH // 16 * _NB):
            c, r = n * (_OCH // (16 * _GC)) + k // _R, k % _R
            rows = pl.ds(_aligned(n * _OCH + 16 * (k // _NB), 16), 16)
            cols = pl.ds((k % _NB) * _T, _T)
            h = pltpu.bitcast(arena[c, _ROW_X + r], bf16).astype(f32)
            b = r % _NB
            s = s_v[c, pl.ds(16 * (r - b) + 32 * (b // 4 * 2 + b % 2) + b // 2 % 2, 16, stride=2), :]
            gated = s * (h + h * jnp.tanh(h))
            o_v[rows, cols] = (xc_v[k % _NB, n * (_OCH // 16) + k // _NB] + gated).astype(bf16)
            yield k

    def down_jobs(n, hid):
        rank = (pltpu.bitcast(key_v[2], i32) - (1 << 28)) >> 11
        score = pltpu.bitcast(jnp.where(rank >= 0x8000, rank - 0x8000, ~rank) << 16, f32)
        y = _rnd(_dot_nt(jnp.concatenate(hid, axis=1), pltpu.bitcast(wd_v[n], bf16)))
        y = 0.5 * (sel_v[n] + _rnd(y * _rnd(jax.nn.sigmoid(score))[:, :_OCH]))
        col = jnp.concatenate([y, jnp.zeros((_T - _C, _OCH), f32)], axis=0).T
        col = pltpu.bitcast(col.astype(bf16), i32)
        token = routed_tokens()

        def scatter(t):
            hit = ((token & (_T - 1)) == lane)[t:t + 1]
            new = jnp.broadcast_to(col[:, t:t + 1], (_OCH // 2, _T))
            where = [(n * (_OCH // (16 * _GC)) + g // _GC,
                      _ROW_X + (g % _GC) * _NB + (token[t, 0] >> 7)) for g in range(_OCH // 16)]
            old = [arena[at] for at in where]
            for g, at in enumerate(where):
                arena[at] = jnp.where(hit, new[8 * g:8 * g + 8], old[g])

        return [lambda t=t: scatter(t) for t in range(_C)]

    def first_output_jobs(c):
        hid, scatter = [], []

        def read():
            hid.extend(pltpu.bitcast(arena[c >> 8, _ROW_W + t], bf16)[:8]
                       for t in range(len(hid), len(hid) + 4))

        return ([(48 * k, read) for k in range(_F // (4 * _T))]
                + [(_G2 - 1, lambda: scatter.extend(down_jobs(0, hid)))]
                + [(_G2 + _S0 + _S1 * t, lambda t=t: scatter[t]()) for t in range(_C)])

    def output_jobs(c):
        n = c - (_NCH - _NO)
        hid = [o_v[hidden_at(t, c >> 8)] for t in range(4)]
        for k in finish(n - 1):
            if k % 12 == 11:
                hid += [o_v[hidden_at(t, c >> 8)] for t in range(len(hid), len(hid) + 4)]
        jobs = [(_S0 + _S1 * t, job) for t, job in enumerate(down_jobs(n, hid))]
        pl.when(n >= _HOLD)(lambda: out_copy(n - 1).start())
        return jobs

    def conv_step(c, cur, nxt, ffn_jobs, delay, pace):
        c_next, c_prev = jnp.minimum(c + 1, _NCH - 1), jnp.maximum(c - 1, 0)
        zero = c >> 8
        fwd_rows, inv_rows, results = [], [], []

        def transform():
            y = _dot(jnp.concatenate(inv_rows, axis=0), pltpu.bitcast(inv_v[...], bf16))
            s_v[c_prev] = y
            results.extend((y, input_spectra(fwd_rows, nxt)))

        def drain(r):
            y, z = results
            arena[c, _ROW_SEL - 1] = pltpu.bitcast(
                y[8 * r:8 * r + 8] + z[2 * (r // _R) + 1][r % _R // 2][r // 8 % 2], i32)

        jobs = sorted(
            ffn_jobs(c)
            + [(delay + 16 * r, lambda r=r: inv_rows.append(w_row(c_prev, r))) for r in range(_R)]
            + [(delay + 16 * r, lambda r=r: fwd_rows.append(arena[c_next, _ROW_X + r]))
               for r in range(_R)]
            + [(delay + 16 * _R, transform)]
            + [(delay + _LAG + 8 * r, lambda r=r: drain(r)) for r in range(2 * _R - 17, 2 * _R, 8)],
            key=lambda job: job[0])

        def run_jobs(done):
            while jobs and done * (delay + 16 * _R) >= (jobs[0][0] - _LEAD) * pace * 18 * _GC:
                jobs.pop(0)[1]()

        run_jobs(0)
        for h in range(2 * _GC):
            for part in range(3):
                for plane in range(3):
                    kf = lambda b: kf_v[c * 2 * _GC + h + (zero >> part), plane * _PLANE + b]
                    uf = lambda b: cur[(zero >> part) + (h * 3 + plane) * _PLANE + b]
                    base = [pltpu.bitcast(arena[c + zero, _ROW_P + plane * 8 + m], f32)
                            for m in range(8) if part and plane]
                    k, u, out = [], [], []
                    for m in range(8):
                        if part == 0:
                            k.append(kf(2 * m))
                            u.append(uf(2 * m) + uf(2 * m + 1))
                        elif part == 1:
                            k.append(kf(2 * m) - kf(2 * m - 1) if m else kf(0))
                            u.append(uf(2 * m + 1))
                        else:
                            k.append(kf(2 * m) - kf(2 * m + 1))
                            u.append(uf(2 * m))
                        y = k[0] * u[m]
                        for j in range(1, m + 1):
                            y = y + k[j] * u[m - j]
                        if plane:
                            y = shared[m] - y if plane == 1 else shared[m] + y
                        out.append(y)
                        if part == 0 or plane == 0:
                            arena[c, _ROW_P + plane * 8 + m] = pltpu.bitcast(y, i32)
                        elif m % 2:
                            r = (h // 2) * _NB + (m - 1 + part - 1) * 2 + h % 2
                            arena[c, _ROW_W + (plane - 1) * _WQ + r] = _interleave(
                                base[m - 1] - out[m - 1], base[m] - y)
                    if plane == 0:
                        shared = out
                    run_jobs((h * 3 + part) * 3 + plane + 1)
        run_jobs(np.inf)

    def phase_c(part, carry):
        for cp in hidden_copies(part):
            cp.wait()

        @pl.when(part == _WD_STEP)
        def _():
            for n in range(_NO):
                down_copy(n).start()

        def pair(i, carry):
            conv_step(2 * i, spec_a, spec_b, hidden_jobs, 240, _PACE)
            conv_step(2 * i + 1, spec_b, spec_a, hidden_jobs, 240, _PACE)

        pairs = (_NCH - _NO) // (2 * _NF)
        lax.fori_loop(part * pairs, (part + 1) * pairs, pair, None)

    def phase_d(n, carry):
        down_copy(n).wait()

        @pl.when(n == _HOLD + _HALF)
        def _():
            for k in range(_HOLD - 1):
                out_copy(k).start()

        c = n + _NCH - _NO
        lax.cond(c & 1 == 0, lambda: conv_step(c, spec_a, spec_b, output_jobs, _G1, _PACE1),
                 lambda: conv_step(c, spec_b, spec_a, output_jobs, _G1, _PACE1))

    with jax.named_scope("C"):
        lax.fori_loop(0, _NF, phase_c, None)
    with jax.named_scope("D"):
        for t in range(_F // _T):
            tile = hid_v[:, t * _T:(t + 1) * _T]
            o_v[hidden_at(t)] = tile
            arena[0, _ROW_W + t] = pltpu.bitcast(jnp.concatenate([tile] * 2, axis=0), i32)
        down_copy(0).wait()
        conv_step(_NCH - _NO + (routed_tokens()[0, 0] >> 11), spec_a, spec_b, first_output_jobs,
                  _G2, _PACE2)
        lax.fori_loop(1, _NO, phase_d, None)
    with jax.named_scope("tail"):
        s_v[_NCH - 1] = _dot(
            jnp.concatenate([w_row(_NCH - 1, r) for r in range(_R)], axis=0), pltpu.bitcast(inv_v[...], bf16))
        for k in finish(_NO - 1):
            if k % _R == _R - 1:
                rows = pl.ds((_NO - 1) * _OCH + k // _R * 16 * _GC, 16 * _GC)
                start("out", o_v.at[rows], o_hbm.at[rows])
    with jax.named_scope("end"):
        for n in range(_NO - 1):
            out_copy(n).wait()
        wait("out")


@jax.jit
def pallas_recurrent_scan__ssm_conv_s4__moe_arch_mod__prompt_kernel(
    A_u: jax.Array,
    A_A_re: jax.Array,
    A_A_im: jax.Array,
    A_B_re: jax.Array,
    A_B_im: jax.Array,
    A_C_re: jax.Array,
    A_C_im: jax.Array,
    A_log_dt: jax.Array,
    A_Dskip: jax.Array,
    B_x: jax.Array,
    B_w_r: jax.Array,
    B_w_gate: jax.Array,
    B_w_up: jax.Array,
    B_w_down: jax.Array,
):
    del B_x
    assert A_u.shape == (1, _L, _D) and A_A_re.shape == (_D, _N) and B_w_gate.shape == (_D, _F)
    assert A_u.dtype == bf16 and A_A_re.dtype == bf16
    hbm = pl.BlockSpec(memory_space=pl.ANY)
    vmem = pltpu.VMEM
    out = pl.pallas_call(
        _kernel,
        out_shape=jax.ShapeDtypeStruct((_D, _L), bf16),
        in_specs=[hbm] * 14,
        out_specs=hbm,
        scratch_shapes=[
            vmem((_D // 2, _L), i32), vmem((_D + 32, _L), bf16),
            vmem((6, _D // 2, _N), i32), vmem((_D,), bf16), vmem((_D,), bf16), vmem((_D,), bf16),
            vmem((_D // 2, _F), i32), vmem((_D // 2, _F), i32), vmem((_NO, _OCH // 2, _F), i32),
            vmem((_T // 2, 2 * _T), i32), vmem((_T, _T), i32),
            vmem((_D // 2, _T), i32), vmem((_NG, 8, _T), i32),
            vmem((_NCH, _ROWS, 8, _T), i32), vmem((_NCH, 16 * _R, _T), f32),
            vmem((_D // 2, _T), i32), vmem((_GA, 2, 4, 8, _N), f32), vmem((_GA, len(_TAPS), 8, _T), i32),
            vmem((2 * _GA, _NB, 8, _T), i32),
            vmem((_NB, _NG, 16, _T), f32), vmem((3, _NB, 8, _T), f32), vmem((3, 8, _T), f32),
            vmem((_NO, 8, _OCH), f32), vmem((8, _F), bf16),
            *[vmem((2 * _GC * 3 * _PLANE, 8, _T), f32)] * 2, vmem((2 * _NG, 3 * _PLANE, 8, _T), f32),
            pltpu.SemaphoreType.DMA((5,)), pltpu.SemaphoreType.DMA((_NF + _NO,)),
            pltpu.SemaphoreType.DMA(()),
        ],
        compiler_params=pltpu.CompilerParams(vmem_limit_bytes=100 * 2**20, flags=_FLAGS),
    )(A_u.reshape(_L, _D).T, A_A_re, A_A_im, A_B_re, A_B_im, A_C_re, A_C_im, A_log_dt, A_Dskip,
      B_w_r, B_w_gate, B_w_up, B_w_down.T, _FWD)
    return out.T.reshape(1, _L, _D)
```

```python
import jax
import jax.numpy as jnp
import numpy as np
from jax import lax
import jax.experimental.pallas as pl
import jax.experimental.pallas.tpu as pltpu

_D, _L, _N, _F, _C = 576, 2048, 128, 4608, 8
_T = 128
_NB = _L // _T
_EPS = 1e-5
_GA = 4
_GC = 2
_NG = _D // 16
_NCH = _NG // _GC
_R = _GC * _NB
_ROW_X, _ROW_W, _ROW_P, _ROWS = 0, _R, 5 * _R + 8, 5 * _R + 8 + 24
_PLANE, _WQ = _NB + 1, 2 * _R + 1
_ROW_SEL = 5 * _R + 3
_MERGE, _HOLD, _PRIO, _G2, _PACE2 = 1, 3, 0, 400, 0.83
_FLAGS, _HALF = None, 0
_KT = -(-_D // _T)
_NO, _OCH = 6, _D // 6
_NF = 3
_FCH = _F // _NF
_LN_STEP = 4
_WD_STEP = 1
_PACE, _PACE1, _LEAD, _LAG, _G1, _S0, _S1 = 0.87, 0.8, 32, 140, 32, 520, 20

f32, bf16, i32 = jnp.float32, jnp.bfloat16, jnp.int32


def _dft_constants():
    theta = (np.pi / 2 + 2 * np.pi * np.arange(_T)) / _T
    ang = np.arange(_T)[:, None] * theta[None, :]
    c, s = np.cos(ang), np.sin(ang)
    fwd = np.concatenate([c, s], axis=1)
    bits = fwd.astype(bf16).view(np.uint16).astype(np.uint32)
    words = (bits[0::2] | bits[1::2] << 16).view(np.int32)
    return words


_FWD = _dft_constants()


def _lag_step(j):
    return max(1, (1 << (j * _T).bit_length()) >> 8)


def _round_lag(p, st):
    if st == 1:
        return p
    return (p + (st // 2 - 1) + ((p >> (st.bit_length() - 1)) & 1)) & ~(st - 1)


assert np.array_equal(
    np.concatenate([j * _T + _round_lag(np.arange(_T), _lag_step(j)) for j in range(_NB)]),
    np.arange(_L).astype(bf16).astype(np.int64))

_PAIRS = (((0, 1), (0, 5)), ((0, 2), (0, 6)), ((0, 3), (0, 7)), ((0, 4), (0, 8)), ((1, 2), (1, 6)),
          ((1, 4), (1, 8)), ((2, 4), (2, 8)), ((3, 4), (3, 8)), ((4, 8), (5, 8)), ((6, 8), (7, 8)))
_TAPS = [k for pair in _PAIRS for k in pair]


def _aligned(i, n):
    return i if isinstance(i, int) else pl.multiple_of(i, n)


def _cmul(a, b):
    return a[0] * b[0] - a[1] * b[1], a[0] * b[1] + a[1] * b[0]


def _csq(a):
    return a[0] * a[0] - a[1] * a[1], (a[0] + a[0]) * a[1]


def _silu(x):
    h = 0.5 * x
    return h + h * jnp.tanh(h)


def _rnd(x):
    return x.astype(bf16).astype(f32)


def _dot(a, b):
    return jnp.dot(a, b, preferred_element_type=f32)


def _dot_nt(a, b):
    return lax.dot_general(a, b, (((1,), (1,)), ((), ())), preferred_element_type=f32)


def _column(v):
    return jnp.broadcast_to(v.reshape(1, _D), (_T, _D)).T


def _even_odd(x):
    return pltpu.bitcast(x << 16, f32), pltpu.bitcast(x & -65536, f32)


def _interleave(even, odd):
    even, odd = [pltpu.bitcast(x, i32) + 0x8000 for x in (even, odd)]
    return lax.shift_right_logical(even, 16) | (odd & -65536)


def _words(x):
    y = jnp.concatenate([x[:8], x[8:]], axis=1).astype(bf16)
    return pltpu.bitcast(jnp.concatenate([y[:, :_T], y[:, _T:]], axis=0), i32)


def _modes(dt, ar, ai, br, bi, cr, ci):
    zr, zi = dt * ar, dt * ai
    mag = jnp.exp(zr)
    return _cmul((cr, ci), (dt * br, dt * bi)) + (mag * jnp.cos(zi), mag * jnp.sin(zi))


def _seeds(w, a1):
    a = {1: a1}
    for n in range(9):
        a[2 << n] = _csq(a[1 << n])
    row = lax.broadcasted_iota(i32, (8, _N), 0)

    def conj(z):
        return z[0], -z[1]

    def mix(z0, z1):
        rolled = [pltpu.roll(x, 4, 0) for x in z1]
        return ([jnp.where(row < 4, x, y) for x, y in zip(z0, rolled)],
                [jnp.where(row < 4, y, x) for x, y in zip(z0, rolled)])

    def dup(z):
        return [[jnp.take_along_axis(x, (row & 3) + 4 * q, axis=0, mode="promise_in_bounds")
                 for x in z] for q in range(2)]

    wa = _cmul(w, a[1])
    return zip(mix((1.0, 0.0), conj(a[128])), dup(conj(a[8])), dup(conj(a[32])),
               mix(wa, _cmul(wa, a[4])), dup(a[1]), dup(a[256]),
               mix(_cmul(a[256], a[4]), a[512]), dup(a[512]))


def _vandermonde(e0, m8, m32, g0, m1, m256, m_top, m512):
    e = [e0]
    for s in range(1, 16):
        e.append(_cmul(e[s - 1], m8) if s < 4 else _cmul(e[s - 4], m32))
    g = [g0]
    for _ in range(3):
        g.append(_cmul(g[-1], m1))
    g += [_cmul(g[1], m256), _cmul(g[3], m256)]
    g += [_cmul(g[3], m512), _cmul(g[5], m512)]
    g.append(_cmul(g[7], m_top))
    g.append(_cmul(g[8], m512))
    re, im = [_dot_nt(jnp.concatenate([z[p] for z in g], axis=0),
                      jnp.concatenate([z[p] for z in e], axis=0)) for p in range(2)]
    return re + im


def _unmix(lo, hi):
    row = lax.broadcasted_iota(i32, (8, _T), 0)
    out = []
    for m in range(len(_PAIRS)):
        x, y = lo[8 * m:8 * m + 8], hi[8 * m:8 * m + 8]
        out += [jnp.where(row < 4, x, y), pltpu.roll(jnp.where(row < 4, y, x), 4, 0)]
    return out


def _lag_blocks(tap, lag0):
    lane = lax.broadcasted_iota(i32, (8, _T), 1)
    row = lax.broadcasted_iota(i32, (8, _T), 0)
    for h in range(2):
        def take(big, r, fine):
            s = ((_T * h + fine) >> 3) & 31
            return jnp.take_along_axis(tap(_TAPS.index((big, r))),
                                       ((s & 15) << 3) + (row ^ ((s >> 4) << 2)),
                                       axis=1, mode="promise_in_bounds")

        top = [take(big, 8, _round_lag(lane, 8) - 8) for big in range(_NB // 2)]
        for big, blk in enumerate(top):
            st = _lag_step(2 * big + h)
            lag = _round_lag(lane, st)
            if h == 0:
                blk = jnp.where(lag == 0, top[big - 1] if big else lag0, blk)
            for r in range(st, 8, st):
                blk = jnp.where((lag & 7) == r, take(big, r, lane), blk)
            yield 2 * big + h, blk


def _kernel(x_hbm, ar_hbm, ai_hbm, br_hbm, bi_hbm, cr_hbm, ci_hbm, ldt_hbm, dsk_hbm, wr_hbm,
            wg_hbm, wu_hbm, wd_hbm, fwd_hbm, o_hbm,
            x_v, o_v, par_v, ldt_v, dsk_v, wr_v, wg_v, wu_v, wd_v, fwd_v, inv_v,
            skip_v, k0_v, arena, s_v, dt_v, mode_v, tap_v, k_v, xc_v, stat_v, key_v, sel_v, hid_v,
            spec_a, spec_b, kf_v, sem, w_sem, o_sem):
    row = lax.broadcasted_iota(i32, (8, _T), 0)
    lane = lax.broadcasted_iota(i32, (8, _T), 1)
    groups = {}

    def start(name, src, dst):
        slot, pairs = groups.setdefault(name, (len(groups), []))
        pairs.append((src, dst))
        pltpu.make_async_copy(src, dst, sem.at[slot]).start()

    def wait(name):
        slot, pairs = groups[name]
        for src, dst in pairs:
            pltpu.make_async_copy(src, dst, sem.at[slot]).wait()

    def hidden_copies(n):
        cols = pl.ds(_aligned(n * _FCH, _FCH), _FCH)
        return [pltpu.make_async_copy(w.bitcast(i32).at[:, cols], v.at[:, cols], w_sem.at[n])
                for w, v in ((wg_hbm, wg_v), (wu_hbm, wu_v))]

    def chunk_rows(n):
        return pl.ds(_aligned(n * _OCH, 32), _OCH)

    def down_copy(n):
        rows = pl.ds(_aligned(n * (_OCH // 2), 16), _OCH // 2)
        return pltpu.make_async_copy(wd_hbm.bitcast(i32).at[rows], wd_v.at[n], w_sem.at[_NF + n])

    def out_copy(n):
        return pltpu.make_async_copy(o_v.at[chunk_rows(n)], o_hbm.at[chunk_rows(n)], o_sem)

    def start_parameters(part, rows):
        for n, src in enumerate((ar_hbm, ai_hbm, br_hbm, bi_hbm, cr_hbm, ci_hbm)):
            start(part, src.bitcast(i32).at[rows], par_v.at[n, rows])

    with jax.named_scope("init"):
        start("vectors", ldt_hbm, ldt_v)
        start("vectors", dsk_hbm, dsk_v)
        start_parameters(0, pl.ds(0, 16 * _GA))
        start(0, fwd_hbm, fwd_v)
        arena[0, _ROW_W:_ROW_P] = jnp.zeros((_ROW_P - _ROW_W, 8, _T), i32)
        tap_v[...] = jnp.zeros(tap_v.shape, i32)
        k_v[:_GA] = jnp.zeros((_GA, _NB, 8, _T), i32)
        key_v[...] = jnp.zeros(key_v.shape, f32)
        wait("vectors")
        start_parameters(1, pl.ds(16 * _GA, _D // 2 - 16 * _GA))
        start("x", x_hbm.bitcast(i32), x_v)
        start("x", wr_hbm, wr_v)
        dt_v[...] = pltpu.bitcast(_column(jnp.exp(ldt_v[...].astype(f32))).astype(bf16), i32)
        skip_v[...] = pltpu.bitcast(_column(dsk_v[...].astype(f32)).astype(bf16), i32)
        wait(0)

    def compact(ref, k, h):
        out = ref[k, 8 * h]
        for s in range(1, 8):
            out = jnp.where(row == s, ref[k, 8 * h + s], out)
        return out

    def layer_norm():
        wait("x")
        for cp in hidden_copies(1):
            cp.start()

        def moments(b, carry):
            cols = pl.ds(_aligned(b * _T, _T), _T)
            pivot = jnp.broadcast_to(_even_odd(x_v[:8, cols])[0][:1], (8, _T))
            s1, s2 = [None] * 2, [None] * 2
            for g in range(_NG):
                words = x_v[pl.ds(8 * g, 8), cols]
                x = pltpu.bitcast(words, bf16).astype(f32)
                xc_v[b, g] = x
                for h in range(2):
                    d = x[8 * h:8 * h + 8] - pivot
                    s1[h] = s1[h] + d if g else d
                    s2[h] = s2[h] + d * d if g else d * d
            for k, s in enumerate((s1, s2)):
                stat_v[k, b] = jnp.broadcast_to(jnp.sum(s[0] + s[1], axis=0, keepdims=True), (8, _T))
            stat_v[2, b] = pivot
            return carry

        lax.fori_loop(0, _NB, moments, 0, unroll=4)
        for h in range(_NB // 8):
            m1, m2, pivot = compact(stat_v, 0, h) / _D, compact(stat_v, 1, h) / _D, compact(stat_v, 2, h)
            var = jnp.maximum(m2 - m1 * m1, 0.0)
            shift = _rnd(pivot + m1)
            gain = 0.5 / _rnd(jnp.sqrt(_rnd(_rnd(var) + _rnd(jnp.full_like(var, _EPS)))))
            for s in range(8):
                stat_v[0, 8 * h + s] = jnp.broadcast_to(shift[s:s + 1], (8, _T))
                stat_v[1, 8 * h + s] = jnp.broadcast_to(gain[s:s + 1], (8, _T))
        inv_v[...] = pltpu.bitcast(fwd_v[...], bf16).astype(f32).T * (2 / _T)
        wr = jnp.broadcast_to(wr_v[...].astype(f32).reshape(1, _D), (8, _D)).astype(bf16)

        def scale(b, carry):
            shift, gain = stat_v[0, b][:1], stat_v[1, b][:1]
            xn = [_words((xc_v[b, g] - shift) * gain) for g in range(_NG)]
            for g in range(_NG):
                arena[g // _GC, _ROW_X + (g % _GC) * _NB + b] = xn[g]
            stat_v[2, b] = _dot(wr, pltpu.bitcast(jnp.concatenate(xn, axis=0), bf16))
            return carry

        lax.fori_loop(0, _NB, scale, 0, unroll=16)
        for h in range(_NB // 8):
            bits = pltpu.bitcast(_rnd(2.0 * compact(stat_v, 2, h)) + 0.0, i32) >> 16
            rank = jnp.where(bits < 0, ~bits, bits + 0x8000)
            token = (8 * h + row) * _T + lane
            key_v[h] = pltpu.bitcast((1 << 28) + rank * _L + (_L - 1 - token), f32)

    def pop_best(c):
        best = jnp.max(jnp.max(jnp.maximum(key_v[0], key_v[1]), axis=0, keepdims=True),
                       axis=1, keepdims=True)
        key_v[2] = jnp.where(row == c, best, key_v[2])
        for h in range(2):
            key_v[h] = jnp.where(key_v[h] == best, 0.0, key_v[h])

    def modes(step):
        for u in range(_GA):
            grp = step * _GA + u
            rows = pl.ds(_aligned(grp * 8, 8), 8)
            par = [_even_odd(dt_v[rows, :])] + [_even_odd(par_v[n, rows, :]) for n in range(6)]
            k0 = []
            for h, skip in enumerate(_even_odd(skip_v[rows, :])):
                z = _modes(*[p[h] for p in par])
                for n in range(4):
                    mode_v[u, h, n] = z[n]
                k0.append(skip + jnp.sum(z[0], axis=1, keepdims=True))
            k0_v[grp] = _interleave(*k0)

    def dft(rows):
        z = _dot(jnp.concatenate([pltpu.bitcast(r, bf16) for r in rows], axis=0),
                 pltpu.bitcast(fwd_v[...], bf16))
        n = min(len(rows), _NB)
        return [[(z[o:o + 8, :_T], z[o:o + 8, _T:])
                 for o in range((h // 2) * 16 * n + 8 * (h % 2), (h // 2 + 1) * 16 * n, 16)]
                for h in range(2 * len(rows) // n)]

    def spread(step, u, slot):
        for j, blk in _lag_blocks(lambda n: tap_v[u, n], k0_v[step * _GA + u]):
            k_v[slot, j] = blk

    def filter_spectra(grp, rows):
        for h, blocks in enumerate(dft(rows)):
            for j, (re, im) in enumerate(blocks):
                for p, val in enumerate((re, re + im, im - re)):
                    kf_v[2 * grp + h, p * _PLANE + j] = val

    def filter_step(i, zero, extra=lambda u: None):
        for u in range(_GA):
            if u % (_GA // 2) == 0:
                old = (u + _GA // 2) % _GA
                filter_spectra(jnp.maximum(i - (1 if u else 2), 0) * _GA + old,
                               [k_v[old + k + zero, j] for k in range(_GA // 2) for j in range(_NB)])
            spread(jnp.maximum(i - 1, 0), u, u)
            v = [[_vandermonde(*seeds) for seeds in _seeds(
                (mode_v[u, h, 0], mode_v[u, h, 1]), (mode_v[u, h, 2], mode_v[u, h, 3]))]
                 for h in range(2)]
            for n, tap in enumerate(_unmix(*map(_interleave, *v))):
                tap_v[u, n] = tap
            extra(u)

    def phase_a(i, carry):
        @pl.when(i == 1)
        def _():
            wait(1)
            for cp in hidden_copies(0):
                cp.start()

        pl.when(i == _LN_STEP)(layer_norm)
        for c in range(2):
            pop_best(2 * (i - _LN_STEP) + c)
        filter_step(i, i >> 8)
        modes(i + 1)

    with jax.named_scope("A"):
        modes(0)
        lax.fori_loop(0, _NG // _GA - 1, phase_a, None)

    def input_spectra(rows, dst):
        z = dft(rows)
        for h, t in enumerate(z):
            for b, (re, im) in enumerate(t):
                if b:
                    re, im = re + t[b - 1][1], im - t[b - 1][0]
                for p, val in enumerate((re + im, im, re)):
                    dst[(h * 3 + p) * _PLANE + b] = val
        return z

    def w_row(c, r):
        return jnp.concatenate(
            [pltpu.bitcast(arena[c, pl.ds(_ROW_W + q * _WQ + 2 * r, 2)].reshape(16, _T), f32)
             for q in range(2)], axis=1)

    def inverse(rows):
        return _dot(jnp.concatenate(rows, axis=0), inv_v[...])

    def routed_tokens():
        return _L - 1 - (pltpu.bitcast(key_v[2], i32) & (_L - 1))

    with jax.named_scope("topk"):
        for n in range(2, _NF):
            for cp in hidden_copies(n):
                cp.start()
        token = routed_tokens()
        picked = []

        def gather(u):
            tokens = range(u * _C // _GA, (u + 1) * _C // _GA)
            blocks = jnp.concatenate(
                [pltpu.bitcast(jnp.concatenate(
                    [arena[g // _GC, _ROW_X + (g % _GC) * _NB + (token[t, 0] >> 7)]
                     for g in range(_NG)], axis=0), bf16) for t in tokens], axis=1)
            pick = jnp.concatenate(
                [jnp.where((row == t) & ((token & (_T - 1)) == lane), 2.0, 0.0) for t in tokens],
                axis=1).astype(bf16)
            picked.append(_dot_nt(pick, blocks))

        filter_step(_NG // _GA - 1, token[0, 0] >> 11, gather if _MERGE else lambda u: None)
        for u in range(0 if _MERGE else _GA):
            gather(u)
        x_sel = sum(picked[1:], picked[0])
        for n in range(_NO):
            sel_v[n] = x_sel[:, n * _OCH:(n + 1) * _OCH]
        x_sel = jnp.concatenate([x_sel, jnp.zeros((8, _KT * _T - _D), f32)], axis=1)
        for n in range(_KT):
            arena[0, _ROW_SEL + n] = pltpu.bitcast(
                jnp.concatenate([x_sel[:, n * _T:(n + 1) * _T]] * 2, axis=0).astype(bf16), i32)
        input_spectra([arena[0, _ROW_X + r] for r in range(_R)], spec_a)
        for u in range(_GA):
            spread(_NG // _GA - 1, u, _GA + u)
        filter_spectra(_NG - 3 * _GA // 2,
                       [k_v[u, j] for u in range(_GA // 2, 2 * _GA) for j in range(_NB)])

    def hidden_jobs(c):
        width = _F // (_NCH - _NO)
        gate = []

        def project(n):
            cols = pl.ds(_aligned(c * width + n // 2 * _T, _T), _T)
            x_sel = jnp.concatenate(
                [pltpu.bitcast(arena[c >> 8, _ROW_SEL + r], bf16) for r in range(_KT)], axis=1)
            gate.append(_rnd(_dot(x_sel[:, :_D], pltpu.bitcast((wu_v if n % 2 else wg_v)[:, cols], bf16))[:8]))
            if n % 2:
                hid_v[:, cols] = (_rnd(_silu(gate[-2])) * gate[-1]).astype(bf16)

        return [(40 * n, lambda n=n: project(n)) for n in range(2 * width // _T)]

    def hidden_at(t, zero=0):
        return pl.ds(_aligned(_D + 8 * (t // _NB + zero), 8), 8), pl.ds((t % _NB) * _T, _T)

    def finish(n):
        for k in range(0, _OCH // 16 * _NB, 2):
            c, r = n * (_OCH // (16 * _GC)) + k // _R, k % _R
            out = []
            for d in range(2):
                h = pltpu.bitcast(arena[c, _ROW_X + r + d], bf16).astype(f32)
                out.append(xc_v[k % _NB + d, n * (_OCH // 16) + k // _NB]
                           + s_v[c, pl.ds(16 * (r + d), 16), :] * (h + h * jnp.tanh(h)))
            o_v[pl.ds(_aligned(n * _OCH + 16 * (k // _NB), 16), 16), pl.ds((k % _NB) * _T, 2 * _T)] = (
                jnp.concatenate(out, axis=1).astype(bf16))
            yield k + 1

    def down_jobs(n, hid):
        rank = (pltpu.bitcast(key_v[2], i32) - (1 << 28)) >> 11
        score = pltpu.bitcast(jnp.where(rank >= 0x8000, rank - 0x8000, ~rank) << 16, f32)
        y = _rnd(_dot_nt(jnp.concatenate(hid, axis=1), pltpu.bitcast(wd_v[n], bf16)))
        y = 0.5 * (sel_v[n] + _rnd(y * _rnd(jax.nn.sigmoid(score))[:, :_OCH]))
        col = jnp.concatenate([y, jnp.zeros((_T - _C, _OCH), f32)], axis=0).T
        col = pltpu.bitcast(col.astype(bf16), i32)
        token = routed_tokens()

        def scatter(t):
            hit = ((token & (_T - 1)) == lane)[t:t + 1]
            new = jnp.broadcast_to(col[:, t:t + 1], (_OCH // 2, _T))
            where = [(n * (_OCH // (16 * _GC)) + g // _GC,
                      _ROW_X + (g % _GC) * _NB + (token[t, 0] >> 7)) for g in range(_OCH // 16)]
            old = [arena[at] for at in where]
            for g, at in enumerate(where):
                arena[at] = jnp.where(hit, new[8 * g:8 * g + 8], old[g])

        return [lambda t=t: scatter(t) for t in range(_C)]

    def first_output_jobs(c):
        hid, scatter = [], []

        def read():
            hid.extend(pltpu.bitcast(arena[c >> 8, _ROW_W + t], bf16)[:8]
                       for t in range(len(hid), len(hid) + 4))

        return ([(48 * k, read) for k in range(_F // (4 * _T))]
                + [(_G2 - 1, lambda: scatter.extend(down_jobs(0, hid)))]
                + [(_G2 + _S0 + _S1 * t, lambda t=t: scatter[t]()) for t in range(_C)])

    def output_jobs(c):
        n = c - (_NCH - _NO)
        hid = [o_v[hidden_at(t, c >> 8)] for t in range(4)]
        for k in finish(n - 1):
            if k % 12 == 11:
                hid += [o_v[hidden_at(t, c >> 8)] for t in range(len(hid), len(hid) + 4)]
        jobs = [(_S0 + _S1 * t, job) for t, job in enumerate(down_jobs(n, hid))]
        pl.when(n >= _HOLD)(lambda: out_copy(n - 1).start())
        return jobs

    def conv_step(c, cur, nxt, ffn_jobs, delay, pace):
        c_next, c_prev = jnp.minimum(c + 1, _NCH - 1), jnp.maximum(c - 1, 0)
        zero = c >> 8
        fwd_rows, inv_rows, results = [], [], []

        def transform():
            y = inverse(inv_rows)
            s_v[c_prev] = y
            results.extend((y, input_spectra(fwd_rows, nxt)))

        def drain(r):
            y, z = results
            arena[c, _ROW_SEL - 1] = pltpu.bitcast(
                y[8 * r:8 * r + 8] + z[2 * (r // _R) + 1][r % _R // 2][r // 8 % 2], i32)

        jobs = sorted(
            ffn_jobs(c)
            + [(delay + 16 * r, lambda r=r: inv_rows.append(w_row(c_prev, r))) for r in range(_R)]
            + [(delay + 16 * r, lambda r=r: fwd_rows.append(arena[c_next, _ROW_X + r]))
               for r in range(_R)]
            + [(delay + 16 * _R, transform)]
            + [(delay + _LAG + 8 * r, lambda r=r: drain(r)) for r in range(2 * _R - 17, 2 * _R, 8)],
            key=lambda job: job[0])

        def run_jobs(done):
            while jobs and done * (delay + 16 * _R) >= (jobs[0][0] - _LEAD) * pace * 18 * _GC:
                jobs.pop(0)[1]()

        run_jobs(0)
        for h in range(2 * _GC):
            for part in range(3):
                for plane in range(3):
                    kf = lambda b: kf_v[c * 2 * _GC + h + (zero >> part), plane * _PLANE + b]
                    uf = lambda b: cur[(zero >> part) + (h * 3 + plane) * _PLANE + b]
                    base = [pltpu.bitcast(arena[c + zero, _ROW_P + plane * 8 + m], f32)
                            for m in range(8) if part and plane]
                    k, u, out = [], [], []
                    for m in range(8):
                        if part == 0:
                            k.append(kf(2 * m))
                            u.append(uf(2 * m) + uf(2 * m + 1))
                        elif part == 1:
                            k.append(kf(2 * m) - kf(2 * m - 1) if m else kf(0))
                            u.append(uf(2 * m + 1))
                        else:
                            k.append(kf(2 * m) - kf(2 * m + 1))
                            u.append(uf(2 * m))
                        y = k[0] * u[m]
                        for j in range(1, m + 1):
                            y = y + k[j] * u[m - j]
                        if plane:
                            y = shared[m] - y if plane == 1 else shared[m] + y
                        out.append(y)
                        if part == 0 or plane == 0:
                            arena[c, _ROW_P + plane * 8 + m] = pltpu.bitcast(y, i32)
                        else:
                            r = ((h // 2) * _NB + 2 * m + part - 1) * 2 + h % 2
                            arena[c, _ROW_W + (plane - 1) * _WQ + r] = pltpu.bitcast(base[m] - y, i32)
                    if plane == 0:
                        shared = out
                    run_jobs((h * 3 + part) * 3 + plane + 1)
        run_jobs(np.inf)

    def phase_c(part, carry):
        for cp in hidden_copies(part):
            cp.wait()

        @pl.when(part == _WD_STEP)
        def _():
            for n in range(_NO):
                down_copy(n).start()

        def pair(i, carry):
            conv_step(2 * i, spec_a, spec_b, hidden_jobs, 240, _PACE)
            conv_step(2 * i + 1, spec_b, spec_a, hidden_jobs, 240, _PACE)

        pairs = (_NCH - _NO) // (2 * _NF)
        lax.fori_loop(part * pairs, (part + 1) * pairs, pair, None)

    def phase_d(n, carry):
        down_copy(n).wait()

        @pl.when(n == _HOLD + _HALF)
        def _():
            for k in range(_HOLD - 1):
                out_copy(k).start()

        c = n + _NCH - _NO
        lax.cond(c & 1 == 0, lambda: conv_step(c, spec_a, spec_b, output_jobs, _G1, _PACE1),
                 lambda: conv_step(c, spec_b, spec_a, output_jobs, _G1, _PACE1))

    with jax.named_scope("C"):
        lax.fori_loop(0, _NF, phase_c, None)
    with jax.named_scope("D"):
        for t in range(_F // _T):
            tile = hid_v[:, t * _T:(t + 1) * _T]
            o_v[hidden_at(t)] = tile
            arena[0, _ROW_W + t] = pltpu.bitcast(jnp.concatenate([tile] * 2, axis=0), i32)
        down_copy(0).wait()
        conv_step(_NCH - _NO + (routed_tokens()[0, 0] >> 11), spec_a, spec_b, first_output_jobs,
                  _G2, _PACE2)
        lax.fori_loop(1, _NO, phase_d, None)
    with jax.named_scope("tail"):
        s_v[_NCH - 1] = inverse([w_row(_NCH - 1, r) for r in range(_R)])
        for k in finish(_NO - 1):
            if k % _R == _R - 1:
                rows = pl.ds((_NO - 1) * _OCH + k // _R * 16 * _GC, 16 * _GC)
                start("out", o_v.at[rows], o_hbm.at[rows])
    with jax.named_scope("end"):
        for n in range(_NO - 1):
            out_copy(n).wait()
        wait("out")


@jax.jit
def pallas_recurrent_scan__ssm_conv_s4__moe_arch_mod__prompt_kernel(
    A_u: jax.Array,
    A_A_re: jax.Array,
    A_A_im: jax.Array,
    A_B_re: jax.Array,
    A_B_im: jax.Array,
    A_C_re: jax.Array,
    A_C_im: jax.Array,
    A_log_dt: jax.Array,
    A_Dskip: jax.Array,
    B_x: jax.Array,
    B_w_r: jax.Array,
    B_w_gate: jax.Array,
    B_w_up: jax.Array,
    B_w_down: jax.Array,
):
    del B_x
    assert A_u.shape == (1, _L, _D) and A_A_re.shape == (_D, _N) and B_w_gate.shape == (_D, _F)
    assert A_u.dtype == bf16 and A_A_re.dtype == bf16
    hbm = pl.BlockSpec(memory_space=pl.ANY)
    vmem = pltpu.VMEM
    out = pl.pallas_call(
        _kernel,
        out_shape=jax.ShapeDtypeStruct((_D, _L), bf16),
        in_specs=[hbm] * 14,
        out_specs=hbm,
        scratch_shapes=[
            vmem((_D // 2, _L), i32), vmem((_D + 32, _L), bf16),
            vmem((6, _D // 2, _N), i32), vmem((_D,), bf16), vmem((_D,), bf16), vmem((_D,), bf16),
            vmem((_D // 2, _F), i32), vmem((_D // 2, _F), i32), vmem((_NO, _OCH // 2, _F), i32),
            vmem((_T // 2, 2 * _T), i32), vmem((2 * _T, _T), f32),
            vmem((_D // 2, _T), i32), vmem((_NG, 8, _T), i32),
            vmem((_NCH, _ROWS, 8, _T), i32), vmem((_NCH, 16 * _R, _T), f32),
            vmem((_D // 2, _T), i32), vmem((_GA, 2, 4, 8, _N), f32), vmem((_GA, len(_TAPS), 8, _T), i32),
            vmem((2 * _GA, _NB, 8, _T), i32),
            vmem((_NB, _NG, 16, _T), f32), vmem((3, _NB, 8, _T), f32), vmem((3, 8, _T), f32),
            vmem((_NO, 8, _OCH), f32), vmem((8, _F), bf16),
            *[vmem((2 * _GC * 3 * _PLANE, 8, _T), f32)] * 2, vmem((2 * _NG, 3 * _PLANE, 8, _T), f32),
            pltpu.SemaphoreType.DMA((5,)), pltpu.SemaphoreType.DMA((_NF + _NO,)),
            pltpu.SemaphoreType.DMA(()),
        ],
        compiler_params=pltpu.CompilerParams(vmem_limit_bytes=100 * 2**20, flags=_FLAGS),
    )(A_u.reshape(_L, _D).T, A_A_re, A_A_im, A_B_re, A_B_im, A_C_re, A_C_im, A_log_dt, A_Dskip,
      B_w_r, B_w_gate, B_w_up, B_w_down.T, _FWD)
    return out.T.reshape(1, _L, _D)
```

```python
import jax
import jax.numpy as jnp
import numpy as np
from jax import lax
import jax.experimental.pallas as pl
import jax.experimental.pallas.tpu as pltpu

_D, _L, _N, _F, _C = 576, 2048, 128, 4608, 8
_T = 128
_NB = _L // _T
_EPS = 1e-5
_GA = 4
_GC = 2
_NG = _D // 16
_NCH = _NG // _GC
_R = _GC * _NB
_ROW_X, _ROW_W, _ROW_P, _ROWS = 0, _R, 5 * _R + 8, 5 * _R + 8 + 24
_PLANE, _WQ = _NB + 1, 2 * _R + 1
_ROW_SEL = 5 * _R + 3
_MERGE, _HOLD, _PRIO, _G2, _PACE2 = 1, 3, 0, 432, 0.87
_FLAGS, _HALF, _FENCE, _INTW, _GD = None, 0, (0, 1, 2), 1, 40
_FORCE = 1
_KT = -(-_D // _T)
_NO, _OCH = 6, _D // 6
_NF = 3
_FCH = _F // _NF
_LN_STEP = 4
_WD_STEP = 1
_PACE, _PACE1, _LEAD, _LAG, _G1, _S0, _S1 = 0.87, 0.8, 32, 140, 32, 560, 14

f32, bf16, i32 = jnp.float32, jnp.bfloat16, jnp.int32


def _dft_constants():
    theta = (np.pi / 2 + 2 * np.pi * np.arange(_T)) / _T
    ang = np.arange(_T)[:, None] * theta[None, :]
    c, s = np.cos(ang), np.sin(ang)
    fwd = np.concatenate([c, s], axis=1)
    bits = fwd.astype(bf16).view(np.uint16).astype(np.uint32)
    words = (bits[0::2] | bits[1::2] << 16).view(np.int32)
    return words


_FWD = _dft_constants()


def _lag_step(j):
    return max(1, (1 << (j * _T).bit_length()) >> 8)


def _round_lag(p, st):
    if st == 1:
        return p
    return (p + (st // 2 - 1) + ((p >> (st.bit_length() - 1)) & 1)) & ~(st - 1)


assert np.array_equal(
    np.concatenate([j * _T + _round_lag(np.arange(_T), _lag_step(j)) for j in range(_NB)]),
    np.arange(_L).astype(bf16).astype(np.int64))

_PAIRS = (((0, 1), (0, 5)), ((0, 2), (0, 6)), ((0, 3), (0, 7)), ((0, 4), (0, 8)), ((1, 2), (1, 6)),
          ((1, 4), (1, 8)), ((2, 4), (2, 8)), ((3, 4), (3, 8)), ((4, 8), (5, 8)), ((6, 8), (7, 8)))
_TAPS = [k for pair in _PAIRS for k in pair]


def _aligned(i, n):
    return i if isinstance(i, int) else pl.multiple_of(i, n)


def _cmul(a, b):
    return a[0] * b[0] - a[1] * b[1], a[0] * b[1] + a[1] * b[0]


def _csq(a):
    return a[0] * a[0] - a[1] * a[1], (a[0] + a[0]) * a[1]


def _silu(x):
    h = 0.5 * x
    return h + h * jnp.tanh(h)


def _rnd(x):
    return x.astype(bf16).astype(f32)


def _dot(a, b):
    return jnp.dot(a, b, preferred_element_type=f32)


def _dot_nt(a, b):
    return lax.dot_general(a, b, (((1,), (1,)), ((), ())), preferred_element_type=f32)


def _column(v):
    return pltpu.bitcast(jnp.broadcast_to(v, (_T, v.shape[1])).T.astype(bf16), i32)


def _even_odd(x):
    return pltpu.bitcast(x << 16, f32), pltpu.bitcast(x & -65536, f32)


def _interleave(even, odd):
    even, odd = [pltpu.bitcast(x, i32) + 0x8000 for x in (even, odd)]
    return lax.shift_right_logical(even, 16) | (odd & -65536)


def _words(x):
    y = jnp.concatenate([x[:8], x[8:]], axis=1).astype(bf16)
    return pltpu.bitcast(jnp.concatenate([y[:, :_T], y[:, _T:]], axis=0), i32)


def _modes(dt, ar, ai, br, bi, cr, ci):
    zr, zi = dt * ar, dt * ai
    mag = jnp.exp(zr)
    return _cmul((cr, ci), (dt * br, dt * bi)) + (mag * jnp.cos(zi), mag * jnp.sin(zi))


def _seeds(w, a1):
    a = {1: a1}
    for n in range(9):
        a[2 << n] = _csq(a[1 << n])
    row = lax.broadcasted_iota(i32, (8, _N), 0)

    def mix(z0, z1):
        rolled = [pltpu.roll(x, 4, 0) for x in z1]
        return ([jnp.where(row < 4, x, y) for x, y in zip(z0, rolled)],
                [jnp.where(row < 4, y, x) for x, y in zip(z0, rolled)])

    def dup(z):
        return [[jnp.take_along_axis(x, (row & 3) + 4 * q, axis=0, mode="promise_in_bounds")
                 for x in z] for q in range(2)]

    wa = _cmul(w, a[1])
    return zip(mix((1.0, 0.0), a[128]), dup(a[8]), dup(a[32]),
               mix(wa, _cmul(wa, a[4])), dup(a[1]), dup(a[256]),
               mix(_cmul(a[256], a[4]), a[512]), dup(a[512]))


def _vandermonde(e0, m8, m32, g0, m1, m256, m_top, m512):
    e = [e0]
    for s in range(1, 16):
        e.append(_cmul(e[s - 1], m8) if s < 4 else _cmul(e[s - 4], m32))
    g = [g0]
    for _ in range(3):
        g.append(_cmul(g[-1], m1))
    g += [_cmul(g[1], m256), _cmul(g[3], m256)]
    g += [_cmul(g[3], m512), _cmul(g[5], m512)]
    g.append(_cmul(g[7], m_top))
    g.append(_cmul(g[8], m512))
    re, im = [_dot_nt(jnp.concatenate([z[p] for z in g], axis=0),
                      jnp.concatenate([z[p] for z in e], axis=0)) for p in range(2)]
    return re - im


def _unmix(lo, hi):
    row = lax.broadcasted_iota(i32, (8, _T), 0)
    out = []
    for m in range(len(_PAIRS)):
        x, y = lo[8 * m:8 * m + 8], hi[8 * m:8 * m + 8]
        out += [jnp.where(row < 4, x, y), pltpu.roll(jnp.where(row < 4, y, x), 4, 0)]
    return out


def _lag_blocks(tap, lag0):
    lane = lax.broadcasted_iota(i32, (8, _T), 1)
    row = lax.broadcasted_iota(i32, (8, _T), 0)
    for h in range(2):
        def take(big, r, fine):
            s = ((_T * h + fine) >> 3) & 31
            return jnp.take_along_axis(tap(_TAPS.index((big, r))),
                                       ((s & 15) << 3) + (row ^ ((s >> 4) << 2)),
                                       axis=1, mode="promise_in_bounds")

        top = [take(big, 8, _round_lag(lane, 8) - 8) for big in range(_NB // 2)]
        for big, blk in enumerate(top):
            st = _lag_step(2 * big + h)
            lag = _round_lag(lane, st)
            if h == 0:
                blk = jnp.where(lag == 0, top[big - 1] if big else lag0, blk)
            for r in range(st, 8, st):
                blk = jnp.where((lag & 7) == r, take(big, r, lane), blk)
            yield 2 * big + h, blk


def _kernel(x_hbm, ar_hbm, ai_hbm, br_hbm, bi_hbm, cr_hbm, ci_hbm, ldt_hbm, dsk_hbm, wr_hbm,
            wg_hbm, wu_hbm, wd_hbm, fwd_hbm, o_hbm,
            x_v, o_v, par_v, ldt_v, dsk_v, wr_v, wg_v, wu_v, wd_v, fwd_v, inv_v,
            skip_v, k0_v, arena, s_v, dt_v, mode_v, tap_v, k_v, xc_v, stat_v, key_v, sel_v, hid_v,
            spec_a, spec_b, kf_v, sem, w_sem, o_sem):
    row = lax.broadcasted_iota(i32, (8, _T), 0)
    lane = lax.broadcasted_iota(i32, (8, _T), 1)
    groups = {}

    def start(name, src, dst):
        slot, pairs = groups.setdefault(name, (len(groups), []))
        pairs.append((src, dst))
        pltpu.make_async_copy(src, dst, sem.at[slot]).start()

    def wait(name):
        slot, pairs = groups[name]
        for src, dst in pairs:
            pltpu.make_async_copy(src, dst, sem.at[slot]).wait()

    def hidden_copies(n):
        cols = pl.ds(_aligned(n * _FCH, _FCH), _FCH)
        return [pltpu.make_async_copy(w.bitcast(i32).at[:, cols], v.at[:, cols], w_sem.at[n])
                for w, v in ((wg_hbm, wg_v), (wu_hbm, wu_v))]

    def chunk_rows(n):
        return pl.ds(_aligned(n * _OCH, 32), _OCH)

    def down_copy(n):
        rows = pl.ds(_aligned(n * (_OCH // 2), 16), _OCH // 2)
        return pltpu.make_async_copy(wd_hbm.bitcast(i32).at[rows], wd_v.at[n], w_sem.at[_NF + n])

    def out_copy(n):
        return pltpu.make_async_copy(o_v.at[chunk_rows(n)], o_hbm.at[chunk_rows(n)], o_sem)

    def start_parameters(part, rows):
        for n, src in enumerate((ar_hbm, ai_hbm, br_hbm, bi_hbm, cr_hbm, ci_hbm)):
            start(part, src.bitcast(i32).at[rows], par_v.at[n, rows])

    with jax.named_scope("init"):
        start("vectors", ldt_hbm, ldt_v)
        start("vectors", dsk_hbm, dsk_v)
        start_parameters(0, pl.ds(0, 8 * _GA))
        start_parameters(2, pl.ds(8 * _GA, 8 * _GA))
        start(2, fwd_hbm, fwd_v)
        arena[0, _ROW_W:_ROW_P] = jnp.zeros((_ROW_P - _ROW_W, 8, _T), i32)
        tap_v[...] = jnp.zeros(tap_v.shape, i32)
        k_v[:_GA] = jnp.zeros((_GA, _NB, 8, _T), i32)
        key_v[...] = jnp.zeros(key_v.shape, f32)
        wait("vectors")
        start_parameters(1, pl.ds(16 * _GA, _D // 2 - 16 * _GA))
        start("x", x_hbm.bitcast(i32), x_v)
        start("x", wr_hbm, wr_v)
        dt = jnp.exp(ldt_v[...].astype(f32)).reshape(1, _D)
        dt_v[:_T // 2] = _column(dt[:, :_T])
        wait(0)

    def compact(ref, k, h):
        out = ref[k, 8 * h]
        for s in range(1, 8):
            out = jnp.where(row == s, ref[k, 8 * h + s], out)
        return out

    def layer_norm():
        wait("x")
        for cp in hidden_copies(1):
            cp.start()

        def moments(b, carry):
            cols = pl.ds(_aligned(b * _T, _T), _T)
            pivot = jnp.broadcast_to(_even_odd(x_v[:8, cols])[0][:1], (8, _T))
            s1, s2 = [None] * 2, [None] * 2
            for g in range(_NG):
                words = x_v[pl.ds(8 * g, 8), cols]
                x = pltpu.bitcast(words, bf16).astype(f32)
                xc_v[b, g] = x
                for h in range(2):
                    d = x[8 * h:8 * h + 8] - pivot
                    s1[h] = s1[h] + d if g else d
                    s2[h] = s2[h] + d * d if g else d * d
            for k, s in enumerate((s1, s2)):
                stat_v[k, b] = jnp.broadcast_to(jnp.sum(s[0] + s[1], axis=0, keepdims=True), (8, _T))
            stat_v[2, b] = pivot
            return carry

        lax.fori_loop(0, _NB, moments, 0, unroll=4)
        for h in range(_NB // 8):
            m1, m2, pivot = compact(stat_v, 0, h) / _D, compact(stat_v, 1, h) / _D, compact(stat_v, 2, h)
            var = jnp.maximum(m2 - m1 * m1, 0.0)
            shift = _rnd(pivot + m1)
            gain = 0.5 / _rnd(jnp.sqrt(_rnd(_rnd(var) + _rnd(jnp.full_like(var, _EPS)))))
            for s in range(8):
                stat_v[0, 8 * h + s] = jnp.broadcast_to(shift[s:s + 1], (8, _T))
                stat_v[1, 8 * h + s] = jnp.broadcast_to(gain[s:s + 1], (8, _T))
        inv_v[...] = pltpu.bitcast(fwd_v[...], bf16).astype(f32).T * (2 / _T)
        wr = jnp.broadcast_to(wr_v[...].astype(f32).reshape(1, _D), (8, _D)).astype(bf16)

        def scale(b, carry):
            shift, gain = stat_v[0, b], stat_v[1, b]
            if _INTW:
                xn = [_interleave(*[(xc_v[b, g, pl.ds(h, 8, stride=2), :] - shift) * gain
                                    for h in range(2)]) for g in range(_NG)]
            else:
                xn = [_words((xc_v[b, g] - shift[:1]) * gain[:1]) for g in range(_NG)]
            for g in range(_NG):
                arena[g // _GC, _ROW_X + (g % _GC) * _NB + b] = xn[g]
            stat_v[2, b] = _dot(wr, pltpu.bitcast(jnp.concatenate(xn, axis=0), bf16))
            return carry

        lax.fori_loop(0, _NB, scale, 0, unroll=16)
        for h in range(_NB // 8):
            bits = pltpu.bitcast(_rnd(2.0 * compact(stat_v, 2, h)) + 0.0, i32) >> 16
            rank = jnp.where(bits < 0, ~bits, bits + 0x8000)
            token = (8 * h + row) * _T + lane
            key_v[h] = pltpu.bitcast((1 << 28) + rank * _L + (_L - 1 - token), f32)

    def pop_best(c):
        best = jnp.max(jnp.max(jnp.maximum(key_v[0], key_v[1]), axis=0, keepdims=True),
                       axis=1, keepdims=True)
        key_v[2] = jnp.where(row == c, best, key_v[2])
        for h in range(2):
            key_v[h] = jnp.where(key_v[h] == best, 0.0, key_v[h])

    def modes(step):
        for u in range(_GA):
            grp = step * _GA + u
            rows = pl.ds(_aligned(grp * 8, 8), 8)
            par = [_even_odd(dt_v[rows, :])] + [_even_odd(par_v[n, rows, :]) for n in range(6)]
            k0 = []
            for h, skip in enumerate(_even_odd(skip_v[rows, :])):
                z = _modes(*[p[h] for p in par])
                for n in range(4):
                    mode_v[u, h, n] = z[n]
                k0.append(skip + jnp.sum(z[0], axis=1, keepdims=True))
            k0_v[grp] = _interleave(*k0)

    def dft(rows):
        z = _dot(jnp.concatenate([pltpu.bitcast(r, bf16) for r in rows], axis=0),
                 pltpu.bitcast(fwd_v[...], bf16))
        n = min(len(rows), _NB)
        return [[(z[o:o + 8, :_T], z[o:o + 8, _T:])
                 for o in range((h // 2) * 16 * n + 8 * (h % 2), (h // 2 + 1) * 16 * n, 16)]
                for h in range(2 * len(rows) // n)]

    def spread(step, u, slot):
        for j, blk in _lag_blocks(lambda n: tap_v[u, n], k0_v[step * _GA + u]):
            k_v[slot, j] = blk

    def filter_spectra(grp, rows):
        z = dft(rows)
        for h, blocks in enumerate(z):
            for j, (re, im) in enumerate(blocks):
                for p, val in enumerate((re, re + im, im - re)):
                    kf_v[2 * grp + h, p * _PLANE + j] = val
        return z

    def filter_step(i, zero, extra=lambda u: None):
        for u in range(_GA):
            if u % (_GA // 2) == 0:
                old = (u + _GA // 2) % _GA
                filter_spectra(jnp.maximum(i - (1 if u else 2), 0) * _GA + old,
                               [k_v[old + k + zero, j] for k in range(_GA // 2) for j in range(_NB)])
            spread(jnp.maximum(i - 1, 0), u, u)
            v = [[_vandermonde(*seeds) for seeds in _seeds(
                (mode_v[u, h, 0], mode_v[u, h, 1]), (mode_v[u, h, 2], mode_v[u, h, 3]))]
                 for h in range(2)]
            for n, tap in enumerate(_unmix(*map(_interleave, *v))):
                tap_v[u, n] = tap
            extra(u)

    def phase_a(i, carry):
        @pl.when(i == 1)
        def _():
            wait(1)
            for cp in hidden_copies(0):
                cp.start()

        pl.when(i == _LN_STEP)(layer_norm)
        for c in range(2):
            pop_best(2 * (i - _LN_STEP) + c)
        filter_step(i, i >> 8)
        modes(i + 1)

    with jax.named_scope("A"):
        skip_v[...] = _column(dsk_v[...].astype(f32).reshape(1, _D))
        dt_v[_T // 2:] = _column(dt[:, _T:])
        modes(0)
        wait(2)
        lax.fori_loop(0, _NG // _GA - 1, phase_a, None)

    def input_spectra(rows, dst):
        z = dft(rows)
        for h, t in enumerate(z):
            for b, (re, im) in enumerate(t):
                if b:
                    re, im = re + t[b - 1][1], im - t[b - 1][0]
                for p, val in enumerate((re + im, im, re)):
                    dst[(h * 3 + p) * _PLANE + b] = val
        return z

    def w_row(c, r):
        return jnp.concatenate(
            [pltpu.bitcast(arena[c, pl.ds(_ROW_W + q * _WQ + 2 * r, 2)].reshape(16, _T), f32)
             for q in range(2)], axis=1)

    def inverse(rows):
        return _dot(jnp.concatenate(rows, axis=0), inv_v[...])

    def routed_tokens():
        return _L - 1 - (pltpu.bitcast(key_v[2], i32) & (_L - 1))

    with jax.named_scope("topk"):
        for n in range(2, _NF):
            for cp in hidden_copies(n):
                cp.start()
        token = routed_tokens()
        picked = []

        def gather(u):
            tokens = range(u * _C // _GA, (u + 1) * _C // _GA)
            blocks = jnp.concatenate(
                [pltpu.bitcast(jnp.concatenate(
                    [arena[g // _GC, _ROW_X + (g % _GC) * _NB + (token[t, 0] >> 7)]
                     for g in range(_NG)], axis=0), bf16) for t in tokens], axis=1)
            pick = jnp.concatenate(
                [jnp.where((row == t) & ((token & (_T - 1)) == lane), 2.0, 0.0) for t in tokens],
                axis=1).astype(bf16)
            picked.append(_dot_nt(pick, blocks))

        filter_step(_NG // _GA - 1, token[0, 0] >> 11, gather if _MERGE else lambda u: None)
        for u in range(0 if _MERGE else _GA):
            gather(u)
        x_sel = sum(picked[1:], picked[0])
        for n in range(_NO):
            sel_v[n] = x_sel[:, n * _OCH:(n + 1) * _OCH]
        x_sel = jnp.concatenate([x_sel, jnp.zeros((8, _KT * _T - _D), f32)], axis=1)
        for n in range(_KT):
            arena[0, _ROW_SEL + n] = pltpu.bitcast(
                jnp.concatenate([x_sel[:, n * _T:(n + 1) * _T]] * 2, axis=0).astype(bf16), i32)
        input_spectra([arena[0, _ROW_X + r] for r in range(_R)], spec_a)
        for u in range(_GA):
            spread(_NG // _GA - 1, u, _GA + u)
        filter_spectra(_NG - 3 * _GA // 2,
                       [k_v[u, j] for u in range(_GA // 2, 2 * _GA) for j in range(_NB)])

    def hidden_jobs(c):
        width = _F // (_NCH - _NO)
        gate = []

        def project(n):
            cols = pl.ds(_aligned(c * width + n // 2 * _T, _T), _T)
            x_sel = jnp.concatenate(
                [pltpu.bitcast(arena[c >> 8, _ROW_SEL + r], bf16) for r in range(_KT)], axis=1)
            gate.append(_rnd(_dot(x_sel[:, :_D], pltpu.bitcast((wu_v if n % 2 else wg_v)[:, cols], bf16))[:8]))
            if n % 2:
                hid_v[:, cols] = (_rnd(_silu(gate[-2])) * gate[-1]).astype(bf16)

        return [(_GD * n, lambda n=n: project(n)) for n in range(2 * width // _T)]

    def hidden_at(t, zero=0):
        return pl.ds(_aligned(_D + 8 * (t // _NB + zero), 8), 8), pl.ds((t % _NB) * _T, _T)

    def finish(n):
        for k in range(0, _OCH // 16 * _NB, 2):
            c, r = n * (_OCH // (16 * _GC)) + k // _R, k % _R
            out = []
            for d in range(2):
                h = pltpu.bitcast(arena[c, _ROW_X + r + d], bf16).astype(f32)
                out.append(xc_v[k % _NB + d, n * (_OCH // 16) + k // _NB]
                           + s_v[c, pl.ds(16 * (r + d), 16), :] * (h + h * jnp.tanh(h)))
            o_v[pl.ds(_aligned(n * _OCH + 16 * (k // _NB), 16), 16), pl.ds((k % _NB) * _T, 2 * _T)] = (
                jnp.concatenate(out, axis=1).astype(bf16))
            yield k + 1

    def down_jobs(n, hid):
        rank = (pltpu.bitcast(key_v[2], i32) - (1 << 28)) >> 11
        score = pltpu.bitcast(jnp.where(rank >= 0x8000, rank - 0x8000, ~rank) << 16, f32)
        y = _rnd(_dot_nt(jnp.concatenate(hid, axis=1), pltpu.bitcast(wd_v[n], bf16)))
        y = 0.5 * (sel_v[n] + _rnd(y * _rnd(jax.nn.sigmoid(score))[:, :_OCH]))
        col = jnp.concatenate([y, jnp.zeros((_T - _C, _OCH), f32)], axis=0).T
        col = pltpu.bitcast(col.astype(bf16), i32)
        token = routed_tokens()

        def scatter(t):
            hit = ((token & (_T - 1)) == lane)[t:t + 1]
            new = jnp.broadcast_to(col[:, t:t + 1], (_OCH // 2, _T))
            where = [(n * (_OCH // (16 * _GC)) + g // _GC,
                      _ROW_X + (g % _GC) * _NB + (token[t, 0] >> 7)) for g in range(_OCH // 16)]
            old = [arena[at] for at in where]
            for g, at in enumerate(where):
                arena[at] = jnp.where(hit, new[8 * g:8 * g + 8], old[g])

        return [lambda t=t: scatter(t) for t in range(_C)]

    def first_output_jobs(c):
        hid, scatter = [], []

        def read():
            hid.extend(pltpu.bitcast(arena[c >> 8, _ROW_W + t], bf16)[:8]
                       for t in range(len(hid), len(hid) + 4))

        return ([(48 * k, read) for k in range(_F // (4 * _T))]
                + [(_G2 - 1, lambda: scatter.extend(down_jobs(0, hid)))]
                + [(_G2 + _S0 + _S1 * t, lambda t=t: scatter[t]()) for t in range(_C)])

    def output_jobs(c):
        n = c - (_NCH - _NO)
        hid = [o_v[hidden_at(t, c >> 8)] for t in range(4)]
        for k in finish(n - 1):
            if k == _OCH // 16 * _NB - 1:
                pl.when(n >= _HOLD)(lambda: out_copy(n - 1).start())
                if _FORCE:
                    o_v[hidden_at(_F // _T, c >> 9)] = hid[0]
            if k % 12 == 11:
                hid += [o_v[hidden_at(t, c >> 8)] for t in range(len(hid), len(hid) + 4)]
        return [(_S0 + _S1 * t, job) for t, job in enumerate(down_jobs(n, hid))]

    def conv_step(c, cur, nxt, ffn_jobs, delay, pace, first=False):
        c_next, c_prev = jnp.minimum(c + 1, _NCH - 1), jnp.maximum(c - 1, 0)
        zero = c >> 8
        fwd_rows, inv_rows, results = [], [], []

        def transform():
            if first:
                y = filter_spectra(_NG - _GC, inv_rows)
            else:
                y = inverse(inv_rows)
                s_v[c_prev] = y
            results.extend((y, input_spectra(fwd_rows, nxt)))

        def drain(r):
            y, z = results
            arena[c, _ROW_SEL - 1] = pltpu.bitcast(
                (y[-1][r % _R // 2][r // 8 % 2] if first else y[8 * r:8 * r + 8]) + z[2 * (r // _R) + 1][r % _R // 2][r // 8 % 2], i32)

        jobs = sorted(
            ffn_jobs(c)
            + [(delay + 16 * r, lambda r=r: inv_rows.append(arena[_NCH - 1 + zero, _ROW_W + r] if first else w_row(c_prev, r))) for r in range(_R)]
            + [(delay + 16 * r, lambda r=r: fwd_rows.append(arena[c_next, _ROW_X + r]))
               for r in range(_R)]
            + [(delay + 16 * _R, transform)]
            + [(delay + _LAG + 8 * r, lambda r=r: drain(r)) for r in range(2 * _R - 17, 2 * _R, 8)],
            key=lambda job: job[0])

        def run_jobs(done):
            while jobs and done * (delay + 16 * _R) >= (jobs[0][0] - _LEAD) * pace * 18 * _GC:
                jobs.pop(0)[1]()

        run_jobs(0)
        for h in range(2 * _GC):
            for part in range(3):
                for plane in range(3):
                    kf = lambda b: kf_v[c * 2 * _GC + h + (zero >> part), plane * _PLANE + b]
                    uf = lambda b: cur[(zero >> part) + (h * 3 + plane) * _PLANE + b]
                    base = [pltpu.bitcast(arena[c + zero, _ROW_P + plane * 8 + m], f32)
                            for m in range(8) if part and plane]
                    k, u, out = [], [], []
                    for m in range(8):
                        if part == 0:
                            k.append(kf(2 * m))
                            u.append(uf(2 * m) + uf(2 * m + 1))
                        elif part == 1:
                            k.append(kf(2 * m) - kf(2 * m - 1) if m else kf(0))
                            u.append(uf(2 * m + 1))
                        else:
                            k.append(kf(2 * m) - kf(2 * m + 1))
                            u.append(uf(2 * m))
                        y = k[0] * u[m]
                        for j in range(1, m + 1):
                            y = y + k[j] * u[m - j]
                        if plane:
                            y = shared[m] - y if plane == 1 else shared[m] + y
                        out.append(y)
                        if part == 0 or plane == 0:
                            arena[c, _ROW_P + plane * 8 + m] = pltpu.bitcast(y, i32)
                        else:
                            r = ((h // 2) * _NB + 2 * m + part - 1) * 2 + h % 2
                            arena[c, _ROW_W + (plane - 1) * _WQ + r] = pltpu.bitcast(base[m] - y, i32)
                    if plane == 0:
                        shared = out
                    if plane in _FENCE:
                        run_jobs((h * 3 + part) * 3 + plane + 1)
        run_jobs(np.inf)

    def phase_c(part, carry):
        for cp in hidden_copies(part):
            cp.wait()

        @pl.when(part == _WD_STEP)
        def _():
            for n in range(_NO):
                down_copy(n).start()

        def pair(i, carry):
            conv_step(2 * i, spec_a, spec_b, hidden_jobs, 6 * _GD, _PACE)
            conv_step(2 * i + 1, spec_b, spec_a, hidden_jobs, 6 * _GD, _PACE)

        pairs = (_NCH - _NO) // (2 * _NF)
        lax.fori_loop(part * pairs, (part + 1) * pairs, pair, None)

    def phase_d(n, carry):
        down_copy(n).wait()

        @pl.when(n == _HOLD + _HALF)
        def _():
            for k in range(_HOLD - 1):
                out_copy(k).start()

        c = n + _NCH - _NO
        lax.cond(c & 1 == 0, lambda: conv_step(c, spec_a, spec_b, output_jobs, _G1, _PACE1),
                 lambda: conv_step(c, spec_b, spec_a, output_jobs, _G1, _PACE1))

    with jax.named_scope("C"):
        lax.fori_loop(0, _NF, phase_c, None)
    with jax.named_scope("D"):
        for t in range(_F // _T):
            tile = hid_v[:, t * _T:(t + 1) * _T]
            o_v[hidden_at(t)] = tile
            arena[0, _ROW_W + t] = pltpu.bitcast(jnp.concatenate([tile] * 2, axis=0), i32)
        down_copy(0).wait()
        conv_step(_NCH - _NO + (routed_tokens()[0, 0] >> 11), spec_a, spec_b, first_output_jobs,
                  _G2, _PACE2)
        lax.fori_loop(1, _NO, phase_d, None)
    with jax.named_scope("tail"):
        s_v[_NCH - 1] = inverse([w_row(_NCH - 1, r) for r in range(_R)])
        for k in finish(_NO - 1):
            if k % _R == _R - 1:
                rows = pl.ds((_NO - 1) * _OCH + k // _R * 16 * _GC, 16 * _GC)
                start("out", o_v.at[rows], o_hbm.at[rows])
    with jax.named_scope("end"):
        for n in range(_NO - 1):
            out_copy(n).wait()
        wait("out")


@jax.jit
def pallas_recurrent_scan__ssm_conv_s4__moe_arch_mod__prompt_kernel(
    A_u: jax.Array,
    A_A_re: jax.Array,
    A_A_im: jax.Array,
    A_B_re: jax.Array,
    A_B_im: jax.Array,
    A_C_re: jax.Array,
    A_C_im: jax.Array,
    A_log_dt: jax.Array,
    A_Dskip: jax.Array,
    B_x: jax.Array,
    B_w_r: jax.Array,
    B_w_gate: jax.Array,
    B_w_up: jax.Array,
    B_w_down: jax.Array,
):
    del B_x
    assert A_u.shape == (1, _L, _D) and A_A_re.shape == (_D, _N) and B_w_gate.shape == (_D, _F)
    assert A_u.dtype == bf16 and A_A_re.dtype == bf16
    hbm = pl.BlockSpec(memory_space=pl.ANY)
    vmem = pltpu.VMEM
    out = pl.pallas_call(
        _kernel,
        out_shape=jax.ShapeDtypeStruct((_D, _L), bf16),
        in_specs=[hbm] * 14,
        out_specs=hbm,
        scratch_shapes=[
            vmem((_D // 2, _L), i32), vmem((_D + 32, _L), bf16),
            vmem((6, _D // 2, _N), i32), vmem((_D,), bf16), vmem((_D,), bf16), vmem((_D,), bf16),
            vmem((_D // 2, _F), i32), vmem((_D // 2, _F), i32), vmem((_NO, _OCH // 2, _F), i32),
            vmem((_T // 2, 2 * _T), i32), vmem((2 * _T, _T), f32),
            vmem((_D // 2, _T), i32), vmem((_NG, 8, _T), i32),
            vmem((_NCH, _ROWS, 8, _T), i32), vmem((_NCH, 16 * _R, _T), f32),
            vmem((_D // 2, _T), i32), vmem((_GA, 2, 4, 8, _N), f32), vmem((_GA, len(_TAPS), 8, _T), i32),
            vmem((2 * _GA, _NB, 8, _T), i32),
            vmem((_NB, _NG, 16, _T), f32), vmem((3, _NB, 8, _T), f32), vmem((3, 8, _T), f32),
            vmem((_NO, 8, _OCH), f32), vmem((8, _F), bf16),
            *[vmem((2 * _GC * 3 * _PLANE, 8, _T), f32)] * 2, vmem((2 * _NG, 3 * _PLANE, 8, _T), f32),
            pltpu.SemaphoreType.DMA((6,)), pltpu.SemaphoreType.DMA((_NF + _NO,)),
            pltpu.SemaphoreType.DMA(()),
        ],
        compiler_params=pltpu.CompilerParams(vmem_limit_bytes=100 * 2**20, flags=_FLAGS),
    )(A_u.reshape(_L, _D).T, A_A_re, A_A_im, A_B_re, A_B_im, A_C_re, A_C_im, A_log_dt, A_Dskip,
      B_w_r, B_w_gate, B_w_up, B_w_down.T, _FWD)
    return out.T.reshape(1, _L, _D)
```

```python
import jax
import jax.numpy as jnp
import numpy as np
from jax import lax
import jax.experimental.pallas as pl
import jax.experimental.pallas.tpu as pltpu

_D, _L, _N, _F, _C = 576, 2048, 128, 4608, 8
_T = 128
_NB = _L // _T
_EPS = 1e-5
_GA = 4
_GC = 2
_NG = _D // 16
_NCH = _NG // _GC
_R = _GC * _NB
_ROW_X, _ROW_W, _ROW_P, _ROWS = 0, _R, 5 * _R + 8, 5 * _R + 8 + 24
_PLANE, _WQ = _NB + 1, 2 * _R + 1
_ROW_SEL = 5 * _R + 3
_MERGE, _HOLD, _PRIO, _G2, _PACE2 = 1, 3, 0, 432, 0.87
_FLAGS, _HALF, _FENCE, _INTW, _GD = None, 0, (0, 1, 2), 1, 40
_FORCE, _COLBF = 1, 1
_KT = -(-_D // _T)
_NO, _OCH = 6, _D // 6
_NF = 3
_FCH = _F // _NF
_LN_STEP = 4
_WD_STEP = 1
_PACE, _PACE1, _LEAD, _LAG, _G1, _S0, _S1 = 0.87, 0.8, 32, 140, 32, 560, 14

f32, bf16, i32 = jnp.float32, jnp.bfloat16, jnp.int32


def _dft_constants():
    theta = (np.pi / 2 + 2 * np.pi * np.arange(_T)) / _T
    ang = np.arange(_T)[:, None] * theta[None, :]
    c, s = np.cos(ang), np.sin(ang)
    fwd = np.concatenate([c, s], axis=1)
    bits = fwd.astype(bf16).view(np.uint16).astype(np.uint32)
    words = (bits[0::2] | bits[1::2] << 16).view(np.int32)
    return words


_FWD = _dft_constants()


def _lag_step(j):
    return max(1, (1 << (j * _T).bit_length()) >> 8)


def _round_lag(p, st):
    if st == 1:
        return p
    return (p + (st // 2 - 1) + ((p >> (st.bit_length() - 1)) & 1)) & ~(st - 1)


assert np.array_equal(
    np.concatenate([j * _T + _round_lag(np.arange(_T), _lag_step(j)) for j in range(_NB)]),
    np.arange(_L).astype(bf16).astype(np.int64))

_PAIRS = (((0, 1), (0, 5)), ((0, 2), (0, 6)), ((0, 3), (0, 7)), ((0, 4), (0, 8)), ((1, 2), (1, 6)),
          ((1, 4), (1, 8)), ((2, 4), (2, 8)), ((3, 4), (3, 8)), ((4, 8), (5, 8)), ((6, 8), (7, 8)))
_TAPS = [k for pair in _PAIRS for k in pair]


def _aligned(i, n):
    return i if isinstance(i, int) else pl.multiple_of(i, n)


def _cmul(a, b):
    return a[0] * b[0] - a[1] * b[1], a[0] * b[1] + a[1] * b[0]


def _csq(a):
    return a[0] * a[0] - a[1] * a[1], (a[0] + a[0]) * a[1]


def _silu(x):
    h = 0.5 * x
    return h + h * jnp.tanh(h)


def _rnd(x):
    return x.astype(bf16).astype(f32)


def _dot(a, b):
    return jnp.dot(a, b, preferred_element_type=f32)


def _dot_nt(a, b):
    return lax.dot_general(a, b, (((1,), (1,)), ((), ())), preferred_element_type=f32)


def _column(v):
    if _COLBF:
        return pltpu.bitcast(jnp.broadcast_to(v, (_T, v.shape[1])).astype(bf16).T, i32)
    return pltpu.bitcast(jnp.broadcast_to(v, (_T, v.shape[1])).T.astype(bf16), i32)


def _even_odd(x):
    return pltpu.bitcast(x << 16, f32), pltpu.bitcast(x & -65536, f32)


def _interleave(even, odd):
    even, odd = [pltpu.bitcast(x, i32) + 0x8000 for x in (even, odd)]
    return lax.shift_right_logical(even, 16) | (odd & -65536)


def _words(x):
    y = jnp.concatenate([x[:8], x[8:]], axis=1).astype(bf16)
    return pltpu.bitcast(jnp.concatenate([y[:, :_T], y[:, _T:]], axis=0), i32)


def _modes(dt, ar, ai, br, bi, cr, ci):
    zr, zi = dt * ar, dt * ai
    mag = jnp.exp(zr)
    return _cmul((cr, ci), (dt * br, dt * bi)) + (mag * jnp.cos(zi), mag * jnp.sin(zi))


def _seeds(w, a1):
    a = {1: a1}
    for n in range(9):
        a[2 << n] = _csq(a[1 << n])
    row = lax.broadcasted_iota(i32, (8, _N), 0)

    def mix(z0, z1):
        rolled = [pltpu.roll(x, 4, 0) for x in z1]
        return ([jnp.where(row < 4, x, y) for x, y in zip(z0, rolled)],
                [jnp.where(row < 4, y, x) for x, y in zip(z0, rolled)])

    def dup(z):
        return [[jnp.take_along_axis(x, (row & 3) + 4 * q, axis=0, mode="promise_in_bounds")
                 for x in z] for q in range(2)]

    wa = _cmul(w, a[1])
    return zip(mix((1.0, 0.0), a[128]), dup(a[8]), dup(a[32]),
               mix(wa, _cmul(wa, a[4])), dup(a[1]), dup(a[256]),
               mix(_cmul(a[256], a[4]), a[512]), dup(a[512]))


def _vandermonde(e0, m8, m32, g0, m1, m256, m_top, m512):
    e = [e0]
    for s in range(1, 16):
        e.append(_cmul(e[s - 1], m8) if s < 4 else _cmul(e[s - 4], m32))
    g = [g0]
    for _ in range(3):
        g.append(_cmul(g[-1], m1))
    g += [_cmul(g[1], m256), _cmul(g[3], m256)]
    g += [_cmul(g[3], m512), _cmul(g[5], m512)]
    g.append(_cmul(g[7], m_top))
    g.append(_cmul(g[8], m512))
    re, im = [_dot_nt(jnp.concatenate([z[p] for z in g], axis=0),
                      jnp.concatenate([z[p] for z in e], axis=0)) for p in range(2)]
    return re - im


def _unmix(lo, hi):
    row = lax.broadcasted_iota(i32, (8, _T), 0)
    out = []
    for m in range(len(_PAIRS)):
        x, y = lo[8 * m:8 * m + 8], hi[8 * m:8 * m + 8]
        out += [jnp.where(row < 4, x, y), pltpu.roll(jnp.where(row < 4, y, x), 4, 0)]
    return out


def _lag_blocks(tap, lag0):
    lane = lax.broadcasted_iota(i32, (8, _T), 1)
    row = lax.broadcasted_iota(i32, (8, _T), 0)
    for h in range(2):
        def take(big, r, fine):
            s = ((_T * h + fine) >> 3) & 31
            return jnp.take_along_axis(tap(_TAPS.index((big, r))),
                                       ((s & 15) << 3) + (row ^ ((s >> 4) << 2)),
                                       axis=1, mode="promise_in_bounds")

        top = [take(big, 8, _round_lag(lane, 8) - 8) for big in range(_NB // 2)]
        for big, blk in enumerate(top):
            st = _lag_step(2 * big + h)
            lag = _round_lag(lane, st)
            if h == 0:
                blk = jnp.where(lag == 0, top[big - 1] if big else lag0, blk)
            for r in range(st, 8, st):
                blk = jnp.where((lag & 7) == r, take(big, r, lane), blk)
            yield 2 * big + h, blk


def _kernel(x_hbm, ar_hbm, ai_hbm, br_hbm, bi_hbm, cr_hbm, ci_hbm, ldt_hbm, dsk_hbm, wr_hbm,
            wg_hbm, wu_hbm, wd_hbm, fwd_hbm, o_hbm,
            x_v, o_v, par_v, ldt_v, dsk_v, wr_v, wg_v, wu_v, wd_v, fwd_v, inv_v,
            skip_v, k0_v, arena, s_v, dt_v, mode_v, tap_v, k_v, xc_v, stat_v, key_v, sel_v, hid_v,
            spec_a, spec_b, kf_v, sem, w_sem, o_sem):
    row = lax.broadcasted_iota(i32, (8, _T), 0)
    lane = lax.broadcasted_iota(i32, (8, _T), 1)
    groups = {}

    def start(name, src, dst):
        slot, pairs = groups.setdefault(name, (len(groups), []))
        pairs.append((src, dst))
        pltpu.make_async_copy(src, dst, sem.at[slot]).start()

    def wait(name):
        slot, pairs = groups[name]
        for src, dst in pairs:
            pltpu.make_async_copy(src, dst, sem.at[slot]).wait()

    def hidden_copies(n):
        cols = pl.ds(_aligned(n * _FCH, _FCH), _FCH)
        return [pltpu.make_async_copy(w.bitcast(i32).at[:, cols], v.at[:, cols], w_sem.at[n])
                for w, v in ((wg_hbm, wg_v), (wu_hbm, wu_v))]

    def chunk_rows(n):
        return pl.ds(_aligned(n * _OCH, 32), _OCH)

    def down_copy(n):
        rows = pl.ds(_aligned(n * (_OCH // 2), 16), _OCH // 2)
        return pltpu.make_async_copy(wd_hbm.bitcast(i32).at[rows], wd_v.at[n], w_sem.at[_NF + n])

    def out_copy(n):
        return pltpu.make_async_copy(o_v.at[chunk_rows(n)], o_hbm.at[chunk_rows(n)], o_sem)

    def start_parameters(part, rows):
        for n, src in enumerate((ar_hbm, ai_hbm, br_hbm, bi_hbm, cr_hbm, ci_hbm)):
            start(part, src.bitcast(i32).at[rows], par_v.at[n, rows])

    with jax.named_scope("init"):
        start("vectors", ldt_hbm, ldt_v)
        start("vectors", dsk_hbm, dsk_v)
        start_parameters(0, pl.ds(0, 8 * _GA))
        start_parameters(2, pl.ds(8 * _GA, 8 * _GA))
        start(2, fwd_hbm, fwd_v)
        arena[0, _ROW_W:_ROW_P] = jnp.zeros((_ROW_P - _ROW_W, 8, _T), i32)
        tap_v[...] = jnp.zeros(tap_v.shape, i32)
        k_v[:_GA] = jnp.zeros((_GA, _NB, 8, _T), i32)
        key_v[...] = jnp.zeros(key_v.shape, f32)
        wait("vectors")
        start_parameters(1, pl.ds(16 * _GA, _D // 2 - 16 * _GA))
        start("x", x_hbm.bitcast(i32), x_v)
        start("x", wr_hbm, wr_v)
        dt = jnp.exp(ldt_v[...].astype(f32)).reshape(1, _D)
        skip = dsk_v[...].astype(f32).reshape(1, _D)
        dt_v[:_T // 2] = _column(dt[:, :_T])
        skip_v[:_T // 2] = _column(skip[:, :_T])
        wait(0)

    def compact(ref, k, h):
        out = ref[k, 8 * h]
        for s in range(1, 8):
            out = jnp.where(row == s, ref[k, 8 * h + s], out)
        return out

    def layer_norm():
        wait("x")
        for cp in hidden_copies(1):
            cp.start()

        def moments(b, carry):
            cols = pl.ds(_aligned(b * _T, _T), _T)
            pivot = jnp.broadcast_to(_even_odd(x_v[:8, cols])[0][:1], (8, _T))
            s1, s2 = [None] * 2, [None] * 2
            for g in range(_NG):
                words = x_v[pl.ds(8 * g, 8), cols]
                x = pltpu.bitcast(words, bf16).astype(f32)
                xc_v[b, g] = x
                for h in range(2):
                    d = x[8 * h:8 * h + 8] - pivot
                    s1[h] = s1[h] + d if g else d
                    s2[h] = s2[h] + d * d if g else d * d
            for k, s in enumerate((s1, s2)):
                stat_v[k, b] = jnp.broadcast_to(jnp.sum(s[0] + s[1], axis=0, keepdims=True), (8, _T))
            stat_v[2, b] = pivot
            return carry

        lax.fori_loop(0, _NB, moments, 0, unroll=4)
        for h in range(_NB // 8):
            m1, m2, pivot = compact(stat_v, 0, h) / _D, compact(stat_v, 1, h) / _D, compact(stat_v, 2, h)
            var = jnp.maximum(m2 - m1 * m1, 0.0)
            shift = _rnd(pivot + m1)
            gain = 0.5 / _rnd(jnp.sqrt(_rnd(_rnd(var) + _rnd(jnp.full_like(var, _EPS)))))
            for s in range(8):
                stat_v[0, 8 * h + s] = jnp.broadcast_to(shift[s:s + 1], (8, _T))
                stat_v[1, 8 * h + s] = jnp.broadcast_to(gain[s:s + 1], (8, _T))
        inv_v[...] = pltpu.bitcast(fwd_v[...], bf16).astype(f32).T * (2 / _T)
        wr = jnp.broadcast_to(wr_v[...].astype(f32).reshape(1, _D), (8, _D)).astype(bf16)

        def scale(b, carry):
            shift, gain = stat_v[0, b], stat_v[1, b]
            if _INTW:
                xn = [_interleave(*[(xc_v[b, g, pl.ds(h, 8, stride=2), :] - shift) * gain
                                    for h in range(2)]) for g in range(_NG)]
            else:
                xn = [_words((xc_v[b, g] - shift[:1]) * gain[:1]) for g in range(_NG)]
            for g in range(_NG):
                arena[g // _GC, _ROW_X + (g % _GC) * _NB + b] = xn[g]
            stat_v[2, b] = _dot(wr, pltpu.bitcast(jnp.concatenate(xn, axis=0), bf16))
            return carry

        lax.fori_loop(0, _NB, scale, 0, unroll=16)
        for h in range(_NB // 8):
            bits = pltpu.bitcast(_rnd(2.0 * compact(stat_v, 2, h)) + 0.0, i32) >> 16
            rank = jnp.where(bits < 0, ~bits, bits + 0x8000)
            token = (8 * h + row) * _T + lane
            key_v[h] = pltpu.bitcast((1 << 28) + rank * _L + (_L - 1 - token), f32)

    def pop_best(c):
        best = jnp.max(jnp.max(jnp.maximum(key_v[0], key_v[1]), axis=0, keepdims=True),
                       axis=1, keepdims=True)
        key_v[2] = jnp.where(row == c, best, key_v[2])
        for h in range(2):
            key_v[h] = jnp.where(key_v[h] == best, 0.0, key_v[h])

    def modes(step):
        for u in range(_GA):
            grp = step * _GA + u
            rows = pl.ds(_aligned(grp * 8, 8), 8)
            par = [_even_odd(dt_v[rows, :])] + [_even_odd(par_v[n, rows, :]) for n in range(6)]
            k0 = []
            for h, skip in enumerate(_even_odd(skip_v[rows, :])):
                z = _modes(*[p[h] for p in par])
                for n in range(4):
                    mode_v[u, h, n] = z[n]
                k0.append(skip + jnp.sum(z[0], axis=1, keepdims=True))
            k0_v[grp] = _interleave(*k0)

    def dft(rows):
        z = _dot(jnp.concatenate([pltpu.bitcast(r, bf16) for r in rows], axis=0),
                 pltpu.bitcast(fwd_v[...], bf16))
        n = min(len(rows), _NB)
        return [[(z[o:o + 8, :_T], z[o:o + 8, _T:])
                 for o in range((h // 2) * 16 * n + 8 * (h % 2), (h // 2 + 1) * 16 * n, 16)]
                for h in range(2 * len(rows) // n)]

    def spread(step, u, slot):
        for j, blk in _lag_blocks(lambda n: tap_v[u, n], k0_v[step * _GA + u]):
            k_v[slot, j] = blk

    def filter_spectra(grp, rows):
        z = dft(rows)
        for h, blocks in enumerate(z):
            for j, (re, im) in enumerate(blocks):
                for p, val in enumerate((re, re + im, im - re)):
                    kf_v[2 * grp + h, p * _PLANE + j] = val
        return z

    def filter_step(i, zero, extra=lambda u: None):
        for u in range(_GA):
            if u % (_GA // 2) == 0:
                old = (u + _GA // 2) % _GA
                filter_spectra(jnp.maximum(i - (1 if u else 2), 0) * _GA + old,
                               [k_v[old + k + zero, j] for k in range(_GA // 2) for j in range(_NB)])
            spread(jnp.maximum(i - 1, 0), u, u)
            v = [[_vandermonde(*seeds) for seeds in _seeds(
                (mode_v[u, h, 0], mode_v[u, h, 1]), (mode_v[u, h, 2], mode_v[u, h, 3]))]
                 for h in range(2)]
            for n, tap in enumerate(_unmix(*map(_interleave, *v))):
                tap_v[u, n] = tap
            extra(u)

    def phase_a(i, carry):
        @pl.when(i == 1)
        def _():
            wait(1)
            for cp in hidden_copies(0):
                cp.start()

        pl.when(i == _LN_STEP)(layer_norm)
        for c in range(2):
            pop_best(2 * (i - _LN_STEP) + c)
        filter_step(i, i >> 8)
        modes(i + 1)

    with jax.named_scope("A"):
        modes(0)
        dt_v[_T // 2:] = _column(dt[:, _T:])
        skip_v[_T // 2:] = _column(skip[:, _T:])
        wait(2)
        lax.fori_loop(0, _NG // _GA - 1, phase_a, None)

    def input_spectra(rows, dst):
        z = dft(rows)
        for h, t in enumerate(z):
            for b, (re, im) in enumerate(t):
                if b:
                    re, im = re + t[b - 1][1], im - t[b - 1][0]
                for p, val in enumerate((re + im, im, re)):
                    dst[(h * 3 + p) * _PLANE + b] = val
        return z

    def w_row(c, r):
        return jnp.concatenate(
            [pltpu.bitcast(arena[c, pl.ds(_ROW_W + q * _WQ + 2 * r, 2)].reshape(16, _T), f32)
             for q in range(2)], axis=1)

    def inverse(rows):
        return _dot(jnp.concatenate(rows, axis=0), inv_v[...])

    def routed_tokens():
        return _L - 1 - (pltpu.bitcast(key_v[2], i32) & (_L - 1))

    with jax.named_scope("topk"):
        for n in range(2, _NF):
            for cp in hidden_copies(n):
                cp.start()
        token = routed_tokens()
        picked = []

        def gather(u):
            tokens = range(u * _C // _GA, (u + 1) * _C // _GA)
            blocks = jnp.concatenate(
                [pltpu.bitcast(jnp.concatenate(
                    [arena[g // _GC, _ROW_X + (g % _GC) * _NB + (token[t, 0] >> 7)]
                     for g in range(_NG)], axis=0), bf16) for t in tokens], axis=1)
            pick = jnp.concatenate(
                [jnp.where((row == t) & ((token & (_T - 1)) == lane), 2.0, 0.0) for t in tokens],
                axis=1).astype(bf16)
            picked.append(_dot_nt(pick, blocks))

        filter_step(_NG // _GA - 1, token[0, 0] >> 11, gather if _MERGE else lambda u: None)
        for u in range(0 if _MERGE else _GA):
            gather(u)
        x_sel = sum(picked[1:], picked[0])
        for n in range(_NO):
            sel_v[n] = x_sel[:, n * _OCH:(n + 1) * _OCH]
        x_sel = jnp.concatenate([x_sel, jnp.zeros((8, _KT * _T - _D), f32)], axis=1)
        for n in range(_KT):
            arena[0, _ROW_SEL + n] = pltpu.bitcast(
                jnp.concatenate([x_sel[:, n * _T:(n + 1) * _T]] * 2, axis=0).astype(bf16), i32)
        input_spectra([arena[0, _ROW_X + r] for r in range(_R)], spec_a)
        for u in range(_GA):
            spread(_NG // _GA - 1, u, _GA + u)
        filter_spectra(_NG - 3 * _GA // 2,
                       [k_v[u, j] for u in range(_GA // 2, 2 * _GA) for j in range(_NB)])

    def hidden_jobs(c):
        width = _F // (_NCH - _NO)
        gate = []

        def project(n):
            cols = pl.ds(_aligned(c * width + n // 2 * _T, _T), _T)
            x_sel = jnp.concatenate(
                [pltpu.bitcast(arena[c >> 8, _ROW_SEL + r], bf16) for r in range(_KT)], axis=1)
            gate.append(_rnd(_dot(x_sel[:, :_D], pltpu.bitcast((wu_v if n % 2 else wg_v)[:, cols], bf16))[:8]))
            if n % 2:
                hid_v[:, cols] = (_rnd(_silu(gate[-2])) * gate[-1]).astype(bf16)

        return [(_GD * n, lambda n=n: project(n)) for n in range(2 * width // _T)]

    def hidden_at(t, zero=0):
        return pl.ds(_aligned(_D + 8 * (t // _NB + zero), 8), 8), pl.ds((t % _NB) * _T, _T)

    def finish(n):
        for k in range(0, _OCH // 16 * _NB, 2):
            c, r = n * (_OCH // (16 * _GC)) + k // _R, k % _R
            out = []
            for d in range(2):
                h = pltpu.bitcast(arena[c, _ROW_X + r + d], bf16).astype(f32)
                out.append(xc_v[k % _NB + d, n * (_OCH // 16) + k // _NB]
                           + s_v[c, pl.ds(16 * (r + d), 16), :] * (h + h * jnp.tanh(h)))
            o_v[pl.ds(_aligned(n * _OCH + 16 * (k // _NB), 16), 16), pl.ds((k % _NB) * _T, 2 * _T)] = (
                jnp.concatenate(out, axis=1).astype(bf16))
            yield k + 1

    def down_jobs(n, hid):
        rank = (pltpu.bitcast(key_v[2], i32) - (1 << 28)) >> 11
        score = pltpu.bitcast(jnp.where(rank >= 0x8000, rank - 0x8000, ~rank) << 16, f32)
        y = _rnd(_dot_nt(jnp.concatenate(hid, axis=1), pltpu.bitcast(wd_v[n], bf16)))
        y = 0.5 * (sel_v[n] + _rnd(y * _rnd(jax.nn.sigmoid(score))[:, :_OCH]))
        col = jnp.concatenate([y, jnp.zeros((_T - _C, _OCH), f32)], axis=0).T
        col = pltpu.bitcast(col.astype(bf16), i32)
        token = routed_tokens()

        def scatter(t):
            hit = ((token & (_T - 1)) == lane)[t:t + 1]
            new = jnp.broadcast_to(col[:, t:t + 1], (_OCH // 2, _T))
            where = [(n * (_OCH // (16 * _GC)) + g // _GC,
                      _ROW_X + (g % _GC) * _NB + (token[t, 0] >> 7)) for g in range(_OCH // 16)]
            old = [arena[at] for at in where]
            for g, at in enumerate(where):
                arena[at] = jnp.where(hit, new[8 * g:8 * g + 8], old[g])

        return [lambda t=t: scatter(t) for t in range(_C)]

    def first_output_jobs(c):
        hid, scatter = [], []

        def read():
            hid.extend(pltpu.bitcast(arena[c >> 8, _ROW_W + t], bf16)[:8]
                       for t in range(len(hid), len(hid) + 4))

        return ([(48 * k, read) for k in range(_F // (4 * _T))]
                + [(_G2 - 1, lambda: scatter.extend(down_jobs(0, hid)))]
                + [(_G2 + _S0 + _S1 * t, lambda t=t: scatter[t]()) for t in range(_C)])

    def output_jobs(c):
        n = c - (_NCH - _NO)
        hid = [o_v[hidden_at(t, c >> 8)] for t in range(4)]
        for k in finish(n - 1):
            if k == _OCH // 16 * _NB - 1:
                pl.when(n >= _HOLD)(lambda: out_copy(n - 1).start())
                if _FORCE:
                    o_v[hidden_at(_F // _T, c >> 9)] = hid[0]
            if k % 12 == 11:
                hid += [o_v[hidden_at(t, c >> 8)] for t in range(len(hid), len(hid) + 4)]
        return [(_S0 + _S1 * t, job) for t, job in enumerate(down_jobs(n, hid))]

    def conv_step(c, cur, nxt, ffn_jobs, delay, pace, first=False):
        c_next, c_prev = jnp.minimum(c + 1, _NCH - 1), jnp.maximum(c - 1, 0)
        zero = c >> 8
        fwd_rows, inv_rows, results = [], [], []

        def transform():
            if first:
                y = filter_spectra(_NG - _GC, inv_rows)
            else:
                y = inverse(inv_rows)
                s_v[c_prev] = y
            results.extend((y, input_spectra(fwd_rows, nxt)))

        def drain(r):
            y, z = results
            arena[c, _ROW_SEL - 1] = pltpu.bitcast(
                (y[-1][r % _R // 2][r // 8 % 2] if first else y[8 * r:8 * r + 8]) + z[2 * (r // _R) + 1][r % _R // 2][r // 8 % 2], i32)

        jobs = sorted(
            ffn_jobs(c)
            + [(delay + 16 * r, lambda r=r: inv_rows.append(arena[_NCH - 1 + zero, _ROW_W + r] if first else w_row(c_prev, r))) for r in range(_R)]
            + [(delay + 16 * r, lambda r=r: fwd_rows.append(arena[c_next, _ROW_X + r]))
               for r in range(_R)]
            + [(delay + 16 * _R, transform)]
            + [(delay + _LAG + 8 * r, lambda r=r: drain(r)) for r in range(2 * _R - 17, 2 * _R, 8)],
            key=lambda job: job[0])

        def run_jobs(done):
            while jobs and done * (delay + 16 * _R) >= (jobs[0][0] - _LEAD) * pace * 18 * _GC:
                jobs.pop(0)[1]()

        run_jobs(0)
        for h in range(2 * _GC):
            for part in range(3):
                for plane in range(3):
                    kf = lambda b: kf_v[c * 2 * _GC + h + (zero >> part), plane * _PLANE + b]
                    uf = lambda b: cur[(zero >> part) + (h * 3 + plane) * _PLANE + b]
                    base = [pltpu.bitcast(arena[c + zero, _ROW_P + plane * 8 + m], f32)
                            for m in range(8) if part and plane]
                    k, u, out = [], [], []
                    for m in range(8):
                        if part == 0:
                            k.append(kf(2 * m))
                            u.append(uf(2 * m) + uf(2 * m + 1))
                        elif part == 1:
                            k.append(kf(2 * m) - kf(2 * m - 1) if m else kf(0))
                            u.append(uf(2 * m + 1))
                        else:
                            k.append(kf(2 * m) - kf(2 * m + 1))
                            u.append(uf(2 * m))
                        y = k[0] * u[m]
                        for j in range(1, m + 1):
                            y = y + k[j] * u[m - j]
                        if plane:
                            y = shared[m] - y if plane == 1 else shared[m] + y
                        out.append(y)
                        if part == 0 or plane == 0:
                            arena[c, _ROW_P + plane * 8 + m] = pltpu.bitcast(y, i32)
                        else:
                            r = ((h // 2) * _NB + 2 * m + part - 1) * 2 + h % 2
                            arena[c, _ROW_W + (plane - 1) * _WQ + r] = pltpu.bitcast(base[m] - y, i32)
                    if plane == 0:
                        shared = out
                    if plane in _FENCE:
                        run_jobs((h * 3 + part) * 3 + plane + 1)
        run_jobs(np.inf)

    def phase_c(part, carry):
        for cp in hidden_copies(part):
            cp.wait()

        @pl.when(part == _WD_STEP)
        def _():
            for n in range(_NO):
                down_copy(n).start()

        def pair(i, carry):
            conv_step(2 * i, spec_a, spec_b, hidden_jobs, 6 * _GD, _PACE)
            conv_step(2 * i + 1, spec_b, spec_a, hidden_jobs, 6 * _GD, _PACE)

        pairs = (_NCH - _NO) // (2 * _NF)
        lax.fori_loop(part * pairs, (part + 1) * pairs, pair, None)

    def phase_d(n, carry):
        down_copy(n).wait()

        @pl.when(n == _HOLD + _HALF)
        def _():
            for k in range(_HOLD - 1):
                out_copy(k).start()

        c = n + _NCH - _NO
        lax.cond(c & 1 == 0, lambda: conv_step(c, spec_a, spec_b, output_jobs, _G1, _PACE1),
                 lambda: conv_step(c, spec_b, spec_a, output_jobs, _G1, _PACE1))

    with jax.named_scope("C"):
        lax.fori_loop(0, _NF, phase_c, None)
    with jax.named_scope("D"):
        for t in range(_F // _T):
            tile = hid_v[:, t * _T:(t + 1) * _T]
            o_v[hidden_at(t)] = tile
            arena[0, _ROW_W + t] = pltpu.bitcast(jnp.concatenate([tile] * 2, axis=0), i32)
        down_copy(0).wait()
        conv_step(_NCH - _NO + (routed_tokens()[0, 0] >> 11), spec_a, spec_b, first_output_jobs,
                  _G2, _PACE2)
        lax.fori_loop(1, _NO, phase_d, None)
    with jax.named_scope("tail"):
        s_v[_NCH - 1] = inverse([w_row(_NCH - 1, r) for r in range(_R)])
        for k in finish(_NO - 1):
            if k % _R == _R - 1:
                rows = pl.ds((_NO - 1) * _OCH + k // _R * 16 * _GC, 16 * _GC)
                start("out", o_v.at[rows], o_hbm.at[rows])
    with jax.named_scope("end"):
        for n in range(_NO - 1):
            out_copy(n).wait()
        wait("out")


@jax.jit
def pallas_recurrent_scan__ssm_conv_s4__moe_arch_mod__prompt_kernel(
    A_u: jax.Array,
    A_A_re: jax.Array,
    A_A_im: jax.Array,
    A_B_re: jax.Array,
    A_B_im: jax.Array,
    A_C_re: jax.Array,
    A_C_im: jax.Array,
    A_log_dt: jax.Array,
    A_Dskip: jax.Array,
    B_x: jax.Array,
    B_w_r: jax.Array,
    B_w_gate: jax.Array,
    B_w_up: jax.Array,
    B_w_down: jax.Array,
):
    del B_x
    assert A_u.shape == (1, _L, _D) and A_A_re.shape == (_D, _N) and B_w_gate.shape == (_D, _F)
    assert A_u.dtype == bf16 and A_A_re.dtype == bf16
    hbm = pl.BlockSpec(memory_space=pl.ANY)
    vmem = pltpu.VMEM
    out = pl.pallas_call(
        _kernel,
        out_shape=jax.ShapeDtypeStruct((_D, _L), bf16),
        in_specs=[hbm] * 14,
        out_specs=hbm,
        scratch_shapes=[
            vmem((_D // 2, _L), i32), vmem((_D + 32, _L), bf16),
            vmem((6, _D // 2, _N), i32), vmem((_D,), bf16), vmem((_D,), bf16), vmem((_D,), bf16),
            vmem((_D // 2, _F), i32), vmem((_D // 2, _F), i32), vmem((_NO, _OCH // 2, _F), i32),
            vmem((_T // 2, 2 * _T), i32), vmem((2 * _T, _T), f32),
            vmem((_D // 2, _T), i32), vmem((_NG, 8, _T), i32),
            vmem((_NCH, _ROWS, 8, _T), i32), vmem((_NCH, 16 * _R, _T), f32),
            vmem((_D // 2, _T), i32), vmem((_GA, 2, 4, 8, _N), f32), vmem((_GA, len(_TAPS), 8, _T), i32),
            vmem((2 * _GA, _NB, 8, _T), i32),
            vmem((_NB, _NG, 16, _T), f32), vmem((3, _NB, 8, _T), f32), vmem((3, 8, _T), f32),
            vmem((_NO, 8, _OCH), f32), vmem((8, _F), bf16),
            *[vmem((2 * _GC * 3 * _PLANE, 8, _T), f32)] * 2, vmem((2 * _NG, 3 * _PLANE, 8, _T), f32),
            pltpu.SemaphoreType.DMA((6,)), pltpu.SemaphoreType.DMA((_NF + _NO,)),
            pltpu.SemaphoreType.DMA(()),
        ],
        compiler_params=pltpu.CompilerParams(vmem_limit_bytes=100 * 2**20, flags=_FLAGS),
    )(A_u.reshape(_L, _D).T, A_A_re, A_A_im, A_B_re, A_B_im, A_C_re, A_C_im, A_log_dt, A_Dskip,
      B_w_r, B_w_gate, B_w_up, B_w_down.T, _FWD)
    return out.T.reshape(1, _L, _D)
```

```python
import jax
import jax.numpy as jnp
import numpy as np
from jax import lax
import jax.experimental.pallas as pl
import jax.experimental.pallas.tpu as pltpu

f32, bf16, i32 = jnp.float32, jnp.bfloat16, jnp.int32

_D, _L, _N, _F, _C = 576, 2048, 128, 4608, 8
_EPS = 1e-5
_T = 128
_NB = _L // _T
_NG = _D // 16
_GA = 4
_GC = 2
_NCH = _NG // _GC
_R = _GC * _NB
_KT = -(-_D // _T)
_NF = 3
_NO, _OCH = 6, _D // 6
_LN_STEP = 4
_OUT_STEP = 3
_ROW_X, _ROW_W, _WQ, _ROW_SEL, _ROW_P = 0, _R, 2 * _R + 1, 5 * _R + 3, 5 * _R + 8
_ROWS = _ROW_P + 3 * _NB // 2
_PLANE = _NB + 1


def _dft_words():
    theta = (np.pi / 2 + 2 * np.pi * np.arange(_T)) / _T
    angle = np.arange(_T)[:, None] * theta[None, :]
    matrix = np.concatenate([np.cos(angle), np.sin(angle)], axis=1)
    bits = matrix.astype(bf16).view(np.uint16).astype(np.uint32)
    return (bits[0::2] | bits[1::2] << 16).view(np.int32)


_DFT = _dft_words()


def _lag_step(j):
    return max(1, (1 << (j * _T).bit_length()) >> 8)


def _round_lag(p, step):
    if step == 1:
        return p
    return (p + (step // 2 - 1) + ((p >> (step.bit_length() - 1)) & 1)) & ~(step - 1)


assert np.array_equal(
    np.concatenate([j * _T + _round_lag(np.arange(_T), _lag_step(j)) for j in range(_NB)]),
    np.arange(_L).astype(bf16).astype(np.int64))

_PAIRS = (((0, 1), (0, 5)), ((0, 2), (0, 6)), ((0, 3), (0, 7)), ((0, 4), (0, 8)), ((1, 2), (1, 6)),
          ((1, 4), (1, 8)), ((2, 4), (2, 8)), ((3, 4), (3, 8)), ((4, 8), (5, 8)), ((6, 8), (7, 8)))
_TAPS = [k for pair in _PAIRS for k in pair]


def _ds(start, size, align):
    return pl.ds(start if isinstance(start, int) else pl.multiple_of(start, align), size)


def _cmul(a, b):
    return a[0] * b[0] - a[1] * b[1], a[0] * b[1] + a[1] * b[0]


def _csq(a):
    return a[0] * a[0] - a[1] * a[1], (a[0] + a[0]) * a[1]


def _silu_of_twice(h):
    return h + h * jnp.tanh(h)


def _rnd(x):
    return x.astype(bf16).astype(f32)


def _dot(a, b):
    return jnp.dot(a, b, preferred_element_type=f32)


def _dot_nt(a, b):
    return lax.dot_general(a, b, (((1,), (1,)), ((), ())), preferred_element_type=f32)


def _column(v):
    return pltpu.bitcast(jnp.broadcast_to(v, (_T, v.shape[1])).astype(bf16).T, i32)


def _even_odd(words):
    return pltpu.bitcast(words << 16, f32), pltpu.bitcast(words & -65536, f32)


def _interleave(even, odd):
    even, odd = [pltpu.bitcast(x, i32) + 0x8000 for x in (even, odd)]
    return lax.shift_right_logical(even, 16) | (odd & -65536)


def _modes(dt, ar, ai, br, bi, cr, ci):
    zr, zi = dt * ar, dt * ai
    mag = jnp.exp(zr)
    return _cmul((cr, ci), (dt * br, dt * bi)) + (mag * jnp.cos(zi), mag * jnp.sin(zi))


def _seeds(w, a1):
    a = {1: a1}
    for n in range(9):
        a[2 << n] = _csq(a[1 << n])
    row = lax.broadcasted_iota(i32, (8, _N), 0)

    def mix(z0, z1):
        rolled = [pltpu.roll(x, 4, 0) for x in z1]
        return ([jnp.where(row < 4, x, y) for x, y in zip(z0, rolled)],
                [jnp.where(row < 4, y, x) for x, y in zip(z0, rolled)])

    def dup(z):
        return [[jnp.take_along_axis(x, (row & 3) + 4 * q, axis=0, mode="promise_in_bounds")
                 for x in z] for q in range(2)]

    wa = _cmul(w, a1)
    return zip(mix((1.0, 0.0), a[128]), dup(a[8]), dup(a[32]),
               mix(wa, _cmul(wa, a[4])), dup(a1), dup(a[256]),
               mix(_cmul(a[256], a[4]), a[512]), dup(a[512]))


def _vandermonde(e0, m8, m32, g0, m1, m256, m_top, m512):
    e = [e0]
    for s in range(1, 16):
        e.append(_cmul(e[s - 1], m8) if s < 4 else _cmul(e[s - 4], m32))
    g = [g0]
    for _ in range(3):
        g.append(_cmul(g[-1], m1))
    g += [_cmul(g[1], m256), _cmul(g[3], m256)]
    g += [_cmul(g[3], m512), _cmul(g[5], m512)]
    g.append(_cmul(g[7], m_top))
    g.append(_cmul(g[8], m512))
    re, im = [_dot_nt(jnp.concatenate([z[p] for z in g], axis=0),
                      jnp.concatenate([z[p] for z in e], axis=0)) for p in range(2)]
    return re - im


def _unmix(lo, hi):
    row = lax.broadcasted_iota(i32, (8, _T), 0)
    for m in range(len(_PAIRS)):
        x, y = lo[8 * m:8 * m + 8], hi[8 * m:8 * m + 8]
        yield jnp.where(row < 4, x, y)
        yield pltpu.roll(jnp.where(row < 4, y, x), 4, 0)


def _lag_blocks(tap, lag0):
    lane = lax.broadcasted_iota(i32, (8, _T), 1)
    row = lax.broadcasted_iota(i32, (8, _T), 0)
    for h in range(2):
        def take(big, r, lag):
            s = ((_T * h + lag) >> 3) & 31
            return jnp.take_along_axis(tap(_TAPS.index((big, r))),
                                       ((s & 15) << 3) + (row ^ ((s >> 4) << 2)),
                                       axis=1, mode="promise_in_bounds")

        top = [take(big, 8, _round_lag(lane, 8) - 8) for big in range(_NB // 2)]
        for big, blk in enumerate(top):
            step = _lag_step(2 * big + h)
            lag = _round_lag(lane, step)
            if h == 0:
                blk = jnp.where(lag == 0, top[big - 1] if big else lag0, blk)
            for r in range(step, 8, step):
                blk = jnp.where((lag & 7) == r, take(big, r, lane), blk)
            yield 2 * big + h, blk


def _kernel(x_hbm, ar_hbm, ai_hbm, br_hbm, bi_hbm, cr_hbm, ci_hbm, ldt_hbm, dsk_hbm, wr_hbm,
            wg_hbm, wu_hbm, wd_hbm, dft_hbm, o_hbm,
            x_v, par_v, ldt_v, dsk_v, wr_v, wg_v, wu_v, wd_v, dft_v, o_v,
            dt_v, skip_v, mode_v, k0_v, tap_v, k_v, kf_v,
            xf_v, stat_v, key_v, sel_v, hid_v,
            inv_v, arena, uf_a, uf_b, s_v, sem, w_sem, o_sem):
    row = lax.broadcasted_iota(i32, (8, _T), 0)
    lane = lax.broadcasted_iota(i32, (8, _T), 1)

    groups = {}

    def start(name, src, dst):
        slot, pairs = groups.setdefault(name, (len(groups), []))
        pairs.append((src, dst))
        pltpu.make_async_copy(src, dst, sem.at[slot]).start()

    def wait(name):
        slot, pairs = groups[name]
        for src, dst in pairs:
            pltpu.make_async_copy(src, dst, sem.at[slot]).wait()

    def start_parameters(name, rows):
        for n, src in enumerate((ar_hbm, ai_hbm, br_hbm, bi_hbm, cr_hbm, ci_hbm)):
            start(name, src.bitcast(i32).at[rows], par_v.at[n, rows])

    def hidden_copies(n):
        cols = _ds(n * (_F // _NF), _F // _NF, _F // _NF)
        return [pltpu.make_async_copy(w.bitcast(i32).at[:, cols], v.at[:, cols], w_sem.at[n])
                for w, v in ((wg_hbm, wg_v), (wu_hbm, wu_v))]

    def down_copy(n):
        return pltpu.make_async_copy(wd_hbm.bitcast(i32).at[_ds(n * (_OCH // 2), _OCH // 2, 16)],
                                     wd_v.at[n], w_sem.at[_NF + n])

    def out_copy(n):
        rows = _ds(n * _OCH, _OCH, 32)
        return pltpu.make_async_copy(o_v.at[rows], o_hbm.at[rows], o_sem)

    def compact(k, h):
        out = stat_v[k, 8 * h]
        for s in range(1, 8):
            out = jnp.where(row == s, stat_v[k, 8 * h + s], out)
        return out

    def layer_norm():
        def moments(b, carry):
            cols = _ds(b * _T, _T, _T)
            pivot = jnp.broadcast_to(_even_odd(x_v[:8, cols])[0][:1], (8, _T))
            s1, s2 = [None] * 2, [None] * 2
            for g in range(_NG):
                x = pltpu.bitcast(x_v[pl.ds(8 * g, 8), cols], bf16).astype(f32)
                xf_v[b, pl.ds(16 * g, 16), :] = x
                for h in range(2):
                    d = x[8 * h:8 * h + 8] - pivot
                    s1[h] = s1[h] + d if g else d
                    s2[h] = s2[h] + d * d if g else d * d
            for k, s in enumerate((s1, s2)):
                stat_v[k, b] = jnp.broadcast_to(jnp.sum(s[0] + s[1], axis=0, keepdims=True), (8, _T))
            stat_v[2, b] = pivot

        lax.fori_loop(0, _NB, moments, None, unroll=4)
        for h in range(_NB // 8):
            m1, m2 = compact(0, h) / _D, compact(1, h) / _D
            mean = _rnd(compact(2, h) + m1)
            var = _rnd(jnp.maximum(m2 - m1 * m1, 0.0))
            gain = 0.5 / _rnd(jnp.sqrt(_rnd(var + _rnd(jnp.full_like(var, _EPS)))))
            for s in range(8):
                stat_v[0, 8 * h + s] = jnp.broadcast_to(mean[s:s + 1], (8, _T))
                stat_v[1, 8 * h + s] = jnp.broadcast_to(gain[s:s + 1], (8, _T))
        wr = jnp.broadcast_to(wr_v[...].astype(f32).reshape(1, _D), (8, _D)).astype(bf16)
        for b in range(_NB):
            mean, gain = stat_v[0, b], stat_v[1, b]
            xn = [_interleave(*[(xf_v[b, pl.ds(16 * g + h, 8, stride=2), :] - mean) * gain
                                for h in range(2)]) for g in range(_NG)]
            for g in range(_NG):
                arena[g // _GC, _ROW_X + (g % _GC) * _NB + b] = xn[g]
            stat_v[2, b] = _dot(wr, pltpu.bitcast(jnp.concatenate(xn, axis=0), bf16))
        for h in range(_NB // 8):
            bits = pltpu.bitcast(_rnd(2.0 * compact(2, h)), i32) >> 16
            rank = jnp.where(bits < 0, 0x8000 - (bits & 0x7FFF), 0x8000 + bits)
            token = (8 * h + row) * _T + lane
            key_v[h] = pltpu.bitcast((1 << 28) + rank * _L + (_L - 1 - token), f32)

    def pop_best(t):
        best = jnp.max(jnp.max(jnp.maximum(key_v[0], key_v[1]), axis=0, keepdims=True),
                       axis=1, keepdims=True)
        key_v[2] = jnp.where(row == t, best, key_v[2])
        for h in range(2):
            key_v[h] = jnp.where(key_v[h] == best, 0.0, key_v[h])

    def routed_tokens():
        return _L - 1 - (pltpu.bitcast(key_v[2], i32) & (_L - 1))

    def routed_scores():
        rank = (pltpu.bitcast(key_v[2], i32) - (1 << 28)) >> 11
        return pltpu.bitcast(jnp.where(rank < 0x8000, 0x10000 - rank, rank - 0x8000) << 16, f32)

    def gather(tokens):
        token = routed_tokens()
        blocks = jnp.concatenate(
            [pltpu.bitcast(jnp.concatenate(
                [arena[g // _GC, _ROW_X + (g % _GC) * _NB + (token[t, 0] >> 7)]
                 for g in range(_NG)], axis=0), bf16) for t in tokens], axis=1)
        pick = jnp.concatenate(
            [jnp.where((row == t) & ((token & (_T - 1)) == lane), 2.0, 0.0) for t in tokens], axis=1)
        return _dot_nt(pick.astype(bf16), blocks)

    def dft(rows):
        z = _dot(jnp.concatenate([pltpu.bitcast(r, bf16) for r in rows], axis=0),
                 pltpu.bitcast(dft_v[...], bf16))
        return [[(z[o:o + 8, :_T], z[o:o + 8, _T:])
                 for o in range(h // 2 * 16 * _NB + 8 * (h % 2), (h // 2 + 1) * 16 * _NB, 16)]
                for h in range(2 * len(rows) // _NB)]

    def modes(step):
        for u in range(_GA):
            grp = step * _GA + u
            rows = _ds(grp * 8, 8, 8)
            par = [_even_odd(dt_v[rows, :])] + [_even_odd(par_v[n, rows, :]) for n in range(6)]
            k0 = []
            for h, skip in enumerate(_even_odd(skip_v[rows, :])):
                z = _modes(*[p[h] for p in par])
                for n in range(4):
                    mode_v[u, h, n] = z[n]
                k0.append(skip + jnp.sum(z[0], axis=1, keepdims=True))
            k0_v[grp] = _interleave(*k0)

    def spread(step, u, slot):
        for j, blk in _lag_blocks(lambda n: tap_v[u, n], k0_v[step * _GA + u]):
            k_v[slot, j] = blk

    def filter_spectra(grp, slots):
        for h, blocks in enumerate(dft([k_v[slot, j] for slot in slots for j in range(_NB)])):
            for j, (re, im) in enumerate(blocks):
                for plane, val in enumerate((re, re + im, im - re)):
                    kf_v[2 * grp + h, plane * _PLANE + j] = val

    def filter_step(i, zero):
        for u in range(_GA):
            if u % (_GA // 2) == 0:
                old = (u + _GA // 2) % _GA
                filter_spectra(jnp.maximum(i - (1 if u else 2), 0) * _GA + old,
                               [old + k + zero for k in range(_GA // 2)])
            spread(jnp.maximum(i - 1, 0), u, u)
            even, odd = [[_vandermonde(*seeds) for seeds in _seeds(
                (mode_v[u, h, 0], mode_v[u, h, 1]), (mode_v[u, h, 2], mode_v[u, h, 3]))]
                         for h in range(2)]
            for n, tap in enumerate(_unmix(*map(_interleave, even, odd))):
                tap_v[u, n] = tap
            yield u

    def hidden_jobs(c):
        width = _F // (_NCH - _NO)
        pre = []

        def project(n):
            cols = _ds(c * width + n // 2 * _T, _T, _T)
            x_sel = jnp.concatenate(
                [pltpu.bitcast(arena[c >> 8, _ROW_SEL + k], bf16) for k in range(_KT)], axis=1)
            weight = pltpu.bitcast((wu_v if n % 2 else wg_v)[:, cols], bf16)
            pre.append(_rnd(_dot(x_sel[:, :_D], weight)[:8]))
            if n % 2:
                hid_v[:, cols] = (_rnd(_silu_of_twice(0.5 * pre[-2])) * pre[-1]).astype(bf16)

        return [(40 * n, lambda n=n: project(n)) for n in range(2 * width // _T)]

    def scatters(n, hid):
        y = _rnd(_dot_nt(jnp.concatenate(hid, axis=1), pltpu.bitcast(wd_v[n], bf16)))
        y = 0.5 * (sel_v[n] + _rnd(y * _rnd(jax.nn.sigmoid(routed_scores()))[:, :_OCH]))
        col = jnp.concatenate([y, jnp.zeros((_T - _C, _OCH), f32)], axis=0).T
        col = pltpu.bitcast(col.astype(bf16), i32)
        token = routed_tokens()

        def scatter(t):
            hit = ((token & (_T - 1)) == lane)[t:t + 1]
            new = jnp.broadcast_to(col[:, t:t + 1], (_OCH // 2, _T))
            where = [(n * (_OCH // (16 * _GC)) + g // _GC,
                      _ROW_X + (g % _GC) * _NB + (token[t, 0] >> 7)) for g in range(_OCH // 16)]
            old = [arena[at] for at in where]
            for g, at in enumerate(where):
                arena[at] = jnp.where(hit, new[8 * g:8 * g + 8], old[g])

        return [lambda t=t: scatter(t) for t in range(_C)]

    def finish(n):
        for k in range(0, _OCH // 16 * _NB, 2):
            c, r = n * (_OCH // (16 * _GC)) + k // _R, k % _R
            rows = _ds(n * _OCH + 16 * (k // _NB), 16, 16)
            out = []
            for d in range(2):
                gate = _silu_of_twice(pltpu.bitcast(arena[c, _ROW_X + r + d], bf16).astype(f32))
                out.append(xf_v[k % _NB + d, rows, :] + s_v[c, pl.ds(16 * (r + d), 16), :] * gate)
            o_v[rows, pl.ds(k % _NB * _T, 2 * _T)] = jnp.concatenate(out, axis=1).astype(bf16)
            yield k + 2

    def spare(t, zero=0):
        return _ds(_D + 8 * (t // _NB + zero), 8, 8), pl.ds(t % _NB * _T, _T)

    def first_output_jobs(c):
        hid, scatter = [], []

        def read():
            hid.extend([pltpu.bitcast(arena[c >> 8, _ROW_W + t], bf16)[:8]
                        for t in range(len(hid), len(hid) + 4)])

        return ([(48 * k, read) for k in range(_F // (4 * _T))]
                + [(431, lambda: scatter.extend(scatters(0, hid)))]
                + [(992 + 14 * t, lambda t=t: scatter[t]()) for t in range(_C)])

    def output_jobs(c):
        n = c - (_NCH - _NO)
        hid = [o_v[spare(t, c >> 8)] for t in range(4)]
        for done in finish(n - 1):
            if done == _OCH // 16 * _NB:
                pl.when(n >= _OUT_STEP)(lambda: out_copy(n - 1).start())
                o_v[spare(_F // _T, c >> 9)] = hid[0]
            if done % 12 == 0:
                hid += [o_v[spare(t, c >> 8)] for t in range(len(hid), len(hid) + 4)]
        return [(560 + 14 * t, job) for t, job in enumerate(scatters(n, hid))]

    def input_spectra(rows, dst):
        z = dft(rows)
        for h, blocks in enumerate(z):
            for b, (re, im) in enumerate(blocks):
                if b:
                    re, im = re + blocks[b - 1][1], im - blocks[b - 1][0]
                for plane, val in enumerate((re + im, im, re)):
                    dst[(h * 3 + plane) * _PLANE + b] = val
        return z

    def output_spectrum(c, r):
        return jnp.concatenate(
            [pltpu.bitcast(arena[c, pl.ds(_ROW_W + q * _WQ + 2 * r, 2)].reshape(16, _T), f32)
             for q in range(2)], axis=1)

    def conv_step(c, cur, nxt, ffn_jobs, delay, pace):
        c_next, c_prev = jnp.minimum(c + 1, _NCH - 1), jnp.maximum(c - 1, 0)
        zero = c >> 8
        fwd_rows, inv_rows, results = [], [], []

        def transform():
            y = _dot(jnp.concatenate(inv_rows, axis=0), inv_v[...])
            s_v[c_prev] = y
            results.extend((y, input_spectra(fwd_rows, nxt)))

        def drain(r):
            y, z = results
            arena[c, _ROW_SEL - 1] = pltpu.bitcast(
                y[8 * r:8 * r + 8] + z[2 * (r // _R) + 1][r % _R // 2][r // 8 % 2], i32)

        jobs = sorted(
            ffn_jobs(c)
            + [(delay + 16 * r, lambda r=r: inv_rows.append(output_spectrum(c_prev, r)))
               for r in range(_R)]
            + [(delay + 16 * r, lambda r=r: fwd_rows.append(arena[c_next, _ROW_X + r]))
               for r in range(_R)]
            + [(delay + 16 * _R, transform)]
            + [(delay + 140 + 8 * r, lambda r=r: drain(r)) for r in range(2 * _R - 17, 2 * _R, 8)],
            key=lambda job: job[0])

        def run_jobs(done):
            while jobs and done * (delay + 16 * _R) >= (jobs[0][0] - 32) * pace * 18 * _GC:
                jobs.pop(0)[1]()

        run_jobs(0)
        for h in range(2 * _GC):
            for part in range(3):
                for plane in range(3):
                    kf = lambda b: kf_v[c * 2 * _GC + h + (zero >> part), plane * _PLANE + b]
                    uf = lambda b: cur[(zero >> part) + (h * 3 + plane) * _PLANE + b]
                    base = [pltpu.bitcast(arena[c + zero, _ROW_P + plane * 8 + m], f32)
                            for m in range(_NB // 2) if part and plane]
                    k, u, out = [], [], []
                    for m in range(_NB // 2):
                        if part == 0:
                            k.append(kf(2 * m))
                            u.append(uf(2 * m) + uf(2 * m + 1))
                        elif part == 1:
                            k.append(kf(2 * m) - kf(2 * m - 1) if m else kf(0))
                            u.append(uf(2 * m + 1))
                        else:
                            k.append(kf(2 * m) - kf(2 * m + 1))
                            u.append(uf(2 * m))
                        y = k[0] * u[m]
                        for j in range(1, m + 1):
                            y = y + k[j] * u[m - j]
                        if plane:
                            y = shared[m] - y if plane == 1 else shared[m] + y
                        out.append(y)
                        if base:
                            r = (h // 2 * _NB + 2 * m + part - 1) * 2 + h % 2
                            arena[c, _ROW_W + (plane - 1) * _WQ + r] = pltpu.bitcast(base[m] - y, i32)
                        else:
                            arena[c, _ROW_P + plane * 8 + m] = pltpu.bitcast(y, i32)
                    if plane == 0:
                        shared = out
                    run_jobs((h * 3 + part) * 3 + plane + 1)
        run_jobs(np.inf)

    start("vectors", ldt_hbm, ldt_v)
    start("vectors", dsk_hbm, dsk_v)
    start_parameters("step 0", pl.ds(0, 8 * _GA))
    start_parameters("step 1", pl.ds(8 * _GA, 8 * _GA))
    start("step 1", dft_hbm, dft_v)
    arena[0, _ROW_W:_ROW_P] = jnp.zeros((_ROW_P - _ROW_W, 8, _T), i32)
    tap_v[...] = jnp.zeros(tap_v.shape, i32)
    k_v[:_GA] = jnp.zeros((_GA, _NB, 8, _T), i32)
    key_v[...] = jnp.zeros(key_v.shape, f32)
    wait("vectors")
    start_parameters("later steps", pl.ds(16 * _GA, _D // 2 - 16 * _GA))
    start("input", x_hbm.bitcast(i32), x_v)
    start("input", wr_hbm, wr_v)
    dt = jnp.exp(ldt_v[...].astype(f32)).reshape(1, _D)
    skip = dsk_v[...].astype(f32).reshape(1, _D)
    dt_v[:_T // 2] = _column(dt[:, :_T])
    skip_v[:_T // 2] = _column(skip[:, :_T])
    wait("step 0")
    modes(0)
    dt_v[_T // 2:] = _column(dt[:, _T:])
    skip_v[_T // 2:] = _column(skip[:, _T:])
    wait("step 1")

    def filter_loop(i, carry):
        @pl.when(i == 1)
        def _():
            wait("later steps")
            for cp in hidden_copies(0):
                cp.start()

        @pl.when(i == _LN_STEP)
        def _():
            wait("input")
            for cp in hidden_copies(1):
                cp.start()
            layer_norm()
            inv_v[...] = pltpu.bitcast(dft_v[...], bf16).astype(f32).T * (2 / _T)

        for t in range(2):
            pop_best(2 * (i - _LN_STEP) + t)
        list(filter_step(i, i >> 8))
        modes(i + 1)

    last = _NG // _GA - 1
    assert 2 * (last - _LN_STEP) == _C
    lax.fori_loop(0, last, filter_loop, None)
    for cp in hidden_copies(2):
        cp.start()
    zero = routed_tokens()[0, 0] >> 11
    parts = [gather(range(u * _C // _GA, (u + 1) * _C // _GA)) for u in filter_step(last, zero)]
    x_sel = sum(parts[1:], parts[0])
    for n in range(_NO):
        sel_v[n] = x_sel[:, n * _OCH:(n + 1) * _OCH]
    x_sel = jnp.concatenate([x_sel, jnp.zeros((8, _KT * _T - _D), f32)], axis=1)
    for k in range(_KT):
        arena[0, _ROW_SEL + k] = pltpu.bitcast(
            jnp.concatenate([x_sel[:, k * _T:(k + 1) * _T]] * 2, axis=0).astype(bf16), i32)
    input_spectra([arena[0, _ROW_X + r] for r in range(_R)], uf_a)
    for u in range(_GA):
        spread(last, u, _GA + u)
    filter_spectra(_NG - 3 * _GA // 2, range(_GA // 2, 2 * _GA))

    def hidden_loop(slab, carry):
        for cp in hidden_copies(slab):
            cp.wait()

        @pl.when(slab == 1)
        def _():
            for n in range(_NO):
                down_copy(n).start()

        def pair(i, carry):
            conv_step(2 * i, uf_a, uf_b, hidden_jobs, 240, 0.87)
            conv_step(2 * i + 1, uf_b, uf_a, hidden_jobs, 240, 0.87)

        pairs = (_NCH - _NO) // (2 * _NF)
        lax.fori_loop(slab * pairs, (slab + 1) * pairs, pair, None)

    def output_loop(n, carry):
        down_copy(n).wait()

        @pl.when(n == _OUT_STEP)
        def _():
            for k in range(_OUT_STEP - 1):
                out_copy(k).start()

        c = n + _NCH - _NO
        lax.cond(c & 1 == 0, lambda: conv_step(c, uf_a, uf_b, output_jobs, 32, 0.8),
                 lambda: conv_step(c, uf_b, uf_a, output_jobs, 32, 0.8))

    lax.fori_loop(0, _NF, hidden_loop, None)
    for t in range(_F // _T):
        tile = hid_v[:, t * _T:(t + 1) * _T]
        o_v[spare(t)] = tile
        arena[0, _ROW_W + t] = pltpu.bitcast(jnp.concatenate([tile] * 2, axis=0), i32)
    down_copy(0).wait()
    conv_step(_NCH - _NO + zero, uf_a, uf_b, first_output_jobs, 432, 0.87)
    lax.fori_loop(1, _NO, output_loop, None)
    s_v[_NCH - 1] = _dot(
        jnp.concatenate([output_spectrum(_NCH - 1, r) for r in range(_R)], axis=0), inv_v[...])
    for done in finish(_NO - 1):
        if done % _R == 0:
            rows = pl.ds((_NO - 1) * _OCH + (done // _R - 1) * 16 * _GC, 16 * _GC)
            start("last slab", o_v.at[rows], o_hbm.at[rows])
    for n in range(_NO - 1):
        out_copy(n).wait()
    wait("last slab")


@jax.jit
def pallas_recurrent_scan__ssm_conv_s4__moe_arch_mod__prompt_kernel(
    A_u: jax.Array,
    A_A_re: jax.Array,
    A_A_im: jax.Array,
    A_B_re: jax.Array,
    A_B_im: jax.Array,
    A_C_re: jax.Array,
    A_C_im: jax.Array,
    A_log_dt: jax.Array,
    A_Dskip: jax.Array,
    B_x: jax.Array,
    B_w_r: jax.Array,
    B_w_gate: jax.Array,
    B_w_up: jax.Array,
    B_w_down: jax.Array,
):
    del B_x
    assert A_u.shape == (1, _L, _D) and A_A_re.shape == (_D, _N) and B_w_gate.shape == (_D, _F)
    assert A_u.dtype == bf16 and A_A_re.dtype == bf16
    hbm = pl.BlockSpec(memory_space=pl.ANY)
    vmem = pltpu.VMEM
    out = pl.pallas_call(
        _kernel,
        out_shape=jax.ShapeDtypeStruct((_D, _L), bf16),
        in_specs=[hbm] * 14,
        out_specs=hbm,
        scratch_shapes=[
            vmem((_D // 2, _L), i32), vmem((6, _D // 2, _N), i32),
            vmem((_D,), bf16), vmem((_D,), bf16), vmem((_D,), bf16),
            vmem((_D // 2, _F), i32), vmem((_D // 2, _F), i32), vmem((_NO, _OCH // 2, _F), i32),
            vmem((_T // 2, 2 * _T), i32), vmem((_D + 32, _L), bf16),
            vmem((_D // 2, _T), i32), vmem((_D // 2, _T), i32), vmem((_GA, 2, 4, 8, _N), f32),
            vmem((_NG, 8, _T), i32), vmem((_GA, len(_TAPS), 8, _T), i32),
            vmem((2 * _GA, _NB, 8, _T), i32), vmem((2 * _NG, 3 * _PLANE, 8, _T), f32),
            vmem((_NB, _D + 8, _T), f32), vmem((3, _NB, 8, _T), f32), vmem((3, 8, _T), f32),
            vmem((_NO, 8, _OCH), f32), vmem((8, _F), bf16),
            vmem((2 * _T, _T), f32), vmem((_NCH, _ROWS, 8, _T), i32),
            vmem((6 * _GC * _PLANE, 8, _T), f32), vmem((6 * _GC * _PLANE, 8, _T), f32),
            vmem((_NCH, 16 * _R, _T), f32),
            pltpu.SemaphoreType.DMA((6,)), pltpu.SemaphoreType.DMA((_NF + _NO,)),
            pltpu.SemaphoreType.DMA(()),
        ],
        compiler_params=pltpu.CompilerParams(vmem_limit_bytes=100 * 2**20),
    )(A_u.reshape(_L, _D).T, A_A_re, A_A_im, A_B_re, A_B_im, A_C_re, A_C_im, A_log_dt, A_Dskip,
      B_w_r, B_w_gate, B_w_up, B_w_down.T, _DFT)
    return out.T.reshape(1, _L, _D)
```

```python
import jax
import jax.numpy as jnp
import numpy as np
from jax import lax
import jax.experimental.pallas as pl
import jax.experimental.pallas.tpu as pltpu

f32, bf16, i32 = jnp.float32, jnp.bfloat16, jnp.int32

_D, _L, _N, _F, _C = 576, 2048, 128, 4608, 8
_EPS = 1e-5
_T = 128
_NB = _L // _T
_NG = _D // 16
_GA = 4
_GC = 2
_NCH = _NG // _GC
_R = _GC * _NB
_KT = -(-_D // _T)
_NF = 3
_NO, _OCH = 6, _D // 6
_LN_STEP = 4
_OUT_STEP = 3
_ROW_X, _ROW_W, _WQ, _ROW_SEL, _ROW_P = 0, _R, 2 * _R + 1, 5 * _R + 3, 5 * _R + 8
_ROWS = _ROW_P + 3 * _NB // 2
_PLANE = _NB + 1
_XP = 32


def _dft_words():
    theta = (np.pi / 2 + 2 * np.pi * np.arange(_T)) / _T
    angle = np.arange(_T)[:, None] * theta[None, :]
    matrix = np.concatenate([np.cos(angle), np.sin(angle)], axis=1)
    bits = matrix.astype(bf16).view(np.uint16).astype(np.uint32)
    return (bits[0::2] | bits[1::2] << 16).view(np.int32)


_DFT = _dft_words()


def _lag_step(j):
    return max(1, (1 << (j * _T).bit_length()) >> 8)


def _round_lag(p, step):
    if step == 1:
        return p
    return (p + (step // 2 - 1) + ((p >> (step.bit_length() - 1)) & 1)) & ~(step - 1)


assert np.array_equal(
    np.concatenate([j * _T + _round_lag(np.arange(_T), _lag_step(j)) for j in range(_NB)]),
    np.arange(_L).astype(bf16).astype(np.int64))

_PAIRS = (((0, 1), (0, 5)), ((0, 2), (0, 6)), ((0, 3), (0, 7)), ((0, 4), (0, 8)), ((1, 2), (1, 6)),
          ((1, 4), (1, 8)), ((2, 4), (2, 8)), ((3, 4), (3, 8)), ((4, 8), (5, 8)), ((6, 8), (7, 8)))
_TAPS = [k for pair in _PAIRS for k in pair]


def _ds(start, size, align):
    return pl.ds(start if isinstance(start, int) else pl.multiple_of(start, align), size)


def _cmul(a, b):
    return a[0] * b[0] - a[1] * b[1], a[0] * b[1] + a[1] * b[0]


def _csq(a):
    return a[0] * a[0] - a[1] * a[1], (a[0] + a[0]) * a[1]


def _silu_of_twice(h):
    return h + h * jnp.tanh(h)


def _rnd(x):
    return x.astype(bf16).astype(f32)


def _dot(a, b):
    return jnp.dot(a, b, preferred_element_type=f32)


def _dot_nt(a, b):
    return lax.dot_general(a, b, (((1,), (1,)), ((), ())), preferred_element_type=f32)


def _column(v):
    return pltpu.bitcast(jnp.broadcast_to(v, (_T, v.shape[1])).astype(bf16).T, i32)


def _even_odd(words):
    return pltpu.bitcast(words << 16, f32), pltpu.bitcast(words & -65536, f32)


def _interleave(even, odd):
    even, odd = [pltpu.bitcast(x, i32) + 0x8000 for x in (even, odd)]
    return lax.shift_right_logical(even, 16) | (odd & -65536)


def _modes(dt, ar, ai, br, bi, cr, ci):
    zr, zi = dt * ar, dt * ai
    mag = jnp.exp(zr)
    return _cmul((cr, ci), (dt * br, dt * bi)) + (mag * jnp.cos(zi), mag * jnp.sin(zi))


def _seeds(w, a1):
    a = {1: a1}
    for n in range(9):
        a[2 << n] = _csq(a[1 << n])
    row = lax.broadcasted_iota(i32, (8, _N), 0)

    def mix(z0, z1):
        rolled = [pltpu.roll(x, 4, 0) for x in z1]
        return ([jnp.where(row < 4, x, y) for x, y in zip(z0, rolled)],
                [jnp.where(row < 4, y, x) for x, y in zip(z0, rolled)])

    def dup(z):
        return [[jnp.take_along_axis(x, (row & 3) + 4 * q, axis=0, mode="promise_in_bounds")
                 for x in z] for q in range(2)]

    wa = _cmul(w, a1)
    return zip(mix((1.0, 0.0), a[128]), dup(a[8]), dup(a[32]),
               mix(wa, _cmul(wa, a[4])), dup(a1), dup(a[256]),
               mix(_cmul(a[256], a[4]), a[512]), dup(a[512]))


def _vandermonde(e0, m8, m32, g0, m1, m256, m_top, m512):
    e = [e0]
    for s in range(1, 16):
        e.append(_cmul(e[s - 1], m8) if s < 4 else _cmul(e[s - 4], m32))
    g = [g0]
    for _ in range(3):
        g.append(_cmul(g[-1], m1))
    g += [_cmul(g[1], m256), _cmul(g[3], m256)]
    g += [_cmul(g[3], m512), _cmul(g[5], m512)]
    g.append(_cmul(g[7], m_top))
    g.append(_cmul(g[8], m512))
    re, im = [_dot_nt(jnp.concatenate([z[p] for z in g], axis=0),
                      jnp.concatenate([z[p] for z in e], axis=0)) for p in range(2)]
    return re - im


def _unmix(lo, hi):
    row = lax.broadcasted_iota(i32, (8, _T), 0)
    for m in range(len(_PAIRS)):
        x, y = lo[8 * m:8 * m + 8], hi[8 * m:8 * m + 8]
        yield jnp.where(row < 4, x, y)
        yield pltpu.roll(jnp.where(row < 4, y, x), 4, 0)


def _lag_blocks(tap, lag0):
    lane = lax.broadcasted_iota(i32, (8, _T), 1)
    row = lax.broadcasted_iota(i32, (8, _T), 0)
    for h in range(2):
        def take(big, r, lag):
            s = ((_T * h + lag) >> 3) & 31
            return jnp.take_along_axis(tap(_TAPS.index((big, r))),
                                       ((s & 15) << 3) + (row ^ ((s >> 4) << 2)),
                                       axis=1, mode="promise_in_bounds")

        top = [take(big, 8, _round_lag(lane, 8) - 8) for big in range(_NB // 2)]
        for big, blk in enumerate(top):
            step = _lag_step(2 * big + h)
            lag = _round_lag(lane, step)
            if h == 0:
                blk = jnp.where(lag == 0, top[big - 1] if big else lag0, blk)
            for r in range(step, 8, step):
                blk = jnp.where((lag & 7) == r, take(big, r, lane), blk)
            yield 2 * big + h, blk


def _kernel(x_hbm, ar_hbm, ai_hbm, br_hbm, bi_hbm, cr_hbm, ci_hbm, ldt_hbm, dsk_hbm, wr_hbm,
            wg_hbm, wu_hbm, wd_hbm, dft_hbm, o_hbm,
            x_v, par_v, wg_v, wu_v, wd_v, dft_v, o_v,
            dt_v, skip_v, mode_v, k0_v, tap_v, k_v, kf_v,
            xf_v, inv_v, arena, uf_a, uf_b, s_v,
            stat_v, key_v, sel_v, hid_v, ldt_v, dsk_v, wr_v, sem, w_sem, o_sem):
    row = lax.broadcasted_iota(i32, (8, _T), 0)
    lane = lax.broadcasted_iota(i32, (8, _T), 1)

    groups = {}

    def start(name, src, dst):
        slot, pairs = groups.setdefault(name, (len(groups), []))
        pairs.append((src, dst))
        pltpu.make_async_copy(src, dst, sem.at[slot]).start()

    def wait(name):
        slot, pairs = groups[name]
        for src, dst in pairs:
            pltpu.make_async_copy(src, dst, sem.at[slot]).wait()

    def start_parameters(name, rows):
        for n, src in enumerate((ar_hbm, ai_hbm, br_hbm, bi_hbm, cr_hbm, ci_hbm)):
            start(name, src.bitcast(i32).at[rows], par_v.at[n, rows])

    def hidden_copies(n):
        cols = _ds(n * (_F // _NF), _F // _NF, _F // _NF)
        return [pltpu.make_async_copy(w.bitcast(i32).at[:, cols], v.at[:, cols], w_sem.at[n])
                for w, v in ((wg_hbm, wg_v), (wu_hbm, wu_v))]

    def down_copy(n):
        return pltpu.make_async_copy(wd_hbm.bitcast(i32).at[_ds(n * (_OCH // 2), _OCH // 2, 16)],
                                     wd_v.at[n], w_sem.at[_NF + n])

    def out_copy(n):
        rows = _ds(n * _OCH, _OCH, 32)
        return pltpu.make_async_copy(o_v.at[rows], o_hbm.at[rows], o_sem)

    def compact(k, h):
        out = stat_v[k, 8 * h]
        for s in range(1, 8):
            out = jnp.where(row == s, stat_v[k, 8 * h + s], out)
        return out

    def layer_norm():
        def moments(b, carry):
            cols = _ds(b * _T, _T, _T)
            pivot = jnp.broadcast_to(_even_odd(x_v[:8, cols])[0][:1], (8, _T))
            s1, s2 = [None] * 2, [None] * 2
            for g in range(_NG):
                x = pltpu.bitcast(x_v[pl.ds(8 * g, 8), cols], bf16).astype(f32)
                xf_v[b, pl.ds(16 * g, 16), :] = x
                for h in range(2):
                    d = x[8 * h:8 * h + 8] - pivot
                    s1[h] = s1[h] + d if g else d
                    s2[h] = s2[h] + d * d if g else d * d
            for k, s in enumerate((s1, s2)):
                stat_v[k, b] = jnp.broadcast_to(jnp.sum(s[0] + s[1], axis=0, keepdims=True), (8, _T))
            stat_v[2, b] = pivot

        lax.fori_loop(0, _NB, moments, None, unroll=4)
        for h in range(_NB // 8):
            m1, m2 = compact(0, h) / _D, compact(1, h) / _D
            mean = _rnd(compact(2, h) + m1)
            var = _rnd(jnp.maximum(m2 - m1 * m1, 0.0))
            gain = 0.5 / _rnd(jnp.sqrt(_rnd(var + _rnd(jnp.full_like(var, _EPS)))))
            for s in range(8):
                stat_v[0, 8 * h + s] = jnp.broadcast_to(mean[s:s + 1], (8, _T))
                stat_v[1, 8 * h + s] = jnp.broadcast_to(gain[s:s + 1], (8, _T))
        wr = jnp.broadcast_to(wr_v[...].astype(f32).reshape(1, _D), (8, _D)).astype(bf16)
        for b in range(_NB):
            mean, gain = stat_v[0, b], stat_v[1, b]
            xn = [_interleave(*[(xf_v[b, pl.ds(16 * g + h, 8, stride=2), :] - mean) * gain
                                for h in range(2)]) for g in range(_NG)]
            for g in range(_NG):
                arena[g // _GC, _ROW_X + (g % _GC) * _NB + b] = xn[g]
            stat_v[2, b] = _dot(wr, pltpu.bitcast(jnp.concatenate(xn, axis=0), bf16))
        for h in range(_NB // 8):
            bits = pltpu.bitcast(_rnd(2.0 * compact(2, h)), i32) >> 16
            rank = jnp.where(bits < 0, 0x8000 - (bits & 0x7FFF), 0x8000 + bits)
            token = (8 * h + row) * _T + lane
            key_v[h] = pltpu.bitcast((1 << 28) + rank * _L + (_L - 1 - token), f32)

    def pop_best(t):
        best = jnp.max(jnp.max(jnp.maximum(key_v[0], key_v[1]), axis=0, keepdims=True),
                       axis=1, keepdims=True)
        key_v[2] = jnp.where(row == t, best, key_v[2])
        for h in range(2):
            key_v[h] = jnp.where(key_v[h] == best, 0.0, key_v[h])

    def routed_tokens():
        return _L - 1 - (pltpu.bitcast(key_v[2], i32) & (_L - 1))

    def routed_scores():
        rank = (pltpu.bitcast(key_v[2], i32) - (1 << 28)) >> 11
        return pltpu.bitcast(jnp.where(rank < 0x8000, 0x10000 - rank, rank - 0x8000) << 16, f32)

    def gather(tokens):
        token = routed_tokens()
        blocks = jnp.concatenate(
            [pltpu.bitcast(jnp.concatenate(
                [arena[g // _GC, _ROW_X + (g % _GC) * _NB + (token[t, 0] >> 7)]
                 for g in range(_NG)], axis=0), bf16) for t in tokens], axis=1)
        pick = jnp.concatenate(
            [jnp.where((row == t) & ((token & (_T - 1)) == lane), 2.0, 0.0) for t in tokens], axis=1)
        return _dot_nt(pick.astype(bf16), blocks)

    def dft(rows):
        z = _dot(jnp.concatenate([pltpu.bitcast(r, bf16) for r in rows], axis=0),
                 pltpu.bitcast(dft_v[...], bf16))
        return [[(z[o:o + 8, :_T], z[o:o + 8, _T:])
                 for o in range(h // 2 * 16 * _NB + 8 * (h % 2), (h // 2 + 1) * 16 * _NB, 16)]
                for h in range(2 * len(rows) // _NB)]

    def modes(step):
        for u in range(_GA):
            grp = step * _GA + u
            rows = _ds(grp * 8, 8, 8)
            par = [_even_odd(dt_v[rows, :])] + [_even_odd(par_v[n, rows, :]) for n in range(6)]
            k0 = []
            for h, skip in enumerate(_even_odd(skip_v[rows, :])):
                z = _modes(*[p[h] for p in par])
                for n in range(4):
                    mode_v[u, h, n] = z[n]
                k0.append(skip + jnp.sum(z[0], axis=1, keepdims=True))
            k0_v[grp] = _interleave(*k0)

    def spread(step, u, slot):
        for j, blk in _lag_blocks(lambda n: tap_v[u, n], k0_v[step * _GA + u]):
            k_v[slot, j] = blk

    def filter_spectra(grp, slots):
        for h, blocks in enumerate(dft([k_v[slot, j] for slot in slots for j in range(_NB)])):
            for j, (re, im) in enumerate(blocks):
                for plane, val in enumerate((re, re + im, im - re)):
                    kf_v[2 * grp + h, plane * _PLANE + j] = val

    def filter_step(i, zero):
        for u in range(_GA):
            if u % (_GA // 2) == 0:
                old = (u + _GA // 2) % _GA
                filter_spectra(jnp.maximum(i - (1 if u else 2), 0) * _GA + old,
                               [old + k + zero for k in range(_GA // 2)])
            spread(jnp.maximum(i - 1, 0), u, u)
            even, odd = [[_vandermonde(*seeds) for seeds in _seeds(
                (mode_v[u, h, 0], mode_v[u, h, 1]), (mode_v[u, h, 2], mode_v[u, h, 3]))]
                         for h in range(2)]
            for n, tap in enumerate(_unmix(*map(_interleave, even, odd))):
                tap_v[u, n] = tap
            yield u

    def hidden_jobs(c):
        width = _F // (_NCH - _NO)
        pre = []

        def project(n):
            cols = _ds(c * width + n // 2 * _T, _T, _T)
            x_sel = jnp.concatenate(
                [pltpu.bitcast(arena[c >> 8, _ROW_SEL + k], bf16) for k in range(_KT)], axis=1)
            weight = pltpu.bitcast((wu_v if n % 2 else wg_v)[:, cols], bf16)
            pre.append(_rnd(_dot(x_sel[:, :_D], weight)[:8]))
            if n % 2:
                hid_v[:, cols] = (_rnd(_silu_of_twice(0.5 * pre[-2])) * pre[-1]).astype(bf16)

        return [(40 * n, lambda n=n: project(n)) for n in range(2 * width // _T)]

    def scatters(n, hid):
        y = _rnd(_dot_nt(jnp.concatenate(hid, axis=1), pltpu.bitcast(wd_v[n], bf16)))
        y = 0.5 * (sel_v[n] + _rnd(y * _rnd(jax.nn.sigmoid(routed_scores()))[:, :_OCH]))
        col = jnp.concatenate([y, jnp.zeros((_T - _C, _OCH), f32)], axis=0).T
        col = pltpu.bitcast(col.astype(bf16), i32)
        token = routed_tokens()

        def scatter(t):
            hit = ((token & (_T - 1)) == lane)[t:t + 1]
            new = jnp.broadcast_to(col[:, t:t + 1], (_OCH // 2, _T))
            where = [(n * (_OCH // (16 * _GC)) + g // _GC,
                      _ROW_X + (g % _GC) * _NB + (token[t, 0] >> 7)) for g in range(_OCH // 16)]
            old = [arena[at] for at in where]
            for g, at in enumerate(where):
                arena[at] = jnp.where(hit, new[8 * g:8 * g + 8], old[g])

        return [lambda t=t: scatter(t) for t in range(_C)]

    def finish(n):
        for k in range(0, _OCH // 16 * _NB, 2):
            c, r = n * (_OCH // (16 * _GC)) + k // _R, k % _R
            rows = _ds(n * _OCH + 16 * (k // _NB), 16, 16)
            out = []
            for d in range(2):
                gate = _silu_of_twice(pltpu.bitcast(arena[c, _ROW_X + r + d], bf16).astype(f32))
                out.append(xf_v[k % _NB + d, rows, :] + s_v[c, pl.ds(16 * (r + d), 16), :] * gate)
            o_v[rows, pl.ds(k % _NB * _T, 2 * _T)] = jnp.concatenate(out, axis=1).astype(bf16)
            yield k + 2

    def spare(t, zero=0):
        return _ds(_D + 8 * (t // _NB + zero), 8, 8), pl.ds(t % _NB * _T, _T)

    def first_output_jobs(c):
        hid, scatter = [], []

        def read():
            hid.extend([pltpu.bitcast(arena[c >> 8, _ROW_W + t], bf16)[:8]
                        for t in range(len(hid), len(hid) + 4)])

        return ([(48 * k, read) for k in range(_F // (4 * _T))]
                + [(431, lambda: scatter.extend(scatters(0, hid)))]
                + [(992 + 14 * t, lambda t=t: scatter[t]()) for t in range(_C)])

    def output_jobs(c):
        n = c - (_NCH - _NO)
        hid = [o_v[spare(t, c >> 8)] for t in range(4)]
        for done in finish(n - 1):
            if done == _OCH // 16 * _NB:
                pl.when(n >= _OUT_STEP)(lambda: out_copy(n - 1).start())
                o_v[spare(_F // _T, c >> 9)] = hid[0]
            if done % 12 == 0:
                hid += [o_v[spare(t, c >> 8)] for t in range(len(hid), len(hid) + 4)]
        return [(560 + 14 * t, job) for t, job in enumerate(scatters(n, hid))]

    def input_spectra(rows, dst):
        z = dft(rows)
        for h, blocks in enumerate(z):
            for b, (re, im) in enumerate(blocks):
                if b:
                    re, im = re + blocks[b - 1][1], im - blocks[b - 1][0]
                for plane, val in enumerate((re + im, im, re)):
                    dst[(h * 3 + plane) * _PLANE + b] = val
        return z

    def output_spectrum(c, r):
        return jnp.concatenate(
            [pltpu.bitcast(arena[c, pl.ds(_ROW_W + q * _WQ + 2 * r, 2)].reshape(16, _T), f32)
             for q in range(2)], axis=1)

    def conv_step(c, cur, nxt, ffn_jobs, delay, pace):
        c_next, c_prev = jnp.minimum(c + 1, _NCH - 1), jnp.maximum(c - 1, 0)
        zero = c >> 8
        fwd_rows, inv_rows, results = [], [], []

        def transform():
            y = _dot(jnp.concatenate(inv_rows, axis=0), inv_v[...])
            s_v[c_prev] = y
            results.extend((y, input_spectra(fwd_rows, nxt)))

        def drain(r):
            y, z = results
            arena[c, _ROW_SEL - 1] = pltpu.bitcast(
                y[8 * r:8 * r + 8] + z[2 * (r // _R) + 1][r % _R // 2][r // 8 % 2], i32)

        jobs = sorted(
            ffn_jobs(c)
            + [(delay + 16 * r, lambda r=r: inv_rows.append(output_spectrum(c_prev, r)))
               for r in range(_R)]
            + [(delay + 16 * r, lambda r=r: fwd_rows.append(arena[c_next, _ROW_X + r]))
               for r in range(_R)]
            + [(delay + 16 * _R, transform)]
            + [(delay + 140 + 8 * r, lambda r=r: drain(r)) for r in range(2 * _R - 17, 2 * _R, 8)],
            key=lambda job: job[0])

        def run_jobs(done):
            while jobs and done * (delay + 16 * _R) >= (jobs[0][0] - 32) * pace * 18 * _GC:
                jobs.pop(0)[1]()

        run_jobs(0)
        for h in range(2 * _GC):
            for part in range(3):
                for plane in range(3):
                    kf = lambda b: kf_v[c * 2 * _GC + h + (zero >> part), plane * _PLANE + b]
                    uf = lambda b: cur[(zero >> part) + (h * 3 + plane) * _PLANE + b]
                    base = [pltpu.bitcast(arena[c + zero, _ROW_P + plane * 8 + m], f32)
                            for m in range(_NB // 2) if part and plane]
                    k, u, out = [], [], []
                    for m in range(_NB // 2):
                        if part == 0:
                            k.append(kf(2 * m))
                            u.append(uf(2 * m) + uf(2 * m + 1))
                        elif part == 1:
                            k.append(kf(2 * m) - kf(2 * m - 1) if m else kf(0))
                            u.append(uf(2 * m + 1))
                        else:
                            k.append(kf(2 * m) - kf(2 * m + 1))
                            u.append(uf(2 * m))
                        y = k[0] * u[m]
                        for j in range(1, m + 1):
                            y = y + k[j] * u[m - j]
                        if plane:
                            y = shared[m] - y if plane == 1 else shared[m] + y
                        out.append(y)
                        if base:
                            r = (h // 2 * _NB + 2 * m + part - 1) * 2 + h % 2
                            arena[c, _ROW_W + (plane - 1) * _WQ + r] = pltpu.bitcast(base[m] - y, i32)
                        else:
                            arena[c, _ROW_P + plane * 8 + m] = pltpu.bitcast(y, i32)
                    if plane == 0:
                        shared = out
                    run_jobs((h * 3 + part) * 3 + plane + 1)
        run_jobs(np.inf)

    start("vectors", ldt_hbm, ldt_v)
    start("vectors", dsk_hbm, dsk_v)
    start_parameters("step 0", pl.ds(0, 8 * _GA))
    start_parameters("step 1", pl.ds(8 * _GA, 8 * _GA))
    start("step 1", dft_hbm, dft_v)
    arena[0, _ROW_W:_ROW_P] = jnp.zeros((_ROW_P - _ROW_W, 8, _T), i32)
    tap_v[...] = jnp.zeros(tap_v.shape, i32)
    k_v[:_GA] = jnp.zeros((_GA, _NB, 8, _T), i32)
    key_v[...] = jnp.zeros(key_v.shape, f32)
    wait("vectors")
    start_parameters("later steps", pl.ds(16 * _GA, _D // 2 - 16 * _GA))
    start("input", x_hbm.bitcast(i32), x_v)
    start("input", wr_hbm, wr_v)
    dt = jnp.exp(ldt_v[...].astype(f32)).reshape(1, _D)
    skip = dsk_v[...].astype(f32).reshape(1, _D)
    dt_v[:_T // 2] = _column(dt[:, :_T])
    skip_v[:_T // 2] = _column(skip[:, :_T])
    wait("step 0")
    modes(0)
    dt_v[_T // 2:] = _column(dt[:, _T:])
    skip_v[_T // 2:] = _column(skip[:, _T:])
    wait("step 1")

    def filter_loop(i, carry):
        @pl.when(i == 1)
        def _():
            wait("later steps")
            for cp in hidden_copies(0):
                cp.start()

        @pl.when(i == _LN_STEP)
        def _():
            wait("input")
            for cp in hidden_copies(1):
                cp.start()
            layer_norm()
            inv_v[...] = pltpu.bitcast(dft_v[...], bf16).astype(f32).T * (2 / _T)

        for t in range(2):
            pop_best(2 * (i - _LN_STEP) + t)
        list(filter_step(i, i >> 8))
        modes(i + 1)

    last = _NG // _GA - 1
    assert 2 * (last - _LN_STEP) == _C
    lax.fori_loop(0, last, filter_loop, None)
    for cp in hidden_copies(2):
        cp.start()
    zero = routed_tokens()[0, 0] >> 11
    parts = [gather(range(u * _C // _GA, (u + 1) * _C // _GA)) for u in filter_step(last, zero)]
    x_sel = sum(parts[1:], parts[0])
    for n in range(_NO):
        sel_v[n] = x_sel[:, n * _OCH:(n + 1) * _OCH]
    x_sel = jnp.concatenate([x_sel, jnp.zeros((8, _KT * _T - _D), f32)], axis=1)
    for k in range(_KT):
        arena[0, _ROW_SEL + k] = pltpu.bitcast(
            jnp.concatenate([x_sel[:, k * _T:(k + 1) * _T]] * 2, axis=0).astype(bf16), i32)
    input_spectra([arena[0, _ROW_X + r] for r in range(_R)], uf_a)
    for u in range(_GA):
        spread(last, u, _GA + u)
    filter_spectra(_NG - 3 * _GA // 2, range(_GA // 2, 2 * _GA))

    def hidden_loop(slab, carry):
        for cp in hidden_copies(slab):
            cp.wait()

        @pl.when(slab == 1)
        def _():
            for n in range(_NO):
                down_copy(n).start()

        def pair(i, carry):
            conv_step(2 * i, uf_a, uf_b, hidden_jobs, 240, 0.87)
            conv_step(2 * i + 1, uf_b, uf_a, hidden_jobs, 240, 0.87)

        pairs = (_NCH - _NO) // (2 * _NF)
        lax.fori_loop(slab * pairs, (slab + 1) * pairs, pair, None)

    def output_loop(n, carry):
        down_copy(n).wait()

        @pl.when(n == _OUT_STEP)
        def _():
            for k in range(_OUT_STEP - 1):
                out_copy(k).start()

        c = n + _NCH - _NO
        lax.cond(c & 1 == 0, lambda: conv_step(c, uf_a, uf_b, output_jobs, 32, 0.8),
                 lambda: conv_step(c, uf_b, uf_a, output_jobs, 32, 0.8))

    lax.fori_loop(0, _NF, hidden_loop, None)
    for t in range(_F // _T):
        tile = hid_v[:, t * _T:(t + 1) * _T]
        o_v[spare(t)] = tile
        arena[0, _ROW_W + t] = pltpu.bitcast(jnp.concatenate([tile] * 2, axis=0), i32)
    down_copy(0).wait()
    conv_step(_NCH - _NO + zero, uf_a, uf_b, first_output_jobs, 432, 0.87)
    lax.fori_loop(1, _NO, output_loop, None)
    s_v[_NCH - 1] = _dot(
        jnp.concatenate([output_spectrum(_NCH - 1, r) for r in range(_R)], axis=0), inv_v[...])
    for done in finish(_NO - 1):
        if done % _R == 0:
            rows = pl.ds((_NO - 1) * _OCH + (done // _R - 1) * 16 * _GC, 16 * _GC)
            start("last slab", o_v.at[rows], o_hbm.at[rows])
    for n in range(_NO - 1):
        out_copy(n).wait()
    wait("last slab")


@jax.jit
def pallas_recurrent_scan__ssm_conv_s4__moe_arch_mod__prompt_kernel(
    A_u: jax.Array,
    A_A_re: jax.Array,
    A_A_im: jax.Array,
    A_B_re: jax.Array,
    A_B_im: jax.Array,
    A_C_re: jax.Array,
    A_C_im: jax.Array,
    A_log_dt: jax.Array,
    A_Dskip: jax.Array,
    B_x: jax.Array,
    B_w_r: jax.Array,
    B_w_gate: jax.Array,
    B_w_up: jax.Array,
    B_w_down: jax.Array,
):
    del B_x
    assert A_u.shape == (1, _L, _D) and A_A_re.shape == (_D, _N) and B_w_gate.shape == (_D, _F)
    assert A_u.dtype == bf16 and A_A_re.dtype == bf16
    hbm = pl.BlockSpec(memory_space=pl.ANY)
    vmem = pltpu.VMEM
    out = pl.pallas_call(
        _kernel,
        out_shape=jax.ShapeDtypeStruct((_D, _L), bf16),
        in_specs=[hbm] * 14,
        out_specs=hbm,
        scratch_shapes=[
            vmem((_D // 2, _L), i32), vmem((6, _D // 2, _N), i32),
            vmem((_D // 2, _F), i32), vmem((_D // 2, _F), i32), vmem((_NO, _OCH // 2, _F), i32),
            vmem((_T // 2, 2 * _T), i32), vmem((_D + 32, _L), bf16),
            vmem((_D // 2, _T), i32), vmem((_D // 2, _T), i32), vmem((_GA, 2, 4, 8, _N), f32),
            vmem((_NG, 8, _T), i32), vmem((_GA, len(_TAPS), 8, _T), i32),
            vmem((2 * _GA, _NB, 8, _T), i32), vmem((2 * _NG, 3 * _PLANE, 8, _T), f32),
            vmem((_NB, _D + _XP, _T), f32), vmem((2 * _T, _T), f32), vmem((_NCH, _ROWS, 8, _T), i32),
            vmem((6 * _GC * _PLANE, 8, _T), f32), vmem((6 * _GC * _PLANE, 8, _T), f32),
            vmem((_NCH, 16 * _R, _T), f32),
            vmem((3, _NB, 8, _T), f32), vmem((3, 8, _T), f32), vmem((_NO, 8, _OCH), f32),
            vmem((8, _F), bf16), vmem((_D,), bf16), vmem((_D,), bf16), vmem((_D,), bf16),
            pltpu.SemaphoreType.DMA((6,)), pltpu.SemaphoreType.DMA((_NF + _NO,)),
            pltpu.SemaphoreType.DMA(()),
        ],
        compiler_params=pltpu.CompilerParams(vmem_limit_bytes=100 * 2**20),
    )(A_u.reshape(_L, _D).T, A_A_re, A_A_im, A_B_re, A_B_im, A_C_re, A_C_im, A_log_dt, A_Dskip,
      B_w_r, B_w_gate, B_w_up, B_w_down.T, _DFT)
    return out.T.reshape(1, _L, _D)
```

```python
import jax
import jax.numpy as jnp
import numpy as np
from jax import lax
import jax.experimental.pallas as pl
import jax.experimental.pallas.tpu as pltpu

f32, bf16, i32 = jnp.float32, jnp.bfloat16, jnp.int32

_D, _L, _N, _F, _C = 576, 2048, 128, 4608, 8
_EPS = 1e-5
_T = 128
_NB = _L // _T
_NG = _D // 16
_GA = 4
_GC = 2
_NCH = _NG // _GC
_R = _GC * _NB
_KT = -(-_D // _T)
_NF = 3
_NO, _OCH = 6, _D // 6
_LN_STEP = 4
_OUT_STEP = 3
_ROW_X, _ROW_W, _WQ, _ROW_SEL, _ROW_P = 0, _R, 2 * _R + 1, 5 * _R + 3, 5 * _R + 8
_ROWS = _ROW_P + 3 * _NB // 2
_PLANE = _NB + 1


def _lag_step(j):
    return max(1, (1 << (j * _T).bit_length()) >> 8)


def _round_lag(p, step):
    if step == 1:
        return p
    return (p + (step // 2 - 1) + ((p >> (step.bit_length() - 1)) & 1)) & ~(step - 1)


assert np.array_equal(
    np.concatenate([j * _T + _round_lag(np.arange(_T), _lag_step(j)) for j in range(_NB)]),
    np.arange(_L).astype(bf16).astype(np.int64))

_PAIRS = (((0, 1), (0, 5)), ((0, 2), (0, 6)), ((0, 3), (0, 7)), ((0, 4), (0, 8)), ((1, 2), (1, 6)),
          ((1, 4), (1, 8)), ((2, 4), (2, 8)), ((3, 4), (3, 8)), ((4, 8), (5, 8)), ((6, 8), (7, 8)))
_TAPS = [k for pair in _PAIRS for k in pair]


def _ds(start, size, align):
    return pl.ds(start if isinstance(start, int) else pl.multiple_of(start, align), size)


def _cmul(a, b):
    return a[0] * b[0] - a[1] * b[1], a[0] * b[1] + a[1] * b[0]


def _csq(a):
    return a[0] * a[0] - a[1] * a[1], (a[0] + a[0]) * a[1]


def _silu_of_twice(h):
    return h + h * jnp.tanh(h)


def _rnd(x):
    return x.astype(bf16).astype(f32)


def _dot(a, b):
    return jnp.dot(a, b, preferred_element_type=f32)


def _dot_nt(a, b):
    return lax.dot_general(a, b, (((1,), (1,)), ((), ())), preferred_element_type=f32)


def _column(v):
    return pltpu.bitcast(jnp.broadcast_to(v, (_T, v.shape[1])).astype(bf16).T, i32)


def _even_odd(words):
    return pltpu.bitcast(words << 16, f32), pltpu.bitcast(words & -65536, f32)


def _interleave(even, odd):
    even, odd = [pltpu.bitcast(x, i32) + 0x8000 for x in (even, odd)]
    return lax.shift_right_logical(even, 16) | (odd & -65536)


def _dft_rows():
    row = lax.broadcasted_iota(i32, (8, _T), 0)
    root = 4 * lax.broadcasted_iota(i32, (8, _T), 1) + 1

    def power(t):
        angle = ((root * t) & (4 * _T - 1)).astype(f32) * (np.pi / (2 * _T))
        return jnp.cos(angle), jnp.sin(angle)

    even, z, z16 = [power(2 * row)], power(1), power(16)
    for _ in range(_T // 16 - 1):
        even.append(_cmul(even[-1], z16))
    return [map(_interleave, e, _cmul(e, z)) for e in even]


def _modes(dt, ar, ai, br, bi, cr, ci):
    zr, zi = dt * ar, dt * ai
    mag = jnp.exp(zr)
    return _cmul((cr, ci), (dt * br, dt * bi)) + (mag * jnp.cos(zi), mag * jnp.sin(zi))


def _seeds(w, a1):
    a = {1: a1}
    for n in range(9):
        a[2 << n] = _csq(a[1 << n])
    row = lax.broadcasted_iota(i32, (8, _N), 0)

    def mix(z0, z1):
        rolled = [pltpu.roll(x, 4, 0) for x in z1]
        return ([jnp.where(row < 4, x, y) for x, y in zip(z0, rolled)],
                [jnp.where(row < 4, y, x) for x, y in zip(z0, rolled)])

    def dup(z):
        return [[jnp.take_along_axis(x, (row & 3) + 4 * q, axis=0, mode="promise_in_bounds")
                 for x in z] for q in range(2)]

    wa = _cmul(w, a1)
    return zip(mix((1.0, 0.0), a[128]), dup(a[8]), dup(a[32]),
               mix(wa, _cmul(wa, a[4])), dup(a1), dup(a[256]),
               mix(_cmul(a[256], a[4]), a[512]), dup(a[512]))


def _vandermonde(e0, m8, m32, g0, m1, m256, m_top, m512):
    e = [e0]
    for s in range(1, 16):
        e.append(_cmul(e[s - 1], m8) if s < 4 else _cmul(e[s - 4], m32))
    g = [g0]
    for _ in range(3):
        g.append(_cmul(g[-1], m1))
    g += [_cmul(g[1], m256), _cmul(g[3], m256)]
    g += [_cmul(g[3], m512), _cmul(g[5], m512)]
    g.append(_cmul(g[7], m_top))
    g.append(_cmul(g[8], m512))
    re, im = [_dot_nt(jnp.concatenate([z[p] for z in g], axis=0),
                      jnp.concatenate([z[p] for z in e], axis=0)) for p in range(2)]
    return re - im


def _unmix(lo, hi):
    row = lax.broadcasted_iota(i32, (8, _T), 0)
    for m in range(len(_PAIRS)):
        x, y = lo[8 * m:8 * m + 8], hi[8 * m:8 * m + 8]
        yield jnp.where(row < 4, x, y)
        yield pltpu.roll(jnp.where(row < 4, y, x), 4, 0)


def _lag_blocks(tap, lag0):
    lane = lax.broadcasted_iota(i32, (8, _T), 1)
    row = lax.broadcasted_iota(i32, (8, _T), 0)
    for h in range(2):
        def take(big, r, lag):
            s = ((_T * h + lag) >> 3) & 31
            return jnp.take_along_axis(tap(_TAPS.index((big, r))),
                                       ((s & 15) << 3) + (row ^ ((s >> 4) << 2)),
                                       axis=1, mode="promise_in_bounds")

        top = [take(big, 8, _round_lag(lane, 8) - 8) for big in range(_NB // 2)]
        for big, blk in enumerate(top):
            step = _lag_step(2 * big + h)
            lag = _round_lag(lane, step)
            if h == 0:
                blk = jnp.where(lag == 0, top[big - 1] if big else lag0, blk)
            for r in range(step, 8, step):
                blk = jnp.where((lag & 7) == r, take(big, r, lane), blk)
            yield 2 * big + h, blk


def _kernel(x_hbm, ar_hbm, ai_hbm, br_hbm, bi_hbm, cr_hbm, ci_hbm, ldt_hbm, dsk_hbm, wr_hbm,
            wg_hbm, wu_hbm, wd_hbm, o_hbm,
            x_v, par_v, wg_v, wu_v, wd_v, dft_v, o_v,
            dt_v, skip_v, mode_v, k0_v, tap_v, k_v, kf_v,
            xf_v, inv_v, arena, uf_a, uf_b, s_v,
            stat_v, key_v, sel_v, hid_v, ldt_v, dsk_v, wr_v, sem, w_sem, o_sem):
    row = lax.broadcasted_iota(i32, (8, _T), 0)
    lane = lax.broadcasted_iota(i32, (8, _T), 1)

    groups = {}

    def start(name, src, dst):
        slot, pairs = groups.setdefault(name, (len(groups), []))
        pairs.append((src, dst))
        pltpu.make_async_copy(src, dst, sem.at[slot]).start()

    def wait(name):
        slot, pairs = groups[name]
        for src, dst in pairs:
            pltpu.make_async_copy(src, dst, sem.at[slot]).wait()

    def start_parameters(name, rows):
        for n, src in enumerate((ar_hbm, ai_hbm, br_hbm, bi_hbm, cr_hbm, ci_hbm)):
            start(name, src.bitcast(i32).at[rows], par_v.at[n, rows])

    def hidden_copies(n):
        cols = _ds(n * (_F // _NF), _F // _NF, _F // _NF)
        return [pltpu.make_async_copy(w.bitcast(i32).at[:, cols], v.at[:, cols], w_sem.at[n])
                for w, v in ((wg_hbm, wg_v), (wu_hbm, wu_v))]

    def down_copy(n):
        return pltpu.make_async_copy(wd_hbm.bitcast(i32).at[_ds(n * (_OCH // 2), _OCH // 2, 16)],
                                     wd_v.at[n], w_sem.at[_NF + n])

    def out_copy(n):
        rows = _ds(n * _OCH, _OCH, 32)
        return pltpu.make_async_copy(o_v.at[rows], o_hbm.at[rows], o_sem)

    def compact(k, h):
        out = stat_v[k, 8 * h]
        for s in range(1, 8):
            out = jnp.where(row == s, stat_v[k, 8 * h + s], out)
        return out

    def layer_norm():
        def moments(b, carry):
            cols = _ds(b * _T, _T, _T)
            pivot = jnp.broadcast_to(_even_odd(x_v[:8, cols])[0][:1], (8, _T))
            s1, s2 = [None] * 2, [None] * 2
            for g in range(_NG):
                x = pltpu.bitcast(x_v[pl.ds(8 * g, 8), cols], bf16).astype(f32)
                xf_v[b, pl.ds(16 * g, 16), :] = x
                for h in range(2):
                    d = x[8 * h:8 * h + 8] - pivot
                    s1[h] = s1[h] + d if g else d
                    s2[h] = s2[h] + d * d if g else d * d
            for k, s in enumerate((s1, s2)):
                stat_v[k, b] = jnp.broadcast_to(jnp.sum(s[0] + s[1], axis=0, keepdims=True), (8, _T))
            stat_v[2, b] = pivot

        lax.fori_loop(0, _NB, moments, None, unroll=4)
        for h in range(_NB // 8):
            m1, m2 = compact(0, h) / _D, compact(1, h) / _D
            mean = _rnd(compact(2, h) + m1)
            var = _rnd(jnp.maximum(m2 - m1 * m1, 0.0))
            gain = 0.5 / _rnd(jnp.sqrt(_rnd(var + _rnd(jnp.full_like(var, _EPS)))))
            for s in range(8):
                stat_v[0, 8 * h + s] = jnp.broadcast_to(mean[s:s + 1], (8, _T))
                stat_v[1, 8 * h + s] = jnp.broadcast_to(gain[s:s + 1], (8, _T))
        wr = jnp.broadcast_to(wr_v[...].astype(f32).reshape(1, _D), (8, _D)).astype(bf16)
        for b in range(_NB):
            mean, gain = stat_v[0, b], stat_v[1, b]
            xn = [_interleave(*[(xf_v[b, pl.ds(16 * g + h, 8, stride=2), :] - mean) * gain
                                for h in range(2)]) for g in range(_NG)]
            for g in range(_NG):
                arena[g // _GC, _ROW_X + (g % _GC) * _NB + b] = xn[g]
            stat_v[2, b] = _dot(wr, pltpu.bitcast(jnp.concatenate(xn, axis=0), bf16))
        for h in range(_NB // 8):
            bits = pltpu.bitcast(_rnd(2.0 * compact(2, h)), i32) >> 16
            rank = jnp.where(bits < 0, 0x8000 - (bits & 0x7FFF), 0x8000 + bits)
            token = (8 * h + row) * _T + lane
            key_v[h] = pltpu.bitcast((1 << 28) + rank * _L + (_L - 1 - token), f32)

    def pop_best(t):
        best = jnp.max(jnp.max(jnp.maximum(key_v[0], key_v[1]), axis=0, keepdims=True),
                       axis=1, keepdims=True)
        key_v[2] = jnp.where(row == t, best, key_v[2])
        for h in range(2):
            key_v[h] = jnp.where(key_v[h] == best, 0.0, key_v[h])

    def routed_tokens():
        return _L - 1 - (pltpu.bitcast(key_v[2], i32) & (_L - 1))

    def routed_scores():
        rank = (pltpu.bitcast(key_v[2], i32) - (1 << 28)) >> 11
        return pltpu.bitcast(jnp.where(rank < 0x8000, 0x10000 - rank, rank - 0x8000) << 16, f32)

    def gather(tokens):
        token = routed_tokens()
        blocks = jnp.concatenate(
            [pltpu.bitcast(jnp.concatenate(
                [arena[g // _GC, _ROW_X + (g % _GC) * _NB + (token[t, 0] >> 7)]
                 for g in range(_NG)], axis=0), bf16) for t in tokens], axis=1)
        pick = jnp.concatenate(
            [jnp.where((row == t) & ((token & (_T - 1)) == lane), 2.0, 0.0) for t in tokens], axis=1)
        return _dot_nt(pick.astype(bf16), blocks)

    def dft(rows):
        z = _dot(jnp.concatenate([pltpu.bitcast(r, bf16) for r in rows], axis=0),
                 pltpu.bitcast(dft_v[...], bf16))
        return [[(z[o:o + 8, :_T], z[o:o + 8, _T:])
                 for o in range(h // 2 * 16 * _NB + 8 * (h % 2), (h // 2 + 1) * 16 * _NB, 16)]
                for h in range(2 * len(rows) // _NB)]

    def modes(step):
        for u in range(_GA):
            grp = step * _GA + u
            rows = _ds(grp * 8, 8, 8)
            par = [_even_odd(dt_v[rows, :])] + [_even_odd(par_v[n, rows, :]) for n in range(6)]
            k0 = []
            for h, skip in enumerate(_even_odd(skip_v[rows, :])):
                z = _modes(*[p[h] for p in par])
                for n in range(4):
                    mode_v[u, h, n] = z[n]
                k0.append(skip + jnp.sum(z[0], axis=1, keepdims=True))
            k0_v[grp] = _interleave(*k0)

    def spread(step, u, slot):
        for j, blk in _lag_blocks(lambda n: tap_v[u, n], k0_v[step * _GA + u]):
            k_v[slot, j] = blk

    def filter_spectra(grp, slots):
        for h, blocks in enumerate(dft([k_v[slot, j] for slot in slots for j in range(_NB)])):
            for j, (re, im) in enumerate(blocks):
                for plane, val in enumerate((re, re + im, im - re)):
                    kf_v[2 * grp + h, plane * _PLANE + j] = val

    def filter_step(i, zero):
        for u in range(_GA):
            if u % (_GA // 2) == 0:
                old = (u + _GA // 2) % _GA
                filter_spectra(jnp.maximum(i - (1 if u else 2), 0) * _GA + old,
                               [old + k + zero for k in range(_GA // 2)])
            spread(jnp.maximum(i - 1, 0), u, u)
            even, odd = [[_vandermonde(*seeds) for seeds in _seeds(
                (mode_v[u, h, 0], mode_v[u, h, 1]), (mode_v[u, h, 2], mode_v[u, h, 3]))]
                         for h in range(2)]
            for n, tap in enumerate(_unmix(*map(_interleave, even, odd))):
                tap_v[u, n] = tap
            yield u

    def hidden_jobs(c):
        width = _F // (_NCH - _NO)
        pre = []

        def project(n):
            cols = _ds(c * width + n // 2 * _T, _T, _T)
            x_sel = jnp.concatenate(
                [pltpu.bitcast(arena[c >> 8, _ROW_SEL + k], bf16) for k in range(_KT)], axis=1)
            weight = pltpu.bitcast((wu_v if n % 2 else wg_v)[:, cols], bf16)
            pre.append(_rnd(_dot(x_sel[:, :_D], weight)[:8]))
            if n % 2:
                hid_v[:, cols] = (_rnd(_silu_of_twice(0.5 * pre[-2])) * pre[-1]).astype(bf16)

        return [(40 * n, lambda n=n: project(n)) for n in range(2 * width // _T)]

    def scatters(n, hid):
        y = _rnd(_dot_nt(jnp.concatenate(hid, axis=1), pltpu.bitcast(wd_v[n], bf16)))
        y = 0.5 * (sel_v[n] + _rnd(y * _rnd(jax.nn.sigmoid(routed_scores()))[:, :_OCH]))
        col = jnp.concatenate([y, jnp.zeros((_T - _C, _OCH), f32)], axis=0).T
        col = pltpu.bitcast(col.astype(bf16), i32)
        token = routed_tokens()

        def scatter(t):
            hit = ((token & (_T - 1)) == lane)[t:t + 1]
            new = jnp.broadcast_to(col[:, t:t + 1], (_OCH // 2, _T))
            where = [(n * (_OCH // (16 * _GC)) + g // _GC,
                      _ROW_X + (g % _GC) * _NB + (token[t, 0] >> 7)) for g in range(_OCH // 16)]
            old = [arena[at] for at in where]
            for g, at in enumerate(where):
                arena[at] = jnp.where(hit, new[8 * g:8 * g + 8], old[g])

        return [lambda t=t: scatter(t) for t in range(_C)]

    def finish(n):
        for k in range(0, _OCH // 16 * _NB, 2):
            c, r = n * (_OCH // (16 * _GC)) + k // _R, k % _R
            rows = _ds(n * _OCH + 16 * (k // _NB), 16, 16)
            out = []
            for d in range(2):
                gate = _silu_of_twice(pltpu.bitcast(arena[c, _ROW_X + r + d], bf16).astype(f32))
                out.append(xf_v[k % _NB + d, rows, :] + s_v[c, pl.ds(16 * (r + d), 16), :] * gate)
            o_v[rows, pl.ds(k % _NB * _T, 2 * _T)] = jnp.concatenate(out, axis=1).astype(bf16)
            yield k + 2

    def spare(t, zero=0):
        return _ds(_D + 8 * (t // _NB + zero), 8, 8), pl.ds(t % _NB * _T, _T)

    def first_output_jobs(c):
        hid, scatter = [], []

        def read():
            hid.extend([pltpu.bitcast(arena[c >> 8, _ROW_W + t], bf16)[:8]
                        for t in range(len(hid), len(hid) + 4)])

        return ([(48 * k, read) for k in range(_F // (4 * _T))]
                + [(431, lambda: scatter.extend(scatters(0, hid)))]
                + [(992 + 14 * t, lambda t=t: scatter[t]()) for t in range(_C)])

    def output_jobs(c):
        n = c - (_NCH - _NO)
        hid = [o_v[spare(t, c >> 8)] for t in range(4)]
        for done in finish(n - 1):
            if done == _OCH // 16 * _NB:
                pl.when(n >= _OUT_STEP)(lambda: out_copy(n - 1).start())
                o_v[spare(_F // _T, c >> 9)] = hid[0]
            if done % 12 == 0:
                hid += [o_v[spare(t, c >> 8)] for t in range(len(hid), len(hid) + 4)]
        return [(560 + 14 * t, job) for t, job in enumerate(scatters(n, hid))]

    def input_spectra(rows, dst):
        z = dft(rows)
        for h, blocks in enumerate(z):
            for b, (re, im) in enumerate(blocks):
                if b:
                    re, im = re + blocks[b - 1][1], im - blocks[b - 1][0]
                for plane, val in enumerate((re + im, im, re)):
                    dst[(h * 3 + plane) * _PLANE + b] = val
        return z

    def output_spectrum(c, r):
        return jnp.concatenate(
            [pltpu.bitcast(arena[c, pl.ds(_ROW_W + q * _WQ + 2 * r, 2)].reshape(16, _T), f32)
             for q in range(2)], axis=1)

    def conv_step(c, cur, nxt, ffn_jobs, delay, pace):
        c_next, c_prev = jnp.minimum(c + 1, _NCH - 1), jnp.maximum(c - 1, 0)
        zero = c >> 8
        fwd_rows, inv_rows, results = [], [], []

        def transform():
            y = _dot(jnp.concatenate(inv_rows, axis=0), inv_v[...])
            s_v[c_prev] = y
            results.extend((y, input_spectra(fwd_rows, nxt)))

        def drain(r):
            y, z = results
            arena[c, _ROW_SEL - 1] = pltpu.bitcast(
                y[8 * r:8 * r + 8] + z[2 * (r // _R) + 1][r % _R // 2][r // 8 % 2], i32)

        jobs = sorted(
            ffn_jobs(c)
            + [(delay + 16 * r, lambda r=r: inv_rows.append(output_spectrum(c_prev, r)))
               for r in range(_R)]
            + [(delay + 16 * r, lambda r=r: fwd_rows.append(arena[c_next, _ROW_X + r]))
               for r in range(_R)]
            + [(delay + 16 * _R, transform)]
            + [(delay + 140 + 8 * r, lambda r=r: drain(r)) for r in range(2 * _R - 17, 2 * _R, 8)],
            key=lambda job: job[0])

        def run_jobs(done):
            while jobs and done * (delay + 16 * _R) >= (jobs[0][0] - 32) * pace * 18 * _GC:
                jobs.pop(0)[1]()

        run_jobs(0)
        for h in range(2 * _GC):
            for part in range(3):
                for plane in range(3):
                    kf = lambda b: kf_v[c * 2 * _GC + h + (zero >> part), plane * _PLANE + b]
                    uf = lambda b: cur[(zero >> part) + (h * 3 + plane) * _PLANE + b]
                    base = [pltpu.bitcast(arena[c + zero, _ROW_P + plane * 8 + m], f32)
                            for m in range(_NB // 2) if part and plane]
                    k, u, out = [], [], []
                    for m in range(_NB // 2):
                        if part == 0:
                            k.append(kf(2 * m))
                            u.append(uf(2 * m) + uf(2 * m + 1))
                        elif part == 1:
                            k.append(kf(2 * m) - kf(2 * m - 1) if m else kf(0))
                            u.append(uf(2 * m + 1))
                        else:
                            k.append(kf(2 * m) - kf(2 * m + 1))
                            u.append(uf(2 * m))
                        y = k[0] * u[m]
                        for j in range(1, m + 1):
                            y = y + k[j] * u[m - j]
                        if plane:
                            y = shared[m] - y if plane == 1 else shared[m] + y
                        out.append(y)
                        if base:
                            r = (h // 2 * _NB + 2 * m + part - 1) * 2 + h % 2
                            arena[c, _ROW_W + (plane - 1) * _WQ + r] = pltpu.bitcast(base[m] - y, i32)
                        else:
                            arena[c, _ROW_P + plane * 8 + m] = pltpu.bitcast(y, i32)
                    if plane == 0:
                        shared = out
                    run_jobs((h * 3 + part) * 3 + plane + 1)
        run_jobs(np.inf)

    start("vectors", ldt_hbm, ldt_v)
    start("vectors", dsk_hbm, dsk_v)
    start_parameters("step 0", pl.ds(0, 8 * _GA))
    start_parameters("step 1", pl.ds(8 * _GA, 8 * _GA))
    start_parameters("later steps", pl.ds(16 * _GA, _D // 2 - 16 * _GA))
    for k, parts in enumerate(_dft_rows()):
        dft_v[pl.ds(8 * k, 8), :] = jnp.concatenate(list(parts), axis=1)
    arena[0, _ROW_W:_ROW_P] = jnp.zeros((_ROW_P - _ROW_W, 8, _T), i32)
    tap_v[...] = jnp.zeros(tap_v.shape, i32)
    k_v[:_GA] = jnp.zeros((_GA, _NB, 8, _T), i32)
    key_v[...] = jnp.zeros(key_v.shape, f32)
    wait("vectors")
    start("input", x_hbm.bitcast(i32), x_v)
    start("input", wr_hbm, wr_v)
    dt = jnp.exp(ldt_v[...].astype(f32)).reshape(1, _D)
    skip = dsk_v[...].astype(f32).reshape(1, _D)
    dt_v[:_T // 2] = _column(dt[:, :_T])
    skip_v[:_T // 2] = _column(skip[:, :_T])
    wait("step 0")
    modes(0)
    dt_v[_T // 2:] = _column(dt[:, _T:])
    skip_v[_T // 2:] = _column(skip[:, _T:])
    wait("step 1")

    def filter_loop(i, carry):
        @pl.when(i == 1)
        def _():
            wait("later steps")
            for cp in hidden_copies(0):
                cp.start()

        @pl.when(i == _LN_STEP)
        def _():
            wait("input")
            for cp in hidden_copies(1):
                cp.start()
            layer_norm()
            inv_v[...] = pltpu.bitcast(dft_v[...], bf16).astype(f32).T * (2 / _T)

        for t in range(2):
            pop_best(2 * (i - _LN_STEP) + t)
        list(filter_step(i, i >> 8))
        modes(i + 1)

    last = _NG // _GA - 1
    assert 2 * (last - _LN_STEP) == _C
    lax.fori_loop(0, last, filter_loop, None)
    for cp in hidden_copies(2):
        cp.start()
    zero = routed_tokens()[0, 0] >> 11
    parts = [gather(range(u * _C // _GA, (u + 1) * _C // _GA)) for u in filter_step(last, zero)]
    x_sel = sum(parts[1:], parts[0])
    for n in range(_NO):
        sel_v[n] = x_sel[:, n * _OCH:(n + 1) * _OCH]
    x_sel = jnp.concatenate([x_sel, jnp.zeros((8, _KT * _T - _D), f32)], axis=1)
    for k in range(_KT):
        arena[0, _ROW_SEL + k] = pltpu.bitcast(
            jnp.concatenate([x_sel[:, k * _T:(k + 1) * _T]] * 2, axis=0).astype(bf16), i32)
    input_spectra([arena[0, _ROW_X + r] for r in range(_R)], uf_a)
    for u in range(_GA):
        spread(last, u, _GA + u)
    filter_spectra(_NG - 3 * _GA // 2, range(_GA // 2, 2 * _GA))

    def hidden_loop(slab, carry):
        for cp in hidden_copies(slab):
            cp.wait()

        @pl.when(slab == 1)
        def _():
            for n in range(_NO):
                down_copy(n).start()

        def pair(i, carry):
            conv_step(2 * i, uf_a, uf_b, hidden_jobs, 240, 0.87)
            conv_step(2 * i + 1, uf_b, uf_a, hidden_jobs, 240, 0.87)

        pairs = (_NCH - _NO) // (2 * _NF)
        lax.fori_loop(slab * pairs, (slab + 1) * pairs, pair, None)

    def output_loop(n, carry):
        down_copy(n).wait()

        @pl.when(n == _OUT_STEP)
        def _():
            for k in range(_OUT_STEP - 1):
                out_copy(k).start()

        c = n + _NCH - _NO
        lax.cond(c & 1 == 0, lambda: conv_step(c, uf_a, uf_b, output_jobs, 32, 0.8),
                 lambda: conv_step(c, uf_b, uf_a, output_jobs, 32, 0.8))

    lax.fori_loop(0, _NF, hidden_loop, None)
    for t in range(_F // _T):
        tile = hid_v[:, t * _T:(t + 1) * _T]
        o_v[spare(t)] = tile
        arena[0, _ROW_W + t] = pltpu.bitcast(jnp.concatenate([tile] * 2, axis=0), i32)
    down_copy(0).wait()
    conv_step(_NCH - _NO + zero, uf_a, uf_b, first_output_jobs, 432, 0.87)
    lax.fori_loop(1, _NO, output_loop, None)
    s_v[_NCH - 1] = _dot(
        jnp.concatenate([output_spectrum(_NCH - 1, r) for r in range(_R)], axis=0), inv_v[...])
    for done in finish(_NO - 1):
        if done % _R == 0:
            rows = pl.ds((_NO - 1) * _OCH + (done // _R - 1) * 16 * _GC, 16 * _GC)
            start("last slab", o_v.at[rows], o_hbm.at[rows])
    for n in range(_NO - 1):
        out_copy(n).wait()
    wait("last slab")


@jax.jit
def pallas_recurrent_scan__ssm_conv_s4__moe_arch_mod__prompt_kernel(
    A_u: jax.Array,
    A_A_re: jax.Array,
    A_A_im: jax.Array,
    A_B_re: jax.Array,
    A_B_im: jax.Array,
    A_C_re: jax.Array,
    A_C_im: jax.Array,
    A_log_dt: jax.Array,
    A_Dskip: jax.Array,
    B_x: jax.Array,
    B_w_r: jax.Array,
    B_w_gate: jax.Array,
    B_w_up: jax.Array,
    B_w_down: jax.Array,
):
    del B_x
    assert A_u.shape == (1, _L, _D) and A_A_re.shape == (_D, _N) and B_w_gate.shape == (_D, _F)
    assert A_u.dtype == bf16 and A_A_re.dtype == bf16
    hbm = pl.BlockSpec(memory_space=pl.ANY)
    vmem = pltpu.VMEM
    out = pl.pallas_call(
        _kernel,
        out_shape=jax.ShapeDtypeStruct((_D, _L), bf16),
        in_specs=[hbm] * 13,
        out_specs=hbm,
        scratch_shapes=[
            vmem((_D // 2, _L), i32), vmem((6, _D // 2, _N), i32),
            vmem((_D // 2, _F), i32), vmem((_D // 2, _F), i32), vmem((_NO, _OCH // 2, _F), i32),
            vmem((_T // 2, 2 * _T), i32), vmem((_D + 32, _L), bf16),
            vmem((_D // 2, _T), i32), vmem((_D // 2, _T), i32), vmem((_GA, 2, 4, 8, _N), f32),
            vmem((_NG, 8, _T), i32), vmem((_GA, len(_TAPS), 8, _T), i32),
            vmem((2 * _GA, _NB, 8, _T), i32), vmem((2 * _NG, 3 * _PLANE, 8, _T), f32),
            vmem((_NB, _D + 32, _T), f32), vmem((2 * _T, _T), f32), vmem((_NCH, _ROWS, 8, _T), i32),
            vmem((6 * _GC * _PLANE, 8, _T), f32), vmem((6 * _GC * _PLANE, 8, _T), f32),
            vmem((_NCH, 16 * _R, _T), f32),
            vmem((3, _NB, 8, _T), f32), vmem((3, 8, _T), f32), vmem((_NO, 8, _OCH), f32),
            vmem((8, _F), bf16), vmem((_D,), bf16), vmem((_D,), bf16), vmem((_D,), bf16),
            pltpu.SemaphoreType.DMA((6,)), pltpu.SemaphoreType.DMA((_NF + _NO,)),
            pltpu.SemaphoreType.DMA(()),
        ],
        compiler_params=pltpu.CompilerParams(vmem_limit_bytes=100 * 2**20),
    )(A_u.reshape(_L, _D).T, A_A_re, A_A_im, A_B_re, A_B_im, A_C_re, A_C_im, A_log_dt, A_Dskip,
      B_w_r, B_w_gate, B_w_up, B_w_down.T)
    return out.T.reshape(1, _L, _D)
```

```python
import jax
import jax.numpy as jnp
import numpy as np
from jax import lax
import jax.experimental.pallas as pl
import jax.experimental.pallas.tpu as pltpu

f32, bf16, i32 = jnp.float32, jnp.bfloat16, jnp.int32

_D, _L, _N, _F, _C = 576, 2048, 128, 4608, 8
_EPS = 1e-5
_T = 128
_NB = _L // _T
_NG = _D // 16
_GA = 4
_GC = 2
_NCH = _NG // _GC
_R = _GC * _NB
_KT = -(-_D // _T)
_NF, _FCH = 6, _F // 6
_NO, _OCH = 6, _D // 6
_LN_STEP = 4
_OUT_STEP = 3
_ROW_X, _ROW_W, _WQ, _ROW_SEL, _ROW_P = 0, _R, 2 * _R + 1, 5 * _R + 3, 5 * _R + 8
_ROWS = _ROW_P + 3 * _NB // 2
_PLANE = _NB + 1


def _lag_step(j):
    return max(1, (1 << (j * _T).bit_length()) >> 8)


def _round_lag(p, step):
    if step == 1:
        return p
    return (p + (step // 2 - 1) + ((p >> (step.bit_length() - 1)) & 1)) & ~(step - 1)


assert np.array_equal(
    np.concatenate([j * _T + _round_lag(np.arange(_T), _lag_step(j)) for j in range(_NB)]),
    np.arange(_L).astype(bf16).astype(np.int64))

_PAIRS = (((0, 1), (0, 5)), ((0, 2), (0, 6)), ((0, 3), (0, 7)), ((0, 4), (0, 8)), ((1, 2), (1, 6)),
          ((1, 4), (1, 8)), ((2, 4), (2, 8)), ((3, 4), (3, 8)), ((4, 8), (5, 8)), ((6, 8), (7, 8)))
_TAPS = [k for pair in _PAIRS for k in pair]


def _ds(start, size, align):
    return pl.ds(start if isinstance(start, int) else pl.multiple_of(start, align), size)


def _cmul(a, b):
    return a[0] * b[0] - a[1] * b[1], a[0] * b[1] + a[1] * b[0]


def _csq(a):
    return a[0] * a[0] - a[1] * a[1], (a[0] + a[0]) * a[1]


def _silu_of_twice(h):
    return h + h * jnp.tanh(h)


def _rnd(x):
    return x.astype(bf16).astype(f32)


def _dot(a, b):
    return jnp.dot(a, b, preferred_element_type=f32)


def _dot_nt(a, b):
    return lax.dot_general(a, b, (((1,), (1,)), ((), ())), preferred_element_type=f32)


def _column(v):
    return pltpu.bitcast(jnp.broadcast_to(v, (_T, v.shape[1])).astype(bf16).T, i32)


def _even_odd(words):
    return pltpu.bitcast(words << 16, f32), pltpu.bitcast(words & -65536, f32)


def _interleave(even, odd):
    even, odd = [pltpu.bitcast(x, i32) + 0x8000 for x in (even, odd)]
    return lax.shift_right_logical(even, 16) | (odd & -65536)


def _dft_rows():
    row = lax.broadcasted_iota(i32, (8, _T), 0)
    root = 4 * lax.broadcasted_iota(i32, (8, _T), 1) + 1

    def power(t):
        angle = ((root * t) & (4 * _T - 1)).astype(f32) * (np.pi / (2 * _T))
        return jnp.cos(angle), jnp.sin(angle)

    even, z, z16 = [power(2 * row)], power(1), power(16)
    for _ in range(_T // 16 - 1):
        even.append(_cmul(even[-1], z16))
    return [map(_interleave, e, _cmul(e, z)) for e in even]


def _modes(dt, ar, ai, br, bi, cr, ci):
    zr, zi = dt * ar, dt * ai
    mag = jnp.exp(zr)
    return _cmul((cr, ci), (dt * br, dt * bi)) + (mag * jnp.cos(zi), mag * jnp.sin(zi))


def _seeds(w, a1):
    a = {1: a1}
    for n in range(9):
        a[2 << n] = _csq(a[1 << n])
    row = lax.broadcasted_iota(i32, (8, _N), 0)

    def mix(z0, z1):
        rolled = [pltpu.roll(x, 4, 0) for x in z1]
        return ([jnp.where(row < 4, x, y) for x, y in zip(z0, rolled)],
                [jnp.where(row < 4, y, x) for x, y in zip(z0, rolled)])

    def dup(z):
        return [[jnp.take_along_axis(x, (row & 3) + 4 * q, axis=0, mode="promise_in_bounds")
                 for x in z] for q in range(2)]

    wa = _cmul(w, a1)
    return zip(mix((1.0, 0.0), a[128]), dup(a[8]), dup(a[32]),
               mix(wa, _cmul(wa, a[4])), dup(a1), dup(a[256]),
               mix(_cmul(a[256], a[4]), a[512]), dup(a[512]))


def _vandermonde(e0, m8, m32, g0, m1, m256, m_top, m512):
    e = [e0]
    for s in range(1, 16):
        e.append(_cmul(e[s - 1], m8) if s < 4 else _cmul(e[s - 4], m32))
    g = [g0]
    for _ in range(3):
        g.append(_cmul(g[-1], m1))
    g += [_cmul(g[1], m256), _cmul(g[3], m256)]
    g += [_cmul(g[3], m512), _cmul(g[5], m512)]
    g.append(_cmul(g[7], m_top))
    g.append(_cmul(g[8], m512))
    re, im = [_dot_nt(jnp.concatenate([z[p] for z in g], axis=0),
                      jnp.concatenate([z[p] for z in e], axis=0)) for p in range(2)]
    return re - im


def _unmix(lo, hi):
    row = lax.broadcasted_iota(i32, (8, _T), 0)
    for m in range(len(_PAIRS)):
        x, y = lo[8 * m:8 * m + 8], hi[8 * m:8 * m + 8]
        yield jnp.where(row < 4, x, y)
        yield pltpu.roll(jnp.where(row < 4, y, x), 4, 0)


def _lag_blocks(tap, lag0):
    lane = lax.broadcasted_iota(i32, (8, _T), 1)
    row = lax.broadcasted_iota(i32, (8, _T), 0)
    for h in range(2):
        def take(big, r, lag):
            s = ((_T * h + lag) >> 3) & 31
            return jnp.take_along_axis(tap(_TAPS.index((big, r))),
                                       ((s & 15) << 3) + (row ^ ((s >> 4) << 2)),
                                       axis=1, mode="promise_in_bounds")

        top = [take(big, 8, _round_lag(lane, 8) - 8) for big in range(_NB // 2)]
        for big, blk in enumerate(top):
            step = _lag_step(2 * big + h)
            lag = _round_lag(lane, step)
            if h == 0:
                blk = jnp.where(lag == 0, top[big - 1] if big else lag0, blk)
            for r in range(step, 8, step):
                blk = jnp.where((lag & 7) == r, take(big, r, lane), blk)
            yield 2 * big + h, blk


def _kernel(x_hbm, ar_hbm, ai_hbm, br_hbm, bi_hbm, cr_hbm, ci_hbm, ldt_hbm, dsk_hbm, wr_hbm,
            wg_hbm, wu_hbm, wd_hbm, o_hbm,
            x_v, par_v, wg_v, wu_v, wd_v, dft_v, o_v,
            dt_v, skip_v, mode_v, k0_v, tap_v, k_v, kf_v,
            xf_v, inv_v, arena, uf_a, uf_b, s_v,
            stat_v, key_v, sel_v, hid_v, ldt_v, dsk_v, wr_v, sem, w_sem, o_sem):
    row = lax.broadcasted_iota(i32, (8, _T), 0)
    lane = lax.broadcasted_iota(i32, (8, _T), 1)

    groups = {}

    def start(name, src, dst):
        slot, pairs = groups.setdefault(name, (len(groups), []))
        pairs.append((src, dst))
        pltpu.make_async_copy(src, dst, sem.at[slot]).start()

    def wait(name):
        slot, pairs = groups[name]
        for src, dst in pairs:
            pltpu.make_async_copy(src, dst, sem.at[slot]).wait()

    def start_parameters(name, rows):
        for n, src in enumerate((ar_hbm, ai_hbm, br_hbm, bi_hbm, cr_hbm, ci_hbm)):
            start(name, src.bitcast(i32).at[rows], par_v.at[n, rows])

    def hidden_copies(n):
        cols = _ds(n * _FCH, _FCH, _FCH)
        return [pltpu.make_async_copy(w.bitcast(i32).at[:, cols], v.at[n], w_sem.at[n])
                for w, v in ((wg_hbm, wg_v), (wu_hbm, wu_v))]

    def down_copy(n):
        return pltpu.make_async_copy(wd_hbm.bitcast(i32).at[_ds(n * (_OCH // 2), _OCH // 2, 16)],
                                     wd_v.at[n], w_sem.at[_NF + n])

    def out_copy(n):
        rows = _ds(n * _OCH, _OCH, 32)
        return pltpu.make_async_copy(o_v.at[rows], o_hbm.at[rows], o_sem)

    def compact(k, h):
        out = stat_v[k, 8 * h]
        for s in range(1, 8):
            out = jnp.where(row == s, stat_v[k, 8 * h + s], out)
        return out

    def layer_norm():
        def moments(b, carry):
            cols = _ds(b * _T, _T, _T)
            pivot = jnp.broadcast_to(_even_odd(x_v[:8, cols])[0][:1], (8, _T))
            s1, s2 = [None] * 2, [None] * 2
            for g in range(_NG):
                x = pltpu.bitcast(x_v[pl.ds(8 * g, 8), cols], bf16).astype(f32)
                xf_v[b, pl.ds(16 * g, 16), :] = x
                for h in range(2):
                    d = x[8 * h:8 * h + 8] - pivot
                    s1[h] = s1[h] + d if g else d
                    s2[h] = s2[h] + d * d if g else d * d
            for k, s in enumerate((s1, s2)):
                stat_v[k, b] = jnp.broadcast_to(jnp.sum(s[0] + s[1], axis=0, keepdims=True), (8, _T))
            stat_v[2, b] = pivot

        lax.fori_loop(0, _NB, moments, None, unroll=4)
        for h in range(_NB // 8):
            m1, m2 = compact(0, h) / _D, compact(1, h) / _D
            mean = _rnd(compact(2, h) + m1)
            var = _rnd(jnp.maximum(m2 - m1 * m1, 0.0))
            gain = 0.5 / _rnd(jnp.sqrt(_rnd(var + _rnd(jnp.full_like(var, _EPS)))))
            for s in range(8):
                stat_v[0, 8 * h + s] = jnp.broadcast_to(mean[s:s + 1], (8, _T))
                stat_v[1, 8 * h + s] = jnp.broadcast_to(gain[s:s + 1], (8, _T))
        wr = jnp.broadcast_to(wr_v[...].astype(f32).reshape(1, _D), (8, _D)).astype(bf16)
        for b in range(_NB):
            mean, gain = stat_v[0, b], stat_v[1, b]
            xn = []
            for g in range(_NG):
                xc = _rnd(jnp.concatenate([xf_v[b, pl.ds(16 * g + h, 8, stride=2), :] - mean
                                           for h in range(2)], axis=1))
                xn.append(_interleave(xc[:, :_T] * gain, xc[:, _T:] * gain))
            for g in range(_NG):
                arena[g // _GC, _ROW_X + (g % _GC) * _NB + b] = xn[g]
            stat_v[2, b] = _dot(wr, pltpu.bitcast(jnp.concatenate(xn, axis=0), bf16))
        for h in range(_NB // 8):
            bits = pltpu.bitcast(_rnd(2.0 * compact(2, h)), i32) >> 16
            rank = jnp.where(bits < 0, 0x8000 - (bits & 0x7FFF), 0x8000 + bits)
            token = (8 * h + row) * _T + lane
            key_v[h] = pltpu.bitcast((1 << 28) + rank * _L + (_L - 1 - token), f32)

    def pop_best(t):
        best = jnp.max(jnp.max(jnp.maximum(key_v[0], key_v[1]), axis=0, keepdims=True),
                       axis=1, keepdims=True)
        key_v[2] = jnp.where(row == t, best, key_v[2])
        for h in range(2):
            key_v[h] = jnp.where(key_v[h] == best, 0.0, key_v[h])

    def routed_tokens():
        return _L - 1 - (pltpu.bitcast(key_v[2], i32) & (_L - 1))

    def routed_scores():
        rank = (pltpu.bitcast(key_v[2], i32) - (1 << 28)) >> 11
        return pltpu.bitcast(jnp.where(rank < 0x8000, 0x10000 - rank, rank - 0x8000) << 16, f32)

    def gather(tokens):
        token = routed_tokens()
        blocks = jnp.concatenate(
            [pltpu.bitcast(jnp.concatenate(
                [arena[g // _GC, _ROW_X + (g % _GC) * _NB + (token[t, 0] >> 7)]
                 for g in range(_NG)], axis=0), bf16) for t in tokens], axis=1)
        pick = jnp.concatenate(
            [jnp.where((row == t) & ((token & (_T - 1)) == lane), 2.0, 0.0) for t in tokens], axis=1)
        return _dot_nt(pick.astype(bf16), blocks)

    def dft(rows):
        z = _dot(jnp.concatenate([pltpu.bitcast(r, bf16) for r in rows], axis=0),
                 pltpu.bitcast(dft_v[...], bf16))
        return [[(z[o:o + 8, :_T], z[o:o + 8, _T:])
                 for o in range(h // 2 * 16 * _NB + 8 * (h % 2), (h // 2 + 1) * 16 * _NB, 16)]
                for h in range(2 * len(rows) // _NB)]

    def modes(step):
        for u in range(_GA):
            grp = step * _GA + u
            rows = _ds(grp * 8, 8, 8)
            par = [_even_odd(dt_v[rows, :])] + [_even_odd(par_v[n, rows, :]) for n in range(6)]
            k0 = []
            for h, skip in enumerate(_even_odd(skip_v[rows, :])):
                z = _modes(*[p[h] for p in par])
                for n in range(4):
                    mode_v[u, h, n] = z[n]
                k0.append(skip + jnp.sum(z[0], axis=1, keepdims=True))
            k0_v[grp] = _interleave(*k0)

    def spread(step, u, slot):
        for j, blk in _lag_blocks(lambda n: tap_v[u, n], k0_v[step * _GA + u]):
            k_v[slot, j] = blk

    def filter_spectra(grp, slots):
        for h, blocks in enumerate(dft([k_v[slot, j] for slot in slots for j in range(_NB)])):
            for j, (re, im) in enumerate(blocks):
                for plane, val in enumerate((re, re + im, im - re)):
                    kf_v[2 * grp + h, plane * _PLANE + j] = val

    def filter_step(i, zero):
        for u in range(_GA):
            if u % (_GA // 2) == 0:
                old = (u + _GA // 2) % _GA
                filter_spectra(jnp.maximum(i - (1 if u else 2), 0) * _GA + old,
                               [old + k + zero for k in range(_GA // 2)])
            spread(jnp.maximum(i - 1, 0), u, u)
            even, odd = [[_vandermonde(*seeds) for seeds in _seeds(
                (mode_v[u, h, 0], mode_v[u, h, 1]), (mode_v[u, h, 2], mode_v[u, h, 3]))]
                         for h in range(2)]
            for n, tap in enumerate(_unmix(*map(_interleave, even, odd))):
                tap_v[u, n] = tap
            yield u

    def hidden_jobs(slab, half):
        pre = []

        def project(n):
            cols = pl.ds(half * _FCH // 2 + n // 2 * _T, _T)
            x_sel = jnp.concatenate(
                [pltpu.bitcast(arena[slab >> 8, _ROW_SEL + k], bf16) for k in range(_KT)], axis=1)
            weight = pltpu.bitcast((wu_v if n % 2 else wg_v)[slab, :, cols], bf16)
            pre.append(_rnd(_dot(x_sel[:, :_D], weight)[:8]))
            if n % 2:
                hid_v[slab, :, cols] = (_rnd(_silu_of_twice(0.5 * pre[-2])) * pre[-1]).astype(bf16)

        return [(40 * n, lambda n=n: project(n)) for n in range(_FCH // _T)]

    def scatters(n, hid):
        y = _rnd(_dot_nt(jnp.concatenate(hid, axis=1), pltpu.bitcast(wd_v[n], bf16)))
        y = 0.5 * (sel_v[n] + _rnd(y * _rnd(jax.nn.sigmoid(routed_scores()))[:, :_OCH]))
        col = jnp.concatenate([y, jnp.zeros((_T - _C, _OCH), f32)], axis=0).T
        col = pltpu.bitcast(col.astype(bf16), i32)
        token = routed_tokens()

        def scatter(t):
            hit = ((token & (_T - 1)) == lane)[t:t + 1]
            new = jnp.broadcast_to(col[:, t:t + 1], (_OCH // 2, _T))
            where = [(n * (_OCH // (16 * _GC)) + g // _GC,
                      _ROW_X + (g % _GC) * _NB + (token[t, 0] >> 7)) for g in range(_OCH // 16)]
            old = [arena[at] for at in where]
            for g, at in enumerate(where):
                arena[at] = jnp.where(hit, new[8 * g:8 * g + 8], old[g])

        return [lambda t=t: scatter(t) for t in range(_C)]

    def finish(n):
        for k in range(0, _OCH // 16 * _NB, 2):
            c, r = n * (_OCH // (16 * _GC)) + k // _R, k % _R
            rows = _ds(n * _OCH + 16 * (k // _NB), 16, 16)
            out = []
            for d in range(2):
                gate = _silu_of_twice(pltpu.bitcast(arena[c, _ROW_X + r + d], bf16).astype(f32))
                out.append(xf_v[k % _NB + d, rows, :] + s_v[c, pl.ds(16 * (r + d), 16), :] * gate)
            o_v[rows, pl.ds(k % _NB * _T, 2 * _T)] = jnp.concatenate(out, axis=1).astype(bf16)
            yield k + 2

    def spare(t, zero=0):
        return _ds(_D + 8 * (t // _NB + zero), 8, 8), pl.ds(t % _NB * _T, _T)

    def first_output_jobs(zero):
        hid, scatter = [], []

        def read():
            hid.extend([pltpu.bitcast(arena[zero, _ROW_W + t], bf16)[:8]
                        for t in range(len(hid), len(hid) + 4)])

        return ([(48 * k, read) for k in range(_F // (4 * _T))]
                + [(431, lambda: scatter.extend(scatters(0, hid)))]
                + [(992 + 14 * t, lambda t=t: scatter[t]()) for t in range(_C)])

    def output_jobs(c):
        n = c - (_NCH - _NO)
        hid = [o_v[spare(t, c >> 8)] for t in range(4)]
        for done in finish(n - 1):
            if done == _OCH // 16 * _NB:
                pl.when(n >= _OUT_STEP)(lambda: out_copy(n - 1).start())
                o_v[spare(_F // _T, c >> 9)] = hid[0]
            if done % 12 == 0:
                hid += [o_v[spare(t, c >> 8)] for t in range(len(hid), len(hid) + 4)]
        return [(560 + 14 * t, job) for t, job in enumerate(scatters(n, hid))]

    def input_spectra(rows, dst):
        z = dft(rows)
        for h, blocks in enumerate(z):
            for b, (re, im) in enumerate(blocks):
                if b:
                    re, im = re + blocks[b - 1][1], im - blocks[b - 1][0]
                for plane, val in enumerate((re + im, im, re)):
                    dst[(h * 3 + plane) * _PLANE + b] = val
        return z

    def output_spectrum(c, r):
        return jnp.concatenate(
            [pltpu.bitcast(arena[c, pl.ds(_ROW_W + q * _WQ + 2 * r, 2)].reshape(16, _T), f32)
             for q in range(2)], axis=1)

    def conv_step(c, cur, nxt, ffn_jobs, delay, pace):
        c_next, c_prev = jnp.minimum(c + 1, _NCH - 1), jnp.maximum(c - 1, 0)
        zero = c >> 8
        fwd_rows, inv_rows, results = [], [], []

        def transform():
            y = _dot(jnp.concatenate(inv_rows, axis=0), inv_v[...])
            s_v[c_prev] = y
            results.extend((y, input_spectra(fwd_rows, nxt)))

        def drain(r):
            y, z = results
            arena[c, _ROW_SEL - 1] = pltpu.bitcast(
                y[8 * r:8 * r + 8] + z[2 * (r // _R) + 1][r % _R // 2][r // 8 % 2], i32)

        jobs = sorted(
            ffn_jobs
            + [(delay + 16 * r, lambda r=r: inv_rows.append(output_spectrum(c_prev, r)))
               for r in range(_R)]
            + [(delay + 16 * r, lambda r=r: fwd_rows.append(arena[c_next, _ROW_X + r]))
               for r in range(_R)]
            + [(delay + 16 * _R, transform)]
            + [(delay + 140 + 8 * r, lambda r=r: drain(r)) for r in range(2 * _R - 17, 2 * _R, 8)],
            key=lambda job: job[0])

        def run_jobs(done):
            while jobs and done * (delay + 16 * _R) >= (jobs[0][0] - 32) * pace * 18 * _GC:
                jobs.pop(0)[1]()

        run_jobs(0)
        for h in range(2 * _GC):
            for part in range(3):
                for plane in range(3):
                    kf = lambda b: kf_v[c * 2 * _GC + h + (zero >> part), plane * _PLANE + b]
                    uf = lambda b: cur[(zero >> part) + (h * 3 + plane) * _PLANE + b]
                    base = [pltpu.bitcast(arena[c + zero, _ROW_P + plane * 8 + m], f32)
                            for m in range(_NB // 2) if part and plane]
                    k, u, out = [], [], []
                    for m in range(_NB // 2):
                        if part == 0:
                            k.append(kf(2 * m))
                            u.append(uf(2 * m) + uf(2 * m + 1))
                        elif part == 1:
                            k.append(kf(2 * m) - kf(2 * m - 1) if m else kf(0))
                            u.append(uf(2 * m + 1))
                        else:
                            k.append(kf(2 * m) - kf(2 * m + 1))
                            u.append(uf(2 * m))
                        y = k[0] * u[m]
                        for j in range(1, m + 1):
                            y = y + k[j] * u[m - j]
                        if plane:
                            y = shared[m] - y if plane == 1 else shared[m] + y
                        out.append(y)
                        if base:
                            r = (h // 2 * _NB + 2 * m + part - 1) * 2 + h % 2
                            arena[c, _ROW_W + (plane - 1) * _WQ + r] = pltpu.bitcast(base[m] - y, i32)
                        else:
                            arena[c, _ROW_P + plane * 8 + m] = pltpu.bitcast(y, i32)
                    if plane == 0:
                        shared = out
                    run_jobs((h * 3 + part) * 3 + plane + 1)
        run_jobs(np.inf)

    start("vectors", ldt_hbm, ldt_v)
    start("vectors", dsk_hbm, dsk_v)
    start_parameters("step 0", pl.ds(0, 8 * _GA))
    start_parameters("step 1", pl.ds(8 * _GA, 8 * _GA))
    start_parameters("later steps", pl.ds(16 * _GA, _D // 2 - 16 * _GA))
    for k, parts in enumerate(_dft_rows()):
        dft_v[pl.ds(8 * k, 8), :] = jnp.concatenate(list(parts), axis=1)
    arena[0, _ROW_W:_ROW_P] = jnp.zeros((_ROW_P - _ROW_W, 8, _T), i32)
    tap_v[...] = jnp.zeros(tap_v.shape, i32)
    k_v[:_GA] = jnp.zeros((_GA, _NB, 8, _T), i32)
    key_v[...] = jnp.zeros(key_v.shape, f32)
    wait("vectors")
    start("input", x_hbm.bitcast(i32), x_v)
    start("input", wr_hbm, wr_v)
    dt = jnp.exp(ldt_v[...].astype(f32)).reshape(1, _D)
    skip = dsk_v[...].astype(f32).reshape(1, _D)
    dt_v[:_T // 2] = _column(dt[:, :_T])
    skip_v[:_T // 2] = _column(skip[:, :_T])
    wait("step 0")
    modes(0)
    dt_v[_T // 2:] = _column(dt[:, _T:])
    skip_v[_T // 2:] = _column(skip[:, _T:])
    wait("step 1")

    def filter_loop(i, carry):
        @pl.when(i == 1)
        def _():
            wait("later steps")
            for cp in hidden_copies(0) + hidden_copies(1):
                cp.start()

        @pl.when(i == _LN_STEP)
        def _():
            wait("input")
            for cp in hidden_copies(2) + hidden_copies(3):
                cp.start()
            layer_norm()
            inv_v[...] = pltpu.bitcast(dft_v[...], bf16).astype(f32).T * (2 / _T)

        for t in range(2):
            pop_best(2 * (i - _LN_STEP) + t)
        list(filter_step(i, i >> 8))
        modes(i + 1)

    last = _NG // _GA - 1
    assert 2 * (last - _LN_STEP) == _C
    lax.fori_loop(0, last, filter_loop, None)
    for cp in hidden_copies(4) + hidden_copies(5):
        cp.start()
    zero = routed_tokens()[0, 0] >> 11
    parts = [gather(range(u * _C // _GA, (u + 1) * _C // _GA)) for u in filter_step(last, zero)]
    x_sel = sum(parts[1:], parts[0])
    for n in range(_NO):
        sel_v[n] = x_sel[:, n * _OCH:(n + 1) * _OCH]
    x_sel = jnp.concatenate([x_sel, jnp.zeros((8, _KT * _T - _D), f32)], axis=1)
    for k in range(_KT):
        arena[0, _ROW_SEL + k] = pltpu.bitcast(
            jnp.concatenate([x_sel[:, k * _T:(k + 1) * _T]] * 2, axis=0).astype(bf16), i32)
    input_spectra([arena[0, _ROW_X + r] for r in range(_R)], uf_a)
    for u in range(_GA):
        spread(last, u, _GA + u)
    filter_spectra(_NG - 3 * _GA // 2, range(_GA // 2, 2 * _GA))

    def hidden_loop(slab, carry):
        for cp in hidden_copies(slab):
            cp.wait()

        @pl.when(slab == 2)
        def _():
            for n in range(_NO):
                down_copy(n).start()

        conv_step(2 * slab, uf_a, uf_b, hidden_jobs(slab, 0), 240, 0.87)
        conv_step(2 * slab + 1, uf_b, uf_a, hidden_jobs(slab, 1), 240, 0.87)

    def output_loop(n, carry):
        down_copy(n).wait()

        @pl.when(n == _OUT_STEP)
        def _():
            for k in range(_OUT_STEP - 1):
                out_copy(k).start()

        c = n + _NCH - _NO
        lax.cond(c & 1 == 0, lambda: conv_step(c, uf_a, uf_b, output_jobs(c), 32, 0.8),
                 lambda: conv_step(c, uf_b, uf_a, output_jobs(c), 32, 0.8))

    lax.fori_loop(0, _NF, hidden_loop, None)
    for t in range(_F // _T):
        tile = hid_v[t * _T // _FCH, :, pl.ds(t * _T % _FCH, _T)]
        o_v[spare(t)] = tile
        arena[0, _ROW_W + t] = pltpu.bitcast(jnp.concatenate([tile] * 2, axis=0), i32)
    down_copy(0).wait()
    conv_step(_NCH - _NO + zero, uf_a, uf_b, first_output_jobs(zero), 432, 0.87)
    lax.fori_loop(1, _NO, output_loop, None)
    s_v[_NCH - 1] = _dot(
        jnp.concatenate([output_spectrum(_NCH - 1, r) for r in range(_R)], axis=0), inv_v[...])
    for done in finish(_NO - 1):
        if done % _R == 0:
            rows = pl.ds((_NO - 1) * _OCH + (done // _R - 1) * 16 * _GC, 16 * _GC)
            start("last slab", o_v.at[rows], o_hbm.at[rows])
    for n in range(_NO - 1):
        out_copy(n).wait()
    wait("last slab")


@jax.jit
def pallas_recurrent_scan__ssm_conv_s4__moe_arch_mod__prompt_kernel(
    A_u: jax.Array,
    A_A_re: jax.Array,
    A_A_im: jax.Array,
    A_B_re: jax.Array,
    A_B_im: jax.Array,
    A_C_re: jax.Array,
    A_C_im: jax.Array,
    A_log_dt: jax.Array,
    A_Dskip: jax.Array,
    B_x: jax.Array,
    B_w_r: jax.Array,
    B_w_gate: jax.Array,
    B_w_up: jax.Array,
    B_w_down: jax.Array,
):
    del B_x
    assert A_u.shape == (1, _L, _D) and A_A_re.shape == (_D, _N) and B_w_gate.shape == (_D, _F)
    assert A_u.dtype == bf16 and A_A_re.dtype == bf16
    hbm = pl.BlockSpec(memory_space=pl.ANY)
    vmem = pltpu.VMEM
    out = pl.pallas_call(
        _kernel,
        out_shape=jax.ShapeDtypeStruct((_D, _L), bf16),
        in_specs=[hbm] * 13,
        out_specs=hbm,
        scratch_shapes=[
            vmem((_D // 2, _L), i32), vmem((6, _D // 2, _N), i32),
            vmem((_NF, _D // 2, _FCH), i32), vmem((_NF, _D // 2, _FCH), i32),
            vmem((_NO, _OCH // 2, _F), i32),
            vmem((_T // 2, 2 * _T), i32), vmem((_D + 32, _L), bf16),
            vmem((_D // 2, _T), i32), vmem((_D // 2, _T), i32), vmem((_GA, 2, 4, 8, _N), f32),
            vmem((_NG, 8, _T), i32), vmem((_GA, len(_TAPS), 8, _T), i32),
            vmem((2 * _GA, _NB, 8, _T), i32), vmem((2 * _NG, 3 * _PLANE, 8, _T), f32),
            vmem((_NB, _D + 32, _T), f32), vmem((2 * _T, _T), f32), vmem((_NCH, _ROWS, 8, _T), i32),
            vmem((6 * _GC * _PLANE, 8, _T), f32), vmem((6 * _GC * _PLANE, 8, _T), f32),
            vmem((_NCH, 16 * _R, _T), f32),
            vmem((3, _NB, 8, _T), f32), vmem((3, 8, _T), f32), vmem((_NO, 8, _OCH), f32),
            vmem((_NF, 8, _FCH), bf16), vmem((_D,), bf16), vmem((_D,), bf16), vmem((_D,), bf16),
            pltpu.SemaphoreType.DMA((6,)), pltpu.SemaphoreType.DMA((_NF + _NO,)),
            pltpu.SemaphoreType.DMA(()),
        ],
        compiler_params=pltpu.CompilerParams(vmem_limit_bytes=100 * 2**20),
    )(A_u.reshape(_L, _D).T, A_A_re, A_A_im, A_B_re, A_B_im, A_C_re, A_C_im, A_log_dt, A_Dskip,
      B_w_r, B_w_gate, B_w_up, B_w_down.T)
    return out.T.reshape(1, _L, _D)
```

```python
import jax
import jax.numpy as jnp
import numpy as np
from jax import lax
import jax.experimental.pallas as pl
import jax.experimental.pallas.tpu as pltpu

f32, bf16, i32 = jnp.float32, jnp.bfloat16, jnp.int32

_D, _L, _N, _F, _C = 576, 2048, 128, 4608, 8
_EPS = 1e-5
_T = 128
_NB = _L // _T
_NG = _D // 16
_GA = 4
_GC = 2
_NCH = _NG // _GC
_R = _GC * _NB
_KT = -(-_D // _T)
_NF, _FCH = 6, _F // 6
_NO, _OCH = 6, _D // 6
_LN_STEP = 4
_OUT_STEP = 3
_ROW_X, _ROW_W, _WQ, _ROW_SEL, _ROW_P = 0, _R, 2 * _R + 1, 5 * _R + 3, 5 * _R + 8
_ROWS = _ROW_P + 3 * _NB // 2
_PLANE = _NB + 1


def _lag_step(j):
    return max(1, (1 << (j * _T).bit_length()) >> 8)


def _round_lag(p, step):
    if step == 1:
        return p
    return (p + (step // 2 - 1) + ((p >> (step.bit_length() - 1)) & 1)) & ~(step - 1)


assert np.array_equal(
    np.concatenate([j * _T + _round_lag(np.arange(_T), _lag_step(j)) for j in range(_NB)]),
    np.arange(_L).astype(bf16).astype(np.int64))

_PAIRS = (((0, 1), (0, 5)), ((0, 2), (0, 6)), ((0, 3), (0, 7)), ((0, 4), (0, 8)), ((1, 2), (1, 6)),
          ((1, 4), (1, 8)), ((2, 4), (2, 8)), ((3, 4), (3, 8)), ((4, 8), (5, 8)), ((6, 8), (7, 8)))
_TAPS = [k for pair in _PAIRS for k in pair]


def _ds(start, size, align):
    return pl.ds(start if isinstance(start, int) else pl.multiple_of(start, align), size)


def _cmul(a, b):
    return a[0] * b[0] - a[1] * b[1], a[0] * b[1] + a[1] * b[0]


def _csq(a):
    return a[0] * a[0] - a[1] * a[1], (a[0] + a[0]) * a[1]


def _silu_of_twice(h):
    return h + h * jnp.tanh(h)


def _rnd(x):
    return x.astype(bf16).astype(f32)


def _dot(a, b):
    return jnp.dot(a, b, preferred_element_type=f32)


def _dot_nt(a, b):
    return lax.dot_general(a, b, (((1,), (1,)), ((), ())), preferred_element_type=f32)


def _column(v):
    return pltpu.bitcast(jnp.broadcast_to(v, (_T, v.shape[1])).astype(bf16).T, i32)


def _even_odd(words):
    return pltpu.bitcast(words << 16, f32), pltpu.bitcast(words & -65536, f32)


def _interleave(even, odd):
    even, odd = [pltpu.bitcast(x, i32) + 0x8000 for x in (even, odd)]
    return lax.shift_right_logical(even, 16) | (odd & -65536)


def _dft_rows():
    row = lax.broadcasted_iota(i32, (8, _T), 0)
    root = 4 * lax.broadcasted_iota(i32, (8, _T), 1) + 1

    def power(t):
        angle = ((root * t) & (4 * _T - 1)).astype(f32) * (np.pi / (2 * _T))
        return jnp.cos(angle), jnp.sin(angle)

    even, z, z16 = [power(2 * row)], power(1), power(16)
    for _ in range(_T // 16 - 1):
        even.append(_cmul(even[-1], z16))
    return [map(_interleave, e, _cmul(e, z)) for e in even]


def _modes(dt, ar, ai, br, bi, cr, ci):
    zr, zi = dt * ar, dt * ai
    mag = 1.0 + jnp.tanh(0.5 * zr) * (1.0 + jnp.exp(zr))
    return _cmul((cr, ci), (dt * br, dt * bi)) + (mag * jnp.cos(zi), mag * jnp.sin(zi))


def _seeds(w, a1):
    a = {1: a1}
    for n in range(9):
        a[2 << n] = _csq(a[1 << n])
    row = lax.broadcasted_iota(i32, (8, _N), 0)

    def mix(z0, z1):
        rolled = [pltpu.roll(x, 4, 0) for x in z1]
        return ([jnp.where(row < 4, x, y) for x, y in zip(z0, rolled)],
                [jnp.where(row < 4, y, x) for x, y in zip(z0, rolled)])

    def dup(z):
        return [[jnp.take_along_axis(x, (row & 3) + 4 * q, axis=0, mode="promise_in_bounds")
                 for x in z] for q in range(2)]

    wa = _cmul(w, a1)
    return zip(mix((1.0, 0.0), a[128]), dup(a[8]), dup(a[32]),
               mix(wa, _cmul(wa, a[4])), dup(a1), dup(a[256]),
               mix(_cmul(a[256], a[4]), a[512]), dup(a[512]))


def _vandermonde(e0, m8, m32, g0, m1, m256, m_top, m512):
    e = [e0]
    for s in range(1, 16):
        e.append(_cmul(e[s - 1], m8) if s < 4 else _cmul(e[s - 4], m32))
    g = [g0]
    for _ in range(3):
        g.append(_cmul(g[-1], m1))
    g += [_cmul(g[1], m256), _cmul(g[3], m256)]
    g += [_cmul(g[3], m512), _cmul(g[5], m512)]
    g.append(_cmul(g[7], m_top))
    g.append(_cmul(g[8], m512))
    re, im = [_dot_nt(jnp.concatenate([z[p] for z in g], axis=0),
                      jnp.concatenate([z[p] for z in e], axis=0)) for p in range(2)]
    return re - im


def _unmix(lo, hi):
    row = lax.broadcasted_iota(i32, (8, _T), 0)
    for m in range(len(_PAIRS)):
        x, y = lo[8 * m:8 * m + 8], hi[8 * m:8 * m + 8]
        yield jnp.where(row < 4, x, y)
        yield pltpu.roll(jnp.where(row < 4, y, x), 4, 0)


def _lag_blocks(tap, lag0):
    lane = lax.broadcasted_iota(i32, (8, _T), 1)
    row = lax.broadcasted_iota(i32, (8, _T), 0)
    for h in range(2):
        def lane_of(lag):
            s = ((_T * h + lag) >> 3) & 31
            return ((s & 15) << 3) + (row ^ ((s >> 4) << 2))

        def take(big, r, at):
            return jnp.take_along_axis(tap(_TAPS.index((big, r))), at, axis=1,
                                       mode="promise_in_bounds")

        at = lane_of(_round_lag(lane, 8) - 8)
        top = [take(big, 8, at) for big in range(_NB // 2)]
        at = lane_of(lane)
        for big, blk in enumerate(top):
            step = _lag_step(2 * big + h)
            lag = _round_lag(lane, step)
            if h == 0:
                blk = jnp.where(lag == 0, top[big - 1] if big else lag0, blk)
            for r in range(step, 8, step):
                blk = jnp.where((lag & 7) == r, take(big, r, at), blk)
            yield 2 * big + h, blk


def _kernel(x_hbm, ar_hbm, ai_hbm, br_hbm, bi_hbm, cr_hbm, ci_hbm, ldt_hbm, dsk_hbm, wr_hbm,
            wg_hbm, wu_hbm, wd_hbm, o_hbm,
            x_v, par_v, wg_v, wu_v, wd_v, dft_v, o_v,
            dt_v, skip_v, mode_v, k0_v, tap_v, k_v, kf_v,
            xf_v, inv_v, arena, uf_a, uf_b, s_v,
            stat_v, key_v, sel_v, hid_v, ldt_v, dsk_v, wr_v, sem, w_sem, o_sem):
    row = lax.broadcasted_iota(i32, (8, _T), 0)
    lane = lax.broadcasted_iota(i32, (8, _T), 1)

    groups = {}

    def start(name, src, dst):
        slot, pairs = groups.setdefault(name, (len(groups), []))
        pairs.append((src, dst))
        pltpu.make_async_copy(src, dst, sem.at[slot]).start()

    def wait(name):
        slot, pairs = groups[name]
        for src, dst in pairs:
            pltpu.make_async_copy(src, dst, sem.at[slot]).wait()

    def start_parameters(name, rows):
        for n, src in enumerate((ar_hbm, ai_hbm, br_hbm, bi_hbm, cr_hbm, ci_hbm)):
            start(name, src.bitcast(i32).at[rows], par_v.at[n, rows])

    def hidden_copies(n):
        cols = _ds(n * _FCH, _FCH, _FCH)
        return [pltpu.make_async_copy(w.bitcast(i32).at[:, cols], v.at[n], w_sem.at[n])
                for w, v in ((wg_hbm, wg_v), (wu_hbm, wu_v))]

    def down_copy(n):
        return pltpu.make_async_copy(wd_hbm.bitcast(i32).at[_ds(n * (_OCH // 2), _OCH // 2, 16)],
                                     wd_v.at[n], w_sem.at[_NF + n])

    def out_copy(n):
        rows = _ds(n * _OCH, _OCH, 32)
        return pltpu.make_async_copy(o_v.at[rows], o_hbm.at[rows], o_sem)

    def compact(k, h):
        out = stat_v[k, 8 * h]
        for s in range(1, 8):
            out = jnp.where(row == s, stat_v[k, 8 * h + s], out)
        return out

    def layer_norm():
        def moments(b, carry):
            cols = _ds(b * _T, _T, _T)
            pivot = jnp.broadcast_to(_even_odd(x_v[:8, cols])[0][:1], (8, _T))
            s1, s2 = [None] * 2, [None] * 2
            for g in range(_NG):
                x = pltpu.bitcast(x_v[pl.ds(8 * g, 8), cols], bf16).astype(f32)
                xf_v[b, pl.ds(16 * g, 16), :] = x
                for h in range(2):
                    d = x[8 * h:8 * h + 8] - pivot
                    s1[h] = s1[h] + d if g else d
                    s2[h] = s2[h] + d * d if g else d * d
            for k, s in enumerate((s1, s2)):
                stat_v[k, b] = jnp.broadcast_to(jnp.sum(s[0] + s[1], axis=0, keepdims=True), (8, _T))
            stat_v[2, b] = pivot

        lax.fori_loop(0, _NB, moments, None, unroll=4)
        for h in range(_NB // 8):
            m1, m2 = compact(0, h) / _D, compact(1, h) / _D
            mean = _rnd(compact(2, h) + m1)
            var = _rnd(jnp.maximum(m2 - m1 * m1, 0.0))
            gain = 0.5 / _rnd(jnp.sqrt(_rnd(var + _rnd(jnp.full_like(var, _EPS)))))
            for s in range(8):
                stat_v[0, 8 * h + s] = jnp.broadcast_to(mean[s:s + 1], (8, _T))
                stat_v[1, 8 * h + s] = jnp.broadcast_to(gain[s:s + 1], (8, _T))
        wr = jnp.broadcast_to(wr_v[...].astype(f32).reshape(1, _D), (8, _D)).astype(bf16)
        for b in range(_NB):
            mean, gain = stat_v[0, b], stat_v[1, b]
            xn = []
            for g in range(_NG):
                xc = _rnd(jnp.concatenate([xf_v[b, pl.ds(16 * g + h, 8, stride=2), :] - mean
                                           for h in range(2)], axis=1))
                xn.append(_interleave(xc[:, :_T] * gain, xc[:, _T:] * gain))
            for g in range(_NG):
                arena[g // _GC, _ROW_X + (g % _GC) * _NB + b] = xn[g]
            stat_v[2, b] = _dot(wr, pltpu.bitcast(jnp.concatenate(xn, axis=0), bf16))
        for h in range(_NB // 8):
            bits = pltpu.bitcast(_rnd(2.0 * compact(2, h)), i32) >> 16
            rank = jnp.where(bits < 0, 0x8000 - (bits & 0x7FFF), 0x8000 + bits)
            token = (8 * h + row) * _T + lane
            key_v[h] = pltpu.bitcast((1 << 28) + rank * _L + (_L - 1 - token), f32)

    def pop_best(t):
        best = jnp.max(jnp.max(jnp.maximum(key_v[0], key_v[1]), axis=0, keepdims=True),
                       axis=1, keepdims=True)
        key_v[2] = jnp.where(row == t, best, key_v[2])
        for h in range(2):
            key_v[h] = jnp.where(key_v[h] == best, 0.0, key_v[h])

    def routed_tokens():
        return _L - 1 - (pltpu.bitcast(key_v[2], i32) & (_L - 1))

    def routed_scores():
        rank = (pltpu.bitcast(key_v[2], i32) - (1 << 28)) >> 11
        return pltpu.bitcast(jnp.where(rank < 0x8000, 0x10000 - rank, rank - 0x8000) << 16, f32)

    def gather(tokens):
        token = routed_tokens()
        blocks = jnp.concatenate(
            [pltpu.bitcast(jnp.concatenate(
                [arena[g // _GC, _ROW_X + (g % _GC) * _NB + b] for g in range(_NG)], axis=0), bf16)
             for b in [token[t, 0] >> 7 for t in tokens]], axis=1)
        pick = jnp.concatenate(
            [jnp.where((row == t) & ((token & (_T - 1)) == lane), 2.0, 0.0) for t in tokens], axis=1)
        return _dot_nt(pick.astype(bf16), blocks)

    def dft(rows):
        z = _dot(jnp.concatenate([pltpu.bitcast(r, bf16) for r in rows], axis=0),
                 pltpu.bitcast(dft_v[...], bf16))
        return [[(z[o:o + 8, :_T], z[o:o + 8, _T:])
                 for o in range(h // 2 * 16 * _NB + 8 * (h % 2), (h // 2 + 1) * 16 * _NB, 16)]
                for h in range(2 * len(rows) // _NB)]

    def modes(step):
        for u in range(_GA):
            grp = step * _GA + u
            rows = _ds(grp * 8, 8, 8)
            par = [_even_odd(dt_v[rows, :])] + [_even_odd(par_v[n, rows, :]) for n in range(6)]
            k0 = []
            for h, skip in enumerate(_even_odd(skip_v[rows, :])):
                z = _modes(*[p[h] for p in par])
                for n in range(4):
                    mode_v[u, h, n] = z[n]
                k0.append(skip + jnp.sum(z[0], axis=1, keepdims=True))
            k0_v[grp] = _interleave(*k0)

    def spread(step, u, slot):
        for j, blk in _lag_blocks(lambda n: tap_v[u, n], k0_v[step * _GA + u]):
            k_v[slot, j] = blk

    def filter_spectra(grp, slots):
        for h, blocks in enumerate(dft([k_v[slot, j] for slot in slots for j in range(_NB)])):
            at = 2 * grp + h
            for j, (re, im) in enumerate(blocks):
                for plane, val in enumerate((re, re + im, im - re)):
                    kf_v[at, plane * _PLANE + j] = val

    def filter_step(i, zero):
        for u in range(_GA):
            if u % (_GA // 2) == 0:
                old = (u + _GA // 2) % _GA
                filter_spectra(jnp.maximum(i - (1 if u else 2), 0) * _GA + old,
                               [old + k + zero for k in range(_GA // 2)])
            spread(jnp.maximum(i - 1, 0), u, u)
            even, odd = [[_vandermonde(*seeds) for seeds in _seeds(
                (mode_v[u, h, 0], mode_v[u, h, 1]), (mode_v[u, h, 2], mode_v[u, h, 3]))]
                         for h in range(2)]
            for n, tap in enumerate(_unmix(*map(_interleave, even, odd))):
                tap_v[u, n] = tap
            yield u

    def hidden_jobs(slab, half):
        pre = []

        def project(n):
            cols = pl.ds(half * _FCH // 2 + n // 2 * _T, _T)
            x_sel = jnp.concatenate(
                [pltpu.bitcast(arena[slab >> 8, _ROW_SEL + k], bf16) for k in range(_KT)], axis=1)
            weight = pltpu.bitcast((wu_v if n % 2 else wg_v)[slab, :, cols], bf16)
            pre.append(_rnd(_dot(x_sel[:, :_D], weight)[:8]))
            if n % 2:
                hid_v[slab, :, cols] = (_rnd(_silu_of_twice(0.5 * pre[-2])) * pre[-1]).astype(bf16)

        return [(40 * n, lambda n=n: project(n)) for n in range(_FCH // _T)]

    def scatters(n, hid):
        y = _rnd(_dot_nt(jnp.concatenate(hid, axis=1), pltpu.bitcast(wd_v[n], bf16)))
        y = 0.5 * (sel_v[n] + _rnd(y * _rnd(jax.nn.sigmoid(routed_scores()))[:, :_OCH]))
        col = jnp.concatenate([y, jnp.zeros((_T - _C, _OCH), f32)], axis=0).T
        col = pltpu.bitcast(col.astype(bf16), i32)
        token = routed_tokens()

        def scatter(t):
            hit = ((token & (_T - 1)) == lane)[t:t + 1]
            new = jnp.broadcast_to(col[:, t:t + 1], (_OCH // 2, _T))
            where = [(n * (_OCH // (16 * _GC)) + g // _GC,
                      _ROW_X + (g % _GC) * _NB + (token[t, 0] >> 7)) for g in range(_OCH // 16)]
            old = [arena[at] for at in where]
            for g, at in enumerate(where):
                arena[at] = jnp.where(hit, new[8 * g:8 * g + 8], old[g])

        return [lambda t=t: scatter(t) for t in range(_C)]

    def finish(n):
        for k in range(0, _OCH // 16 * _NB, 2):
            c, r = n * (_OCH // (16 * _GC)) + k // _R, k % _R
            rows = _ds(n * _OCH + 16 * (k // _NB), 16, 16)
            out = []
            for d in range(2):
                gate = _silu_of_twice(pltpu.bitcast(arena[c, _ROW_X + r + d], bf16).astype(f32))
                out.append(xf_v[k % _NB + d, rows, :] + s_v[c, pl.ds(16 * (r + d), 16), :] * gate)
            o_v[rows, pl.ds(k % _NB * _T, 2 * _T)] = jnp.concatenate(out, axis=1).astype(bf16)
            yield k + 2

    def spare(t, zero=0):
        return _ds(_D + 8 * (t // _NB + zero), 8, 8), pl.ds(t % _NB * _T, _T)

    def first_output_jobs(zero):
        hid, scatter = [], []

        def read():
            hid.extend([pltpu.bitcast(arena[zero, _ROW_W + t], bf16)[:8]
                        for t in range(len(hid), len(hid) + 4)])

        return ([(48 * k, read) for k in range(_F // (4 * _T))]
                + [(431, lambda: scatter.extend(scatters(0, hid)))]
                + [(992 + 14 * t, lambda t=t: scatter[t]()) for t in range(_C)])

    def output_jobs(c):
        n = c - (_NCH - _NO)
        hid = [o_v[spare(t, c >> 8)] for t in range(4)]
        for done in finish(n - 1):
            if done == _OCH // 16 * _NB:
                pl.when(n >= _OUT_STEP)(lambda: out_copy(n - 1).start())
                o_v[spare(_F // _T, c >> 9)] = hid[0]
            if done % 12 == 0:
                hid += [o_v[spare(t, c >> 8)] for t in range(len(hid), len(hid) + 4)]
        return [(560 + 14 * t, job) for t, job in enumerate(scatters(n, hid))]

    def input_spectra(rows, dst):
        z = dft(rows)
        for h, blocks in enumerate(z):
            for b, (re, im) in enumerate(blocks):
                if b:
                    re, im = re + blocks[b - 1][1], im - blocks[b - 1][0]
                for plane, val in enumerate((re + im, im, re)):
                    dst[h, plane * _PLANE + b] = val
        return z

    def output_spectrum(c, r):
        return jnp.concatenate(
            [pltpu.bitcast(arena[c, pl.ds(_ROW_W + q * _WQ + 2 * r, 2)].reshape(16, _T), f32)
             for q in range(2)], axis=1)

    def conv_step(c, cur, nxt, ffn_jobs, delay, pace):
        c_next, c_prev = jnp.minimum(c + 1, _NCH - 1), jnp.maximum(c - 1, 0)
        zero = c >> 8
        c_again = c + zero
        fwd_rows, inv_rows, results = [], [], []

        def transform():
            y = _dot(jnp.concatenate(inv_rows, axis=0), inv_v[...])
            s_v[c_prev] = y
            results.extend((y, input_spectra(fwd_rows, nxt)))

        def drain(r):
            y, z = results
            arena[c, _ROW_SEL - 1] = pltpu.bitcast(
                y[8 * r:8 * r + 8] + z[2 * (r // _R) + 1][r % _R // 2][r // 8 % 2], i32)

        jobs = sorted(
            ffn_jobs
            + [(delay + 16 * r, lambda r=r: inv_rows.append(output_spectrum(c_prev, r)))
               for r in range(_R)]
            + [(delay + 16 * r, lambda r=r: fwd_rows.append(arena[c_next, _ROW_X + r]))
               for r in range(_R)]
            + [(delay + 16 * _R, transform)]
            + [(delay + 140 + 8 * r, lambda r=r: drain(r)) for r in range(2 * _R - 17, 2 * _R, 8)],
            key=lambda job: job[0])

        def run_jobs(done):
            while jobs and done * (delay + 16 * _R) >= (jobs[0][0] - 32) * pace * 18 * _GC:
                jobs.pop(0)[1]()

        run_jobs(0)
        for h in range(2 * _GC):
            for part in range(3):
                at_k, at_u = c * 2 * _GC + h + (zero >> part), h + (zero >> part)
                for plane in range(3):
                    kf = lambda b: kf_v[at_k, plane * _PLANE + b]
                    uf = lambda b: cur[at_u, plane * _PLANE + b]
                    base = [pltpu.bitcast(arena[c_again, _ROW_P + plane * 8 + m], f32)
                            for m in range(_NB // 2) if part and plane]
                    k, u, out = [], [], []
                    for m in range(_NB // 2):
                        if part == 0:
                            k.append(kf(2 * m))
                            u.append(uf(2 * m) + uf(2 * m + 1))
                        elif part == 1:
                            k.append(kf(2 * m) - kf(2 * m - 1) if m else kf(0))
                            u.append(uf(2 * m + 1))
                        else:
                            k.append(kf(2 * m) - kf(2 * m + 1))
                            u.append(uf(2 * m))
                        y = k[0] * u[m]
                        for j in range(1, m + 1):
                            y = y + k[j] * u[m - j]
                        if plane:
                            y = shared[m] - y if plane == 1 else shared[m] + y
                        out.append(y)
                        if base:
                            r = (h // 2 * _NB + 2 * m + part - 1) * 2 + h % 2
                            arena[c, _ROW_W + (plane - 1) * _WQ + r] = pltpu.bitcast(base[m] - y, i32)
                        else:
                            arena[c, _ROW_P + plane * 8 + m] = pltpu.bitcast(y, i32)
                    if plane == 0:
                        shared = out
                    run_jobs((h * 3 + part) * 3 + plane + 1)
        run_jobs(np.inf)

    start("vectors", ldt_hbm, ldt_v)
    start("vectors", dsk_hbm, dsk_v)
    start_parameters("step 0", pl.ds(0, 8 * _GA))
    start_parameters("step 1", pl.ds(8 * _GA, 8 * _GA))
    start_parameters("later steps", pl.ds(16 * _GA, _D // 2 - 16 * _GA))
    for k, parts in enumerate(_dft_rows()):
        dft_v[pl.ds(8 * k, 8), :] = jnp.concatenate(list(parts), axis=1)
    arena[0, _ROW_W:_ROW_P] = jnp.zeros((_ROW_P - _ROW_W, 8, _T), i32)
    tap_v[...] = jnp.zeros(tap_v.shape, i32)
    k_v[:_GA] = jnp.zeros((_GA, _NB, 8, _T), i32)
    key_v[...] = jnp.zeros(key_v.shape, f32)
    wait("vectors")
    start("input", x_hbm.bitcast(i32), x_v)
    start("input", wr_hbm, wr_v)
    dt = jnp.exp(ldt_v[...].astype(f32)).reshape(1, _D)
    skip = dsk_v[...].astype(f32).reshape(1, _D)
    dt_v[:_T // 2] = _column(dt[:, :_T])
    skip_v[:_T // 2] = _column(skip[:, :_T])
    wait("step 0")
    modes(0)
    dt_v[_T // 2:] = _column(dt[:, _T:])
    skip_v[_T // 2:] = _column(skip[:, _T:])
    wait("step 1")

    def filter_loop(i, carry):
        @pl.when(i == 1)
        def _():
            wait("later steps")
            for cp in hidden_copies(0) + hidden_copies(1):
                cp.start()

        @pl.when(i == _LN_STEP)
        def _():
            wait("input")
            for cp in hidden_copies(2) + hidden_copies(3):
                cp.start()
            layer_norm()
            inv_v[...] = pltpu.bitcast(dft_v[...], bf16).astype(f32).T * (2 / _T)

        for t in range(2):
            pop_best(2 * (i - _LN_STEP) + t)
        list(filter_step(i, i >> 8))
        modes(i + 1)

    last = _NG // _GA - 1
    assert 2 * (last - _LN_STEP) == _C
    lax.fori_loop(0, last, filter_loop, None)
    for cp in hidden_copies(4) + hidden_copies(5):
        cp.start()
    zero = routed_tokens()[0, 0] >> 11
    parts = [gather(range(u * _C // _GA, (u + 1) * _C // _GA)) for u in filter_step(last, zero)]
    x_sel = sum(parts[1:], parts[0])
    for n in range(_NO):
        sel_v[n] = x_sel[:, n * _OCH:(n + 1) * _OCH]
    x_sel = jnp.concatenate([x_sel, jnp.zeros((8, _KT * _T - _D), f32)], axis=1)
    for k in range(_KT):
        arena[0, _ROW_SEL + k] = pltpu.bitcast(
            jnp.concatenate([x_sel[:, k * _T:(k + 1) * _T]] * 2, axis=0).astype(bf16), i32)
    input_spectra([arena[0, _ROW_X + r] for r in range(_R)], uf_a)
    for u in range(_GA):
        spread(last, u, _GA + u)
    filter_spectra(_NG - 3 * _GA // 2, range(_GA // 2, 2 * _GA))

    def hidden_loop(slab, carry):
        for cp in hidden_copies(slab):
            cp.wait()

        @pl.when(slab == 2)
        def _():
            for n in range(_NO):
                down_copy(n).start()

        conv_step(2 * slab, uf_a, uf_b, hidden_jobs(slab, 0), 240, 0.87)
        conv_step(2 * slab + 1, uf_b, uf_a, hidden_jobs(slab, 1), 240, 0.87)

    def output_loop(n, carry):
        down_copy(n).wait()

        @pl.when(n == _OUT_STEP)
        def _():
            for k in range(_OUT_STEP - 1):
                out_copy(k).start()

        c = n + _NCH - _NO
        lax.cond(c & 1 == 0, lambda: conv_step(c, uf_a, uf_b, output_jobs(c), 32, 0.8),
                 lambda: conv_step(c, uf_b, uf_a, output_jobs(c), 32, 0.8))

    lax.fori_loop(0, _NF, hidden_loop, None)
    for t in range(_F // _T):
        tile = hid_v[t * _T // _FCH, :, pl.ds(t * _T % _FCH, _T)]
        o_v[spare(t)] = tile
        arena[0, _ROW_W + t] = pltpu.bitcast(jnp.concatenate([tile] * 2, axis=0), i32)
    down_copy(0).wait()
    conv_step(_NCH - _NO + zero, uf_a, uf_b, first_output_jobs(zero >> 1), 432, 0.87)
    lax.fori_loop(1, _NO, output_loop, None)
    s_v[_NCH - 1] = _dot(
        jnp.concatenate([output_spectrum(_NCH - 1, r) for r in range(_R)], axis=0), inv_v[...])
    for done in finish(_NO - 1):
        if done % _R == 0:
            rows = pl.ds((_NO - 1) * _OCH + (done // _R - 1) * 16 * _GC, 16 * _GC)
            start("last slab", o_v.at[rows], o_hbm.at[rows])
    for n in range(_NO - 1):
        out_copy(n).wait()
    wait("last slab")


@jax.jit
def pallas_recurrent_scan__ssm_conv_s4__moe_arch_mod__prompt_kernel(
    A_u: jax.Array,
    A_A_re: jax.Array,
    A_A_im: jax.Array,
    A_B_re: jax.Array,
    A_B_im: jax.Array,
    A_C_re: jax.Array,
    A_C_im: jax.Array,
    A_log_dt: jax.Array,
    A_Dskip: jax.Array,
    B_x: jax.Array,
    B_w_r: jax.Array,
    B_w_gate: jax.Array,
    B_w_up: jax.Array,
    B_w_down: jax.Array,
):
    del B_x
    assert A_u.shape == (1, _L, _D) and A_A_re.shape == (_D, _N) and B_w_gate.shape == (_D, _F)
    assert A_u.dtype == bf16 and A_A_re.dtype == bf16
    hbm = pl.BlockSpec(memory_space=pl.ANY)
    vmem = pltpu.VMEM
    out = pl.pallas_call(
        _kernel,
        out_shape=jax.ShapeDtypeStruct((_D, _L), bf16),
        in_specs=[hbm] * 13,
        out_specs=hbm,
        scratch_shapes=[
            vmem((_D // 2, _L), i32), vmem((6, _D // 2, _N), i32),
            vmem((_NF, _D // 2, _FCH), i32), vmem((_NF, _D // 2, _FCH), i32),
            vmem((_NO, _OCH // 2, _F), i32),
            vmem((_T // 2, 2 * _T), i32), vmem((_D + 32, _L), bf16),
            vmem((_D // 2, _T), i32), vmem((_D // 2, _T), i32), vmem((_GA, 2, 4, 8, _N), f32),
            vmem((_NG, 8, _T), i32), vmem((_GA, len(_TAPS), 8, _T), i32),
            vmem((2 * _GA, _NB, 8, _T), i32), vmem((2 * _NG, 3 * _PLANE, 8, _T), f32),
            vmem((_NB, _D + 32, _T), f32), vmem((2 * _T, _T), f32), vmem((_NCH, _ROWS, 8, _T), i32),
            vmem((2 * _GC, 3 * _PLANE, 8, _T), f32), vmem((2 * _GC, 3 * _PLANE, 8, _T), f32),
            vmem((_NCH, 16 * _R, _T), f32),
            vmem((3, _NB, 8, _T), f32), vmem((3, 8, _T), f32), vmem((_NO, 8, _OCH), f32),
            vmem((_NF, 8, _FCH), bf16), vmem((_D,), bf16), vmem((_D,), bf16), vmem((_D,), bf16),
            pltpu.SemaphoreType.DMA((6,)), pltpu.SemaphoreType.DMA((_NF + _NO,)),
            pltpu.SemaphoreType.DMA(()),
        ],
        compiler_params=pltpu.CompilerParams(vmem_limit_bytes=100 * 2**20),
    )(A_u.reshape(_L, _D).T, A_A_re, A_A_im, A_B_re, A_B_im, A_C_re, A_C_im, A_log_dt, A_Dskip,
      B_w_r, B_w_gate, B_w_up, B_w_down.T)
    return out.T.reshape(1, _L, _D)
```
